```python
import jax
import jax.numpy as jnp

def _softmax(x, axis=-1):
    return jax.nn.softmax(x, axis=axis)

def _gelu(x):
    return jax.nn.gelu(x, approximate=True)

def _silu(x):
    return jax.nn.silu(x)

def _sigmoid(x):
    return jax.nn.sigmoid(x)

def _layernorm(x, axis=-1, eps=1e-05):
    m = jnp.mean(x, axis=axis, keepdims=True)
    v = jnp.var(x, axis=axis, keepdims=True)
    return (x - m) / jnp.sqrt(v + eps)

def _scatter_add(tgt, idx, src, axis=0):
    return tgt.at[idx].add(src)

def _segment_sum(src, seg, n):
    return jax.ops.segment_sum(src, seg, n)

class _Rng:

    def __init__(self, key):
        self._k = key

    def _next(self):
        self._k, sub = jax.random.split(self._k)
        return sub

    def normal(self, shape):
        return jax.random.normal(self._next(), shape, dtype=jnp.bfloat16)

    def randint(self, lo, hi, shape):
        return jax.random.randint(self._next(), shape, lo, hi, dtype=jnp.int32)

    def uniform(self, shape, lo=0.0, hi=1.0):
        return jax.random.uniform(self._next(), shape, jnp.bfloat16, lo, hi)

    def permutation(self, n):
        return jax.random.permutation(self._next(), n)
kernel_name = 'interleave_layers__memory_aug_recurrent_mem_tr__sliding_local_dilated__prompt'

def setup_inputs():
    _rng = _Rng(jax.random.key(int.from_bytes(__import__("os").urandom(4), "little")))
    _w = lambda a: (lambda t: t.astype(jnp.bfloat16) if jnp.issubdtype(t.dtype, jnp.floating) else t)(jnp.asarray(a))

    def _A_setup():
        B, S, Dm = (1, 2048, 640)
        H, Dh = (32, 192)
        M, seg = (8, 32)
        seg = min(seg, S)
        S = S // seg * seg
        return {'x': _w((lambda *s: _rng.normal(s) * 0.05)(B, S, Dm)), 'mem0': _w((lambda *s: _rng.normal(s) * 0.05)(B, M, Dm)), 'Wq': _w((lambda *s: _rng.normal(s) * 0.05)(Dm, H, Dh) * Dm ** (-0.5)), 'Wk': _w((lambda *s: _rng.normal(s) * 0.05)(Dm, H, Dh) * Dm ** (-0.5)), 'Wv': _w((lambda *s: _rng.normal(s) * 0.05)(Dm, H, Dh) * Dm ** (-0.5)), 'Wo': _w((lambda *s: _rng.normal(s) * 0.05)(H, Dh, Dm) * (H * Dh) ** (-0.5)), 'seg_len': seg}
    _A_in = _A_setup()

    def _B_setup():
        B, S, D = (1, 2048, 640)
        return {'x': _w((lambda *s: _rng.normal(s) * 0.05)(B, S, D)), 'wqkv': _w((lambda *s: _rng.normal(s) * 0.05)(D, 3 * D)), 'wo': _w((lambda *s: _rng.normal(s) * 0.05)(D, D))}
    _B_in = _B_setup()
    return {'A_x': _A_in['x'], 'A_mem0': _A_in['mem0'], 'A_Wq': _A_in['Wq'], 'A_Wk': _A_in['Wk'], 'A_Wv': _A_in['Wv'], 'A_Wo': _A_in['Wo'], 'A_seg_len': _A_in['seg_len'], 'B_x': _B_in['x'], 'B_wqkv': _B_in['wqkv'], 'B_wo': _B_in['wo']}

def reference(A_x, A_mem0, A_Wq, A_Wk, A_Wv, A_Wo, A_seg_len, B_x, B_wqkv, B_wo):

    def _A_ref(x, mem0, Wq, Wk, Wv, Wo, seg_len):
        B, S, Dm = x.shape
        H, Dh = (Wq.shape[1], Wq.shape[2])
        M = mem0.shape[1]
        scale = Dh ** (-0.5)
        n_seg = S // seg_len
        L = M + seg_len
        idx = jnp.arange(L)
        mask = (idx[:, None] < M) | (idx[:, None] >= idx[None, :])
        mem = mem0
        outs = []
        for s in range(n_seg):
            xs = x[:, s * seg_len:(s + 1) * seg_len, :].copy()
            h = jnp.concatenate([mem, xs], axis=1)
            q = jnp.einsum('btd,dhe->bhte', h, Wq)
            k = jnp.einsum('btd,dhe->bhte', h, Wk)
            v = jnp.einsum('btd,dhe->bhte', h, Wv)
            scores = jnp.einsum('bhqe,bhke->bhqk', q, k) * scale
            scores = jnp.where(mask[None, None], scores, -1000000000.0)
            p = _softmax(scores, axis=-1)
            o = jnp.einsum('bhqk,bhke->bhqe', p, v)
            o = jnp.einsum('bhte,hed->btd', o, Wo)
            mem = o[:, :M, :].copy()
            outs.append(o[:, M:, :])
        return jnp.concatenate(outs, axis=1)

    def _B_ref(x, wqkv, wo):
        B, S, D = x.shape
        H = 32
        Dh = D // H
        W, dil = (8, 2)
        qkv = (lambda x, *d: x.transpose(*d))((x @ wqkv).reshape(B, S, 3, H, Dh), 2, 0, 3, 1, 4)
        q, k, v = (qkv[0], qkv[1], qkv[2])
        scale = Dh ** (-0.5)
        pos = jnp.arange(S)
        off = jnp.arange(W) * dil
        idx = pos[:, None] - off[None, :]
        mask = idx >= 0
        idx_c = jnp.where(mask, idx, 0).reshape(-1)
        kg = k[:, :, idx_c, :].reshape(B, H, S, W, Dh)
        vg = v[:, :, idx_c, :].reshape(B, H, S, W, Dh)
        logits = jnp.einsum('bhsd,bhswd->bhsw', q, kg) * scale
        logits = jnp.where(mask[None, None, :, :], logits, -1000000000.0)
        attn = _softmax(logits, axis=-1)
        o = jnp.einsum('bhsw,bhswd->bhsd', attn, vg)
        return (lambda x, *d: x.transpose(*d))(o, 0, 2, 1, 3).reshape(B, S, D) @ wo
    x = A_x
    x = x + _A_ref(_layernorm(x, axis=-1), A_mem0, A_Wq, A_Wk, A_Wv, A_Wo, A_seg_len)
    x = x + _B_ref(_layernorm(x, axis=-1), B_wqkv, B_wo)
    x = x + _A_ref(_layernorm(x, axis=-1), A_mem0, A_Wq, A_Wk, A_Wv, A_Wo, A_seg_len)
    x = x + _B_ref(_layernorm(x, axis=-1), B_wqkv, B_wo)
    return x
```

```python
import functools

import jax
import jax.numpy as jnp
from jax import lax
import jax.experimental.pallas as pl
import jax.experimental.pallas.tpu as pltpu

F32 = jnp.float32
BF16 = jnp.bfloat16

_NT = (((1,), (1,)), ((), ()))
_NN = (((1,), (0,)), ((), ()))

HB = 32
WIN = 8
DIL = 2
HIST = 16
LANES = 128
NEG = -1000000000.0


def _dot(a, b, dims):
    return lax.dot_general(a, b, dims, preferred_element_type=F32)


def _ln(x):
    m = jnp.mean(x, axis=-1, keepdims=True)
    xc = x - m
    v = jnp.mean(xc * xc, axis=-1, keepdims=True)
    return xc * lax.rsqrt(v + 1e-05)


def _a_pass(h, wq_ref, wk_ref, wv_ref, wo_ref, *, n_pairs, dh, m_len, l_len):
    L = l_len
    R = 2 * L
    pw = 2 * dh
    half = dh - LANES
    scale = dh ** (-0.5)
    lo_rows = ((L + 15) // 16) * 16
    hi_start = R - lo_rows

    row = lax.broadcasted_iota(jnp.int32, (R, R), 0)
    col = lax.broadcasted_iota(jnp.int32, (R, R), 1)
    col_lo = col < L
    diag = (row < L) == col_lo
    r_in = jnp.where(row < L, row, row - L)
    c_in = jnp.where(col_lo, col, col - L)
    allowed = (r_in < m_len) | (r_in >= c_in)
    lane = lax.broadcasted_iota(jnp.int32, (L, LANES), 1)
    lane_lo = lane < half

    def swap(a):
        return jnp.concatenate([a[L:], a[:L]], axis=0)

    def split_shared(a):
        a1, a2 = a[:L], a[L:]
        z = jnp.zeros_like(a1)
        first = jnp.concatenate(
            [jnp.where(lane_lo, a1, z), jnp.where(lane_lo, z, a1)], axis=0)
        second = jnp.concatenate(
            [jnp.where(lane_lo, z, a2), jnp.where(lane_lo, a2, z)], axis=0)
        return first.astype(BF16), second.astype(BF16)

    def merge_rows(a, b):
        return jnp.concatenate([a[:L], b[L - hi_start:]], axis=0)

    acc = None
    for p in range(n_pairs):
        c0 = p * pw
        q = _dot(h, wq_ref[c0:c0 + pw, :], _NT).astype(BF16)
        k = _dot(h, wk_ref[c0:c0 + pw, :], _NT)
        v = _dot(h, wv_ref[c0:c0 + pw, :], _NT)

        k0 = k[:, :LANES].astype(BF16)
        k2 = swap(k[:, 2 * LANES:]).astype(BF16)
        k1a, k1b = split_shared(k[:, LANES:2 * LANES])
        r0 = _dot(q[:, :LANES], k0, _NT)
        r2 = _dot(q[:, 2 * LANES:], k2, _NT)
        r1a = _dot(q[:lo_rows, LANES:2 * LANES], k1a, _NT)
        r1b = _dot(q[hi_start:, LANES:2 * LANES], k1b, _NT)
        s = jnp.where(diag, r0, r2) + merge_rows(r1a, r1b)
        s = jnp.where(allowed, s * scale, NEG)

        m_lo = jnp.max(jnp.where(col_lo, s, -jnp.inf), axis=1, keepdims=True)
        m_hi = jnp.max(jnp.where(col_lo, -jnp.inf, s), axis=1, keepdims=True)
        e = jnp.exp(s - jnp.where(col_lo, m_lo, m_hi))
        e_lo = jnp.where(col_lo, e, 0.0)
        e_hi = jnp.where(col_lo, 0.0, e)
        p_lo = e_lo * (1.0 / jnp.sum(e_lo, axis=1, keepdims=True))
        p_hi = e_hi * (1.0 / jnp.sum(e_hi, axis=1, keepdims=True))
        p_all = (p_lo + p_hi).astype(BF16)
        p_diag = jnp.concatenate([p_lo[:L], p_hi[L:]], axis=0).astype(BF16)
        p_off = jnp.concatenate([p_hi[:L], p_lo[L:]], axis=0).astype(BF16)

        v0 = v[:, :LANES].astype(BF16)
        v2 = swap(v[:, 2 * LANES:]).astype(BF16)
        v1a, v1b = split_shared(v[:, LANES:2 * LANES])
        o0 = _dot(p_diag, v0, _NN)
        o2 = _dot(p_off, v2, _NN)
        o1 = merge_rows(_dot(p_all[:lo_rows], v1a, _NN),
                        _dot(p_all[hi_start:], v1b, _NN))
        o = jnp.concatenate([o0, o1, o2], axis=1).astype(BF16)
        part = _dot(o, wo_ref[c0:c0 + pw, :], _NN)
        acc = part if acc is None else acc + part
    return acc


def _b_pass(y, starts, wqkv_ref, wo_ref, kv_ref, *, seg, d):
    n = len(starts)
    db = d // HB
    scale = db ** (-0.5)
    nt = d // LANES
    yn = _ln(y).astype(BF16)
    qkv = _dot(yn, wqkv_ref[...], _NN)
    rows = lax.broadcasted_iota(jnp.int32, (seg, LANES), 0)
    outs = []
    for i in range(n):
        r0 = i * seg
        q = qkv[r0:r0 + seg, :d] * scale
        kv_ref[i, HIST:, :] = qkv[r0:r0 + seg, d:]
        pos = rows + starts[i]
        logits = []
        for w in range(WIN):
            off = HIST - w * DIL
            prod = q * kv_ref[i, off:off + seg, :d]
            t = prod[:, :LANES]
            for c in range(1, nt):
                t = t + prod[:, c * LANES:(c + 1) * LANES]
            t = t + pltpu.roll(t, 64, 1)
            t = t + pltpu.roll(t, 32, 1)
            if w > 0:
                t = jnp.where(pos >= w * DIL, t, NEG)
            logits.append(t)
        m = logits[0]
        for w in range(1, WIN):
            m = jnp.maximum(m, logits[w])
        es = [jnp.exp(t - m) for t in logits]
        den = es[0]
        for w in range(1, WIN):
            den = den + es[w]
        inv = 1.0 / den
        o = None
        for w in range(WIN):
            off = HIST - w * DIL
            pw_ = es[w] * inv
            term = (jnp.concatenate([pw_] * nt, axis=1)
                    * kv_ref[i, off:off + seg, d:])
            o = term if o is None else o + term
        outs.append(o)
        kv_ref[i, :HIST, :] = kv_ref[i, seg:, :]
    o = outs[0] if n == 1 else jnp.concatenate(outs, axis=0)
    return y + _dot(o.astype(BF16), wo_ref[...], _NN)


def _kernel(x_hbm, mem_hbm, wq_hbm, wk_hbm, wv_hbm, wo_hbm, bqkv_hbm, bo_hbm,
            out_hbm,
            x_v, mem_v, wq_v, wk_v, wv_v, wo_v, bqkv_v, bo_v, bqkv_p, bo_p,
            out_v, h_s, ra_s, y_s, kv_s, sems,
            *, seg, n_seg, m_len, n_pairs, dh, d):
    L = m_len + seg
    db = d // HB

    srcs = (x_hbm, mem_hbm, bqkv_hbm, bo_hbm, wq_hbm, wk_hbm, wv_hbm, wo_hbm)
    dsts = (x_v, mem_v, bqkv_v, bo_v, wq_v, wk_v, wv_v, wo_v)
    copies = [pltpu.make_async_copy(s_, d_, sems.at[i])
              for i, (s_, d_) in enumerate(zip(srcs, dsts))]
    for c in copies:
        c.start()
    for c in copies[:4]:
        c.wait()

    ii = lax.broadcasted_iota(jnp.int32, (d, d), 0)
    jj = lax.broadcasted_iota(jnp.int32, (d, d), 1)
    perm = (ii == (jj % HB) * db + jj // HB).astype(BF16)
    perm_t = (jj == (ii % HB) * db + ii // HB).astype(BF16)
    for c in range(3):
        bqkv_p[:, c * d:(c + 1) * d] = _dot(
            bqkv_v[:, c * d:(c + 1) * d], perm, _NN).astype(BF16)
    bo_p[...] = _dot(perm_t, bo_v[...], _NN).astype(BF16)

    mem0 = mem_v[...].astype(F32)
    zero_seg = jnp.zeros((seg, d), F32)
    h_s[...] = jnp.concatenate(
        [mem0, _ln(x_v[0:seg, :].astype(F32)), mem0, zero_seg],
        axis=0).astype(BF16)
    ra_s[...] = zero_seg
    y_s[...] = jnp.zeros(y_s.shape, F32)
    kv_s[...] = jnp.zeros(kv_s.shape, F32)

    for c in copies[4:]:
        c.wait()

    def step(t, carry):
        yb = _b_pass(y_s[...], ((t - 1) * seg, (t - 3) * seg),
                     bqkv_p, bo_p, kv_s, seg=seg, d=d)
        x2 = yb[:seg]
        o_row = pl.multiple_of(jnp.maximum(t - 3, 0) * seg, seg)
        out_v[pl.ds(o_row, seg), :] = yb[seg:].astype(out_v.dtype)

        acc = _a_pass(h_s[...], wq_v, wk_v, wv_v, wo_v,
                      n_pairs=n_pairs, dh=dh, m_len=m_len, l_len=L)
        x_row = pl.multiple_of(jnp.minimum(t, n_seg - 1) * seg, seg)
        x0 = x_v[pl.ds(x_row, seg), :].astype(F32)
        y_s[:seg, :] = x0 + acc[m_len:L]
        y_s[seg:, :] = ra_s[...] + acc[L + m_len:]
        ra_s[...] = x2

        n_row = pl.multiple_of(jnp.minimum(t + 1, n_seg - 1) * seg, seg)
        xn = x_v[pl.ds(n_row, seg), :].astype(F32)
        mem2 = jnp.where(t < 2, mem_v[...].astype(F32), acc[L:L + m_len])
        h_s[...] = jnp.concatenate(
            [acc[:m_len], _ln(xn), mem2, _ln(x2)], axis=0).astype(BF16)
        return carry

    lax.fori_loop(0, n_seg + 2, step, 0)

    yb = _b_pass(y_s[seg:, :], ((n_seg - 1) * seg,), bqkv_p, bo_p,
                 kv_s.at[1:], seg=seg, d=d)
    out_v[(n_seg - 1) * seg:, :] = yb.astype(out_v.dtype)

    out_copy = pltpu.make_async_copy(out_v, out_hbm, sems.at[8])
    out_copy.start()
    out_copy.wait()


@functools.partial(jax.jit, static_argnames=("A_seg_len",))
def pallas_interleave_layers__memory_aug_recurrent_mem_tr__sliding_local_dilated__prompt_kernel(
    A_x: jax.Array,
    A_mem0: jax.Array,
    A_Wq: jax.Array,
    A_Wk: jax.Array,
    A_Wv: jax.Array,
    A_Wo: jax.Array,
    A_seg_len,
    B_x: jax.Array,
    B_wqkv: jax.Array,
    B_wo: jax.Array,
):
    del B_x
    bsz, s_len, d = A_x.shape
    m_len = A_mem0.shape[1]
    n_heads, dh = A_Wq.shape[1], A_Wq.shape[2]
    seg = int(A_seg_len)
    n_seg = s_len // seg
    assert bsz == 1 and s_len % seg == 0 and n_seg >= 3
    assert seg % 16 == 0 and m_len % 8 == 0 and (2 * (m_len + seg)) % 16 == 0
    assert 2 * (m_len + seg) <= LANES and seg >= HIST
    assert n_heads % 2 == 0 and 2 * dh == 3 * LANES and d % LANES == 0
    assert d % HB == 0 and LANES == 4 * HB
    hd = n_heads * dh
    L = m_len + seg

    wq_t = jnp.transpose(A_Wq, (1, 2, 0)).reshape(hd, d)
    wk_t = jnp.transpose(A_Wk, (1, 2, 0)).reshape(hd, d)
    wv_t = jnp.transpose(A_Wv, (1, 2, 0)).reshape(hd, d)
    wo = A_Wo.reshape(hd, d)

    kernel = functools.partial(
        _kernel, seg=seg, n_seg=n_seg, m_len=m_len, n_pairs=n_heads // 2,
        dh=dh, d=d)
    any_spec = pl.BlockSpec(memory_space=pl.ANY)
    out = pl.pallas_call(
        kernel,
        out_shape=jax.ShapeDtypeStruct((s_len, d), A_x.dtype),
        in_specs=[any_spec] * 8,
        out_specs=any_spec,
        scratch_shapes=[
            pltpu.VMEM((s_len, d), BF16),
            pltpu.VMEM((m_len, d), BF16),
            pltpu.VMEM((hd, d), BF16),
            pltpu.VMEM((hd, d), BF16),
            pltpu.VMEM((hd, d), BF16),
            pltpu.VMEM((hd, d), BF16),
            pltpu.VMEM((d, 3 * d), BF16),
            pltpu.VMEM((d, d), BF16),
            pltpu.VMEM((d, 3 * d), BF16),
            pltpu.VMEM((d, d), BF16),
            pltpu.VMEM((s_len, d), A_x.dtype),
            pltpu.VMEM((2 * L, d), BF16),
            pltpu.VMEM((seg, d), F32),
            pltpu.VMEM((2 * seg, d), F32),
            pltpu.VMEM((2, HIST + seg, 2 * d), F32),
            pltpu.SemaphoreType.DMA((9,)),
        ],
        compiler_params=pltpu.CompilerParams(
            vmem_limit_bytes=100 * 1024 * 1024),
    )(A_x.reshape(s_len, d), A_mem0.reshape(m_len, d), wq_t, wk_t, wv_t, wo,
      B_wqkv, B_wo)
    return out.reshape(bsz, s_len, d)
```

```python
import functools

import jax
import jax.numpy as jnp
from jax import lax
import jax.experimental.pallas as pl
import jax.experimental.pallas.tpu as pltpu

F32 = jnp.float32
BF16 = jnp.bfloat16

_NT = (((1,), (1,)), ((), ()))
_NN = (((1,), (0,)), ((), ()))

HB = 32
WIN = 8
DIL = 2
HIST = 16
LANES = 128
NEG = -1000000000.0


def _dot(a, b, dims):
    return lax.dot_general(a, b, dims, preferred_element_type=F32)


def _recip(x):
    r = pl.reciprocal(x, approx=True)
    return r * (2.0 - x * r)


def _ln(x):
    m = jnp.mean(x, axis=-1, keepdims=True)
    xc = x - m
    v = jnp.mean(xc * xc, axis=-1, keepdims=True)
    return xc * lax.rsqrt(v + 1e-05)


class _APass:
    def __init__(self, h, wq_ref, wk_ref, wv_ref, wo_ref, *, dh, m_len, l_len):
        self.h = h
        self.wq, self.wk, self.wv, self.wo = wq_ref, wk_ref, wv_ref, wo_ref
        L = self.L = l_len
        R = 2 * L
        self.pw = 2 * dh
        half = dh - LANES
        self.scale = dh ** (-0.5)
        self.lo_rows = ((L + 15) // 16) * 16
        self.hi_start = R - self.lo_rows
        row = lax.broadcasted_iota(jnp.int32, (R, R), 0)
        col = lax.broadcasted_iota(jnp.int32, (R, R), 1)
        self.col_lo = col < L
        self.diag = (row < L) == self.col_lo
        r_in = jnp.where(row < L, row, row - L)
        c_in = jnp.where(self.col_lo, col, col - L)
        self.allowed = (r_in < m_len) | (r_in >= c_in)
        lane = lax.broadcasted_iota(jnp.int32, (L, LANES), 1)
        self.lane_lo = lane < half
        self.q, self.k, self.v, self.p, self.o = {}, {}, {}, {}, {}
        self.acc = None

    def _swap(self, a):
        return jnp.concatenate([a[self.L:], a[:self.L]], axis=0)

    def _tiles(self, a):
        L, lo = self.L, self.lane_lo
        a1, a2 = a[:L, LANES:2 * LANES], a[L:, LANES:2 * LANES]
        z = jnp.zeros_like(a1)
        first = jnp.concatenate(
            [jnp.where(lo, a1, z), jnp.where(lo, z, a1)], axis=0)
        second = jnp.concatenate(
            [jnp.where(lo, z, a2), jnp.where(lo, a2, z)], axis=0)
        return (a[:, :LANES].astype(BF16), first.astype(BF16),
                second.astype(BF16), self._swap(a[:, 2 * LANES:]).astype(BF16))

    def _merge_rows(self, a, b):
        return jnp.concatenate(
            [a[:self.L], b[self.L - self.hi_start:]], axis=0)

    def _w(self, ref, p):
        return ref[p * self.pw:(p + 1) * self.pw, :]

    def proj_q(self, p):
        self.q[p] = _dot(self.h, self._w(self.wq, p), _NT).astype(BF16)

    def proj_k(self, p):
        self.k[p] = self._tiles(_dot(self.h, self._w(self.wk, p), _NT))

    def proj_v(self, p):
        self.v[p] = self._tiles(_dot(self.h, self._w(self.wv, p), _NT))

    def scores(self, p):
        L, col_lo = self.L, self.col_lo
        q = self.q.pop(p)
        k0, k1a, k1b, k2 = self.k.pop(p)
        r0 = _dot(q[:, :LANES], k0, _NT)
        r2 = _dot(q[:, 2 * LANES:], k2, _NT)
        r1a = _dot(q[:self.lo_rows, LANES:2 * LANES], k1a, _NT)
        r1b = _dot(q[self.hi_start:, LANES:2 * LANES], k1b, _NT)
        s = jnp.where(self.diag, r0, r2) + self._merge_rows(r1a, r1b)
        s = jnp.where(self.allowed, s * self.scale, NEG)
        m_lo = jnp.max(jnp.where(col_lo, s, -jnp.inf), axis=1, keepdims=True)
        m_hi = jnp.max(jnp.where(col_lo, -jnp.inf, s), axis=1, keepdims=True)
        e = jnp.exp(s - jnp.where(col_lo, m_lo, m_hi))
        d_lo = jnp.sum(jnp.where(col_lo, e, 0.0), axis=1, keepdims=True)
        d_hi = jnp.sum(jnp.where(col_lo, 0.0, e), axis=1, keepdims=True)
        p_all = e * _recip(jnp.where(col_lo, d_lo, d_hi))
        p_diag = jnp.where(self.diag, p_all, 0.0)
        p_off = jnp.where(self.diag, 0.0, p_all)
        self.p[p] = (p_all.astype(BF16), p_diag.astype(BF16),
                     p_off.astype(BF16))

    def pv(self, p):
        p_all, p_diag, p_off = self.p.pop(p)
        v0, v1a, v1b, v2 = self.v.pop(p)
        o0 = _dot(p_diag, v0, _NN)
        o2 = _dot(p_off, v2, _NN)
        o1 = self._merge_rows(_dot(p_all[:self.lo_rows], v1a, _NN),
                              _dot(p_all[self.hi_start:], v1b, _NN))
        self.o[p] = jnp.concatenate([o0, o1, o2], axis=1).astype(BF16)

    def out(self, p):
        part = _dot(self.o.pop(p), self._w(self.wo, p), _NN)
        self.acc = part if self.acc is None else self.acc + part


def _b_attn(y, starts, wqkv_ref, kv_ref, *, seg, d):
    n = len(starts)
    db = d // HB
    scale = db ** (-0.5)
    nt = d // LANES
    yn = _ln(y).astype(BF16)
    qkv = _dot(yn, wqkv_ref[...], _NN)
    rows = lax.broadcasted_iota(jnp.int32, (seg, LANES), 0)
    outs = []
    for i in range(n):
        r0 = i * seg
        q = qkv[r0:r0 + seg, :d] * scale
        kv_ref[i, HIST:, :] = qkv[r0:r0 + seg, d:]
        pos = rows + starts[i]
        logits = []
        for w in range(WIN):
            off = HIST - w * DIL
            prod = q * kv_ref[i, off:off + seg, :d]
            t = prod[:, :LANES]
            for c in range(1, nt):
                t = t + prod[:, c * LANES:(c + 1) * LANES]
            t = t + pltpu.roll(t, 64, 1)
            t = t + pltpu.roll(t, 32, 1)
            if w > 0:
                t = jnp.where(pos >= w * DIL, t, NEG)
            logits.append(t)
        m = logits[0]
        for w in range(1, WIN):
            m = jnp.maximum(m, logits[w])
        es = [jnp.exp(t - m) for t in logits]
        den = es[0]
        for w in range(1, WIN):
            den = den + es[w]
        inv = _recip(den)
        o = None
        for w in range(WIN):
            off = HIST - w * DIL
            pw_ = es[w] * inv
            term = (jnp.concatenate([pw_] * nt, axis=1)
                    * kv_ref[i, off:off + seg, d:])
            o = term if o is None else o + term
        outs.append(o)
        kv_ref[i, :HIST, :] = kv_ref[i, seg:, :]
    o = outs[0] if n == 1 else jnp.concatenate(outs, axis=0)
    return o.astype(BF16)


def _kernel(x_hbm, mem_hbm, wq_hbm, wk_hbm, wv_hbm, wo_hbm, bqkv_hbm, bo_hbm,
            out_hbm,
            x_v, mem_v, wq_v, wk_v, wv_v, wo_v, bqkv_v, bo_v, bqkv_p, bo_p,
            out_v, h_s, ra_s, y_s, kv_s, sems,
            *, seg, n_seg, m_len, n_pairs, dh, d):
    L = m_len + seg
    db = d // HB

    srcs = (x_hbm, mem_hbm, bqkv_hbm, bo_hbm, wq_hbm, wk_hbm, wv_hbm, wo_hbm)
    dsts = (x_v, mem_v, bqkv_v, bo_v, wq_v, wk_v, wv_v, wo_v)
    copies = [pltpu.make_async_copy(s_, d_, sems.at[i])
              for i, (s_, d_) in enumerate(zip(srcs, dsts))]
    for c in copies:
        c.start()
    for c in copies[:4]:
        c.wait()

    ii = lax.broadcasted_iota(jnp.int32, (d, d), 0)
    jj = lax.broadcasted_iota(jnp.int32, (d, d), 1)
    perm = (ii == (jj % HB) * db + jj // HB).astype(BF16)
    perm_t = (jj == (ii % HB) * db + ii // HB).astype(BF16)
    for c in range(3):
        bqkv_p[:, c * d:(c + 1) * d] = _dot(
            bqkv_v[:, c * d:(c + 1) * d], perm, _NN).astype(BF16)
    bo_p[...] = _dot(perm_t, bo_v[...], _NN).astype(BF16)

    mem0 = mem_v[...].astype(F32)
    zero_seg = jnp.zeros((seg, d), F32)
    h_s[...] = jnp.concatenate(
        [mem0, _ln(x_v[0:seg, :].astype(F32)), mem0, zero_seg],
        axis=0).astype(BF16)
    ra_s[...] = zero_seg
    y_s[...] = jnp.zeros(y_s.shape, F32)
    kv_s[...] = jnp.zeros(kv_s.shape, F32)

    for c in copies[4:]:
        c.wait()

    def step(t, carry):
        a = _APass(h_s[...], wq_v, wk_v, wv_v, wo_v,
                   dh=dh, m_len=m_len, l_len=L)
        ob = None
        for p in range(n_pairs):
            a.proj_q(p)
            a.proj_k(p)
            if p > 0:
                a.pv(p - 1)
            a.proj_v(p)
            a.scores(p)
            if p == 0:
                ob = _b_attn(y_s[...], ((t - 1) * seg, (t - 3) * seg),
                             bqkv_p, kv_s, seg=seg, d=d)
            elif p < n_pairs - 1:
                a.out(p - 1)
        yb = y_s[...] + _dot(ob, bo_p[...], _NN)
        a.pv(n_pairs - 1)
        a.out(n_pairs - 2)
        a.out(n_pairs - 1)
        acc = a.acc

        x2 = yb[:seg]
        o_row = pl.multiple_of(jnp.maximum(t - 3, 0) * seg, seg)
        out_v[pl.ds(o_row, seg), :] = yb[seg:].astype(out_v.dtype)

        x_row = pl.multiple_of(jnp.minimum(t, n_seg - 1) * seg, seg)
        x0 = x_v[pl.ds(x_row, seg), :].astype(F32)
        y_s[:seg, :] = x0 + acc[m_len:L]
        y_s[seg:, :] = ra_s[...] + acc[L + m_len:]
        ra_s[...] = x2

        n_row = pl.multiple_of(jnp.minimum(t + 1, n_seg - 1) * seg, seg)
        xn = x_v[pl.ds(n_row, seg), :].astype(F32)
        mem2 = jnp.where(t < 2, mem_v[...].astype(F32), acc[L:L + m_len])
        h_s[...] = jnp.concatenate(
            [acc[:m_len], _ln(xn), mem2, _ln(x2)], axis=0).astype(BF16)
        return carry

    lax.fori_loop(0, n_seg + 2, step, 0)

    ob = _b_attn(y_s[seg:, :], ((n_seg - 1) * seg,), bqkv_p, kv_s.at[1:],
                 seg=seg, d=d)
    yb = y_s[seg:, :] + _dot(ob, bo_p[...], _NN)
    out_v[(n_seg - 1) * seg:, :] = yb.astype(out_v.dtype)

    out_copy = pltpu.make_async_copy(out_v, out_hbm, sems.at[8])
    out_copy.start()
    out_copy.wait()


@functools.partial(jax.jit, static_argnames=("A_seg_len",))
def pallas_interleave_layers__memory_aug_recurrent_mem_tr__sliding_local_dilated__prompt_kernel(
    A_x: jax.Array,
    A_mem0: jax.Array,
    A_Wq: jax.Array,
    A_Wk: jax.Array,
    A_Wv: jax.Array,
    A_Wo: jax.Array,
    A_seg_len,
    B_x: jax.Array,
    B_wqkv: jax.Array,
    B_wo: jax.Array,
):
    del B_x
    bsz, s_len, d = A_x.shape
    m_len = A_mem0.shape[1]
    n_heads, dh = A_Wq.shape[1], A_Wq.shape[2]
    seg = int(A_seg_len)
    n_seg = s_len // seg
    assert bsz == 1 and s_len % seg == 0 and n_seg >= 3
    assert seg % 16 == 0 and m_len % 8 == 0 and (2 * (m_len + seg)) % 16 == 0
    assert 2 * (m_len + seg) <= LANES and seg >= HIST
    assert n_heads % 2 == 0 and 2 * dh == 3 * LANES and d % LANES == 0
    assert d % HB == 0 and LANES == 4 * HB
    hd = n_heads * dh
    L = m_len + seg

    wq_t = jnp.transpose(A_Wq, (1, 2, 0)).reshape(hd, d)
    wk_t = jnp.transpose(A_Wk, (1, 2, 0)).reshape(hd, d)
    wv_t = jnp.transpose(A_Wv, (1, 2, 0)).reshape(hd, d)
    wo = A_Wo.reshape(hd, d)

    kernel = functools.partial(
        _kernel, seg=seg, n_seg=n_seg, m_len=m_len, n_pairs=n_heads // 2,
        dh=dh, d=d)
    any_spec = pl.BlockSpec(memory_space=pl.ANY)
    out = pl.pallas_call(
        kernel,
        out_shape=jax.ShapeDtypeStruct((s_len, d), A_x.dtype),
        in_specs=[any_spec] * 8,
        out_specs=any_spec,
        scratch_shapes=[
            pltpu.VMEM((s_len, d), BF16),
            pltpu.VMEM((m_len, d), BF16),
            pltpu.VMEM((hd, d), BF16),
            pltpu.VMEM((hd, d), BF16),
            pltpu.VMEM((hd, d), BF16),
            pltpu.VMEM((hd, d), BF16),
            pltpu.VMEM((d, 3 * d), BF16),
            pltpu.VMEM((d, d), BF16),
            pltpu.VMEM((d, 3 * d), BF16),
            pltpu.VMEM((d, d), BF16),
            pltpu.VMEM((s_len, d), A_x.dtype),
            pltpu.VMEM((2 * L, d), BF16),
            pltpu.VMEM((seg, d), F32),
            pltpu.VMEM((2 * seg, d), F32),
            pltpu.VMEM((2, HIST + seg, 2 * d), F32),
            pltpu.SemaphoreType.DMA((9,)),
        ],
        compiler_params=pltpu.CompilerParams(
            vmem_limit_bytes=100 * 1024 * 1024),
    )(A_x.reshape(s_len, d), A_mem0.reshape(m_len, d), wq_t, wk_t, wv_t, wo,
      B_wqkv, B_wo)
    return out.reshape(bsz, s_len, d)
```

```python
import functools

import jax
import jax.numpy as jnp
from jax import lax
import jax.experimental.pallas as pl
import jax.experimental.pallas.tpu as pltpu

F32 = jnp.float32
BF16 = jnp.bfloat16

_NT = (((1,), (1,)), ((), ()))
_NN = (((1,), (0,)), ((), ()))

HB = 32
WIN = 8
DIL = 2
HIST = 16
LANES = 128
PRE = 16
PRE_CHUNK = 128
LAG = 2
NSLOT = 3
NEG = -1000000000.0


def _dot(a, b, dims):
    return lax.dot_general(a, b, dims, preferred_element_type=F32)


def _recip(x):
    r = pl.reciprocal(x, approx=True)
    return r * (2.0 - x * r)


def _ln(x):
    m = jnp.mean(x, axis=-1, keepdims=True)
    xc = x - m
    v = jnp.mean(xc * xc, axis=-1, keepdims=True)
    return xc * lax.rsqrt(v + 1e-05)


def _tile(a, c):
    return a[:, c * LANES:(c + 1) * LANES]


def _keep(mask, a):
    return jnp.where(mask, a, jnp.zeros_like(a))


def _drop(mask, a):
    return jnp.where(mask, jnp.zeros_like(a), a)


def _pair_softmax(s, col_a):
    m_a = jnp.max(jnp.where(col_a, s, -jnp.inf), axis=1, keepdims=True)
    m_b = jnp.max(jnp.where(col_a, -jnp.inf, s), axis=1, keepdims=True)
    e = jnp.exp(s - jnp.where(col_a, m_a, m_b))
    d_a = jnp.sum(jnp.where(col_a, e, 0.0), axis=1, keepdims=True)
    d_b = jnp.sum(jnp.where(col_a, 0.0, e), axis=1, keepdims=True)
    return e * _recip(jnp.where(col_a, d_a, d_b))


class _PassBase:
    def __init__(self, h, w_ref, wo_ref, dh):
        self.h, self.w, self.wo = h, w_ref, wo_ref
        self.pw = 2 * dh
        self.half = dh - LANES
        self.scale = dh ** (-0.5)
        self.q, self.k, self.v, self.p, self.o = {}, {}, {}, {}, {}
        self.acc = None

    def _lane_lo(self, rows):
        return lax.broadcasted_iota(jnp.int32, (rows, LANES), 1) < self.half

    def _project(self, p, j):
        return _dot(self.h, self.w[p, :, j * self.pw:(j + 1) * self.pw], _NN)

    def out(self, p):
        w = self.wo[p * self.pw:(p + 1) * self.pw, :]
        part = _dot(self.o.pop(p), w, _NN)
        self.acc = part if self.acc is None else self.acc + part

    def run(self, n_pairs, early, late):
        last = n_pairs - 1
        for p in range(n_pairs):
            self.proj_q(p)
            self.proj_k(p)
            if p > 0:
                self.pv(p - 1)
            self.proj_v(p)
            self.scores(p)
            if p == 0:
                early()
            elif p < last - 1:
                self.out(p - 1)
        self.out(last - 2)
        late()
        self.pv(last)
        self.out(last - 1)
        self.out(last)
        return self.acc


class _TwoLayerPass(_PassBase):
    def __init__(self, h, pre_ref, pre_row, w_ref, wo_ref, *, dh, m_len, seg):
        super().__init__(h, w_ref, wo_ref, dh)
        self.pre, self.pre_row = pre_ref, pre_row
        self.m, self.seg = m_len, seg
        m2 = 2 * m_len
        n = m2 + 2 * seg
        row = lax.broadcasted_iota(jnp.int32, (n, n), 0)
        col = lax.broadcasted_iota(jnp.int32, (n, n), 1)

        def first_layer(i):
            return (i < m_len) | ((i >= m2) & (i < m2 + seg))

        def token(i):
            return jnp.where(i < m2 + seg, i - m2, i - m2 - seg)

        self.col_a = first_layer(col)
        self.diag = first_layer(row) == self.col_a
        self.allowed = (row < m2) | (col < m2) | (token(row) >= token(col))
        self.lo_m = self._lane_lo(m_len)
        self.lo_x = self._lane_lo(seg)

    def _proj(self, p, j):
        m, pw = self.m, self.pw
        a = self._project(p, j)
        pre = self.pre[p, pl.ds(self.pre_row, PRE), j * pw:(j + 1) * pw]
        rest = a[2 * m:].astype(BF16)
        n1 = self.seg - PRE
        x1 = jnp.concatenate([pre, rest[:n1]], axis=0)
        return a[:m], a[m:2 * m], x1, rest[n1:]

    @staticmethod
    def _cat(ma, mb, xa, xb):
        mm = jnp.concatenate([ma, mb], axis=0).astype(BF16)
        return jnp.concatenate([mm, xa, xb], axis=0)

    def _tiles(self, m1, m2, x1, x2):
        cat, lm, lx = self._cat, self.lo_m, self.lo_x
        t0 = cat(_tile(m1, 0), _tile(m2, 0), _tile(x1, 0), _tile(x2, 0))
        t2 = cat(_tile(m2, 2), _tile(m1, 2), _tile(x2, 2), _tile(x1, 2))
        m1, m2, x1, x2 = (_tile(a, 1) for a in (m1, m2, x1, x2))
        t1a = cat(_keep(lm, m1), _drop(lm, m1), _keep(lx, x1), _drop(lx, x1))
        t1b = cat(_drop(lm, m2), _keep(lm, m2), _drop(lx, x2), _keep(lx, x2))
        return t0, t1a, t1b, t2

    def _rows_a(self, a):
        return a[:2 * self.m + self.seg]

    def _rows_b(self, a):
        m2 = 2 * self.m
        return jnp.concatenate([a[:m2], a[m2 + self.seg:]], axis=0)

    def _merge_rows(self, a, b):
        m = self.m
        return jnp.concatenate([a[:m], b[m:2 * m], a[2 * m:], b[2 * m:]],
                               axis=0)

    def proj_q(self, p):
        self.q[p] = self._cat(*self._proj(p, 0))

    def proj_k(self, p):
        self.k[p] = self._tiles(*self._proj(p, 1))

    def proj_v(self, p):
        self.v[p] = self._tiles(*self._proj(p, 2))

    def scores(self, p):
        q = self.q.pop(p)
        k0, k1a, k1b, k2 = self.k.pop(p)
        q1 = _tile(q, 1)
        r0 = _dot(_tile(q, 0), k0, _NT)
        r2 = _dot(_tile(q, 2), k2, _NT)
        r1a = _dot(self._rows_a(q1), k1a, _NT)
        r1b = _dot(self._rows_b(q1), k1b, _NT)
        s = jnp.where(self.diag, r0, r2) + self._merge_rows(r1a, r1b)
        s = jnp.where(self.allowed, s * self.scale, NEG)
        p_all = _pair_softmax(s, self.col_a)
        self.p[p] = (p_all.astype(BF16), _keep(self.diag, p_all).astype(BF16),
                     _drop(self.diag, p_all).astype(BF16))

    def pv(self, p):
        p_all, p_diag, p_off = self.p.pop(p)
        v0, v1a, v1b, v2 = self.v.pop(p)
        o0 = _dot(p_diag, v0, _NN)
        o2 = _dot(p_off, v2, _NN)
        o1 = self._merge_rows(_dot(self._rows_a(p_all), v1a, _NN),
                              _dot(self._rows_b(p_all), v1b, _NN))
        self.o[p] = jnp.concatenate([o0, o1, o2], axis=1).astype(BF16)


class _OneLayerPass(_PassBase):
    def __init__(self, h, w_ref, wo_ref, *, dh, m_len, seg):
        super().__init__(h, w_ref, wo_ref, dh)
        n = m_len + seg
        row = lax.broadcasted_iota(jnp.int32, (n, 2 * n), 0)
        col = lax.broadcasted_iota(jnp.int32, (n, 2 * n), 1)
        self.col_a = col < n
        key = jnp.where(self.col_a, col, col - n)
        self.allowed = (row < m_len) | (row >= key)
        lane = lax.broadcasted_iota(jnp.int32, (n, self.pw), 1)
        self.head0 = lane < dh

    def _block_diag(self, a):
        return jnp.concatenate([_keep(self.head0, a), _drop(self.head0, a)],
                               axis=0).astype(BF16)

    def proj_q(self, p):
        self.q[p] = self._project(p, 0).astype(BF16)

    def proj_k(self, p):
        self.k[p] = self._block_diag(self._project(p, 1))

    def proj_v(self, p):
        self.v[p] = self._block_diag(self._project(p, 2))

    def scores(self, p):
        s = _dot(self.q.pop(p), self.k.pop(p), _NT)
        s = jnp.where(self.allowed, s * self.scale, NEG)
        self.p[p] = _pair_softmax(s, self.col_a).astype(BF16)

    def pv(self, p):
        self.o[p] = _dot(self.p.pop(p), self.v.pop(p), _NN).astype(BF16)


def _b_attn(y, starts, wqkv_ref, kv_ref, *, seg, d):
    n = len(starts)
    db = d // HB
    scale = db ** (-0.5)
    nt = d // LANES
    yn = _ln(y).astype(BF16)
    qa, ka, va = (_dot(yn, wqkv_ref[j], _NN) for j in range(3))
    rows = lax.broadcasted_iota(jnp.int32, (8, LANES), 0)
    outs = []
    for i in range(n):
        r0 = i * seg
        for c in range(nt):
            kv_ref[i, c, HIST:, :] = _tile(ka[r0:r0 + seg], c)
            kv_ref[i, nt + c, HIST:, :] = _tile(va[r0:r0 + seg], c)
        for g in range(seg // 8):
            q = [_tile(qa[r0 + 8 * g:r0 + 8 * g + 8], c) for c in range(nt)]
            pos = rows + (starts[i] + 8 * g)
            logits = []
            for w in range(WIN):
                off = HIST + 8 * g - w * DIL
                t = q[0] * kv_ref[i, 0, off:off + 8, :]
                for c in range(1, nt):
                    t = t + q[c] * kv_ref[i, c, off:off + 8, :]
                t = t + pltpu.roll(t, 64, 1)
                t = (t + pltpu.roll(t, 32, 1)) * scale
                if 8 * g < w * DIL:
                    t = jnp.where(pos >= w * DIL, t, NEG)
                logits.append(t)
            m = logits[0]
            for w in range(1, WIN):
                m = jnp.maximum(m, logits[w])
            es = [jnp.exp(t - m) for t in logits]
            den = es[0]
            for w in range(1, WIN):
                den = den + es[w]
            inv = _recip(den)
            o = []
            for c in range(nt):
                acc = None
                for w in range(WIN):
                    off = HIST + 8 * g - w * DIL
                    term = es[w] * kv_ref[i, nt + c, off:off + 8, :]
                    acc = term if acc is None else acc + term
                o.append(acc * inv)
            outs.append(jnp.concatenate(o, axis=1))
        kv_ref[i, :, :HIST, :] = kv_ref[i, :, seg:, :]
    return jnp.concatenate(outs, axis=0).astype(BF16)


def _kernel(x_hbm, mem_hbm, wq_hbm, wk_hbm, wv_hbm, wo_hbm, bqkv_hbm, bo_hbm,
            out_hbm,
            x_v, mem_v, wst_v, w_v, wo_v, bq_st, bo_st, tq_s, to_s, bqkv_p,
            bo_p, out_v, xn_s, pre_s, h_s, h1_s, ra_s, y_s, kv_s,
            sems, w_sems, wo_sems, bq_sems, bo_sems,
            *, seg, n_seg, m_len, n_pairs, dh, d):
    db = d // HB
    nt = d // LANES
    pw = 2 * dh
    m2 = 2 * m_len
    n_pre = (n_seg - LAG) * PRE
    n_bq = 3 * nt

    def w_copy(p, j):
        src = (wq_hbm, wk_hbm, wv_hbm)[j]
        slot = p % NSLOT
        return pltpu.make_async_copy(
            src.at[pl.ds(p * pw, pw), :],
            wst_v.at[slot, pl.ds(j * pw, pw), :], w_sems.at[3 * slot + j])

    def wo_copy(p):
        return pltpu.make_async_copy(wo_hbm.at[pl.ds(p * pw, pw), :],
                                     wo_v.at[pl.ds(p * pw, pw), :],
                                     wo_sems.at[p])

    def bq_copy(i):
        row = pl.multiple_of((i % nt) * LANES, LANES)
        col = pl.multiple_of((i // nt) * d, LANES)
        return pltpu.make_async_copy(
            bqkv_hbm.at[pl.ds(row, LANES), pl.ds(col, d)], bq_st.at[i],
            bq_sems.at[i])

    def bo_copy(i):
        col = pl.multiple_of(i * LANES, LANES)
        return pltpu.make_async_copy(bo_hbm.at[:, pl.ds(col, LANES)],
                                     bo_st.at[i], bo_sems.at[i])

    xa_copy = pltpu.make_async_copy(x_hbm.at[:, :PRE, :], x_v.at[:, :PRE, :],
                                    sems.at[0])
    xb_copy = pltpu.make_async_copy(x_hbm.at[:, PRE:, :], x_v.at[:, PRE:, :],
                                    sems.at[1])
    mem_copy = pltpu.make_async_copy(mem_hbm, mem_v, sems.at[2])

    xa_copy.start()
    for p in range(2):
        bq_copy(p).start()
        bo_copy(p).start()
        for j in range(3):
            w_copy(p, j).start()
    mem_copy.start()
    xb_copy.start()

    ra_s[...] = jnp.zeros(ra_s.shape, F32)
    y_s[...] = jnp.zeros(y_s.shape, F32)
    kv_s[...] = jnp.zeros(kv_s.shape, F32)

    xa_copy.wait()
    for s in range(LAG, n_seg):
        xn_s[(s - LAG) * PRE:(s - LAG + 1) * PRE, :] = _ln(
            x_v[s, :PRE, :].astype(F32)).astype(BF16)

    def permute_rows(tmp_ref):
        return jnp.concatenate(
            [tmp_ref[pl.ds(j, HB, stride=db), :] for j in range(db)], axis=0)

    def pre_pair(p, carry):
        for j in range(3):
            w_copy(p, j).wait()

        @pl.when(p < n_bq)
        def _():
            bq_copy(p).wait()

        @pl.when(p < nt)
        def _():
            bo_copy(p).wait()

        @pl.when(p + 2 < n_pairs)
        def _():
            for j in range(3):
                w_copy(p + 2, j).start()

        @pl.when(p + 2 < n_bq)
        def _():
            bq_copy(p + 2).start()

        @pl.when(p + 2 < nt)
        def _():
            bo_copy(p + 2).start()

        wo_copy(p).start()

        slot = p % NSLOT
        for r0 in range(0, n_pre, PRE_CHUNK):
            r1 = min(r0 + PRE_CHUNK, n_pre)
            pre_s[p, r0:r1, :] = _dot(
                xn_s[r0:r1, :], wst_v[slot], _NT).astype(BF16)
        for n in range(3 * pw // LANES):
            w_v[p, :, n * LANES:(n + 1) * LANES] = (
                wst_v[slot, n * LANES:(n + 1) * LANES, :].T)

        i = jnp.minimum(p, n_bq - 1)
        tq_s[...] = bq_st[i].astype(F32).T
        row = pl.multiple_of((i % nt) * LANES, LANES)
        bqkv_p[i // nt, pl.ds(row, LANES), :] = (
            permute_rows(tq_s).T.astype(BF16))
        i = jnp.minimum(p, nt - 1)
        to_s[...] = bo_st[i].astype(F32)
        bo_p[i] = permute_rows(to_s).astype(BF16)
        return carry

    lax.fori_loop(0, n_pairs, pre_pair, 0)

    mem_copy.wait()
    xb_copy.wait()
    for p in range(n_pairs):
        wo_copy(p).wait()
    h1_s[...] = jnp.concatenate(
        [mem_v[...].astype(F32), _ln(x_v[0].astype(F32))],
        axis=0).astype(BF16)

    def b_stages(t):
        res = {}

        def early():
            res["o"] = _b_attn(y_s[...], ((t - 1) * seg, (t - 1 - LAG) * seg),
                               bqkv_p, kv_s, seg=seg, d=d)

        def late():
            proj = jnp.concatenate(
                [_dot(res["o"], bo_p[c], _NN) for c in range(nt)], axis=1)
            yb = y_s[...] + proj
            out_v[jnp.maximum(t - 1 - LAG, 0)] = yb[seg:].astype(out_v.dtype)
            res["x2"] = yb[:seg]

        return early, late, res

    def two_layer_step(t, carry):
        early, late, res = b_stages(t)
        a = _TwoLayerPass(h_s[...], pre_s,
                          pl.multiple_of((t - LAG) * PRE, PRE), w_v, wo_v,
                          dh=dh, m_len=m_len, seg=seg)
        acc = a.run(n_pairs, early, late)
        x2 = res["x2"]
        y_s[:seg, :] = x_v[t].astype(F32) + acc[m2:m2 + seg]
        y_s[seg:, :] = ra_s[...] + acc[m2 + seg:]
        ra_s[...] = x2
        xn = x_v[jnp.minimum(t + 1, n_seg - 1), PRE:, :].astype(F32)
        h_s[:m2, :] = acc[:m2].astype(BF16)
        h_s[m2:, :] = jnp.concatenate([_ln(xn), _ln(x2)],
                                      axis=0).astype(BF16)
        return carry

    def one_layer_step(t, carry):
        first = t < LAG
        early, late, res = b_stages(t)
        a = _OneLayerPass(h1_s[...], w_v, wo_v, dh=dh, m_len=m_len, seg=seg)
        acc = a.run(n_pairs, early, late)
        x2 = res["x2"]
        x0 = x_v[jnp.minimum(t, n_seg - 1)].astype(F32)
        y = jnp.where(first, x0, ra_s[...]) + acc[m_len:]
        y_s[:seg, :] = y
        y_s[seg:, :] = y
        ra_s[...] = x2
        xn = _ln(x_v[jnp.minimum(t + 1, n_seg - 1)].astype(F32))
        x2n = _ln(x2)
        mem = acc[:m_len]
        h1_s[...] = jnp.concatenate(
            [mem, jnp.where(first, xn, x2n)], axis=0).astype(BF16)
        h_s[...] = jnp.concatenate(
            [mem, mem_v[...].astype(F32), xn[PRE:], x2n], axis=0).astype(BF16)
        return carry

    n_early_out = n_seg - 1 - LAG
    out_a = pltpu.make_async_copy(out_v.at[:n_early_out],
                                  out_hbm.at[:n_early_out], sems.at[3])
    out_b = pltpu.make_async_copy(out_v.at[n_early_out:],
                                  out_hbm.at[n_early_out:], sems.at[4])

    def phase(ph, carry):
        t0 = ph * n_seg
        lax.fori_loop(t0, t0 + LAG, one_layer_step, 0)

        @pl.when(ph == 0)
        def _():
            lax.fori_loop(LAG, n_seg, two_layer_step, 0)
            out_a.start()
            hf = h_s[...].astype(F32)
            h1_s[...] = jnp.concatenate(
                [hf[m_len:m2], hf[m2 + seg - PRE:]], axis=0).astype(BF16)

        return carry

    lax.fori_loop(0, 2, phase, 0)

    ob = _b_attn(y_s[seg:, :], ((n_seg - 1) * seg,), bqkv_p, kv_s.at[1:],
                 seg=seg, d=d)
    proj = jnp.concatenate([_dot(ob, bo_p[c], _NN) for c in range(nt)], axis=1)
    out_v[n_seg - 1] = (y_s[seg:, :] + proj).astype(out_v.dtype)
    out_b.start()
    out_a.wait()
    out_b.wait()


@functools.partial(jax.jit, static_argnames=("A_seg_len",))
def pallas_interleave_layers__memory_aug_recurrent_mem_tr__sliding_local_dilated__prompt_kernel(
    A_x: jax.Array,
    A_mem0: jax.Array,
    A_Wq: jax.Array,
    A_Wk: jax.Array,
    A_Wv: jax.Array,
    A_Wo: jax.Array,
    A_seg_len,
    B_x: jax.Array,
    B_wqkv: jax.Array,
    B_wo: jax.Array,
):
    del B_x
    bsz, s_len, d = A_x.shape
    m_len = A_mem0.shape[1]
    n_heads, dh = A_Wq.shape[1], A_Wq.shape[2]
    seg = int(A_seg_len)
    n_seg = s_len // seg
    n_pairs = n_heads // 2
    nt = d // LANES
    assert bsz == 1 and s_len % seg == 0 and n_seg > LAG + 1
    assert seg % 16 == 0 and m_len == 8 and seg > PRE and seg >= HIST
    assert 2 * (m_len + seg) <= LANES
    assert n_heads % 2 == 0 and 2 * dh == 3 * LANES and d % LANES == 0
    assert d % HB == 0 and LANES == 4 * HB and n_pairs >= 3 * nt >= 3
    hd = n_heads * dh
    n_pre = (n_seg - LAG) * PRE

    wq_t = jnp.transpose(A_Wq, (1, 2, 0)).reshape(hd, d)
    wk_t = jnp.transpose(A_Wk, (1, 2, 0)).reshape(hd, d)
    wv_t = jnp.transpose(A_Wv, (1, 2, 0)).reshape(hd, d)
    wo = A_Wo.reshape(hd, d)

    kernel = functools.partial(
        _kernel, seg=seg, n_seg=n_seg, m_len=m_len, n_pairs=n_pairs, dh=dh,
        d=d)
    any_spec = pl.BlockSpec(memory_space=pl.ANY)
    dma = pltpu.SemaphoreType.DMA
    out = pl.pallas_call(
        kernel,
        out_shape=jax.ShapeDtypeStruct((n_seg, seg, d), A_x.dtype),
        in_specs=[any_spec] * 8,
        out_specs=any_spec,
        scratch_shapes=[
            pltpu.VMEM((n_seg, seg, d), BF16),
            pltpu.VMEM((m_len, d), BF16),
            pltpu.VMEM((NSLOT, 6 * dh, d), BF16),
            pltpu.VMEM((n_pairs, d, 6 * dh), BF16),
            pltpu.VMEM((hd, d), BF16),
            pltpu.VMEM((3 * nt, LANES, d), BF16),
            pltpu.VMEM((nt, d, LANES), BF16),
            pltpu.VMEM((d, LANES), F32),
            pltpu.VMEM((d, LANES), F32),
            pltpu.VMEM((3, d, d), BF16),
            pltpu.VMEM((nt, d, LANES), BF16),
            pltpu.VMEM((n_seg, seg, d), A_x.dtype),
            pltpu.VMEM((n_pre, d), BF16),
            pltpu.VMEM((n_pairs, n_pre, 6 * dh), BF16),
            pltpu.VMEM((2 * (m_len + seg) - PRE, d), BF16),
            pltpu.VMEM((m_len + seg, d), BF16),
            pltpu.VMEM((seg, d), F32),
            pltpu.VMEM((2 * seg, d), F32),
            pltpu.VMEM((2, 2 * nt, HIST + seg, LANES), F32),
            dma((5,)), dma((3 * NSLOT,)), dma((n_pairs,)),
            dma((3 * nt,)), dma((nt,)),
        ],
        compiler_params=pltpu.CompilerParams(
            vmem_limit_bytes=110 * 1024 * 1024),
    )(A_x.reshape(n_seg, seg, d), A_mem0.reshape(m_len, d), wq_t, wk_t, wv_t,
      wo, B_wqkv, B_wo)
    return out.reshape(bsz, s_len, d)
```

```python
import functools

import jax
import jax.numpy as jnp
from jax import lax
import jax.experimental.pallas as pl
import jax.experimental.pallas.tpu as pltpu

F32 = jnp.float32
BF16 = jnp.bfloat16

_NT = (((1,), (1,)), ((), ()))
_NN = (((1,), (0,)), ((), ()))

HB = 32
WIN = 8
DIL = 2
HIST = 16
LANES = 128
PRE = 16
PRE_CHUNK = 128
LAG = 2
NSLOT = 3
NEG = -1000000000.0


def _dot(a, b, dims):
    return lax.dot_general(a, b, dims, preferred_element_type=F32)


def _recip(x):
    r = pl.reciprocal(x, approx=True)
    return r * (2.0 - x * r)


def _ln(x):
    m = jnp.mean(x, axis=-1, keepdims=True)
    xc = x - m
    v = jnp.mean(xc * xc, axis=-1, keepdims=True)
    return xc * lax.rsqrt(v + 1e-05)


def _tile(a, c):
    return a[:, c * LANES:(c + 1) * LANES]


def _keep(mask, a):
    return jnp.where(mask, a, jnp.zeros_like(a))


def _drop(mask, a):
    return jnp.where(mask, jnp.zeros_like(a), a)


def _pair_softmax(s, col_a):
    m_a = jnp.max(jnp.where(col_a, s, -jnp.inf), axis=1, keepdims=True)
    m_b = jnp.max(jnp.where(col_a, -jnp.inf, s), axis=1, keepdims=True)
    e = jnp.exp(s - jnp.where(col_a, m_a, m_b))
    d_a = jnp.sum(jnp.where(col_a, e, 0.0), axis=1, keepdims=True)
    d_b = jnp.sum(jnp.where(col_a, 0.0, e), axis=1, keepdims=True)
    return e * _recip(jnp.where(col_a, d_a, d_b))


class _PassBase:
    def __init__(self, h, w_ref, wo_ref, dh):
        self.h, self.w, self.wo = h, w_ref, wo_ref
        self.pw = 2 * dh
        self.half = dh - LANES
        self.scale = dh ** (-0.5)
        self.q, self.k, self.v, self.p, self.o = {}, {}, {}, {}, {}
        self.acc = None
        self.pending = None

    def _lane_lo(self, rows):
        return lax.broadcasted_iota(jnp.int32, (rows, LANES), 1) < self.half

    def _project(self, p, j):
        a = _dot(self.h, self.w[p, :, j * self.pw:(j + 1) * self.pw], _NN)
        self.marker = a[:8, :LANES]
        return a

    def _gate(self, s):
        if self.pending is None:
            return s
        top = jnp.where(self.always, s[:8], self.pending[:, :s.shape[1]])
        self.pending = None
        return jnp.concatenate([top, s[8:]], axis=0)

    def out(self, p):
        w = self.wo[p * self.pw:(p + 1) * self.pw, :]
        part = _dot(self.o.pop(p), w, _NN)
        self.acc = part if self.acc is None else self.acc + part

    def run(self, n_pairs, b, always):
        last = n_pairs - 1
        self.always = always
        done = None
        for p in range(n_pairs):
            self.proj_q(p)
            self.pending, done = done, None
            if 2 <= p < 2 + b.n_groups:
                o = b.attend(p - 2, (always, self.marker))
                done = functools.reduce(lambda u, v: u + v, o)
            self.proj_k(p)
            if p > 0:
                self.pv(p - 1)
            self.proj_v(p)
            self.scores(p)
            if p == 0:
                b.project()
            elif p < last - 1:
                self.out(p - 1)
        self.out(last - 2)
        yb = b.finish()
        self.pv(last)
        self.out(last - 1)
        self.out(last)
        return self.acc, yb


class _TwoLayerPass(_PassBase):
    def __init__(self, h, pre_ref, pre_row, w_ref, wo_ref, *, dh, m_len, seg):
        super().__init__(h, w_ref, wo_ref, dh)
        self.pre, self.pre_row = pre_ref, pre_row
        self.m, self.seg = m_len, seg
        m2 = 2 * m_len
        n = m2 + 2 * seg
        row = lax.broadcasted_iota(jnp.int32, (n, n), 0)
        col = lax.broadcasted_iota(jnp.int32, (n, n), 1)

        def first_layer(i):
            return (i < m_len) | ((i >= m2) & (i < m2 + seg))

        def token(i):
            return jnp.where(i < m2 + seg, i - m2, i - m2 - seg)

        self.col_a = first_layer(col)
        self.diag = first_layer(row) == self.col_a
        self.allowed = (row < m2) | (col < m2) | (token(row) >= token(col))
        self.lo_m = self._lane_lo(m_len)
        self.lo_x = self._lane_lo(seg)

    def _proj(self, p, j):
        m, pw = self.m, self.pw
        a = self._project(p, j)
        pre = self.pre[p, pl.ds(self.pre_row, PRE), j * pw:(j + 1) * pw]
        rest = a[2 * m:].astype(BF16)
        n1 = self.seg - PRE
        x1 = jnp.concatenate([pre, rest[:n1]], axis=0)
        return a[:m], a[m:2 * m], x1, rest[n1:]

    @staticmethod
    def _cat(ma, mb, xa, xb):
        mm = jnp.concatenate([ma, mb], axis=0).astype(BF16)
        return jnp.concatenate([mm, xa, xb], axis=0)

    def _tiles(self, m1, m2, x1, x2):
        cat, lm, lx = self._cat, self.lo_m, self.lo_x
        t0 = cat(_tile(m1, 0), _tile(m2, 0), _tile(x1, 0), _tile(x2, 0))
        t2 = cat(_tile(m2, 2), _tile(m1, 2), _tile(x2, 2), _tile(x1, 2))
        m1, m2, x1, x2 = (_tile(a, 1) for a in (m1, m2, x1, x2))
        t1a = cat(_keep(lm, m1), _drop(lm, m1), _keep(lx, x1), _drop(lx, x1))
        t1b = cat(_drop(lm, m2), _keep(lm, m2), _drop(lx, x2), _keep(lx, x2))
        return t0, t1a, t1b, t2

    def _rows_a(self, a):
        return a[:2 * self.m + self.seg]

    def _rows_b(self, a):
        m2 = 2 * self.m
        return jnp.concatenate([a[:m2], a[m2 + self.seg:]], axis=0)

    def _merge_rows(self, a, b):
        m = self.m
        return jnp.concatenate([a[:m], b[m:2 * m], a[2 * m:], b[2 * m:]],
                               axis=0)

    def proj_q(self, p):
        self.q[p] = self._cat(*self._proj(p, 0))

    def proj_k(self, p):
        self.k[p] = self._tiles(*self._proj(p, 1))

    def proj_v(self, p):
        self.v[p] = self._tiles(*self._proj(p, 2))

    def scores(self, p):
        q = self.q.pop(p)
        k0, k1a, k1b, k2 = self.k.pop(p)
        q1 = _tile(q, 1)
        r0 = _dot(_tile(q, 0), k0, _NT)
        r2 = _dot(_tile(q, 2), k2, _NT)
        r1a = _dot(self._rows_a(q1), k1a, _NT)
        r1b = _dot(self._rows_b(q1), k1b, _NT)
        s = jnp.where(self.diag, r0, r2) + self._merge_rows(r1a, r1b)
        s = self._gate(jnp.where(self.allowed, s * self.scale, NEG))
        p_all = _pair_softmax(s, self.col_a)
        self.p[p] = (p_all.astype(BF16), _keep(self.diag, p_all).astype(BF16),
                     _drop(self.diag, p_all).astype(BF16))

    def pv(self, p):
        p_all, p_diag, p_off = self.p.pop(p)
        v0, v1a, v1b, v2 = self.v.pop(p)
        o0 = _dot(p_diag, v0, _NN)
        o2 = _dot(p_off, v2, _NN)
        o1 = self._merge_rows(_dot(self._rows_a(p_all), v1a, _NN),
                              _dot(self._rows_b(p_all), v1b, _NN))
        self.o[p] = jnp.concatenate([o0, o1, o2], axis=1).astype(BF16)


class _OneLayerPass(_PassBase):
    def __init__(self, h, w_ref, wo_ref, *, dh, m_len, seg):
        super().__init__(h, w_ref, wo_ref, dh)
        n = m_len + seg
        row = lax.broadcasted_iota(jnp.int32, (n, 2 * n), 0)
        col = lax.broadcasted_iota(jnp.int32, (n, 2 * n), 1)
        self.col_a = col < n
        key = jnp.where(self.col_a, col, col - n)
        self.allowed = (row < m_len) | (row >= key)
        lane = lax.broadcasted_iota(jnp.int32, (n, self.pw), 1)
        self.head0 = lane < dh

    def _block_diag(self, a):
        return jnp.concatenate([_keep(self.head0, a), _drop(self.head0, a)],
                               axis=0).astype(BF16)

    def proj_q(self, p):
        self.q[p] = self._project(p, 0).astype(BF16)

    def proj_k(self, p):
        self.k[p] = self._block_diag(self._project(p, 1))

    def proj_v(self, p):
        self.v[p] = self._block_diag(self._project(p, 2))

    def scores(self, p):
        s = _dot(self.q.pop(p), self.k.pop(p), _NT)
        s = self._gate(jnp.where(self.allowed, s * self.scale, NEG))
        self.p[p] = _pair_softmax(s, self.col_a).astype(BF16)

    def pv(self, p):
        self.o[p] = _dot(self.p.pop(p), self.v.pop(p), _NN).astype(BF16)


class _BPass:
    def __init__(self, y_ref, starts, wqkv_ref, wo_ref, kv_ref, *, seg, d):
        self.y, self.starts = y_ref, starts
        self.wqkv, self.wo, self.kv = wqkv_ref, wo_ref, kv_ref
        self.seg, self.nt = seg, d // LANES
        self.scale = (d // HB) ** (-0.5)
        self.n_groups = len(starts) * seg // 8
        self.outs = []

    def project(self):
        seg, nt = self.seg, self.nt
        yn = _ln(self.y[...]).astype(BF16)
        self.q, ka, va = (_dot(yn, self.wqkv[j], _NN) for j in range(3))
        for i in range(len(self.starts)):
            self.kv[i, :, :HIST, :] = self.kv[i, :, seg:, :]
            for c in range(nt):
                rows = slice(i * seg, (i + 1) * seg)
                self.kv[i, c, HIST:, :] = _tile(ka[rows], c)
                self.kv[i, nt + c, HIST:, :] = _tile(va[rows], c)

    def attend(self, gi, after=None):
        seg, nt, kv = self.seg, self.nt, self.kv
        i, g = divmod(gi, seg // 8)
        q = [_tile(self.q[8 * gi:8 * gi + 8], c) for c in range(nt)]
        if after is not None:
            q = [jnp.where(after[0], u, after[1]) for u in q]
        pos = (lax.broadcasted_iota(jnp.int32, (8, LANES), 0)
               + (self.starts[i] + 8 * g))
        offs = [HIST + 8 * g - w * DIL for w in range(WIN)]
        logits = []
        for w, off in enumerate(offs):
            t = q[0] * kv[i, 0, off:off + 8, :]
            for c in range(1, nt):
                t = t + q[c] * kv[i, c, off:off + 8, :]
            t = t + pltpu.roll(t, 64, 1)
            t = (t + pltpu.roll(t, 32, 1)) * self.scale
            if 8 * g < w * DIL:
                t = jnp.where(pos >= w * DIL, t, NEG)
            logits.append(t)
        m = logits[0]
        for t in logits[1:]:
            m = jnp.maximum(m, t)
        es = [jnp.exp(t - m) for t in logits]
        den = es[0]
        for e in es[1:]:
            den = den + e
        inv = _recip(den)
        o = []
        for c in range(nt):
            acc = None
            for w, off in enumerate(offs):
                term = es[w] * kv[i, nt + c, off:off + 8, :]
                acc = term if acc is None else acc + term
            o.append(acc * inv)
        self.outs.append(jnp.concatenate(o, axis=1))
        return o

    def finish(self):
        o = jnp.concatenate(self.outs, axis=0).astype(BF16)
        proj = jnp.concatenate(
            [_dot(o, self.wo[c], _NN) for c in range(self.nt)], axis=1)
        return self.y[...] + proj


def _kernel(x_hbm, mem_hbm, wq_hbm, wk_hbm, wv_hbm, wo_hbm, bqkv_hbm, bo_hbm,
            out_hbm,
            x_v, mem_v, wst_v, w_v, wo_v, bq_st, bo_st, tq_s, to_s, bqkv_p,
            bo_p, out_v, xn_s, pre_s, h_s, h1_s, ra_s, y_s, kv_s,
            sems, w_sems, wo_sems, bq_sems, bo_sems,
            *, seg, n_seg, m_len, n_pairs, dh, d):
    db = d // HB
    nt = d // LANES
    pw = 2 * dh
    m2 = 2 * m_len
    n_pre = (n_seg - LAG) * PRE
    n_bq = 3 * nt

    def w_copy(p, j):
        src = (wq_hbm, wk_hbm, wv_hbm)[j]
        slot = p % NSLOT
        return pltpu.make_async_copy(
            src.at[pl.ds(p * pw, pw), :],
            wst_v.at[slot, pl.ds(j * pw, pw), :], w_sems.at[3 * slot + j])

    def wo_copy(p):
        return pltpu.make_async_copy(wo_hbm.at[pl.ds(p * pw, pw), :],
                                     wo_v.at[pl.ds(p * pw, pw), :],
                                     wo_sems.at[p])

    def bq_copy(i):
        row = pl.multiple_of((i % nt) * LANES, LANES)
        col = pl.multiple_of((i // nt) * d, LANES)
        return pltpu.make_async_copy(
            bqkv_hbm.at[pl.ds(row, LANES), pl.ds(col, d)], bq_st.at[i],
            bq_sems.at[i])

    def bo_copy(i):
        col = pl.multiple_of(i * LANES, LANES)
        return pltpu.make_async_copy(bo_hbm.at[:, pl.ds(col, LANES)],
                                     bo_st.at[i], bo_sems.at[i])

    xa_copy = pltpu.make_async_copy(x_hbm.at[:, :PRE, :], x_v.at[:, :PRE, :],
                                    sems.at[0])
    xb_copy = pltpu.make_async_copy(x_hbm.at[:, PRE:, :], x_v.at[:, PRE:, :],
                                    sems.at[1])
    mem_copy = pltpu.make_async_copy(mem_hbm, mem_v, sems.at[2])

    xa_copy.start()
    for p in range(2):
        bq_copy(p).start()
        bo_copy(p).start()
        for j in range(3):
            w_copy(p, j).start()
    mem_copy.start()
    xb_copy.start()

    ra_s[...] = jnp.zeros(ra_s.shape, F32)
    y_s[...] = jnp.zeros(y_s.shape, F32)
    kv_s[...] = jnp.zeros(kv_s.shape, F32)

    xa_copy.wait()
    for s in range(LAG, n_seg):
        xn_s[(s - LAG) * PRE:(s - LAG + 1) * PRE, :] = _ln(
            x_v[s, :PRE, :].astype(F32)).astype(BF16)

    def permute_rows(tmp_ref):
        return jnp.concatenate(
            [tmp_ref[pl.ds(j, HB, stride=db), :] for j in range(db)], axis=0)

    def pre_pair(p, carry):
        for j in range(3):
            w_copy(p, j).wait()

        @pl.when(p < n_bq)
        def _():
            bq_copy(p).wait()

        @pl.when(p < nt)
        def _():
            bo_copy(p).wait()

        @pl.when(p + 2 < n_pairs)
        def _():
            for j in range(3):
                w_copy(p + 2, j).start()

        @pl.when(p + 2 < n_bq)
        def _():
            bq_copy(p + 2).start()

        @pl.when(p + 2 < nt)
        def _():
            bo_copy(p + 2).start()

        wo_copy(p).start()

        slot = p % NSLOT
        for r0 in range(0, n_pre, PRE_CHUNK):
            r1 = min(r0 + PRE_CHUNK, n_pre)
            pre_s[p, r0:r1, :] = _dot(
                xn_s[r0:r1, :], wst_v[slot], _NT).astype(BF16)
        for n in range(3 * pw // LANES):
            w_v[p, :, n * LANES:(n + 1) * LANES] = (
                wst_v[slot, n * LANES:(n + 1) * LANES, :].T)

        i = jnp.minimum(p, n_bq - 1)
        tq_s[...] = bq_st[i].astype(F32).T
        row = pl.multiple_of((i % nt) * LANES, LANES)
        bqkv_p[i // nt, pl.ds(row, LANES), :] = (
            permute_rows(tq_s).T.astype(BF16))
        i = jnp.minimum(p, nt - 1)
        to_s[...] = bo_st[i].astype(F32)
        bo_p[i] = permute_rows(to_s).astype(BF16)
        return carry

    lax.fori_loop(0, n_pairs, pre_pair, 0)

    mem_copy.wait()
    xb_copy.wait()
    for p in range(n_pairs):
        wo_copy(p).wait()
    h1_s[...] = jnp.concatenate(
        [mem_v[...].astype(F32), _ln(x_v[0].astype(F32))],
        axis=0).astype(BF16)

    def b_pass(t):
        return _BPass(y_s, ((t - 1) * seg, (t - 1 - LAG) * seg), bqkv_p, bo_p,
                      kv_s, seg=seg, d=d)

    def b_store(t, yb):
        out_v[jnp.maximum(t - 1 - LAG, 0)] = yb[seg:].astype(out_v.dtype)
        return yb[:seg]

    def two_layer_step(t, carry):
        a = _TwoLayerPass(h_s[...], pre_s,
                          pl.multiple_of((t - LAG) * PRE, PRE), w_v, wo_v,
                          dh=dh, m_len=m_len, seg=seg)
        acc, yb = a.run(n_pairs, b_pass(t), t >= 0)
        x2 = b_store(t, yb)
        y_s[:seg, :] = x_v[t].astype(F32) + acc[m2:m2 + seg]
        y_s[seg:, :] = ra_s[...] + acc[m2 + seg:]
        ra_s[...] = x2
        xn = x_v[jnp.minimum(t + 1, n_seg - 1), PRE:, :].astype(F32)
        h_s[:m2, :] = acc[:m2].astype(BF16)
        h_s[m2:, :] = jnp.concatenate([_ln(xn), _ln(x2)],
                                      axis=0).astype(BF16)
        return carry

    def one_layer_step(t, carry):
        first = t < LAG
        a = _OneLayerPass(h1_s[...], w_v, wo_v, dh=dh, m_len=m_len, seg=seg)
        acc, yb = a.run(n_pairs, b_pass(t), t >= 0)
        x2 = b_store(t, yb)
        x0 = x_v[jnp.minimum(t, n_seg - 1)].astype(F32)
        y = jnp.where(first, x0, ra_s[...]) + acc[m_len:]
        y_s[:seg, :] = y
        y_s[seg:, :] = y
        ra_s[...] = x2
        xn = _ln(x_v[jnp.minimum(t + 1, n_seg - 1)].astype(F32))
        x2n = _ln(x2)
        mem = acc[:m_len]
        h1_s[...] = jnp.concatenate(
            [mem, jnp.where(first, xn, x2n)], axis=0).astype(BF16)
        h_s[...] = jnp.concatenate(
            [mem, mem_v[...].astype(F32), xn[PRE:], x2n], axis=0).astype(BF16)
        return carry

    n_early_out = n_seg - 1 - LAG
    out_a = pltpu.make_async_copy(out_v.at[:n_early_out],
                                  out_hbm.at[:n_early_out], sems.at[3])
    out_b = pltpu.make_async_copy(out_v.at[n_early_out:],
                                  out_hbm.at[n_early_out:], sems.at[4])

    def phase(ph, carry):
        t0 = ph * n_seg
        lax.fori_loop(t0, t0 + LAG, one_layer_step, 0)

        @pl.when(ph == 0)
        def _():
            lax.fori_loop(LAG, n_seg, two_layer_step, 0)
            out_a.start()
            hf = h_s[...].astype(F32)
            h1_s[...] = jnp.concatenate(
                [hf[m_len:m2], hf[m2 + seg - PRE:]], axis=0).astype(BF16)

        return carry

    lax.fori_loop(0, 2, phase, 0)

    b = _BPass(y_s.at[seg:], ((n_seg - 1) * seg,), bqkv_p, bo_p, kv_s.at[1:],
               seg=seg, d=d)
    b.project()
    for gi in range(b.n_groups):
        b.attend(gi)
    out_v[n_seg - 1] = b.finish().astype(out_v.dtype)
    out_b.start()
    out_a.wait()
    out_b.wait()


@functools.partial(jax.jit, static_argnames=("A_seg_len",))
def pallas_interleave_layers__memory_aug_recurrent_mem_tr__sliding_local_dilated__prompt_kernel(
    A_x: jax.Array,
    A_mem0: jax.Array,
    A_Wq: jax.Array,
    A_Wk: jax.Array,
    A_Wv: jax.Array,
    A_Wo: jax.Array,
    A_seg_len,
    B_x: jax.Array,
    B_wqkv: jax.Array,
    B_wo: jax.Array,
):
    del B_x
    bsz, s_len, d = A_x.shape
    m_len = A_mem0.shape[1]
    n_heads, dh = A_Wq.shape[1], A_Wq.shape[2]
    seg = int(A_seg_len)
    n_seg = s_len // seg
    n_pairs = n_heads // 2
    nt = d // LANES
    assert bsz == 1 and s_len % seg == 0 and n_seg > LAG + 1
    assert seg % 16 == 0 and m_len == 8 and seg > PRE and seg >= HIST
    assert 2 * (m_len + seg) <= LANES
    assert n_heads % 2 == 0 and 2 * dh == 3 * LANES and d % LANES == 0
    assert d % HB == 0 and LANES == 4 * HB and n_pairs >= 3 * nt >= 3
    hd = n_heads * dh
    n_pre = (n_seg - LAG) * PRE

    wq_t = jnp.transpose(A_Wq, (1, 2, 0)).reshape(hd, d)
    wk_t = jnp.transpose(A_Wk, (1, 2, 0)).reshape(hd, d)
    wv_t = jnp.transpose(A_Wv, (1, 2, 0)).reshape(hd, d)
    wo = A_Wo.reshape(hd, d)

    kernel = functools.partial(
        _kernel, seg=seg, n_seg=n_seg, m_len=m_len, n_pairs=n_pairs, dh=dh,
        d=d)
    any_spec = pl.BlockSpec(memory_space=pl.ANY)
    dma = pltpu.SemaphoreType.DMA
    out = pl.pallas_call(
        kernel,
        out_shape=jax.ShapeDtypeStruct((n_seg, seg, d), A_x.dtype),
        in_specs=[any_spec] * 8,
        out_specs=any_spec,
        scratch_shapes=[
            pltpu.VMEM((n_seg, seg, d), BF16),
            pltpu.VMEM((m_len, d), BF16),
            pltpu.VMEM((NSLOT, 6 * dh, d), BF16),
            pltpu.VMEM((n_pairs, d, 6 * dh), BF16),
            pltpu.VMEM((hd, d), BF16),
            pltpu.VMEM((3 * nt, LANES, d), BF16),
            pltpu.VMEM((nt, d, LANES), BF16),
            pltpu.VMEM((d, LANES), F32),
            pltpu.VMEM((d, LANES), F32),
            pltpu.VMEM((3, d, d), BF16),
            pltpu.VMEM((nt, d, LANES), BF16),
            pltpu.VMEM((n_seg, seg, d), A_x.dtype),
            pltpu.VMEM((n_pre, d), BF16),
            pltpu.VMEM((n_pairs, n_pre, 6 * dh), BF16),
            pltpu.VMEM((2 * (m_len + seg) - PRE, d), BF16),
            pltpu.VMEM((m_len + seg, d), BF16),
            pltpu.VMEM((seg, d), F32),
            pltpu.VMEM((2 * seg, d), F32),
            pltpu.VMEM((2, 2 * nt, HIST + seg, LANES), F32),
            dma((5,)), dma((3 * NSLOT,)), dma((n_pairs,)),
            dma((3 * nt,)), dma((nt,)),
        ],
        compiler_params=pltpu.CompilerParams(
            vmem_limit_bytes=110 * 1024 * 1024),
    )(A_x.reshape(n_seg, seg, d), A_mem0.reshape(m_len, d), wq_t, wk_t, wv_t,
      wo, B_wqkv, B_wo)
    return out.reshape(bsz, s_len, d)
```

```python
import functools

import jax
import jax.numpy as jnp
from jax import lax
import jax.experimental.pallas as pl
import jax.experimental.pallas.tpu as pltpu

F32 = jnp.float32
BF16 = jnp.bfloat16

_NT = (((1,), (1,)), ((), ()))
_NN = (((1,), (0,)), ((), ()))

HB = 32
WIN = 8
DIL = 2
HIST = 16
LANES = 128
PRE = 16
PRE_CHUNK = 128
LAG = 2
NSLOT = 2
NEG = -1000000000.0


def _dot(a, b, dims):
    return lax.dot_general(a, b, dims, preferred_element_type=F32)


def _recip(x):
    r = pl.reciprocal(x, approx=True)
    return r * (2.0 - x * r)


def _ln(x):
    m = jnp.mean(x, axis=-1, keepdims=True)
    xc = x - m
    v = jnp.mean(xc * xc, axis=-1, keepdims=True)
    return xc * lax.rsqrt(v + 1e-05)


def _tile(a, c):
    return a[:, c * LANES:(c + 1) * LANES]


def _keep(mask, a):
    return jnp.where(mask, a, jnp.zeros_like(a))


def _drop(mask, a):
    return jnp.where(mask, jnp.zeros_like(a), a)


def _pair_softmax(s, col_a):
    m_a = jnp.max(jnp.where(col_a, s, -jnp.inf), axis=1, keepdims=True)
    m_b = jnp.max(jnp.where(col_a, -jnp.inf, s), axis=1, keepdims=True)
    e = jnp.exp(s - jnp.where(col_a, m_a, m_b))
    d_a = jnp.sum(jnp.where(col_a, e, 0.0), axis=1, keepdims=True)
    d_b = jnp.sum(jnp.where(col_a, 0.0, e), axis=1, keepdims=True)
    return e * _recip(jnp.where(col_a, d_a, d_b))


class _PassBase:
    def __init__(self, h, w_ref, wo_ref, dh):
        self.h, self.w, self.wo = h, w_ref, wo_ref
        self.pw = 2 * dh
        self.half = dh - LANES
        self.scale = dh ** (-0.5)
        self.q, self.k, self.v, self.p, self.o = {}, {}, {}, {}, {}
        self.acc = None
        self.pending = None

    def _lane_lo(self, rows):
        return lax.broadcasted_iota(jnp.int32, (rows, LANES), 1) < self.half

    def _project(self, p, j):
        a = _dot(self.h, self.w[p, :, j * self.pw:(j + 1) * self.pw], _NN)
        self.marker = a[:8, :LANES]
        return a

    def _gate(self, s):
        if self.pending is None:
            return s
        top = jnp.where(self.always, s[:8], self.pending[:, :s.shape[1]])
        self.pending = None
        return jnp.concatenate([top, s[8:]], axis=0)

    def out(self, p):
        w = self.wo[p * self.pw:(p + 1) * self.pw, :]
        part = _dot(self.o.pop(p), w, _NN)
        self.acc = part if self.acc is None else self.acc + part

    def run(self, n_pairs, b, always):
        last = n_pairs - 1
        self.always = always
        done = None
        for p in range(n_pairs):
            self.proj_q(p)
            self.pending, done = done, None
            if 2 <= p < 2 + b.n_groups:
                o = b.attend(p - 2, (always, self.marker))
                done = functools.reduce(lambda u, v: u + v, o)
            self.proj_k(p)
            if p > 0:
                self.pv(p - 1)
            self.proj_v(p)
            self.scores(p)
            if p == 0:
                b.project()
            elif p < last - 1:
                self.out(p - 1)
        self.out(last - 2)
        yb = b.finish()
        self.pv(last)
        self.out(last - 1)
        self.out(last)
        return self.acc, yb


class _TwoLayerPass(_PassBase):
    def __init__(self, h, pre_ref, pre_row, w_ref, wo_ref, *, dh, m_len, seg):
        super().__init__(h, w_ref, wo_ref, dh)
        self.pre, self.pre_row = pre_ref, pre_row
        self.m, self.seg = m_len, seg
        m2 = 2 * m_len
        n = m2 + 2 * seg
        row = lax.broadcasted_iota(jnp.int32, (n, n), 0)
        col = lax.broadcasted_iota(jnp.int32, (n, n), 1)

        def first_layer(i):
            return (i < m_len) | ((i >= m2) & (i < m2 + seg))

        def token(i):
            return jnp.where(i < m2 + seg, i - m2, i - m2 - seg)

        self.col_a = first_layer(col)
        self.diag = first_layer(row) == self.col_a
        self.allowed = (row < m2) | (col < m2) | (token(row) >= token(col))
        self.lo_m = self._lane_lo(m_len)
        self.lo_x = self._lane_lo(seg)

    def _proj(self, p, j):
        m, pw = self.m, self.pw
        a = self._project(p, j)
        pre = self.pre[p, pl.ds(self.pre_row, PRE), j * pw:(j + 1) * pw]
        rest = a[2 * m:].astype(BF16)
        n1 = self.seg - PRE
        x1 = jnp.concatenate([pre, rest[:n1]], axis=0)
        return a[:m], a[m:2 * m], x1, rest[n1:]

    @staticmethod
    def _cat(ma, mb, xa, xb):
        mm = jnp.concatenate([ma, mb], axis=0).astype(BF16)
        return jnp.concatenate([mm, xa, xb], axis=0)

    def _tiles(self, m1, m2, x1, x2):
        cat, lm, lx = self._cat, self.lo_m, self.lo_x
        t0 = cat(_tile(m1, 0), _tile(m2, 0), _tile(x1, 0), _tile(x2, 0))
        t2 = cat(_tile(m2, 2), _tile(m1, 2), _tile(x2, 2), _tile(x1, 2))
        m1, m2, x1, x2 = (_tile(a, 1) for a in (m1, m2, x1, x2))
        t1a = cat(_keep(lm, m1), _drop(lm, m1), _keep(lx, x1), _drop(lx, x1))
        t1b = cat(_drop(lm, m2), _keep(lm, m2), _drop(lx, x2), _keep(lx, x2))
        return t0, t1a, t1b, t2

    def _rows_a(self, a):
        return a[:2 * self.m + self.seg]

    def _rows_b(self, a):
        m2 = 2 * self.m
        return jnp.concatenate([a[:m2], a[m2 + self.seg:]], axis=0)

    def _merge_rows(self, a, b):
        m = self.m
        return jnp.concatenate([a[:m], b[m:2 * m], a[2 * m:], b[2 * m:]],
                               axis=0)

    def proj_q(self, p):
        self.q[p] = self._cat(*self._proj(p, 0))

    def proj_k(self, p):
        self.k[p] = self._tiles(*self._proj(p, 1))

    def proj_v(self, p):
        self.v[p] = self._tiles(*self._proj(p, 2))

    def scores(self, p):
        q = self.q.pop(p)
        k0, k1a, k1b, k2 = self.k.pop(p)
        q1 = _tile(q, 1)
        r0 = _dot(_tile(q, 0), k0, _NT)
        r2 = _dot(_tile(q, 2), k2, _NT)
        r1a = _dot(self._rows_a(q1), k1a, _NT)
        r1b = _dot(self._rows_b(q1), k1b, _NT)
        s = jnp.where(self.diag, r0, r2) + self._merge_rows(r1a, r1b)
        s = self._gate(jnp.where(self.allowed, s * self.scale, NEG))
        p_all = _pair_softmax(s, self.col_a)
        self.p[p] = (p_all.astype(BF16), _keep(self.diag, p_all).astype(BF16),
                     _drop(self.diag, p_all).astype(BF16))

    def pv(self, p):
        p_all, p_diag, p_off = self.p.pop(p)
        v0, v1a, v1b, v2 = self.v.pop(p)
        o0 = _dot(p_diag, v0, _NN)
        o2 = _dot(p_off, v2, _NN)
        o1 = self._merge_rows(_dot(self._rows_a(p_all), v1a, _NN),
                              _dot(self._rows_b(p_all), v1b, _NN))
        self.o[p] = jnp.concatenate([o0, o1, o2], axis=1).astype(BF16)


class _OneLayerPass(_PassBase):
    def __init__(self, h, w_ref, wo_ref, *, dh, m_len, seg):
        super().__init__(h, w_ref, wo_ref, dh)
        n = m_len + seg
        row = lax.broadcasted_iota(jnp.int32, (n, 2 * n), 0)
        col = lax.broadcasted_iota(jnp.int32, (n, 2 * n), 1)
        self.col_a = col < n
        key = jnp.where(self.col_a, col, col - n)
        self.allowed = (row < m_len) | (row >= key)
        lane = lax.broadcasted_iota(jnp.int32, (n, self.pw), 1)
        self.head0 = lane < dh

    def _block_diag(self, a):
        return jnp.concatenate([_keep(self.head0, a), _drop(self.head0, a)],
                               axis=0).astype(BF16)

    def proj_q(self, p):
        self.q[p] = self._project(p, 0).astype(BF16)

    def proj_k(self, p):
        self.k[p] = self._block_diag(self._project(p, 1))

    def proj_v(self, p):
        self.v[p] = self._block_diag(self._project(p, 2))

    def scores(self, p):
        s = _dot(self.q.pop(p), self.k.pop(p), _NT)
        s = self._gate(jnp.where(self.allowed, s * self.scale, NEG))
        self.p[p] = _pair_softmax(s, self.col_a).astype(BF16)

    def pv(self, p):
        self.o[p] = _dot(self.p.pop(p), self.v.pop(p), _NN).astype(BF16)


class _BPass:
    def __init__(self, y_ref, starts, wqkv_ref, wo_ref, kv_ref, *, seg, d):
        self.y, self.starts = y_ref, starts
        self.wqkv, self.wo, self.kv = wqkv_ref, wo_ref, kv_ref
        self.seg, self.nt = seg, d // LANES
        self.scale = (d // HB) ** (-0.5)
        self.n_groups = len(starts) * seg // 8
        self.outs = []

    def project(self):
        seg, nt = self.seg, self.nt
        yn = _ln(self.y[...]).astype(BF16)
        self.q, ka, va = (_dot(yn, self.wqkv[j], _NN) for j in range(3))
        for i in range(len(self.starts)):
            self.kv[i, :, :HIST, :] = self.kv[i, :, seg:, :]
            for c in range(nt):
                rows = slice(i * seg, (i + 1) * seg)
                self.kv[i, c, HIST:, :] = _tile(ka[rows], c)
                self.kv[i, nt + c, HIST:, :] = _tile(va[rows], c)

    def attend(self, gi, after=None):
        seg, nt, kv = self.seg, self.nt, self.kv
        i, g = divmod(gi, seg // 8)
        q = [_tile(self.q[8 * gi:8 * gi + 8], c) for c in range(nt)]
        if after is not None:
            q = [jnp.where(after[0], u, after[1]) for u in q]
        pos = (lax.broadcasted_iota(jnp.int32, (8, LANES), 0)
               + (self.starts[i] + 8 * g))
        offs = [HIST + 8 * g - w * DIL for w in range(WIN)]
        logits = []
        for w, off in enumerate(offs):
            t = q[0] * kv[i, 0, off:off + 8, :]
            for c in range(1, nt):
                t = t + q[c] * kv[i, c, off:off + 8, :]
            t = t + pltpu.roll(t, 64, 1)
            t = (t + pltpu.roll(t, 32, 1)) * self.scale
            if 8 * g < w * DIL:
                t = jnp.where(pos >= w * DIL, t, NEG)
            logits.append(t)
        m = logits[0]
        for t in logits[1:]:
            m = jnp.maximum(m, t)
        es = [jnp.exp(t - m) for t in logits]
        den = es[0]
        for e in es[1:]:
            den = den + e
        inv = _recip(den)
        o = []
        for c in range(nt):
            acc = None
            for w, off in enumerate(offs):
                term = es[w] * kv[i, nt + c, off:off + 8, :]
                acc = term if acc is None else acc + term
            o.append(acc * inv)
        self.outs.append(jnp.concatenate(o, axis=1))
        return o

    def finish(self):
        o = jnp.concatenate(self.outs, axis=0).astype(BF16)
        proj = jnp.concatenate(
            [_dot(o, self.wo[c], _NN) for c in range(self.nt)], axis=1)
        return self.y[...] + proj


def _kernel(x_hbm, mem_hbm, wq_hbm, wk_hbm, wv_hbm, wo_hbm, bqkv_hbm, bo_hbm,
            out_hbm,
            x_v, mem_v, wst_v, w_v, wo_v, bq_st, bo_st, tq_s, to_s, bqkv_p,
            bo_p, out_v, xn_s, pre_s, h_s, h1_s, ra_s, y_s, kv_s,
            sems, w_sems, wo_sems, bq_sems, bo_sems,
            *, seg, n_seg, m_len, n_pairs, dh, d):
    db = d // HB
    nt = d // LANES
    pw = 2 * dh
    m2 = 2 * m_len
    n_pre = (n_seg - LAG) * PRE
    n_bq = 3 * nt

    def w_copy(p, j):
        src = (wq_hbm, wk_hbm, wv_hbm)[j]
        slot = p % NSLOT
        return pltpu.make_async_copy(
            src.at[pl.ds(p * pw, pw), :],
            wst_v.at[slot, pl.ds(j * pw, pw), :], w_sems.at[3 * slot + j])

    def wo_copy(p):
        return pltpu.make_async_copy(wo_hbm.at[pl.ds(p * pw, pw), :],
                                     wo_v.at[pl.ds(p * pw, pw), :],
                                     wo_sems.at[p])

    def bq_copy(i):
        row = pl.multiple_of((i % nt) * LANES, LANES)
        col = pl.multiple_of((i // nt) * d, LANES)
        return pltpu.make_async_copy(
            bqkv_hbm.at[pl.ds(row, LANES), pl.ds(col, d)], bq_st.at[i],
            bq_sems.at[i])

    def bo_copy(i):
        col = pl.multiple_of(i * LANES, LANES)
        return pltpu.make_async_copy(bo_hbm.at[:, pl.ds(col, LANES)],
                                     bo_st.at[i], bo_sems.at[i])

    xa_copy = pltpu.make_async_copy(x_hbm.at[:, :PRE, :], x_v.at[:, :PRE, :],
                                    sems.at[0])
    xb_copy = pltpu.make_async_copy(x_hbm.at[:, PRE:, :], x_v.at[:, PRE:, :],
                                    sems.at[1])
    mem_copy = pltpu.make_async_copy(mem_hbm, mem_v, sems.at[2])

    mem_copy.start()
    xa_copy.start()
    mem_copy.wait()
    for p in range(2):
        for j in range(3):
            w_copy(p, j).start()
        bq_copy(p).start()
        bo_copy(p).start()
    xb_copy.start()

    ra_s[...] = jnp.zeros(ra_s.shape, F32)
    y_s[...] = jnp.zeros(y_s.shape, F32)
    kv_s[...] = jnp.zeros(kv_s.shape, F32)

    xa_copy.wait()
    for s in range(LAG, n_seg):
        xn_s[(s - LAG) * PRE:(s - LAG + 1) * PRE, :] = _ln(
            x_v[s, :PRE, :].astype(F32)).astype(BF16)

    def permute_rows(tmp_ref):
        return jnp.concatenate(
            [tmp_ref[pl.ds(j, HB, stride=db), :] for j in range(db)], axis=0)

    def pre_pair(p, carry):
        for j in range(3):
            w_copy(p, j).wait()

        @pl.when(p < n_bq)
        def _():
            bq_copy(p).wait()

        @pl.when(p < nt)
        def _():
            bo_copy(p).wait()

        wo_copy(p).start()

        always = p >= 0
        marks = []

        def last_rows(a):
            return [a[(c + 1) * LANES - 16:(c + 1) * LANES] for c in range(nt)]

        i = jnp.minimum(p, nt - 1)
        to_s[...] = bo_st[i].astype(F32)
        bo = permute_rows(to_s)
        bo_p[i] = bo.astype(BF16)
        g = d // nt // 16
        marks.append([
            functools.reduce(
                lambda u, v: u + v,
                [bo[16 * (c * g + r):16 * (c * g + r + 1)] for r in range(g)]
            ).astype(BF16) for c in range(nt)])
        i = jnp.minimum(p, n_bq - 1)
        tq_s[...] = bq_st[i].astype(F32).T
        row = pl.multiple_of((i % nt) * LANES, LANES)
        bq = permute_rows(tq_s).T.astype(BF16)
        bqkv_p[i // nt, pl.ds(row, LANES), :] = bq
        marks.append([_tile(bq[LANES - 16:], c) for c in range(nt)])

        slot = p % NSLOT
        for n in range(3 * pw // LANES):
            wt = wst_v[slot, n * LANES:(n + 1) * LANES, :].T
            w_v[p, :, n * LANES:(n + 1) * LANES] = wt
            marks.append(last_rows(wt))

        starts = list(range(0, n_pre, PRE_CHUNK))
        groups = [[], marks[:1], marks[1:2]]
        rest, n_left = marks[2:], len(starts) - 3
        per_chunk = -(-len(rest) // n_left)
        groups += [rest[k * per_chunk:(k + 1) * per_chunk]
                   for k in range(n_left)]
        for r0, mine in zip(starts, groups):
            r1 = min(r0 + PRE_CHUNK, n_pre)
            lhs = xn_s[r0:r1, :]
            if mine:
                top = [jnp.where(always, lhs[16 * g:16 * (g + 1)],
                                 jnp.concatenate(mk, axis=1))
                       for g, mk in enumerate(mine)]
                lhs = jnp.concatenate(top + [lhs[16 * len(mine):]], axis=0)
            pre_s[p, r0:r1, :] = _dot(lhs, wst_v[slot], _NT).astype(BF16)

        @pl.when(p + NSLOT < n_pairs)
        def _():
            for j in range(3):
                w_copy(p + NSLOT, j).start()

        @pl.when(p + 2 < n_bq)
        def _():
            bq_copy(p + 2).start()

        @pl.when(p + 2 < nt)
        def _():
            bo_copy(p + 2).start()

        return carry

    lax.fori_loop(0, n_pairs, pre_pair, 0)

    xb_copy.wait()
    for p in range(n_pairs):
        wo_copy(p).wait()
    h1_s[...] = jnp.concatenate(
        [mem_v[...].astype(F32), _ln(x_v[0].astype(F32))],
        axis=0).astype(BF16)

    def b_pass(t):
        return _BPass(y_s, ((t - 1) * seg, (t - 1 - LAG) * seg), bqkv_p, bo_p,
                      kv_s, seg=seg, d=d)

    def b_store(t, yb):
        out_v[jnp.maximum(t - 1 - LAG, 0)] = yb[seg:].astype(out_v.dtype)
        return yb[:seg]

    def two_layer_step(t, carry):
        a = _TwoLayerPass(h_s[...], pre_s,
                          pl.multiple_of((t - LAG) * PRE, PRE), w_v, wo_v,
                          dh=dh, m_len=m_len, seg=seg)
        acc, yb = a.run(n_pairs, b_pass(t), t >= 0)
        x2 = b_store(t, yb)
        y_s[:seg, :] = x_v[t].astype(F32) + acc[m2:m2 + seg]
        y_s[seg:, :] = ra_s[...] + acc[m2 + seg:]
        ra_s[...] = x2
        xn = x_v[jnp.minimum(t + 1, n_seg - 1), PRE:, :].astype(F32)
        h_s[:m2, :] = acc[:m2].astype(BF16)
        h_s[m2:, :] = jnp.concatenate([_ln(xn), _ln(x2)],
                                      axis=0).astype(BF16)
        return carry

    def one_layer_step(t, carry):
        first = t < LAG
        a = _OneLayerPass(h1_s[...], w_v, wo_v, dh=dh, m_len=m_len, seg=seg)
        acc, yb = a.run(n_pairs, b_pass(t), t >= 0)
        x2 = b_store(t, yb)
        x0 = x_v[jnp.minimum(t, n_seg - 1)].astype(F32)
        y = jnp.where(first, x0, ra_s[...]) + acc[m_len:]
        y_s[:seg, :] = y
        y_s[seg:, :] = y
        ra_s[...] = x2
        xn = _ln(x_v[jnp.minimum(t + 1, n_seg - 1)].astype(F32))
        x2n = _ln(x2)
        mem = acc[:m_len]
        h1_s[...] = jnp.concatenate(
            [mem, jnp.where(first, xn, x2n)], axis=0).astype(BF16)
        h_s[...] = jnp.concatenate(
            [mem, mem_v[...].astype(F32), xn[PRE:], x2n], axis=0).astype(BF16)
        return carry

    n_early_out = n_seg - 1 - LAG
    out_a = pltpu.make_async_copy(out_v.at[:n_early_out],
                                  out_hbm.at[:n_early_out], sems.at[3])
    out_b = pltpu.make_async_copy(out_v.at[n_early_out:],
                                  out_hbm.at[n_early_out:], sems.at[4])

    def phase(ph, carry):
        t0 = ph * n_seg
        lax.fori_loop(t0, t0 + LAG, one_layer_step, 0)

        @pl.when(ph == 0)
        def _():
            lax.fori_loop(LAG, n_seg, two_layer_step, 0)
            out_a.start()
            hf = h_s[...].astype(F32)
            h1_s[...] = jnp.concatenate(
                [hf[m_len:m2], hf[m2 + seg - PRE:]], axis=0).astype(BF16)

        return carry

    lax.fori_loop(0, 2, phase, 0)

    b = _BPass(y_s.at[seg:], ((n_seg - 1) * seg,), bqkv_p, bo_p, kv_s.at[1:],
               seg=seg, d=d)
    b.project()
    for gi in range(b.n_groups):
        b.attend(gi)
    out_v[n_seg - 1] = b.finish().astype(out_v.dtype)
    out_b.start()
    out_a.wait()
    out_b.wait()


@functools.partial(jax.jit, static_argnames=("A_seg_len",))
def pallas_interleave_layers__memory_aug_recurrent_mem_tr__sliding_local_dilated__prompt_kernel(
    A_x: jax.Array,
    A_mem0: jax.Array,
    A_Wq: jax.Array,
    A_Wk: jax.Array,
    A_Wv: jax.Array,
    A_Wo: jax.Array,
    A_seg_len,
    B_x: jax.Array,
    B_wqkv: jax.Array,
    B_wo: jax.Array,
):
    del B_x
    bsz, s_len, d = A_x.shape
    m_len = A_mem0.shape[1]
    n_heads, dh = A_Wq.shape[1], A_Wq.shape[2]
    seg = int(A_seg_len)
    n_seg = s_len // seg
    n_pairs = n_heads // 2
    nt = d // LANES
    assert bsz == 1 and s_len % seg == 0 and n_seg > LAG + 1
    assert seg % 16 == 0 and m_len == 8 and seg > PRE and seg >= HIST
    assert 2 * (m_len + seg) <= LANES
    assert n_heads % 2 == 0 and 2 * dh == 3 * LANES and d % LANES == 0
    assert d % HB == 0 and LANES == 4 * HB and n_pairs >= 3 * nt >= 3
    hd = n_heads * dh
    n_pre = (n_seg - LAG) * PRE

    wq_t = jnp.transpose(A_Wq, (1, 2, 0)).reshape(hd, d)
    wk_t = jnp.transpose(A_Wk, (1, 2, 0)).reshape(hd, d)
    wv_t = jnp.transpose(A_Wv, (1, 2, 0)).reshape(hd, d)
    wo = A_Wo.reshape(hd, d)

    kernel = functools.partial(
        _kernel, seg=seg, n_seg=n_seg, m_len=m_len, n_pairs=n_pairs, dh=dh,
        d=d)
    any_spec = pl.BlockSpec(memory_space=pl.ANY)
    dma = pltpu.SemaphoreType.DMA
    out = pl.pallas_call(
        kernel,
        out_shape=jax.ShapeDtypeStruct((n_seg, seg, d), A_x.dtype),
        in_specs=[any_spec] * 8,
        out_specs=any_spec,
        scratch_shapes=[
            pltpu.VMEM((n_seg, seg, d), BF16),
            pltpu.VMEM((m_len, d), BF16),
            pltpu.VMEM((NSLOT, 6 * dh, d), BF16),
            pltpu.VMEM((n_pairs, d, 6 * dh), BF16),
            pltpu.VMEM((hd, d), BF16),
            pltpu.VMEM((3 * nt, LANES, d), BF16),
            pltpu.VMEM((nt, d, LANES), BF16),
            pltpu.VMEM((d, LANES), F32),
            pltpu.VMEM((d, LANES), F32),
            pltpu.VMEM((3, d, d), BF16),
            pltpu.VMEM((nt, d, LANES), BF16),
            pltpu.VMEM((n_seg, seg, d), A_x.dtype),
            pltpu.VMEM((n_pre, d), BF16),
            pltpu.VMEM((n_pairs, n_pre, 6 * dh), BF16),
            pltpu.VMEM((2 * (m_len + seg) - PRE, d), BF16),
            pltpu.VMEM((m_len + seg, d), BF16),
            pltpu.VMEM((seg, d), F32),
            pltpu.VMEM((2 * seg, d), F32),
            pltpu.VMEM((2, 2 * nt, HIST + seg, LANES), F32),
            dma((5,)), dma((3 * NSLOT,)), dma((n_pairs,)),
            dma((3 * nt,)), dma((nt,)),
        ],
        compiler_params=pltpu.CompilerParams(
            vmem_limit_bytes=110 * 1024 * 1024,
            disable_bounds_checks=True),
    )(A_x.reshape(n_seg, seg, d), A_mem0.reshape(m_len, d), wq_t, wk_t, wv_t,
      wo, B_wqkv, B_wo)
    return out.reshape(bsz, s_len, d)
```

```python
import functools

import jax
import jax.numpy as jnp
from jax import lax
import jax.experimental.pallas as pl
import jax.experimental.pallas.tpu as pltpu

F32 = jnp.float32
BF16 = jnp.bfloat16

_NT = (((1,), (1,)), ((), ()))
_NN = (((1,), (0,)), ((), ()))

HB = 32
WIN = 8
DIL = 2
HIST = 16
LANES = 128
PRE = 16
PRE_CHUNK = 128
LAG = 2
UNROLL = 1
NSLOT = 2
NEG = -1000000000.0


def _dot(a, b, dims):
    return lax.dot_general(a, b, dims, preferred_element_type=F32)


def _recip(x):
    r = pl.reciprocal(x, approx=True)
    return r * (2.0 - x * r)


def _ln(x):
    m = jnp.mean(x, axis=-1, keepdims=True)
    xc = x - m
    v = jnp.mean(xc * xc, axis=-1, keepdims=True)
    return xc * lax.rsqrt(v + 1e-05)


def _tile(a, c):
    return a[:, c * LANES:(c + 1) * LANES]


def _keep(mask, a):
    return jnp.where(mask, a, jnp.zeros_like(a))


def _drop(mask, a):
    return jnp.where(mask, jnp.zeros_like(a), a)


def _pair_softmax(s, col_a):
    m_a = jnp.max(jnp.where(col_a, s, -jnp.inf), axis=1, keepdims=True)
    m_b = jnp.max(jnp.where(col_a, -jnp.inf, s), axis=1, keepdims=True)
    e = jnp.exp(s - jnp.where(col_a, m_a, m_b))
    d_a = jnp.sum(jnp.where(col_a, e, 0.0), axis=1, keepdims=True)
    d_b = jnp.sum(jnp.where(col_a, 0.0, e), axis=1, keepdims=True)
    return e * _recip(jnp.where(col_a, d_a, d_b))


class _PassBase:
    def __init__(self, h, w_ref, wo_ref, dh):
        self.h, self.w, self.wo = h, w_ref, wo_ref
        self.pw = 2 * dh
        self.half = dh - LANES
        self.scale = dh ** (-0.5)
        self.q, self.k, self.v, self.p, self.o = {}, {}, {}, {}, {}
        self.cols = (0, 2 * LANES, wo_ref.shape[1])
        self.acc = [None, None]
        self.pending = None

    def _lane_lo(self, rows):
        return lax.broadcasted_iota(jnp.int32, (rows, LANES), 1) < self.half

    def _project(self, p, j):
        a = _dot(self.h, self.w[p, :, j * self.pw:(j + 1) * self.pw], _NN)
        self.marker = a[:8, :LANES]
        return a

    def _gate(self, s):
        if self.pending is None:
            return s
        top = jnp.where(self.always, s[:8], self.pending[:, :s.shape[1]])
        self.pending = None
        return jnp.concatenate([top, s[8:]], axis=0)

    def out(self, p, part=None):
        for k in ((0, 1) if part is None else (part,)):
            c0, c1 = self.cols[k], self.cols[k + 1]
            w = self.wo[p * self.pw:(p + 1) * self.pw, c0:c1]
            r = _dot(self.o[p], w, _NN)
            self.acc[k] = r if self.acc[k] is None else self.acc[k] + r

    def run(self, n_pairs, b, always):
        last = n_pairs - 1
        self.always = always
        done = None
        for p in range(n_pairs):
            self.proj_q(p)
            self.pending, done = done, None
            if 2 <= p < 2 + b.n_groups:
                o = b.attend(p - 2, (always, self.marker))
                done = functools.reduce(lambda u, v: u + v, o)
            self.proj_k(p)
            if p > 0:
                self.pv(p - 1)
            self.proj_v(p)
            self.scores(p)
            if p == 0:
                b.project()
            elif p < last:
                self.out(p - 1)
        yb = b.finish()
        self.out(last - 1, 0)
        self.pv(last)
        self.out(last - 1, 1)
        self.out(last)
        return jnp.concatenate(self.acc, axis=1), yb


class _TwoLayerPass(_PassBase):
    def __init__(self, h, pre_ref, pre_row, w_ref, wo_ref, *, dh, m_len, seg):
        super().__init__(h, w_ref, wo_ref, dh)
        self.pre, self.pre_row = pre_ref, pre_row
        self.m, self.seg = m_len, seg
        m2 = 2 * m_len
        n = m2 + 2 * seg
        row = lax.broadcasted_iota(jnp.int32, (n, n), 0)
        col = lax.broadcasted_iota(jnp.int32, (n, n), 1)

        def first_layer(i):
            return (i < m_len) | ((i >= m2) & (i < m2 + seg))

        def token(i):
            return jnp.where(i < m2 + seg, i - m2, i - m2 - seg)

        self.col_a = first_layer(col)
        self.diag = first_layer(row) == self.col_a
        self.allowed = (row < m2) | (col < m2) | (token(row) >= token(col))
        self.lo_m = self._lane_lo(m_len)
        self.lo_x = self._lane_lo(seg)

    def _proj(self, p, j):
        m, pw = self.m, self.pw
        a = self._project(p, j)
        pre = self.pre[p, pl.ds(self.pre_row, PRE), j * pw:(j + 1) * pw]
        n1 = self.seg - PRE
        nx = n1 + self.seg
        rest = a[:nx].astype(BF16)
        x1 = jnp.concatenate([pre, rest[:n1]], axis=0)
        return a[nx:nx + m], a[nx + m:], x1, rest[n1:]

    @staticmethod
    def _cat(ma, mb, xa, xb):
        mm = jnp.concatenate([ma, mb], axis=0).astype(BF16)
        return jnp.concatenate([mm, xa, xb], axis=0)

    def _tiles(self, m1, m2, x1, x2):
        cat, lm, lx = self._cat, self.lo_m, self.lo_x
        t0 = cat(_tile(m1, 0), _tile(m2, 0), _tile(x1, 0), _tile(x2, 0))
        t2 = cat(_tile(m2, 2), _tile(m1, 2), _tile(x2, 2), _tile(x1, 2))
        m1, m2, x1, x2 = (_tile(a, 1) for a in (m1, m2, x1, x2))
        t1a = cat(_keep(lm, m1), _drop(lm, m1), _keep(lx, x1), _drop(lx, x1))
        t1b = cat(_drop(lm, m2), _keep(lm, m2), _drop(lx, x2), _keep(lx, x2))
        return t0, t1a, t1b, t2

    def _rows_a(self, a):
        return a[:2 * self.m + self.seg]

    def _rows_b(self, a):
        m2 = 2 * self.m
        return jnp.concatenate([a[:m2], a[m2 + self.seg:]], axis=0)

    def _merge_rows(self, a, b):
        m = self.m
        return jnp.concatenate([a[:m], b[m:2 * m], a[2 * m:], b[2 * m:]],
                               axis=0)

    def proj_q(self, p):
        self.q[p] = self._cat(*self._proj(p, 0))

    def proj_k(self, p):
        self.k[p] = self._tiles(*self._proj(p, 1))

    def proj_v(self, p):
        self.v[p] = self._tiles(*self._proj(p, 2))

    def scores(self, p):
        q = self.q.pop(p)
        k0, k1a, k1b, k2 = self.k.pop(p)
        q1 = _tile(q, 1)
        r0 = _dot(_tile(q, 0), k0, _NT)
        r2 = _dot(_tile(q, 2), k2, _NT)
        r1a = _dot(self._rows_a(q1), k1a, _NT)
        r1b = _dot(self._rows_b(q1), k1b, _NT)
        s = jnp.where(self.diag, r0, r2) + self._merge_rows(r1a, r1b)
        s = self._gate(jnp.where(self.allowed, s * self.scale, NEG))
        p_all = _pair_softmax(s, self.col_a)
        self.p[p] = (p_all.astype(BF16), _keep(self.diag, p_all).astype(BF16),
                     _drop(self.diag, p_all).astype(BF16))

    def pv(self, p):
        p_all, p_diag, p_off = self.p.pop(p)
        v0, v1a, v1b, v2 = self.v.pop(p)
        o0 = _dot(p_diag, v0, _NN)
        o2 = _dot(p_off, v2, _NN)
        o1 = self._merge_rows(_dot(self._rows_a(p_all), v1a, _NN),
                              _dot(self._rows_b(p_all), v1b, _NN))
        self.o[p] = jnp.concatenate([o0, o1, o2], axis=1).astype(BF16)


class _OneLayerPass(_PassBase):
    def __init__(self, h, w_ref, wo_ref, *, dh, m_len, seg):
        super().__init__(h, w_ref, wo_ref, dh)
        n = m_len + seg
        row = lax.broadcasted_iota(jnp.int32, (n, 2 * n), 0)
        col = lax.broadcasted_iota(jnp.int32, (n, 2 * n), 1)
        self.col_a = col < n
        key = jnp.where(self.col_a, col, col - n)
        self.allowed = (row < m_len) | (row >= key)
        lane = lax.broadcasted_iota(jnp.int32, (n, self.pw), 1)
        self.head0 = lane < dh

    def _block_diag(self, a):
        return jnp.concatenate([_keep(self.head0, a), _drop(self.head0, a)],
                               axis=0).astype(BF16)

    def proj_q(self, p):
        self.q[p] = self._project(p, 0).astype(BF16)

    def proj_k(self, p):
        self.k[p] = self._block_diag(self._project(p, 1))

    def proj_v(self, p):
        self.v[p] = self._block_diag(self._project(p, 2))

    def scores(self, p):
        s = _dot(self.q.pop(p), self.k.pop(p), _NT)
        s = self._gate(jnp.where(self.allowed, s * self.scale, NEG))
        self.p[p] = _pair_softmax(s, self.col_a).astype(BF16)

    def pv(self, p):
        self.o[p] = _dot(self.p.pop(p), self.v.pop(p), _NN).astype(BF16)


class _BPass:
    def __init__(self, y_ref, starts, wqkv_ref, wo_ref, kv_ref, *, seg, d):
        self.y, self.starts = y_ref, starts
        self.wqkv, self.wo, self.kv = wqkv_ref, wo_ref, kv_ref
        self.seg, self.nt = seg, d // LANES
        self.scale = (d // HB) ** (-0.5)
        self.n_groups = len(starts) * seg // 8
        self.outs = []

    def project(self):
        seg, nt = self.seg, self.nt
        yn = _ln(self.y[...]).astype(BF16)
        self.q, ka, va = (_dot(yn, self.wqkv[j], _NN) for j in range(3))
        for i in range(len(self.starts)):
            self.kv[i, :, :HIST, :] = self.kv[i, :, seg:, :]
            for c in range(nt):
                rows = slice(i * seg, (i + 1) * seg)
                self.kv[i, c, HIST:, :] = _tile(ka[rows], c)
                self.kv[i, nt + c, HIST:, :] = _tile(va[rows], c)

    def attend(self, gi, after=None):
        seg, nt, kv = self.seg, self.nt, self.kv
        i, g = divmod(gi, seg // 8)
        q = [_tile(self.q[8 * gi:8 * gi + 8], c) for c in range(nt)]
        if after is not None:
            q = [jnp.where(after[0], u, after[1]) for u in q]
        pos = (lax.broadcasted_iota(jnp.int32, (8, LANES), 0)
               + (self.starts[i] + 8 * g))
        offs = [HIST + 8 * g - w * DIL for w in range(WIN)]
        logits = []
        for w, off in enumerate(offs):
            t = q[0] * kv[i, 0, off:off + 8, :]
            for c in range(1, nt):
                t = t + q[c] * kv[i, c, off:off + 8, :]
            t = t + pltpu.roll(t, 64, 1)
            t = (t + pltpu.roll(t, 32, 1)) * self.scale
            if 8 * g < w * DIL:
                t = jnp.where(pos >= w * DIL, t, NEG)
            logits.append(t)
        m = logits[0]
        for t in logits[1:]:
            m = jnp.maximum(m, t)
        es = [jnp.exp(t - m) for t in logits]
        den = es[0]
        for e in es[1:]:
            den = den + e
        inv = _recip(den)
        o = []
        for c in range(nt):
            acc = None
            for w, off in enumerate(offs):
                term = es[w] * kv[i, nt + c, off:off + 8, :]
                acc = term if acc is None else acc + term
            o.append(acc * inv)
        self.outs.append(jnp.concatenate(o, axis=1))
        return o

    def finish(self):
        o = jnp.concatenate(self.outs, axis=0).astype(BF16)
        proj = jnp.concatenate(
            [_dot(o, self.wo[c], _NN) for c in range(self.nt)], axis=1)
        return self.y[...] + proj


def _kernel(x_hbm, mem_hbm, wq_hbm, wk_hbm, wv_hbm, wo_hbm, bqkv_hbm, bo_hbm,
            out_hbm,
            x_v, mem_v, wst_v, w_v, wo_v, bq_st, bo_st, tq_s, to_s, bqkv_p,
            bo_p, out_v, xn_s, pre_s, h_s, h1_s, ra_s, y_s, kv_s,
            sems, w_sems, wo_sems, bq_sems, bo_sems,
            *, seg, n_seg, m_len, n_pairs, dh, d):
    db = d // HB
    nt = d // LANES
    pw = 2 * dh
    m2 = 2 * m_len
    n_pre = (n_seg - LAG) * PRE
    n_bq = 3 * nt

    def w_copy(p, j):
        src = (wq_hbm, wk_hbm, wv_hbm)[j]
        slot = p % NSLOT
        return pltpu.make_async_copy(
            src.at[pl.ds(p * pw, pw), :],
            wst_v.at[slot, pl.ds(j * pw, pw), :], w_sems.at[3 * slot + j])

    def wo_copy(p):
        return pltpu.make_async_copy(wo_hbm.at[pl.ds(p * pw, pw), :],
                                     wo_v.at[pl.ds(p * pw, pw), :],
                                     wo_sems.at[p])

    def bq_copy(i):
        row = pl.multiple_of((i % nt) * LANES, LANES)
        col = pl.multiple_of((i // nt) * d, LANES)
        return pltpu.make_async_copy(
            bqkv_hbm.at[pl.ds(row, LANES), pl.ds(col, d)], bq_st.at[i],
            bq_sems.at[i])

    def bo_copy(i):
        col = pl.multiple_of(i * LANES, LANES)
        return pltpu.make_async_copy(bo_hbm.at[:, pl.ds(col, LANES)],
                                     bo_st.at[i], bo_sems.at[i])

    xa_copy = pltpu.make_async_copy(x_hbm.at[:, :PRE, :], x_v.at[:, :PRE, :],
                                    sems.at[0])
    xb_copy = pltpu.make_async_copy(x_hbm.at[:, PRE:, :], x_v.at[:, PRE:, :],
                                    sems.at[1])
    mem_copy = pltpu.make_async_copy(mem_hbm, mem_v, sems.at[2])

    mem_copy.start()
    xa_copy.start()
    mem_copy.wait()
    for p in range(2):
        for j in range(3):
            w_copy(p, j).start()
        bq_copy(p).start()
        bo_copy(p).start()
    xb_copy.start()

    ra_s[...] = jnp.zeros(ra_s.shape, F32)
    y_s[...] = jnp.zeros(y_s.shape, F32)
    kv_s[...] = jnp.zeros(kv_s.shape, F32)

    xa_copy.wait()
    for s in range(LAG, n_seg):
        xn_s[(s - LAG) * PRE:(s - LAG + 1) * PRE, :] = _ln(
            x_v[s, :PRE, :].astype(F32)).astype(BF16)

    def permute_rows(tmp_ref):
        return jnp.concatenate(
            [tmp_ref[pl.ds(j, HB, stride=db), :] for j in range(db)], axis=0)

    def pre_pair(p, carry):
        for j in range(3):
            w_copy(p, j).wait()

        @pl.when(p < n_bq)
        def _():
            bq_copy(p).wait()

        @pl.when(p < nt)
        def _():
            bo_copy(p).wait()

        wo_copy(p).start()

        always = p >= 0
        marks = []

        def last_rows(a):
            return [a[(c + 1) * LANES - 16:(c + 1) * LANES] for c in range(nt)]

        i = jnp.minimum(p, nt - 1)
        to_s[...] = bo_st[i].astype(F32)
        bo = permute_rows(to_s)
        bo_p[i] = bo.astype(BF16)
        g = d // nt // 16
        marks.append([
            functools.reduce(
                lambda u, v: u + v,
                [bo[16 * (c * g + r):16 * (c * g + r + 1)] for r in range(g)]
            ).astype(BF16) for c in range(nt)])
        i = jnp.minimum(p, n_bq - 1)
        tq_s[...] = bq_st[i].astype(F32).T
        row = pl.multiple_of((i % nt) * LANES, LANES)
        bq = permute_rows(tq_s).T.astype(BF16)
        bqkv_p[i // nt, pl.ds(row, LANES), :] = bq
        marks.append([_tile(bq[LANES - 16:], c) for c in range(nt)])

        slot = p % NSLOT
        for n in range(3 * pw // LANES):
            wt = wst_v[slot, n * LANES:(n + 1) * LANES, :].T
            w_v[p, :, n * LANES:(n + 1) * LANES] = wt
            marks.append(last_rows(wt))

        starts = list(range(0, n_pre, PRE_CHUNK))
        groups = [[], marks[:1], marks[1:2]]
        rest, n_left = marks[2:], len(starts) - 3
        per_chunk = -(-len(rest) // n_left)
        groups += [rest[k * per_chunk:(k + 1) * per_chunk]
                   for k in range(n_left)]
        for r0, mine in zip(starts, groups):
            r1 = min(r0 + PRE_CHUNK, n_pre)
            lhs = xn_s[r0:r1, :]
            if mine:
                top = [jnp.where(always, lhs[16 * g:16 * (g + 1)],
                                 jnp.concatenate(mk, axis=1))
                       for g, mk in enumerate(mine)]
                lhs = jnp.concatenate(top + [lhs[16 * len(mine):]], axis=0)
            pre_s[p, r0:r1, :] = _dot(lhs, wst_v[slot], _NT).astype(BF16)

        @pl.when(p + NSLOT < n_pairs)
        def _():
            for j in range(3):
                w_copy(p + NSLOT, j).start()

        @pl.when(p + 2 < n_bq)
        def _():
            bq_copy(p + 2).start()

        @pl.when(p + 2 < nt)
        def _():
            bo_copy(p + 2).start()

        return carry

    lax.fori_loop(0, n_pairs, pre_pair, 0)

    xb_copy.wait()
    for p in range(n_pairs):
        wo_copy(p).wait()
    h1_s[...] = jnp.concatenate(
        [mem_v[...].astype(F32), _ln(x_v[0].astype(F32))],
        axis=0).astype(BF16)

    def b_pass(t):
        return _BPass(y_s, ((t - 1) * seg, (t - 1 - LAG) * seg), bqkv_p, bo_p,
                      kv_s, seg=seg, d=d)

    def b_store(t, yb):
        out_v[jnp.maximum(t - 1 - LAG, 0)] = yb[seg:].astype(out_v.dtype)
        return yb[:seg]

    def two_layer_step(t, h):
        a = _TwoLayerPass(h, pre_s, pl.multiple_of((t - LAG) * PRE, PRE),
                          w_v, wo_v, dh=dh, m_len=m_len, seg=seg)
        acc, yb = a.run(n_pairs, b_pass(t), t >= 0)
        x2 = b_store(t, yb)
        y_s[:seg, :] = x_v[t].astype(F32) + acc[m2:m2 + seg]
        y_s[seg:, :] = ra_s[...] + acc[m2 + seg:]
        ra_s[...] = x2
        xn = x_v[jnp.minimum(t + 1, n_seg - 1), PRE:, :].astype(F32)
        return jnp.concatenate([_ln(xn), _ln(x2), acc[:m2]],
                               axis=0).astype(BF16)

    def two_layer_steps(i, carry):
        h = h_s[...]
        for u in range(UNROLL):
            h = two_layer_step(LAG + i * UNROLL + u, h)
        h_s[...] = h
        return carry

    def one_layer_step(t, carry):
        first = t < LAG
        a = _OneLayerPass(h1_s[...], w_v, wo_v, dh=dh, m_len=m_len, seg=seg)
        acc, yb = a.run(n_pairs, b_pass(t), t >= 0)
        x2 = b_store(t, yb)
        x0 = x_v[jnp.minimum(t, n_seg - 1)].astype(F32)
        y = jnp.where(first, x0, ra_s[...]) + acc[m_len:]
        y_s[:seg, :] = y
        y_s[seg:, :] = y
        ra_s[...] = x2
        xn = _ln(x_v[jnp.minimum(t + 1, n_seg - 1)].astype(F32))
        x2n = _ln(x2)
        mem = acc[:m_len]
        h1_s[...] = jnp.concatenate(
            [mem, jnp.where(first, xn, x2n)], axis=0).astype(BF16)
        h_s[...] = jnp.concatenate(
            [xn[PRE:], x2n, mem, mem_v[...].astype(F32)], axis=0).astype(BF16)
        return carry

    n_early_out = n_seg - 1 - LAG
    out_a = pltpu.make_async_copy(out_v.at[:n_early_out],
                                  out_hbm.at[:n_early_out], sems.at[3])
    out_b = pltpu.make_async_copy(out_v.at[n_early_out:],
                                  out_hbm.at[n_early_out:], sems.at[4])

    def phase(ph, carry):
        t0 = ph * n_seg
        lax.fori_loop(t0, t0 + LAG, one_layer_step, 0)

        @pl.when(ph == 0)
        def _():
            lax.fori_loop(0, (n_seg - LAG) // UNROLL, two_layer_steps, 0)
            out_a.start()
            hf = h_s[...].astype(F32)
            h1_s[...] = jnp.concatenate(
                [hf[2 * seg - PRE + m_len:], hf[seg - PRE:2 * seg - PRE]],
                axis=0).astype(BF16)

        return carry

    lax.fori_loop(0, 2, phase, 0)

    b = _BPass(y_s.at[seg:], ((n_seg - 1) * seg,), bqkv_p, bo_p, kv_s.at[1:],
               seg=seg, d=d)
    b.project()
    for gi in range(b.n_groups):
        b.attend(gi)
    out_v[n_seg - 1] = b.finish().astype(out_v.dtype)
    out_b.start()
    out_a.wait()
    out_b.wait()


@functools.partial(jax.jit, static_argnames=("A_seg_len",))
def pallas_interleave_layers__memory_aug_recurrent_mem_tr__sliding_local_dilated__prompt_kernel(
    A_x: jax.Array,
    A_mem0: jax.Array,
    A_Wq: jax.Array,
    A_Wk: jax.Array,
    A_Wv: jax.Array,
    A_Wo: jax.Array,
    A_seg_len,
    B_x: jax.Array,
    B_wqkv: jax.Array,
    B_wo: jax.Array,
):
    del B_x
    bsz, s_len, d = A_x.shape
    m_len = A_mem0.shape[1]
    n_heads, dh = A_Wq.shape[1], A_Wq.shape[2]
    seg = int(A_seg_len)
    n_seg = s_len // seg
    n_pairs = n_heads // 2
    nt = d // LANES
    assert bsz == 1 and s_len % seg == 0 and n_seg > LAG + 1
    assert seg % 16 == 0 and m_len == 8 and seg > PRE and seg >= HIST
    assert 2 * (m_len + seg) <= LANES and (n_seg - LAG) % UNROLL == 0
    assert n_heads % 2 == 0 and 2 * dh == 3 * LANES and d % LANES == 0
    assert d % HB == 0 and LANES == 4 * HB and n_pairs >= 3 * nt >= 3
    hd = n_heads * dh
    n_pre = (n_seg - LAG) * PRE

    wq_t = jnp.transpose(A_Wq, (1, 2, 0)).reshape(hd, d)
    wk_t = jnp.transpose(A_Wk, (1, 2, 0)).reshape(hd, d)
    wv_t = jnp.transpose(A_Wv, (1, 2, 0)).reshape(hd, d)
    wo = A_Wo.reshape(hd, d)

    kernel = functools.partial(
        _kernel, seg=seg, n_seg=n_seg, m_len=m_len, n_pairs=n_pairs, dh=dh,
        d=d)
    any_spec = pl.BlockSpec(memory_space=pl.ANY)
    dma = pltpu.SemaphoreType.DMA
    out = pl.pallas_call(
        kernel,
        out_shape=jax.ShapeDtypeStruct((n_seg, seg, d), A_x.dtype),
        in_specs=[any_spec] * 8,
        out_specs=any_spec,
        scratch_shapes=[
            pltpu.VMEM((n_seg, seg, d), BF16),
            pltpu.VMEM((m_len, d), BF16),
            pltpu.VMEM((NSLOT, 6 * dh, d), BF16),
            pltpu.VMEM((n_pairs, d, 6 * dh), BF16),
            pltpu.VMEM((hd, d), BF16),
            pltpu.VMEM((3 * nt, LANES, d), BF16),
            pltpu.VMEM((nt, d, LANES), BF16),
            pltpu.VMEM((d, LANES), F32),
            pltpu.VMEM((d, LANES), F32),
            pltpu.VMEM((3, d, d), BF16),
            pltpu.VMEM((nt, d, LANES), BF16),
            pltpu.VMEM((n_seg, seg, d), A_x.dtype),
            pltpu.VMEM((n_pre, d), BF16),
            pltpu.VMEM((n_pairs, n_pre, 6 * dh), BF16),
            pltpu.VMEM((2 * (m_len + seg) - PRE, d), BF16),
            pltpu.VMEM((m_len + seg, d), BF16),
            pltpu.VMEM((seg, d), F32),
            pltpu.VMEM((2 * seg, d), F32),
            pltpu.VMEM((2, 2 * nt, HIST + seg, LANES), F32),
            dma((5,)), dma((3 * NSLOT,)), dma((n_pairs,)),
            dma((3 * nt,)), dma((nt,)),
        ],
        compiler_params=pltpu.CompilerParams(
            vmem_limit_bytes=110 * 1024 * 1024,
            disable_bounds_checks=True),
    )(A_x.reshape(n_seg, seg, d), A_mem0.reshape(m_len, d), wq_t, wk_t, wv_t,
      wo, B_wqkv, B_wo)
    return out.reshape(bsz, s_len, d)
```

```python
import functools

import jax
import jax.numpy as jnp
from jax import lax
import jax.experimental.pallas as pl
import jax.experimental.pallas.tpu as pltpu

F32 = jnp.float32
BF16 = jnp.bfloat16

_NT = (((1,), (1,)), ((), ()))
_NN = (((1,), (0,)), ((), ()))

HB = 32
WIN = 8
DIL = 2
HIST = 16
LANES = 128
PRE = 16
PRE_CHUNK = 128
LN_SEGS = 16
LAG = 2
UNROLL = 2
NSLOT = 2
NEG = -1000000000.0


def _dot(a, b, dims):
    return lax.dot_general(a, b, dims, preferred_element_type=F32)


def _recip(x):
    r = pl.reciprocal(x, approx=True)
    return r * (2.0 - x * r)


def _ln(x):
    m = jnp.mean(x, axis=-1, keepdims=True)
    xc = x - m
    v = jnp.mean(xc * xc, axis=-1, keepdims=True)
    return xc * lax.rsqrt(v + 1e-05)


def _tile(a, c):
    return a[:, c * LANES:(c + 1) * LANES]


def _keep(mask, a):
    return jnp.where(mask, a, jnp.zeros_like(a))


def _drop(mask, a):
    return jnp.where(mask, jnp.zeros_like(a), a)


def _pair_softmax(s, col_a):
    m_a = jnp.max(jnp.where(col_a, s, -jnp.inf), axis=1, keepdims=True)
    m_b = jnp.max(jnp.where(col_a, -jnp.inf, s), axis=1, keepdims=True)
    e = jnp.exp(s - jnp.where(col_a, m_a, m_b))
    d_a = jnp.sum(jnp.where(col_a, e, 0.0), axis=1, keepdims=True)
    d_b = jnp.sum(jnp.where(col_a, 0.0, e), axis=1, keepdims=True)
    return e * _recip(jnp.where(col_a, d_a, d_b))


class _PassBase:
    def __init__(self, h, w_ref, wo_ref, dh):
        self.h, self.w, self.wo = h, w_ref, wo_ref
        self.pw = 2 * dh
        self.half = dh - LANES
        self.scale = dh ** (-0.5)
        self.q, self.k, self.v, self.p, self.o = {}, {}, {}, {}, {}
        self.cols = (0, 2 * LANES, wo_ref.shape[1])
        self.acc = [None, None]
        self.pending = None

    def _lane_lo(self, rows):
        return lax.broadcasted_iota(jnp.int32, (rows, LANES), 1) < self.half

    def _project(self, p, j):
        a = _dot(self.h, self.w[p, :, j * self.pw:(j + 1) * self.pw], _NN)
        self.marker = a[:8, :LANES]
        return a

    def _gate(self, s):
        if self.pending is None:
            return s
        top = jnp.where(self.always, s[:8], self.pending[:, :s.shape[1]])
        self.pending = None
        return jnp.concatenate([top, s[8:]], axis=0)

    def out(self, p, part=None):
        for k in ((0, 1) if part is None else (part,)):
            c0, c1 = self.cols[k], self.cols[k + 1]
            w = self.wo[p * self.pw:(p + 1) * self.pw, c0:c1]
            r = _dot(self.o[p], w, _NN)
            self.acc[k] = r if self.acc[k] is None else self.acc[k] + r

    def run(self, n_pairs, b, always):
        last = n_pairs - 1
        self.always = always
        done = None
        for p in range(n_pairs):
            self.proj_q(p)
            self.pending, done = done, None
            if 2 <= p < 2 + b.n_groups:
                o = b.attend(p - 2, (always, self.marker))
                done = functools.reduce(lambda u, v: u + v, o)
            self.proj_k(p)
            if p > 0:
                self.pv(p - 1)
            self.proj_v(p)
            self.scores(p)
            if p == 0:
                b.project()
            elif p < last:
                self.out(p - 1)
        yb = b.finish()
        self.out(last - 1, 0)
        self.pv(last)
        self.out(last - 1, 1)
        self.out(last)
        return jnp.concatenate(self.acc, axis=1), yb


class _TwoLayerPass(_PassBase):
    def __init__(self, h, pre_ref, pre_row, w_ref, wo_ref, *, dh, m_len, seg):
        super().__init__(h, w_ref, wo_ref, dh)
        self.pre, self.pre_row = pre_ref, pre_row
        self.m, self.seg = m_len, seg
        m2 = 2 * m_len
        n = m2 + 2 * seg
        row = lax.broadcasted_iota(jnp.int32, (n, n), 0)
        col = lax.broadcasted_iota(jnp.int32, (n, n), 1)

        def first_layer(i):
            return (i < m_len) | ((i >= m2) & (i < m2 + seg))

        def token(i):
            return jnp.where(i < m2 + seg, i - m2, i - m2 - seg)

        self.col_a = first_layer(col)
        self.diag = first_layer(row) == self.col_a
        self.allowed = (row < m2) | (col < m2) | (token(row) >= token(col))
        self.lo_m = self._lane_lo(m_len)
        self.lo_x = self._lane_lo(seg)

    def _proj(self, p, j):
        m, pw = self.m, self.pw
        a = self._project(p, j)
        pre = self.pre[p, pl.ds(self.pre_row, PRE), j * pw:(j + 1) * pw]
        n1 = self.seg - PRE
        nx = n1 + self.seg
        rest = a[:nx].astype(BF16)
        x1 = jnp.concatenate([pre, rest[:n1]], axis=0)
        return a[nx:nx + m], a[nx + m:], x1, rest[n1:]

    @staticmethod
    def _cat(ma, mb, xa, xb):
        mm = jnp.concatenate([ma, mb], axis=0).astype(BF16)
        return jnp.concatenate([mm, xa, xb], axis=0)

    def _tiles(self, m1, m2, x1, x2):
        cat, lm, lx = self._cat, self.lo_m, self.lo_x
        t0 = cat(_tile(m1, 0), _tile(m2, 0), _tile(x1, 0), _tile(x2, 0))
        t2 = cat(_tile(m2, 2), _tile(m1, 2), _tile(x2, 2), _tile(x1, 2))
        m1, m2, x1, x2 = (_tile(a, 1) for a in (m1, m2, x1, x2))
        t1a = cat(_keep(lm, m1), _drop(lm, m1), _keep(lx, x1), _drop(lx, x1))
        t1b = cat(_drop(lm, m2), _keep(lm, m2), _drop(lx, x2), _keep(lx, x2))
        return t0, t1a, t1b, t2

    def _rows_a(self, a):
        return a[:2 * self.m + self.seg]

    def _rows_b(self, a):
        m2 = 2 * self.m
        return jnp.concatenate([a[:m2], a[m2 + self.seg:]], axis=0)

    def _merge_rows(self, a, b):
        m = self.m
        return jnp.concatenate([a[:m], b[m:2 * m], a[2 * m:], b[2 * m:]],
                               axis=0)

    def proj_q(self, p):
        self.q[p] = self._cat(*self._proj(p, 0))

    def proj_k(self, p):
        self.k[p] = self._tiles(*self._proj(p, 1))

    def proj_v(self, p):
        self.v[p] = self._tiles(*self._proj(p, 2))

    def scores(self, p):
        q = self.q.pop(p)
        k0, k1a, k1b, k2 = self.k.pop(p)
        q1 = _tile(q, 1)
        r0 = _dot(_tile(q, 0), k0, _NT)
        r2 = _dot(_tile(q, 2), k2, _NT)
        r1a = _dot(self._rows_a(q1), k1a, _NT)
        r1b = _dot(self._rows_b(q1), k1b, _NT)
        s = jnp.where(self.diag, r0, r2) + self._merge_rows(r1a, r1b)
        s = self._gate(jnp.where(self.allowed, s * self.scale, NEG))
        p_all = _pair_softmax(s, self.col_a)
        self.p[p] = (p_all.astype(BF16), _keep(self.diag, p_all).astype(BF16),
                     _drop(self.diag, p_all).astype(BF16))

    def pv(self, p):
        p_all, p_diag, p_off = self.p.pop(p)
        v0, v1a, v1b, v2 = self.v.pop(p)
        o0 = _dot(p_diag, v0, _NN)
        o2 = _dot(p_off, v2, _NN)
        o1 = self._merge_rows(_dot(self._rows_a(p_all), v1a, _NN),
                              _dot(self._rows_b(p_all), v1b, _NN))
        self.o[p] = jnp.concatenate([o0, o1, o2], axis=1).astype(BF16)


class _OneLayerPass(_PassBase):
    def __init__(self, h, pre_ref, pre_row, w_ref, wo_ref, *, dh, m_len, seg):
        super().__init__(h, w_ref, wo_ref, dh)
        self.pre, self.pre_row = pre_ref, pre_row
        n = self.n = m_len + seg
        row = lax.broadcasted_iota(jnp.int32, (n, 2 * n), 0)
        col = lax.broadcasted_iota(jnp.int32, (n, 2 * n), 1)
        self.col_a = col < n
        key = jnp.where(self.col_a, col, col - n)
        self.allowed = (row < m_len) | (row >= key)
        lane = lax.broadcasted_iota(jnp.int32, (n, self.pw), 1)
        self.head0 = lane < dh

    def _project(self, p, j):
        a = super()._project(p, j)
        n, pw = self.n, self.pw
        self.pre[p, pl.ds(self.pre_row, a.shape[0] - n),
                 j * pw:(j + 1) * pw] = a[n:].astype(BF16)
        return a[:n]

    def _block_diag(self, a):
        return jnp.concatenate([_keep(self.head0, a), _drop(self.head0, a)],
                               axis=0).astype(BF16)

    def proj_q(self, p):
        self.q[p] = self._project(p, 0).astype(BF16)

    def proj_k(self, p):
        self.k[p] = self._block_diag(self._project(p, 1))

    def proj_v(self, p):
        self.v[p] = self._block_diag(self._project(p, 2))

    def scores(self, p):
        s = _dot(self.q.pop(p), self.k.pop(p), _NT)
        s = self._gate(jnp.where(self.allowed, s * self.scale, NEG))
        self.p[p] = _pair_softmax(s, self.col_a).astype(BF16)

    def pv(self, p):
        self.o[p] = _dot(self.p.pop(p), self.v.pop(p), _NN).astype(BF16)


class _BPass:
    def __init__(self, y_ref, starts, wqkv_ref, wo_ref, kv_ref, *, seg, d):
        self.y, self.starts = y_ref, starts
        self.wqkv, self.wo, self.kv = wqkv_ref, wo_ref, kv_ref
        self.seg, self.nt = seg, d // LANES
        self.scale = (d // HB) ** (-0.5)
        self.n_groups = len(starts) * seg // 8
        self.outs = []

    def project(self):
        seg, nt = self.seg, self.nt
        yn = _ln(self.y[...]).astype(BF16)
        self.q, ka, va = (_dot(yn, self.wqkv[j], _NN) for j in range(3))
        for i in range(len(self.starts)):
            self.kv[i, :, :HIST, :] = self.kv[i, :, seg:, :]
            for c in range(nt):
                rows = slice(i * seg, (i + 1) * seg)
                self.kv[i, c, HIST:, :] = _tile(ka[rows], c)
                self.kv[i, nt + c, HIST:, :] = _tile(va[rows], c)

    def attend(self, gi, after=None):
        seg, nt, kv = self.seg, self.nt, self.kv
        i, g = divmod(gi, seg // 8)
        q = [_tile(self.q[8 * gi:8 * gi + 8], c) for c in range(nt)]
        if after is not None:
            q = [jnp.where(after[0], u, after[1]) for u in q]
        pos = (lax.broadcasted_iota(jnp.int32, (8, LANES), 0)
               + (self.starts[i] + 8 * g))
        offs = [HIST + 8 * g - w * DIL for w in range(WIN)]
        logits = []
        for w, off in enumerate(offs):
            t = q[0] * kv[i, 0, off:off + 8, :]
            for c in range(1, nt):
                t = t + q[c] * kv[i, c, off:off + 8, :]
            t = t + pltpu.roll(t, 64, 1)
            t = (t + pltpu.roll(t, 32, 1)) * self.scale
            if 8 * g < w * DIL:
                t = jnp.where(pos >= w * DIL, t, NEG)
            logits.append(t)
        m = logits[0]
        for t in logits[1:]:
            m = jnp.maximum(m, t)
        es = [jnp.exp(t - m) for t in logits]
        den = es[0]
        for e in es[1:]:
            den = den + e
        inv = _recip(den)
        o = []
        for c in range(nt):
            acc = None
            for w, off in enumerate(offs):
                term = es[w] * kv[i, nt + c, off:off + 8, :]
                acc = term if acc is None else acc + term
            o.append(acc * inv)
        self.outs.append(jnp.concatenate(o, axis=1))
        return o

    def finish(self):
        o = jnp.concatenate(self.outs, axis=0).astype(BF16)
        proj = jnp.concatenate(
            [_dot(o, self.wo[c], _NN) for c in range(self.nt)], axis=1)
        return self.y[...] + proj


def _kernel(x_hbm, mem_hbm, wq_hbm, wk_hbm, wv_hbm, wo_hbm, bqkv_hbm, bo_hbm,
            out_hbm,
            x_v, mem_v, wst_v, w_v, wo_v, bq_st, bo_st, tq_s, to_s, bqkv_p,
            bo_p, out_v, xn_s, pre_s, h_s, h1_s, ra_s, y_s, kv_s,
            sems, w_sems, wo_sems, bq_sems, bo_sems,
            *, seg, n_seg, m_len, n_pairs, dh, d):
    db = d // HB
    nt = d // LANES
    pw = 2 * dh
    m2 = 2 * m_len
    n_pre = (n_seg - 1 - LAG) * PRE
    n_bq = 3 * nt

    def w_copy(p, j):
        src = (wq_hbm, wk_hbm, wv_hbm)[j]
        slot = p % NSLOT
        return pltpu.make_async_copy(
            src.at[pl.ds(p * pw, pw), :],
            wst_v.at[slot, pl.ds(j * pw, pw), :], w_sems.at[3 * slot + j])

    def wo_copy(p):
        return pltpu.make_async_copy(wo_hbm.at[pl.ds(p * pw, pw), :],
                                     wo_v.at[pl.ds(p * pw, pw), :],
                                     wo_sems.at[p])

    def bq_copy(i):
        row = pl.multiple_of((i % nt) * LANES, LANES)
        col = pl.multiple_of((i // nt) * d, LANES)
        return pltpu.make_async_copy(
            bqkv_hbm.at[pl.ds(row, LANES), pl.ds(col, d)], bq_st.at[i],
            bq_sems.at[i])

    def bo_copy(i):
        col = pl.multiple_of(i * LANES, LANES)
        return pltpu.make_async_copy(bo_hbm.at[:, pl.ds(col, LANES)],
                                     bo_st.at[i], bo_sems.at[i])

    xa_copy = pltpu.make_async_copy(x_hbm.at[:, :PRE, :], x_v.at[:, :PRE, :],
                                    sems.at[0])
    xb_copy = pltpu.make_async_copy(x_hbm.at[:, PRE:, :], x_v.at[:, PRE:, :],
                                    sems.at[1])
    mem_copy = pltpu.make_async_copy(mem_hbm, mem_v, sems.at[2])

    mem_copy.start()
    xa_copy.start()
    mem_copy.wait()
    for p in range(2):
        for j in range(3):
            w_copy(p, j).start()
        bq_copy(p).start()
        bo_copy(p).start()
    xb_copy.start()

    ra_s[...] = jnp.zeros(ra_s.shape, F32)
    y_s[...] = jnp.zeros(y_s.shape, F32)
    kv_s[...] = jnp.zeros(kv_s.shape, F32)

    xa_copy.wait()

    def ln_block(i, carry):
        s0 = pl.multiple_of(i * LN_SEGS, LN_SEGS)
        xb = x_v[pl.ds(s0, LN_SEGS), :PRE, :].astype(F32)
        xn_s[pl.ds(pl.multiple_of(s0 * PRE, PRE), LN_SEGS * PRE), :] = _ln(
            xb.reshape(LN_SEGS * PRE, d)).astype(BF16)
        return carry

    lax.fori_loop(0, n_seg // LN_SEGS, ln_block, 0)

    def permute_rows(tmp_ref):
        return jnp.concatenate(
            [tmp_ref[pl.ds(j, HB, stride=db), :] for j in range(db)], axis=0)

    def pre_pair(p, carry):
        for j in range(3):
            w_copy(p, j).wait()

        @pl.when(p < n_bq)
        def _():
            bq_copy(p).wait()

        @pl.when(p < nt)
        def _():
            bo_copy(p).wait()

        wo_copy(p).start()

        always = p >= 0
        marks = []

        def last_rows(a):
            return [a[(c + 1) * LANES - 16:(c + 1) * LANES] for c in range(nt)]

        i = jnp.minimum(p, nt - 1)
        to_s[...] = bo_st[i].astype(F32)
        bo = permute_rows(to_s)
        bo_p[i] = bo.astype(BF16)
        g = d // nt // 16
        marks.append([
            functools.reduce(
                lambda u, v: u + v,
                [bo[16 * (c * g + r):16 * (c * g + r + 1)] for r in range(g)]
            ).astype(BF16) for c in range(nt)])
        i = jnp.minimum(p, n_bq - 1)
        tq_s[...] = bq_st[i].astype(F32).T
        row = pl.multiple_of((i % nt) * LANES, LANES)
        bq = permute_rows(tq_s).T.astype(BF16)
        bqkv_p[i // nt, pl.ds(row, LANES), :] = bq
        marks.append([_tile(bq[LANES - 16:], c) for c in range(nt)])

        slot = p % NSLOT
        for n in range(3 * pw // LANES):
            wt = wst_v[slot, n * LANES:(n + 1) * LANES, :].T
            w_v[p, :, n * LANES:(n + 1) * LANES] = wt
            marks.append(last_rows(wt))

        starts = list(range(0, n_pre, PRE_CHUNK))
        groups = [[], marks[:1], marks[1:2]]
        rest, n_left = marks[2:], len(starts) - 3
        per_chunk = -(-len(rest) // n_left)
        groups += [rest[k * per_chunk:(k + 1) * per_chunk]
                   for k in range(n_left)]
        for r0, mine in zip(starts, groups):
            r1 = min(r0 + PRE_CHUNK, n_pre)
            lhs = xn_s[LAG * PRE + r0:LAG * PRE + r1, :]
            if mine:
                top = [jnp.where(always, lhs[16 * g:16 * (g + 1)],
                                 jnp.concatenate(mk, axis=1))
                       for g, mk in enumerate(mine)]
                lhs = jnp.concatenate(top + [lhs[16 * len(mine):]], axis=0)
            pre_s[p, r0:r1, :] = _dot(lhs, wst_v[slot], _NT).astype(BF16)

        @pl.when(p + NSLOT < n_pairs)
        def _():
            for j in range(3):
                w_copy(p + NSLOT, j).start()

        @pl.when(p + 2 < n_bq)
        def _():
            bq_copy(p + 2).start()

        @pl.when(p + 2 < nt)
        def _():
            bo_copy(p + 2).start()

        return carry

    lax.fori_loop(0, n_pairs, pre_pair, 0)

    xb_copy.wait()
    for p in range(n_pairs):
        wo_copy(p).wait()
    n1 = m_len + seg
    last_xn = (n_seg - 1) * PRE
    h1_s[:n1, :] = jnp.concatenate(
        [mem_v[...].astype(F32), _ln(x_v[0].astype(F32))],
        axis=0).astype(BF16)
    h1_s[n1:, :] = xn_s[last_xn:last_xn + m_len, :]

    def b_pass(t):
        return _BPass(y_s, ((t - 1) * seg, (t - 1 - LAG) * seg), bqkv_p, bo_p,
                      kv_s, seg=seg, d=d)

    def b_store(t, yb):
        out_v[jnp.maximum(t - 1 - LAG, 0)] = yb[seg:].astype(out_v.dtype)
        return yb[:seg]

    def two_layer_step(t, h):
        a = _TwoLayerPass(h, pre_s, pl.multiple_of((t - LAG) * PRE, PRE),
                          w_v, wo_v, dh=dh, m_len=m_len, seg=seg)
        acc, yb = a.run(n_pairs, b_pass(t), t >= 0)
        x2 = b_store(t, yb)
        y_s[:seg, :] = x_v[t].astype(F32) + acc[m2:m2 + seg]
        y_s[seg:, :] = ra_s[...] + acc[m2 + seg:]
        ra_s[...] = x2
        xn = x_v[jnp.minimum(t + 1, n_seg - 1), PRE:, :].astype(F32)
        return jnp.concatenate([_ln(xn), _ln(x2), acc[:m2]],
                               axis=0).astype(BF16)

    def two_layer_steps(i, carry):
        h = h_s[...]
        for u in range(UNROLL):
            h = two_layer_step(LAG + i * UNROLL + u, h)
        h_s[...] = h
        return carry

    def one_layer_step(t, carry):
        first = t < LAG
        extra_row = pl.multiple_of(n_pre + jnp.minimum(t, 1) * m_len, m_len)
        a = _OneLayerPass(h1_s[...], pre_s, extra_row, w_v, wo_v,
                          dh=dh, m_len=m_len, seg=seg)
        acc, yb = a.run(n_pairs, b_pass(t), t >= 0)
        x2 = b_store(t, yb)
        x0 = x_v[jnp.minimum(t, n_seg - 1)].astype(F32)
        y = jnp.where(first, x0, ra_s[...]) + acc[m_len:]
        y_s[:seg, :] = y
        y_s[seg:, :] = y
        ra_s[...] = x2
        xn = _ln(x_v[jnp.minimum(t + 1, n_seg - 1)].astype(F32))
        x2n = _ln(x2)
        mem = acc[:m_len]
        h1_s[:n1, :] = jnp.concatenate(
            [mem, jnp.where(first, xn, x2n)], axis=0).astype(BF16)
        h1_s[n1:, :] = xn_s[last_xn + m_len:, :]
        h_s[...] = jnp.concatenate(
            [xn[PRE:], x2n, mem, mem_v[...].astype(F32)], axis=0).astype(BF16)
        return carry

    n_early_out = n_seg - 1 - LAG
    out_a = pltpu.make_async_copy(out_v.at[:n_early_out],
                                  out_hbm.at[:n_early_out], sems.at[3])
    out_b = pltpu.make_async_copy(out_v.at[n_early_out:],
                                  out_hbm.at[n_early_out:], sems.at[4])

    def phase(ph, carry):
        t0 = ph * n_seg
        lax.fori_loop(t0, t0 + LAG, one_layer_step, 0)

        @pl.when(ph == 0)
        def _():
            lax.fori_loop(0, (n_seg - LAG) // UNROLL, two_layer_steps, 0)
            out_a.start()
            hf = h_s[...].astype(F32)
            h1_s[:n1, :] = jnp.concatenate(
                [hf[2 * seg - PRE + m_len:], hf[seg - PRE:2 * seg - PRE]],
                axis=0).astype(BF16)

        return carry

    lax.fori_loop(0, 2, phase, 0)

    b = _BPass(y_s.at[seg:], ((n_seg - 1) * seg,), bqkv_p, bo_p, kv_s.at[1:],
               seg=seg, d=d)
    b.project()
    for gi in range(b.n_groups):
        b.attend(gi)
    out_v[n_seg - 1] = b.finish().astype(out_v.dtype)
    out_b.start()
    out_a.wait()
    out_b.wait()


@functools.partial(jax.jit, static_argnames=("A_seg_len",))
def pallas_interleave_layers__memory_aug_recurrent_mem_tr__sliding_local_dilated__prompt_kernel(
    A_x: jax.Array,
    A_mem0: jax.Array,
    A_Wq: jax.Array,
    A_Wk: jax.Array,
    A_Wv: jax.Array,
    A_Wo: jax.Array,
    A_seg_len,
    B_x: jax.Array,
    B_wqkv: jax.Array,
    B_wo: jax.Array,
):
    del B_x
    bsz, s_len, d = A_x.shape
    m_len = A_mem0.shape[1]
    n_heads, dh = A_Wq.shape[1], A_Wq.shape[2]
    seg = int(A_seg_len)
    n_seg = s_len // seg
    n_pairs = n_heads // 2
    nt = d // LANES
    assert bsz == 1 and s_len % seg == 0 and n_seg > LAG + 1
    assert seg % 16 == 0 and m_len == 8 and seg > PRE and seg >= HIST
    assert LAG == 2 and LAG * m_len == PRE and n_seg % LN_SEGS == 0
    assert 2 * (m_len + seg) <= LANES and (n_seg - LAG) % UNROLL == 0
    assert n_heads % 2 == 0 and 2 * dh == 3 * LANES and d % LANES == 0
    assert d % HB == 0 and LANES == 4 * HB and n_pairs >= 3 * nt >= 3
    hd = n_heads * dh
    n_pre = (n_seg - LAG) * PRE

    wq_t = jnp.transpose(A_Wq, (1, 2, 0)).reshape(hd, d)
    wk_t = jnp.transpose(A_Wk, (1, 2, 0)).reshape(hd, d)
    wv_t = jnp.transpose(A_Wv, (1, 2, 0)).reshape(hd, d)
    wo = A_Wo.reshape(hd, d)

    kernel = functools.partial(
        _kernel, seg=seg, n_seg=n_seg, m_len=m_len, n_pairs=n_pairs, dh=dh,
        d=d)
    any_spec = pl.BlockSpec(memory_space=pl.ANY)
    dma = pltpu.SemaphoreType.DMA
    out = pl.pallas_call(
        kernel,
        out_shape=jax.ShapeDtypeStruct((n_seg, seg, d), A_x.dtype),
        in_specs=[any_spec] * 8,
        out_specs=any_spec,
        scratch_shapes=[
            pltpu.VMEM((n_seg, seg, d), BF16),
            pltpu.VMEM((m_len, d), BF16),
            pltpu.VMEM((NSLOT, 6 * dh, d), BF16),
            pltpu.VMEM((n_pairs, d, 6 * dh), BF16),
            pltpu.VMEM((hd, d), BF16),
            pltpu.VMEM((3 * nt, LANES, d), BF16),
            pltpu.VMEM((nt, d, LANES), BF16),
            pltpu.VMEM((d, LANES), F32),
            pltpu.VMEM((d, LANES), F32),
            pltpu.VMEM((3, d, d), BF16),
            pltpu.VMEM((nt, d, LANES), BF16),
            pltpu.VMEM((n_seg, seg, d), A_x.dtype),
            pltpu.VMEM((n_seg * PRE, d), BF16),
            pltpu.VMEM((n_pairs, n_pre, 6 * dh), BF16),
            pltpu.VMEM((2 * (m_len + seg) - PRE, d), BF16),
            pltpu.VMEM((2 * m_len + seg, d), BF16),
            pltpu.VMEM((seg, d), F32),
            pltpu.VMEM((2 * seg, d), F32),
            pltpu.VMEM((2, 2 * nt, HIST + seg, LANES), F32),
            dma((5,)), dma((3 * NSLOT,)), dma((n_pairs,)),
            dma((3 * nt,)), dma((nt,)),
        ],
        compiler_params=pltpu.CompilerParams(
            vmem_limit_bytes=110 * 1024 * 1024,
            disable_bounds_checks=True),
    )(A_x.reshape(n_seg, seg, d), A_mem0.reshape(m_len, d), wq_t, wk_t, wv_t,
      wo, B_wqkv, B_wo)
    return out.reshape(bsz, s_len, d)
```

```python
import functools

import jax
import jax.numpy as jnp
from jax import lax
import jax.experimental.pallas as pl
import jax.experimental.pallas.tpu as pltpu

F32 = jnp.float32
BF16 = jnp.bfloat16

_NT = (((1,), (1,)), ((), ()))
_NN = (((1,), (0,)), ((), ()))

HB = 32
WIN = 8
DIL = 2
HIST = 16
LANES = 128
PRE = 16
PRE_CHUNK = 128
LN_SEGS = 16
LAG = 2
UNROLL = 2
NSLOT = 2
NEG = -1000000000.0


def _dot(a, b, dims):
    return lax.dot_general(a, b, dims, preferred_element_type=F32)


def _recip(x):
    r = pl.reciprocal(x, approx=True)
    return r * (2.0 - x * r)


def _ln(x):
    m = jnp.mean(x, axis=-1, keepdims=True)
    xc = x - m
    v = jnp.mean(xc * xc, axis=-1, keepdims=True)
    return xc * lax.rsqrt(v + 1e-05)


def _tile(a, c):
    return a[:, c * LANES:(c + 1) * LANES]


def _keep(mask, a):
    return jnp.where(mask, a, jnp.zeros_like(a))


def _drop(mask, a):
    return jnp.where(mask, jnp.zeros_like(a), a)


def _pair_softmax(s, col_a):
    m_a = jnp.max(jnp.where(col_a, s, -jnp.inf), axis=1, keepdims=True)
    m_b = jnp.max(jnp.where(col_a, -jnp.inf, s), axis=1, keepdims=True)
    e = jnp.exp(s - jnp.where(col_a, m_a, m_b))
    d_a = jnp.sum(jnp.where(col_a, e, 0.0), axis=1, keepdims=True)
    d_b = jnp.sum(jnp.where(col_a, 0.0, e), axis=1, keepdims=True)
    return e * _recip(jnp.where(col_a, d_a, d_b))


class _PassBase:
    def __init__(self, h, w_ref, wo_ref, dh):
        self.h, self.w, self.wo = h, w_ref, wo_ref
        self.pw = 2 * dh
        self.half = dh - LANES
        self.scale = dh ** (-0.5)
        self.q, self.k, self.v, self.p, self.o = {}, {}, {}, {}, {}
        self.cols = (0, 2 * LANES, wo_ref.shape[1])
        self.pending = None

    def _lane_lo(self, rows):
        return lax.broadcasted_iota(jnp.int32, (rows, LANES), 1) < self.half

    def _project(self, p, j):
        a = _dot(self.h, self.w[p, :, j * self.pw:(j + 1) * self.pw], _NN)
        self.marker = a[:8, :LANES]
        return a

    def _gate(self, s):
        if self.pending is None:
            return s
        top = jnp.where(self.always, s[:8], self.pending[:, :s.shape[1]])
        self.pending = None
        return jnp.concatenate([top, s[8:]], axis=0)

    def out(self, p, part=None):
        for k in ((0, 1) if part is None else (part,)):
            c0, c1 = self.cols[k], self.cols[k + 1]
            w = self.wo[p * self.pw:(p + 1) * self.pw, c0:c1]
            self.acc[k] = self.acc[k] + _dot(self.o[p], w, _NN)

    def run(self, n_pairs, init, b, always):
        last = n_pairs - 1
        self.acc = [init[:, :self.cols[1]], init[:, self.cols[1]:]]
        self.always = always
        done = None
        for p in range(n_pairs):
            self.proj_q(p)
            self.pending, done = done, None
            if 2 <= p < 2 + b.n_groups:
                o = b.attend(p - 2, (always, self.marker))
                done = functools.reduce(lambda u, v: u + v, o)
            self.proj_k(p)
            if p > 0:
                self.pv(p - 1)
            self.proj_v(p)
            self.scores(p)
            if p == 0:
                b.project()
            elif p < last:
                self.out(p - 1)
        yb = b.finish()
        self.out(last - 1, 0)
        self.pv(last)
        self.out(last - 1, 1)
        self.out(last)
        return jnp.concatenate(self.acc, axis=1), yb


class _TwoLayerPass(_PassBase):
    def __init__(self, h, pre_ref, pre_row, w_ref, wo_ref, *, dh, m_len, seg):
        super().__init__(h, w_ref, wo_ref, dh)
        self.pre, self.pre_row = pre_ref, pre_row
        self.m, self.seg = m_len, seg
        m2 = 2 * m_len
        n = m2 + 2 * seg
        row = lax.broadcasted_iota(jnp.int32, (n, n), 0)
        col = lax.broadcasted_iota(jnp.int32, (n, n), 1)

        def first_layer(i):
            return (i < m_len) | ((i >= m2) & (i < m2 + seg))

        def token(i):
            return jnp.where(i < m2 + seg, i - m2, i - m2 - seg)

        self.col_a = first_layer(col)
        self.diag = first_layer(row) == self.col_a
        self.allowed = (row < m2) | (col < m2) | (token(row) >= token(col))
        self.lo_m = self._lane_lo(m_len)
        self.lo_x = self._lane_lo(seg)

    def _proj(self, p, j):
        m, pw = self.m, self.pw
        a = self._project(p, j)
        pre = self.pre[p, pl.ds(self.pre_row, PRE), j * pw:(j + 1) * pw]
        n1 = self.seg - PRE
        nx = n1 + self.seg
        rest = a[:nx].astype(BF16)
        x1 = jnp.concatenate([pre, rest[:n1]], axis=0)
        return a[nx:nx + m], a[nx + m:], x1, rest[n1:]

    @staticmethod
    def _cat(ma, mb, xa, xb):
        mm = jnp.concatenate([ma, mb], axis=0).astype(BF16)
        return jnp.concatenate([mm, xa, xb], axis=0)

    def _tiles(self, m1, m2, x1, x2):
        cat, lm, lx = self._cat, self.lo_m, self.lo_x
        t0 = cat(_tile(m1, 0), _tile(m2, 0), _tile(x1, 0), _tile(x2, 0))
        t2 = cat(_tile(m2, 2), _tile(m1, 2), _tile(x2, 2), _tile(x1, 2))
        m1, m2, x1, x2 = (_tile(a, 1) for a in (m1, m2, x1, x2))
        t1a = cat(_keep(lm, m1), _drop(lm, m1), _keep(lx, x1), _drop(lx, x1))
        t1b = cat(_drop(lm, m2), _keep(lm, m2), _drop(lx, x2), _keep(lx, x2))
        return t0, t1a, t1b, t2

    def _rows_a(self, a):
        return a[:2 * self.m + self.seg]

    def _rows_b(self, a):
        m2 = 2 * self.m
        return jnp.concatenate([a[:m2], a[m2 + self.seg:]], axis=0)

    def _merge_rows(self, a, b):
        m = self.m
        return jnp.concatenate([a[:m], b[m:2 * m], a[2 * m:], b[2 * m:]],
                               axis=0)

    def proj_q(self, p):
        self.q[p] = self._cat(*self._proj(p, 0))

    def proj_k(self, p):
        self.k[p] = self._tiles(*self._proj(p, 1))

    def proj_v(self, p):
        self.v[p] = self._tiles(*self._proj(p, 2))

    def scores(self, p):
        q = self.q.pop(p)
        k0, k1a, k1b, k2 = self.k.pop(p)
        q1 = _tile(q, 1)
        r0 = _dot(_tile(q, 0), k0, _NT)
        r2 = _dot(_tile(q, 2), k2, _NT)
        r1a = _dot(self._rows_a(q1), k1a, _NT)
        r1b = _dot(self._rows_b(q1), k1b, _NT)
        s = jnp.where(self.diag, r0, r2) + self._merge_rows(r1a, r1b)
        s = self._gate(jnp.where(self.allowed, s * self.scale, NEG))
        p_all = _pair_softmax(s, self.col_a)
        self.p[p] = (p_all.astype(BF16), _keep(self.diag, p_all).astype(BF16),
                     _drop(self.diag, p_all).astype(BF16))

    def pv(self, p):
        p_all, p_diag, p_off = self.p.pop(p)
        v0, v1a, v1b, v2 = self.v.pop(p)
        o0 = _dot(p_diag, v0, _NN)
        o2 = _dot(p_off, v2, _NN)
        o1 = self._merge_rows(_dot(self._rows_a(p_all), v1a, _NN),
                              _dot(self._rows_b(p_all), v1b, _NN))
        self.o[p] = jnp.concatenate([o0, o1, o2], axis=1).astype(BF16)


class _OneLayerPass(_PassBase):
    def __init__(self, h, pre_ref, pre_row, w_ref, wo_ref, *, dh, m_len, seg):
        super().__init__(h, w_ref, wo_ref, dh)
        self.pre, self.pre_row = pre_ref, pre_row
        n = self.n = m_len + seg
        row = lax.broadcasted_iota(jnp.int32, (n, 2 * n), 0)
        col = lax.broadcasted_iota(jnp.int32, (n, 2 * n), 1)
        self.col_a = col < n
        key = jnp.where(self.col_a, col, col - n)
        self.allowed = (row < m_len) | (row >= key)
        lane = lax.broadcasted_iota(jnp.int32, (n, self.pw), 1)
        self.head0 = lane < dh

    def _project(self, p, j):
        a = super()._project(p, j)
        n, pw = self.n, self.pw
        self.pre[p, pl.ds(self.pre_row, a.shape[0] - n),
                 j * pw:(j + 1) * pw] = a[n:].astype(BF16)
        return a[:n]

    def _block_diag(self, a):
        return jnp.concatenate([_keep(self.head0, a), _drop(self.head0, a)],
                               axis=0).astype(BF16)

    def proj_q(self, p):
        self.q[p] = self._project(p, 0).astype(BF16)

    def proj_k(self, p):
        self.k[p] = self._block_diag(self._project(p, 1))

    def proj_v(self, p):
        self.v[p] = self._block_diag(self._project(p, 2))

    def scores(self, p):
        s = _dot(self.q.pop(p), self.k.pop(p), _NT)
        s = self._gate(jnp.where(self.allowed, s * self.scale, NEG))
        self.p[p] = _pair_softmax(s, self.col_a).astype(BF16)

    def pv(self, p):
        self.o[p] = _dot(self.p.pop(p), self.v.pop(p), _NN).astype(BF16)


class _BPass:
    def __init__(self, y_ref, starts, wqkv_ref, wo_ref, kv_ref, *, seg, d):
        self.y, self.starts = y_ref, starts
        self.wqkv, self.wo, self.kv = wqkv_ref, wo_ref, kv_ref
        self.seg, self.nt = seg, d // LANES
        self.scale = (d // HB) ** (-0.5)
        self.n_groups = len(starts) * seg // 8
        self.outs = []

    def project(self):
        seg, nt = self.seg, self.nt
        yn = _ln(self.y[...]).astype(BF16)
        self.q, ka, va = (_dot(yn, self.wqkv[j], _NN) for j in range(3))
        for i in range(len(self.starts)):
            self.kv[i, :, :HIST, :] = self.kv[i, :, seg:, :]
            for c in range(nt):
                rows = slice(i * seg, (i + 1) * seg)
                self.kv[i, c, HIST:, :] = _tile(ka[rows], c)
                self.kv[i, nt + c, HIST:, :] = _tile(va[rows], c)

    def attend(self, gi, after=None):
        seg, nt, kv = self.seg, self.nt, self.kv
        i, g = divmod(gi, seg // 8)
        q = [_tile(self.q[8 * gi:8 * gi + 8], c) for c in range(nt)]
        if after is not None:
            q = [jnp.where(after[0], u, after[1]) for u in q]
        pos = (lax.broadcasted_iota(jnp.int32, (8, LANES), 0)
               + (self.starts[i] + 8 * g))
        offs = [HIST + 8 * g - w * DIL for w in range(WIN)]
        logits = []
        for w, off in enumerate(offs):
            t = q[0] * kv[i, 0, off:off + 8, :]
            for c in range(1, nt):
                t = t + q[c] * kv[i, c, off:off + 8, :]
            t = t + pltpu.roll(t, 64, 1)
            t = (t + pltpu.roll(t, 32, 1)) * self.scale
            if 8 * g < w * DIL:
                t = jnp.where(pos >= w * DIL, t, NEG)
            logits.append(t)
        m = logits[0]
        for t in logits[1:]:
            m = jnp.maximum(m, t)
        es = [jnp.exp(t - m) for t in logits]
        den = es[0]
        for e in es[1:]:
            den = den + e
        inv = _recip(den)
        o = []
        for c in range(nt):
            acc = None
            for w, off in enumerate(offs):
                term = es[w] * kv[i, nt + c, off:off + 8, :]
                acc = term if acc is None else acc + term
            o.append(acc * inv)
        self.outs.append(jnp.concatenate(o, axis=1))
        return o

    def finish(self):
        o = jnp.concatenate(self.outs, axis=0).astype(BF16)
        proj = jnp.concatenate(
            [_dot(o, self.wo[c], _NN) for c in range(self.nt)], axis=1)
        return self.y[...] + proj


def _kernel(x_hbm, mem_hbm, wq_hbm, wk_hbm, wv_hbm, wo_hbm, bqkv_hbm, bo_hbm,
            out_hbm,
            x_v, mem_v, wst_v, w_v, wo_v, bq_st, bo_st, tq_s, to_s, bqkv_p,
            bo_p, out_v, xn_s, pre_s, h_s, h1_s, ra_s, y_s, kv_s,
            sems, w_sems, wo_sems, bq_sems, bo_sems,
            *, seg, n_seg, m_len, n_pairs, dh, d):
    db = d // HB
    nt = d // LANES
    pw = 2 * dh
    m2 = 2 * m_len
    n_pre = (n_seg - 1 - LAG) * PRE
    n_bq = 3 * nt

    def w_copy(p, j):
        src = (wq_hbm, wk_hbm, wv_hbm)[j]
        slot = p % NSLOT
        return pltpu.make_async_copy(
            src.at[pl.ds(p * pw, pw), :],
            wst_v.at[slot, pl.ds(j * pw, pw), :], w_sems.at[3 * slot + j])

    def wo_copy(p):
        return pltpu.make_async_copy(wo_hbm.at[pl.ds(p * pw, pw), :],
                                     wo_v.at[pl.ds(p * pw, pw), :],
                                     wo_sems.at[p])

    def bq_copy(i):
        row = pl.multiple_of((i % nt) * LANES, LANES)
        col = pl.multiple_of((i // nt) * d, LANES)
        return pltpu.make_async_copy(
            bqkv_hbm.at[pl.ds(row, LANES), pl.ds(col, d)], bq_st.at[i],
            bq_sems.at[i])

    def bo_copy(i):
        col = pl.multiple_of(i * LANES, LANES)
        return pltpu.make_async_copy(bo_hbm.at[:, pl.ds(col, LANES)],
                                     bo_st.at[i], bo_sems.at[i])

    xa_copy = pltpu.make_async_copy(x_hbm.at[:, :PRE, :], x_v.at[:, :PRE, :],
                                    sems.at[0])
    xb_copy = pltpu.make_async_copy(x_hbm.at[:, PRE:, :], x_v.at[:, PRE:, :],
                                    sems.at[1])
    mem_copy = pltpu.make_async_copy(mem_hbm, mem_v, sems.at[2])

    mem_copy.start()
    xa_copy.start()
    mem_copy.wait()
    for p in range(2):
        for j in range(3):
            w_copy(p, j).start()
        bq_copy(p).start()
        bo_copy(p).start()
    xb_copy.start()

    ra_s[...] = jnp.zeros(ra_s.shape, F32)
    y_s[...] = jnp.zeros(y_s.shape, F32)
    kv_s[...] = jnp.zeros(kv_s.shape, F32)

    xa_copy.wait()

    def ln_block(i, carry):
        s0 = pl.multiple_of(i * LN_SEGS, LN_SEGS)
        xb = x_v[pl.ds(s0, LN_SEGS), :PRE, :].astype(F32)
        xn_s[pl.ds(pl.multiple_of(s0 * PRE, PRE), LN_SEGS * PRE), :] = _ln(
            xb.reshape(LN_SEGS * PRE, d)).astype(BF16)
        return carry

    lax.fori_loop(0, n_seg // LN_SEGS, ln_block, 0)

    def permute_rows(tmp_ref):
        return jnp.concatenate(
            [tmp_ref[pl.ds(j, HB, stride=db), :] for j in range(db)], axis=0)

    def pre_pair(p, carry):
        for j in range(3):
            w_copy(p, j).wait()

        @pl.when(p < n_bq)
        def _():
            bq_copy(p).wait()

        @pl.when(p < nt)
        def _():
            bo_copy(p).wait()

        wo_copy(p).start()

        always = p >= 0
        marks = []

        def last_rows(a):
            return [a[(c + 1) * LANES - 16:(c + 1) * LANES] for c in range(nt)]

        i = jnp.minimum(p, nt - 1)
        to_s[...] = bo_st[i].astype(F32)
        bo = permute_rows(to_s)
        bo_p[i] = bo.astype(BF16)
        g = d // nt // 16
        marks.append([
            functools.reduce(
                lambda u, v: u + v,
                [bo[16 * (c * g + r):16 * (c * g + r + 1)] for r in range(g)]
            ).astype(BF16) for c in range(nt)])
        i = jnp.minimum(p, n_bq - 1)
        tq_s[...] = bq_st[i].astype(F32).T
        row = pl.multiple_of((i % nt) * LANES, LANES)
        bq = permute_rows(tq_s).T.astype(BF16)
        bqkv_p[i // nt, pl.ds(row, LANES), :] = bq
        marks.append([_tile(bq[LANES - 16:], c) for c in range(nt)])

        slot = p % NSLOT
        for n in range(3 * pw // LANES):
            wt = wst_v[slot, n * LANES:(n + 1) * LANES, :].T
            w_v[p, :, n * LANES:(n + 1) * LANES] = wt
            marks.append(last_rows(wt))

        starts = list(range(0, n_pre, PRE_CHUNK))
        groups = [[], marks[:1], marks[1:2]]
        rest, n_left = marks[2:], len(starts) - 3
        per_chunk = -(-len(rest) // n_left)
        groups += [rest[k * per_chunk:(k + 1) * per_chunk]
                   for k in range(n_left)]
        for r0, mine in zip(starts, groups):
            r1 = min(r0 + PRE_CHUNK, n_pre)
            lhs = xn_s[LAG * PRE + r0:LAG * PRE + r1, :]
            if mine:
                top = [jnp.where(always, lhs[16 * g:16 * (g + 1)],
                                 jnp.concatenate(mk, axis=1))
                       for g, mk in enumerate(mine)]
                lhs = jnp.concatenate(top + [lhs[16 * len(mine):]], axis=0)
            pre_s[p, r0:r1, :] = _dot(lhs, wst_v[slot], _NT).astype(BF16)

        @pl.when(p + NSLOT < n_pairs)
        def _():
            for j in range(3):
                w_copy(p + NSLOT, j).start()

        @pl.when(p + 2 < n_bq)
        def _():
            bq_copy(p + 2).start()

        @pl.when(p + 2 < nt)
        def _():
            bo_copy(p + 2).start()

        return carry

    lax.fori_loop(0, n_pairs, pre_pair, 0)

    xb_copy.wait()
    for p in range(n_pairs):
        wo_copy(p).wait()
    n1 = m_len + seg
    last_xn = (n_seg - 1) * PRE
    h1_s[:n1, :] = jnp.concatenate(
        [mem_v[...].astype(F32), _ln(x_v[0].astype(F32))],
        axis=0).astype(BF16)
    h1_s[n1:, :] = xn_s[last_xn:last_xn + m_len, :]

    def b_pass(t):
        return _BPass(y_s, ((t - 1) * seg, (t - 1 - LAG) * seg), bqkv_p, bo_p,
                      kv_s, seg=seg, d=d)

    def b_store(t, yb):
        out_v[jnp.maximum(t - 1 - LAG, 0)] = yb[seg:].astype(out_v.dtype)
        return yb[:seg]

    def two_layer_step(t, h):
        a = _TwoLayerPass(h, pre_s, pl.multiple_of((t - LAG) * PRE, PRE),
                          w_v, wo_v, dh=dh, m_len=m_len, seg=seg)
        init = jnp.concatenate(
            [jnp.zeros((m2, d), F32), x_v[t].astype(F32), ra_s[...]], axis=0)
        acc, yb = a.run(n_pairs, init, b_pass(t), t >= 0)
        x2 = b_store(t, yb)
        y_s[...] = acc[m2:]
        ra_s[...] = x2
        xn = x_v[jnp.minimum(t + 1, n_seg - 1), PRE:, :].astype(F32)
        return jnp.concatenate([_ln(xn), _ln(x2), acc[:m2]],
                               axis=0).astype(BF16)

    def two_layer_steps(i, carry):
        h = h_s[...]
        for u in range(UNROLL):
            h = two_layer_step(LAG + i * UNROLL + u, h)
        h_s[...] = h
        return carry

    def one_layer_step(t, carry):
        first = t < LAG
        extra_row = pl.multiple_of(n_pre + jnp.minimum(t, 1) * m_len, m_len)
        a = _OneLayerPass(h1_s[...], pre_s, extra_row, w_v, wo_v,
                          dh=dh, m_len=m_len, seg=seg)
        x0 = x_v[jnp.minimum(t, n_seg - 1)].astype(F32)
        init = jnp.concatenate(
            [jnp.zeros((m_len, d), F32), jnp.where(first, x0, ra_s[...])],
            axis=0)
        acc, yb = a.run(n_pairs, init, b_pass(t), t >= 0)
        x2 = b_store(t, yb)
        y = acc[m_len:]
        y_s[:seg, :] = y
        y_s[seg:, :] = y
        ra_s[...] = x2
        xn = _ln(x_v[jnp.minimum(t + 1, n_seg - 1)].astype(F32))
        x2n = _ln(x2)
        mem = acc[:m_len]
        h1_s[:n1, :] = jnp.concatenate(
            [mem, jnp.where(first, xn, x2n)], axis=0).astype(BF16)
        h1_s[n1:, :] = xn_s[last_xn + m_len:, :]
        h_s[...] = jnp.concatenate(
            [xn[PRE:], x2n, mem, mem_v[...].astype(F32)], axis=0).astype(BF16)
        return carry

    n_early_out = n_seg - 1 - LAG
    out_a = pltpu.make_async_copy(out_v.at[:n_early_out],
                                  out_hbm.at[:n_early_out], sems.at[3])
    out_b = pltpu.make_async_copy(out_v.at[n_early_out:],
                                  out_hbm.at[n_early_out:], sems.at[4])

    def phase(ph, carry):
        t0 = ph * n_seg
        lax.fori_loop(t0, t0 + LAG, one_layer_step, 0)

        @pl.when(ph == 0)
        def _():
            lax.fori_loop(0, (n_seg - LAG) // UNROLL, two_layer_steps, 0)
            out_a.start()
            hf = h_s[...].astype(F32)
            h1_s[:n1, :] = jnp.concatenate(
                [hf[2 * seg - PRE + m_len:], hf[seg - PRE:2 * seg - PRE]],
                axis=0).astype(BF16)

        return carry

    lax.fori_loop(0, 2, phase, 0)

    b = _BPass(y_s.at[seg:], ((n_seg - 1) * seg,), bqkv_p, bo_p, kv_s.at[1:],
               seg=seg, d=d)
    b.project()
    for gi in range(b.n_groups):
        b.attend(gi)
    out_v[n_seg - 1] = b.finish().astype(out_v.dtype)
    out_b.start()
    out_a.wait()
    out_b.wait()


@functools.partial(jax.jit, static_argnames=("A_seg_len",))
def pallas_interleave_layers__memory_aug_recurrent_mem_tr__sliding_local_dilated__prompt_kernel(
    A_x: jax.Array,
    A_mem0: jax.Array,
    A_Wq: jax.Array,
    A_Wk: jax.Array,
    A_Wv: jax.Array,
    A_Wo: jax.Array,
    A_seg_len,
    B_x: jax.Array,
    B_wqkv: jax.Array,
    B_wo: jax.Array,
):
    del B_x
    bsz, s_len, d = A_x.shape
    m_len = A_mem0.shape[1]
    n_heads, dh = A_Wq.shape[1], A_Wq.shape[2]
    seg = int(A_seg_len)
    n_seg = s_len // seg
    n_pairs = n_heads // 2
    nt = d // LANES
    assert bsz == 1 and s_len % seg == 0 and n_seg > LAG + 1
    assert seg % 16 == 0 and m_len == 8 and seg > PRE and seg >= HIST
    assert LAG == 2 and LAG * m_len == PRE and n_seg % LN_SEGS == 0
    assert 2 * (m_len + seg) <= LANES and (n_seg - LAG) % UNROLL == 0
    assert n_heads % 2 == 0 and 2 * dh == 3 * LANES and d % LANES == 0
    assert d % HB == 0 and LANES == 4 * HB and n_pairs >= 3 * nt >= 3
    hd = n_heads * dh
    n_pre = (n_seg - LAG) * PRE

    wq_t = jnp.transpose(A_Wq, (1, 2, 0)).reshape(hd, d)
    wk_t = jnp.transpose(A_Wk, (1, 2, 0)).reshape(hd, d)
    wv_t = jnp.transpose(A_Wv, (1, 2, 0)).reshape(hd, d)
    wo = A_Wo.reshape(hd, d)

    kernel = functools.partial(
        _kernel, seg=seg, n_seg=n_seg, m_len=m_len, n_pairs=n_pairs, dh=dh,
        d=d)
    any_spec = pl.BlockSpec(memory_space=pl.ANY)
    dma = pltpu.SemaphoreType.DMA
    out = pl.pallas_call(
        kernel,
        out_shape=jax.ShapeDtypeStruct((n_seg, seg, d), A_x.dtype),
        in_specs=[any_spec] * 8,
        out_specs=any_spec,
        scratch_shapes=[
            pltpu.VMEM((n_seg, seg, d), BF16),
            pltpu.VMEM((m_len, d), BF16),
            pltpu.VMEM((NSLOT, 6 * dh, d), BF16),
            pltpu.VMEM((n_pairs, d, 6 * dh), BF16),
            pltpu.VMEM((hd, d), BF16),
            pltpu.VMEM((3 * nt, LANES, d), BF16),
            pltpu.VMEM((nt, d, LANES), BF16),
            pltpu.VMEM((d, LANES), F32),
            pltpu.VMEM((d, LANES), F32),
            pltpu.VMEM((3, d, d), BF16),
            pltpu.VMEM((nt, d, LANES), BF16),
            pltpu.VMEM((n_seg, seg, d), A_x.dtype),
            pltpu.VMEM((n_seg * PRE, d), BF16),
            pltpu.VMEM((n_pairs, n_pre, 6 * dh), BF16),
            pltpu.VMEM((2 * (m_len + seg) - PRE, d), BF16),
            pltpu.VMEM((2 * m_len + seg, d), BF16),
            pltpu.VMEM((seg, d), F32),
            pltpu.VMEM((2 * seg, d), F32),
            pltpu.VMEM((2, 2 * nt, HIST + seg, LANES), F32),
            dma((5,)), dma((3 * NSLOT,)), dma((n_pairs,)),
            dma((3 * nt,)), dma((nt,)),
        ],
        compiler_params=pltpu.CompilerParams(
            vmem_limit_bytes=110 * 1024 * 1024,
            disable_bounds_checks=True),
    )(A_x.reshape(n_seg, seg, d), A_mem0.reshape(m_len, d), wq_t, wk_t, wv_t,
      wo, B_wqkv, B_wo)
    return out.reshape(bsz, s_len, d)
```

```python
import functools

import jax
import jax.numpy as jnp
from jax import lax
import jax.experimental.pallas as pl
import jax.experimental.pallas.tpu as pltpu

F32 = jnp.float32
BF16 = jnp.bfloat16

_NT = (((1,), (1,)), ((), ()))
_NN = (((1,), (0,)), ((), ()))

HB = 32
WIN = 8
DIL = 2
HIST = 16
LANES = 128
PRE = 16
PRE_CHUNK = 256
LN_SEGS = 16
LAG = 2
UNROLL = 2
NSLOT = 2
NEG = -1000000000.0


def _dot(a, b, dims):
    return lax.dot_general(a, b, dims, preferred_element_type=F32)


def _recip(x):
    r = pl.reciprocal(x, approx=True)
    return r * (2.0 - x * r)


def _ln(x):
    m = jnp.mean(x, axis=-1, keepdims=True)
    xc = x - m
    v = jnp.mean(xc * xc, axis=-1, keepdims=True)
    return xc * lax.rsqrt(v + 1e-05)


def _tile(a, c):
    return a[:, c * LANES:(c + 1) * LANES]


def _keep(mask, a):
    return jnp.where(mask, a, jnp.zeros_like(a))


def _drop(mask, a):
    return jnp.where(mask, jnp.zeros_like(a), a)


def _pair_softmax(s, col_a):
    m_a = jnp.max(jnp.where(col_a, s, -jnp.inf), axis=1, keepdims=True)
    m_b = jnp.max(jnp.where(col_a, -jnp.inf, s), axis=1, keepdims=True)
    e = jnp.exp(s - jnp.where(col_a, m_a, m_b))
    d_a = jnp.sum(jnp.where(col_a, e, 0.0), axis=1, keepdims=True)
    d_b = jnp.sum(jnp.where(col_a, 0.0, e), axis=1, keepdims=True)
    return e * _recip(jnp.where(col_a, d_a, d_b))


class _PassBase:
    def __init__(self, h, w_ref, wo_ref, dh):
        self.h, self.w, self.wo = h, w_ref, wo_ref
        self.pw = 2 * dh
        self.half = dh - LANES
        self.scale = dh ** (-0.5)
        self.q, self.k, self.v, self.p, self.o = {}, {}, {}, {}, {}
        self.cols = (0, 2 * LANES, wo_ref.shape[1])
        self.pending = None

    def _lane_lo(self, rows):
        return lax.broadcasted_iota(jnp.int32, (rows, LANES), 1) < self.half

    def _project(self, p, j):
        a = _dot(self.h, self.w[p, :, j * self.pw:(j + 1) * self.pw], _NN)
        self.marker = a[:8, :LANES]
        return a

    def _gate(self, s):
        if self.pending is None:
            return s
        top = jnp.where(self.always, s[:8], self.pending[:, :s.shape[1]])
        self.pending = None
        return jnp.concatenate([top, s[8:]], axis=0)

    def out(self, p, part=None):
        for k in ((0, 1) if part is None else (part,)):
            c0, c1 = self.cols[k], self.cols[k + 1]
            w = self.wo[p * self.pw:(p + 1) * self.pw, c0:c1]
            self.acc[k] = self.acc[k] + _dot(self.o[p], w, _NN)

    def run(self, n_pairs, init, b, always):
        last = n_pairs - 1
        self.acc = [init[:, :self.cols[1]], init[:, self.cols[1]:]]
        self.always = always
        done = None
        for p in range(n_pairs):
            self.proj_q(p)
            self.pending, done = done, None
            if 2 <= p < 2 + b.n_groups:
                o = b.attend(p - 2, (always, self.marker))
                done = functools.reduce(lambda u, v: u + v, o)
            self.proj_k(p)
            if p > 0:
                self.pv(p - 1)
            self.proj_v(p)
            self.scores(p)
            if p == 0:
                b.project()
            elif p < last:
                self.out(p - 1)
        yb = b.finish()
        self.out(last - 1, 0)
        self.pv(last)
        self.out(last - 1, 1)
        self.out(last)
        return jnp.concatenate(self.acc, axis=1), yb


class _TwoLayerPass(_PassBase):
    def __init__(self, h, pre_ref, pre_row, w_ref, wo_ref, *, dh, m_len, seg):
        super().__init__(h, w_ref, wo_ref, dh)
        self.pre, self.pre_row = pre_ref, pre_row
        self.m, self.seg = m_len, seg
        m2 = 2 * m_len
        n = m2 + 2 * seg
        row = lax.broadcasted_iota(jnp.int32, (n, n), 0)
        col = lax.broadcasted_iota(jnp.int32, (n, n), 1)

        def first_layer(i):
            return (i < m_len) | ((i >= m2) & (i < m2 + seg))

        def token(i):
            return jnp.where(i < m2 + seg, i - m2, i - m2 - seg)

        self.col_a = first_layer(col)
        self.diag = first_layer(row) == self.col_a
        self.allowed = (row < m2) | (col < m2) | (token(row) >= token(col))
        self.lo_m = self._lane_lo(m_len)
        self.lo_x = self._lane_lo(seg)

    def _proj(self, p, j):
        m, pw = self.m, self.pw
        a = self._project(p, j)
        pre = self.pre[p, pl.ds(self.pre_row, PRE), j * pw:(j + 1) * pw]
        n1 = self.seg - PRE
        nx = n1 + self.seg
        rest = a[:nx].astype(BF16)
        x1 = jnp.concatenate([pre, rest[:n1]], axis=0)
        return a[nx:nx + m], a[nx + m:], x1, rest[n1:]

    @staticmethod
    def _cat(ma, mb, xa, xb):
        mm = jnp.concatenate([ma, mb], axis=0).astype(BF16)
        return jnp.concatenate([mm, xa, xb], axis=0)

    def _tiles(self, m1, m2, x1, x2):
        cat, lm, lx = self._cat, self.lo_m, self.lo_x
        t0 = cat(_tile(m1, 0), _tile(m2, 0), _tile(x1, 0), _tile(x2, 0))
        t2 = cat(_tile(m2, 2), _tile(m1, 2), _tile(x2, 2), _tile(x1, 2))
        m1, m2, x1, x2 = (_tile(a, 1) for a in (m1, m2, x1, x2))
        t1a = cat(_keep(lm, m1), _drop(lm, m1), _keep(lx, x1), _drop(lx, x1))
        t1b = cat(_drop(lm, m2), _keep(lm, m2), _drop(lx, x2), _keep(lx, x2))
        return t0, t1a, t1b, t2

    def _rows_a(self, a):
        return a[:2 * self.m + self.seg]

    def _rows_b(self, a):
        m2 = 2 * self.m
        return jnp.concatenate([a[:m2], a[m2 + self.seg:]], axis=0)

    def _merge_rows(self, a, b):
        m = self.m
        return jnp.concatenate([a[:m], b[m:2 * m], a[2 * m:], b[2 * m:]],
                               axis=0)

    def proj_q(self, p):
        self.q[p] = self._cat(*self._proj(p, 0))

    def proj_k(self, p):
        self.k[p] = self._tiles(*self._proj(p, 1))

    def proj_v(self, p):
        self.v[p] = self._tiles(*self._proj(p, 2))

    def scores(self, p):
        q = self.q.pop(p)
        k0, k1a, k1b, k2 = self.k.pop(p)
        q1 = _tile(q, 1)
        r0 = _dot(_tile(q, 0), k0, _NT)
        r2 = _dot(_tile(q, 2), k2, _NT)
        r1a = _dot(self._rows_a(q1), k1a, _NT)
        r1b = _dot(self._rows_b(q1), k1b, _NT)
        s = jnp.where(self.diag, r0, r2) + self._merge_rows(r1a, r1b)
        s = self._gate(jnp.where(self.allowed, s * self.scale, NEG))
        p_all = _pair_softmax(s, self.col_a)
        self.p[p] = (p_all.astype(BF16), _keep(self.diag, p_all).astype(BF16),
                     _drop(self.diag, p_all).astype(BF16))

    def pv(self, p):
        p_all, p_diag, p_off = self.p.pop(p)
        v0, v1a, v1b, v2 = self.v.pop(p)
        o0 = _dot(p_diag, v0, _NN)
        o2 = _dot(p_off, v2, _NN)
        o1 = self._merge_rows(_dot(self._rows_a(p_all), v1a, _NN),
                              _dot(self._rows_b(p_all), v1b, _NN))
        self.o[p] = jnp.concatenate([o0, o1, o2], axis=1).astype(BF16)


class _OneLayerPass(_PassBase):
    def __init__(self, h, pre_ref, pre_row, w_ref, wo_ref, *, dh, m_len, seg):
        super().__init__(h, w_ref, wo_ref, dh)
        self.pre, self.pre_row = pre_ref, pre_row
        n = self.n = m_len + seg
        row = lax.broadcasted_iota(jnp.int32, (n, 2 * n), 0)
        col = lax.broadcasted_iota(jnp.int32, (n, 2 * n), 1)
        self.col_a = col < n
        key = jnp.where(self.col_a, col, col - n)
        self.allowed = (row < m_len) | (row >= key)
        lane = lax.broadcasted_iota(jnp.int32, (n, self.pw), 1)
        self.head0 = lane < dh

    def _project(self, p, j):
        a = super()._project(p, j)
        n, pw = self.n, self.pw
        self.pre[p, pl.ds(self.pre_row, a.shape[0] - n),
                 j * pw:(j + 1) * pw] = a[n:].astype(BF16)
        return a[:n]

    def _block_diag(self, a):
        return jnp.concatenate([_keep(self.head0, a), _drop(self.head0, a)],
                               axis=0).astype(BF16)

    def proj_q(self, p):
        self.q[p] = self._project(p, 0).astype(BF16)

    def proj_k(self, p):
        self.k[p] = self._block_diag(self._project(p, 1))

    def proj_v(self, p):
        self.v[p] = self._block_diag(self._project(p, 2))

    def scores(self, p):
        s = _dot(self.q.pop(p), self.k.pop(p), _NT)
        s = self._gate(jnp.where(self.allowed, s * self.scale, NEG))
        self.p[p] = _pair_softmax(s, self.col_a).astype(BF16)

    def pv(self, p):
        self.o[p] = _dot(self.p.pop(p), self.v.pop(p), _NN).astype(BF16)


class _BPass:
    def __init__(self, y_ref, starts, wqkv_ref, wo_ref, kv_ref, *, seg, d):
        self.y, self.starts = y_ref, starts
        self.wqkv, self.wo, self.kv = wqkv_ref, wo_ref, kv_ref
        self.seg, self.nt = seg, d // LANES
        self.scale = (d // HB) ** (-0.5)
        self.n_groups = len(starts) * seg // 8
        self.outs = []

    def project(self):
        seg, nt = self.seg, self.nt
        yn = _ln(self.y[...]).astype(BF16)
        self.q, ka, va = (_dot(yn, self.wqkv[j], _NN) for j in range(3))
        for i in range(len(self.starts)):
            self.kv[i, :, :HIST, :] = self.kv[i, :, seg:, :]
            for c in range(nt):
                rows = slice(i * seg, (i + 1) * seg)
                self.kv[i, c, HIST:, :] = _tile(ka[rows], c)
                self.kv[i, nt + c, HIST:, :] = _tile(va[rows], c)

    def attend(self, gi, after=None):
        seg, nt, kv = self.seg, self.nt, self.kv
        i, g = divmod(gi, seg // 8)
        q = [_tile(self.q[8 * gi:8 * gi + 8], c) for c in range(nt)]
        if after is not None:
            q = [jnp.where(after[0], u, after[1]) for u in q]
        pos = (lax.broadcasted_iota(jnp.int32, (8, LANES), 0)
               + (self.starts[i] + 8 * g))
        offs = [HIST + 8 * g - w * DIL for w in range(WIN)]
        logits = []
        for w, off in enumerate(offs):
            t = q[0] * kv[i, 0, off:off + 8, :]
            for c in range(1, nt):
                t = t + q[c] * kv[i, c, off:off + 8, :]
            t = t + pltpu.roll(t, 64, 1)
            t = (t + pltpu.roll(t, 32, 1)) * self.scale
            if 8 * g < w * DIL:
                t = jnp.where(pos >= w * DIL, t, NEG)
            logits.append(t)
        m = logits[0]
        for t in logits[1:]:
            m = jnp.maximum(m, t)
        es = [jnp.exp(t - m) for t in logits]
        den = es[0]
        for e in es[1:]:
            den = den + e
        inv = _recip(den)
        o = []
        for c in range(nt):
            acc = None
            for w, off in enumerate(offs):
                term = es[w] * kv[i, nt + c, off:off + 8, :]
                acc = term if acc is None else acc + term
            o.append(acc * inv)
        self.outs.append(jnp.concatenate(o, axis=1))
        return o

    def finish(self):
        o = jnp.concatenate(self.outs, axis=0).astype(BF16)
        proj = jnp.concatenate(
            [_dot(o, self.wo[c], _NN) for c in range(self.nt)], axis=1)
        return self.y[...] + proj


def _kernel(x_hbm, mem_hbm, wq_hbm, wk_hbm, wv_hbm, wo_hbm, bqkv_hbm, bo_hbm,
            out_hbm,
            x_v, mem_v, wst_v, w_v, wo_v, bq_st, bo_st, tq_s, to_s, bqkv_p,
            bo_p, out_v, xn_s, pre_s, h_s, h1_s, ra_s, y_s, kv_s,
            sems, w_sems, wo_sems, bq_sems, bo_sems,
            *, seg, n_seg, m_len, n_pairs, dh, d):
    db = d // HB
    nt = d // LANES
    pw = 2 * dh
    m2 = 2 * m_len
    n_pre = (n_seg - 1 - LAG) * PRE
    n_bq = 3 * nt

    def w_copy(p, j):
        src = (wq_hbm, wk_hbm, wv_hbm)[j]
        slot = p % NSLOT
        return pltpu.make_async_copy(
            src.at[pl.ds(p * pw, pw), :],
            wst_v.at[slot, pl.ds(j * pw, pw), :], w_sems.at[3 * slot + j])

    def wo_copy(p):
        return pltpu.make_async_copy(wo_hbm.at[pl.ds(p * pw, pw), :],
                                     wo_v.at[pl.ds(p * pw, pw), :],
                                     wo_sems.at[p])

    def bq_copy(i):
        row = pl.multiple_of((i % nt) * LANES, LANES)
        col = pl.multiple_of((i // nt) * d, LANES)
        return pltpu.make_async_copy(
            bqkv_hbm.at[pl.ds(row, LANES), pl.ds(col, d)], bq_st.at[i + 1],
            bq_sems.at[i])

    def bo_copy(i):
        col = pl.multiple_of(i * LANES, LANES)
        return pltpu.make_async_copy(bo_hbm.at[:, pl.ds(col, LANES)],
                                     bo_st.at[i + 1], bo_sems.at[i])

    xa_copy = pltpu.make_async_copy(x_hbm.at[:, :PRE, :], x_v.at[:, :PRE, :],
                                    sems.at[0])
    xb_copy = pltpu.make_async_copy(x_hbm.at[:, PRE:, :], x_v.at[:, PRE:, :],
                                    sems.at[1])
    mem_copy = pltpu.make_async_copy(mem_hbm, mem_v, sems.at[2])

    mem_copy.start()
    xa_copy.start()
    mem_copy.wait()
    for j in range(3):
        w_copy(0, j).start()

    ra_s[...] = jnp.zeros(ra_s.shape, F32)
    y_s[...] = jnp.zeros(y_s.shape, F32)
    kv_s[...] = jnp.zeros(kv_s.shape, F32)
    bq_st[0] = jnp.zeros(bq_st.shape[1:], BF16)
    bo_st[0] = jnp.zeros(bo_st.shape[1:], BF16)

    xa_copy.wait()
    for j in range(3):
        w_copy(1, j).start()
    bq_copy(0).start()
    bo_copy(0).start()
    xb_copy.start()

    def ln_block(i, carry):
        s0 = pl.multiple_of(i * LN_SEGS, LN_SEGS)
        xb = x_v[pl.ds(s0, LN_SEGS), :PRE, :].astype(F32)
        xn_s[pl.ds(pl.multiple_of(s0 * PRE, PRE), LN_SEGS * PRE), :] = _ln(
            xb.reshape(LN_SEGS * PRE, d)).astype(BF16)
        return carry

    lax.fori_loop(0, n_seg // LN_SEGS, ln_block, 0)

    def permute_rows(tmp_ref):
        return jnp.concatenate(
            [tmp_ref[pl.ds(j, HB, stride=db), :] for j in range(db)], axis=0)

    def pre_pair(p, carry):
        always = p >= 0
        slot = p % NSLOT
        n_chunk = -(-n_pre // PRE_CHUNK)
        rows16 = n_pre // 16
        bounds = [16 * (rows16 * c // n_chunk) for c in range(n_chunk + 1)]

        def last_rows(a):
            return [a[(c + 1) * LANES - 16:(c + 1) * LANES] for c in range(nt)]

        def relayout_bo():
            k = jnp.minimum(p, nt)
            to_s[...] = bo_st[k].astype(F32)
            bo = permute_rows(to_s)
            bo_p[jnp.maximum(k - 1, 0)] = bo.astype(BF16)
            g = d // nt // 16
            return [functools.reduce(
                lambda u, v: u + v,
                [bo[16 * (c * g + r):16 * (c * g + r + 1)] for r in range(g)]
            ).astype(BF16) for c in range(nt)]

        def relayout_bq():
            k = jnp.minimum(p, n_bq)
            i = jnp.maximum(k - 1, 0)
            tq_s[...] = bq_st[k].astype(F32).T
            row = pl.multiple_of((i % nt) * LANES, LANES)
            bq = permute_rows(tq_s).T.astype(BF16)
            bqkv_p[i // nt, pl.ds(row, LANES), :] = bq
            return [_tile(bq[LANES - 16:], c) for c in range(nt)]

        def transpose_w(n):
            wt = wst_v[slot, n * LANES:(n + 1) * LANES, :].T
            w_v[p, :, n * LANES:(n + 1) * LANES] = wt
            return last_rows(wt)

        for j in range(3):
            w_copy(p, j).wait()

        @pl.when((p >= 1) & (p <= n_bq))
        def _():
            bq_copy(p - 1).wait()

        @pl.when((p >= 1) & (p <= nt))
        def _():
            bo_copy(p - 1).wait()

        wo_copy(p).start()

        jobs = [functools.partial(transpose_w, n)
                for n in range(3 * pw // LANES)]
        jobs = [None, relayout_bo, relayout_bq] + jobs
        for c in range(n_chunk):
            r0, r1 = bounds[c], bounds[c + 1]
            for j in range(3):
                lhs = xn_s[LAG * PRE + r0:LAG * PRE + r1, :]
                job = jobs.pop(0) if jobs else None
                if job is not None:
                    top = jnp.where(always, lhs[:16],
                                    jnp.concatenate(job(), axis=1))
                    lhs = jnp.concatenate([top, lhs[16:]], axis=0)
                pre_s[p, r0:r1, j * pw:(j + 1) * pw] = _dot(
                    lhs, wst_v[slot, j * pw:(j + 1) * pw, :],
                    _NT).astype(BF16)
        assert not jobs

        @pl.when(p + NSLOT < n_pairs)
        def _():
            for j in range(3):
                w_copy(p + NSLOT, j).start()

        @pl.when(p + 1 < n_bq)
        def _():
            bq_copy(p + 1).start()

        @pl.when(p + 1 < nt)
        def _():
            bo_copy(p + 1).start()

        return carry

    lax.fori_loop(0, n_pairs, pre_pair, 0)

    xb_copy.wait()
    for p in range(n_pairs):
        wo_copy(p).wait()
    n1 = m_len + seg
    last_xn = (n_seg - 1) * PRE
    h1_s[:n1, :] = jnp.concatenate(
        [mem_v[...].astype(F32), _ln(x_v[0].astype(F32))],
        axis=0).astype(BF16)
    h1_s[n1:, :] = xn_s[last_xn:last_xn + m_len, :]

    def b_pass(t):
        return _BPass(y_s, ((t - 1) * seg, (t - 1 - LAG) * seg), bqkv_p, bo_p,
                      kv_s, seg=seg, d=d)

    def b_store(t, yb):
        out_v[jnp.maximum(t - 1 - LAG, 0)] = yb[seg:].astype(out_v.dtype)
        return yb[:seg]

    def two_layer_step(t, h):
        a = _TwoLayerPass(h, pre_s, pl.multiple_of((t - LAG) * PRE, PRE),
                          w_v, wo_v, dh=dh, m_len=m_len, seg=seg)
        init = jnp.concatenate(
            [jnp.zeros((m2, d), F32), x_v[t].astype(F32), ra_s[...]], axis=0)
        acc, yb = a.run(n_pairs, init, b_pass(t), t >= 0)
        x2 = b_store(t, yb)
        y_s[...] = acc[m2:]
        ra_s[...] = x2
        xn = x_v[jnp.minimum(t + 1, n_seg - 1), PRE:, :].astype(F32)
        return jnp.concatenate([_ln(xn), _ln(x2), acc[:m2]],
                               axis=0).astype(BF16)

    def two_layer_steps(i, carry):
        h = h_s[...]
        for u in range(UNROLL):
            h = two_layer_step(LAG + i * UNROLL + u, h)
        h_s[...] = h
        return carry

    def one_layer_step(t, carry):
        first = t < LAG
        extra_row = pl.multiple_of(n_pre + jnp.minimum(t, 1) * m_len, m_len)
        a = _OneLayerPass(h1_s[...], pre_s, extra_row, w_v, wo_v,
                          dh=dh, m_len=m_len, seg=seg)
        x0 = x_v[jnp.minimum(t, n_seg - 1)].astype(F32)
        init = jnp.concatenate(
            [jnp.zeros((m_len, d), F32), jnp.where(first, x0, ra_s[...])],
            axis=0)
        acc, yb = a.run(n_pairs, init, b_pass(t), t >= 0)
        x2 = b_store(t, yb)
        y = acc[m_len:]
        y_s[:seg, :] = y
        y_s[seg:, :] = y
        ra_s[...] = x2
        xn = _ln(x_v[jnp.minimum(t + 1, n_seg - 1)].astype(F32))
        x2n = _ln(x2)
        mem = acc[:m_len]
        h1_s[:n1, :] = jnp.concatenate(
            [mem, jnp.where(first, xn, x2n)], axis=0).astype(BF16)
        h1_s[n1:, :] = xn_s[last_xn + m_len:, :]
        h_s[...] = jnp.concatenate(
            [xn[PRE:], x2n, mem, mem_v[...].astype(F32)], axis=0).astype(BF16)
        return carry

    n_early_out = n_seg - 1 - LAG
    out_a = pltpu.make_async_copy(out_v.at[:n_early_out],
                                  out_hbm.at[:n_early_out], sems.at[3])
    out_b = pltpu.make_async_copy(out_v.at[n_early_out:],
                                  out_hbm.at[n_early_out:], sems.at[4])

    def phase(ph, carry):
        t0 = ph * n_seg
        lax.fori_loop(t0, t0 + LAG, one_layer_step, 0)

        @pl.when(ph == 0)
        def _():
            lax.fori_loop(0, (n_seg - LAG) // UNROLL, two_layer_steps, 0)
            out_a.start()
            hf = h_s[...].astype(F32)
            h1_s[:n1, :] = jnp.concatenate(
                [hf[2 * seg - PRE + m_len:], hf[seg - PRE:2 * seg - PRE]],
                axis=0).astype(BF16)

        return carry

    lax.fori_loop(0, 2, phase, 0)

    b = _BPass(y_s.at[seg:], ((n_seg - 1) * seg,), bqkv_p, bo_p, kv_s.at[1:],
               seg=seg, d=d)
    b.project()
    for gi in range(b.n_groups):
        b.attend(gi)
    out_v[n_seg - 1] = b.finish().astype(out_v.dtype)
    out_b.start()
    out_a.wait()
    out_b.wait()


@functools.partial(jax.jit, static_argnames=("A_seg_len",))
def pallas_interleave_layers__memory_aug_recurrent_mem_tr__sliding_local_dilated__prompt_kernel(
    A_x: jax.Array,
    A_mem0: jax.Array,
    A_Wq: jax.Array,
    A_Wk: jax.Array,
    A_Wv: jax.Array,
    A_Wo: jax.Array,
    A_seg_len,
    B_x: jax.Array,
    B_wqkv: jax.Array,
    B_wo: jax.Array,
):
    del B_x
    bsz, s_len, d = A_x.shape
    m_len = A_mem0.shape[1]
    n_heads, dh = A_Wq.shape[1], A_Wq.shape[2]
    seg = int(A_seg_len)
    n_seg = s_len // seg
    n_pairs = n_heads // 2
    nt = d // LANES
    assert bsz == 1 and s_len % seg == 0 and n_seg > LAG + 1
    assert seg % 16 == 0 and m_len == 8 and seg > PRE and seg >= HIST
    assert LAG == 2 and LAG * m_len == PRE and n_seg % LN_SEGS == 0
    assert 2 * (m_len + seg) <= LANES and (n_seg - LAG) % UNROLL == 0
    assert n_heads % 2 == 0 and 2 * dh == 3 * LANES and d % LANES == 0
    assert d % HB == 0 and LANES == 4 * HB and n_pairs > 3 * nt
    hd = n_heads * dh
    n_pre = (n_seg - LAG) * PRE

    wq_t = jnp.transpose(A_Wq, (1, 2, 0)).reshape(hd, d)
    wk_t = jnp.transpose(A_Wk, (1, 2, 0)).reshape(hd, d)
    wv_t = jnp.transpose(A_Wv, (1, 2, 0)).reshape(hd, d)
    wo = A_Wo.reshape(hd, d)

    kernel = functools.partial(
        _kernel, seg=seg, n_seg=n_seg, m_len=m_len, n_pairs=n_pairs, dh=dh,
        d=d)
    any_spec = pl.BlockSpec(memory_space=pl.ANY)
    dma = pltpu.SemaphoreType.DMA
    out = pl.pallas_call(
        kernel,
        out_shape=jax.ShapeDtypeStruct((n_seg, seg, d), A_x.dtype),
        in_specs=[any_spec] * 8,
        out_specs=any_spec,
        scratch_shapes=[
            pltpu.VMEM((n_seg, seg, d), BF16),
            pltpu.VMEM((m_len, d), BF16),
            pltpu.VMEM((NSLOT, 6 * dh, d), BF16),
            pltpu.VMEM((n_pairs, d, 6 * dh), BF16),
            pltpu.VMEM((hd, d), BF16),
            pltpu.VMEM((3 * nt + 1, LANES, d), BF16),
            pltpu.VMEM((nt + 1, d, LANES), BF16),
            pltpu.VMEM((d, LANES), F32),
            pltpu.VMEM((d, LANES), F32),
            pltpu.VMEM((3, d, d), BF16),
            pltpu.VMEM((nt, d, LANES), BF16),
            pltpu.VMEM((n_seg, seg, d), A_x.dtype),
            pltpu.VMEM((n_seg * PRE, d), BF16),
            pltpu.VMEM((n_pairs, n_pre, 6 * dh), BF16),
            pltpu.VMEM((2 * (m_len + seg) - PRE, d), BF16),
            pltpu.VMEM((2 * m_len + seg, d), BF16),
            pltpu.VMEM((seg, d), F32),
            pltpu.VMEM((2 * seg, d), F32),
            pltpu.VMEM((2, 2 * nt, HIST + seg, LANES), F32),
            dma((5,)), dma((3 * NSLOT,)), dma((n_pairs,)),
            dma((3 * nt,)), dma((nt,)),
        ],
        compiler_params=pltpu.CompilerParams(
            vmem_limit_bytes=110 * 1024 * 1024,
            disable_bounds_checks=True),
    )(A_x.reshape(n_seg, seg, d), A_mem0.reshape(m_len, d), wq_t, wk_t, wv_t,
      wo, B_wqkv, B_wo)
    return out.reshape(bsz, s_len, d)
```

```python
import functools

import jax
import jax.numpy as jnp
from jax import lax
import jax.experimental.pallas as pl
import jax.experimental.pallas.tpu as pltpu

F32 = jnp.float32
BF16 = jnp.bfloat16

_NT = (((1,), (1,)), ((), ()))
_NN = (((1,), (0,)), ((), ()))

HB = 32
WIN = 8
DIL = 2
HIST = 16
LANES = 128
PRE = 16
PRE_CHUNK = 256
LN_SEGS = 16
LAG = 2
UNROLL = 2
NSLOT = 2
NEG = -1000000000.0


def _dot(a, b, dims):
    return lax.dot_general(a, b, dims, preferred_element_type=F32)


def _recip(x):
    r = pl.reciprocal(x, approx=True)
    return r * (2.0 - x * r)


def _ln(x):
    m = jnp.mean(x, axis=-1, keepdims=True)
    xc = x - m
    v = jnp.mean(xc * xc, axis=-1, keepdims=True)
    return xc * lax.rsqrt(v + 1e-05)


def _tile(a, c):
    return a[:, c * LANES:(c + 1) * LANES]


def _keep(mask, a):
    return jnp.where(mask, a, jnp.zeros_like(a))


def _drop(mask, a):
    return jnp.where(mask, jnp.zeros_like(a), a)


def _pair_softmax(s, col_a):
    m_a = jnp.max(jnp.where(col_a, s, -jnp.inf), axis=1, keepdims=True)
    m_b = jnp.max(jnp.where(col_a, -jnp.inf, s), axis=1, keepdims=True)
    e = jnp.exp(s - jnp.where(col_a, m_a, m_b))
    d_a = jnp.sum(jnp.where(col_a, e, 0.0), axis=1, keepdims=True)
    d_b = jnp.sum(jnp.where(col_a, 0.0, e), axis=1, keepdims=True)
    return e * _recip(jnp.where(col_a, d_a, d_b))


class _PassBase:
    def __init__(self, h, w_ref, wo_ref, dh):
        self.h, self.w, self.wo = h, w_ref, wo_ref
        self.pw = 2 * dh
        self.half = dh - LANES
        self.scale = dh ** (-0.5)
        self.q, self.k, self.v, self.p, self.o = {}, {}, {}, {}, {}
        self.cols = (0, 2 * LANES, wo_ref.shape[1])
        self.pending = None

    def _lane_lo(self, rows):
        return lax.broadcasted_iota(jnp.int32, (rows, LANES), 1) < self.half

    def _project(self, p, j):
        a = _dot(self.h, self.w[p, :, j * self.pw:(j + 1) * self.pw], _NN)
        self.marker = a[:8, :LANES]
        return a

    def _gate(self, s):
        if self.pending is None:
            return s
        top = jnp.where(self.always, s[:8], self.pending[:, :s.shape[1]])
        self.pending = None
        return jnp.concatenate([top, s[8:]], axis=0)

    def out(self, p, part=None):
        for k in ((0, 1) if part is None else (part,)):
            c0, c1 = self.cols[k], self.cols[k + 1]
            w = self.wo[p * self.pw:(p + 1) * self.pw, c0:c1]
            self.acc[k] = self.acc[k] + _dot(self.o[p], w, _NN)

    def run(self, n_pairs, init, b, always):
        last = n_pairs - 1
        self.acc = [init[:, :self.cols[1]], init[:, self.cols[1]:]]
        self.always = always
        done = None
        for p in range(n_pairs):
            self.proj_q(p)
            self.pending, done = done, None
            if 2 <= p < 2 + b.n_groups:
                o = b.attend(p - 2, (always, self.marker))
                done = functools.reduce(lambda u, v: u + v, o)
            self.proj_k(p)
            if p > 0:
                self.pv(p - 1)
            self.proj_v(p)
            self.scores(p)
            if p == 0:
                b.project()
            elif p < last:
                self.out(p - 1)
        yb = b.finish()
        self.out(last - 1, 0)
        self.pv(last)
        self.out(last - 1, 1)
        self.out(last)
        return jnp.concatenate(self.acc, axis=1), yb


class _TwoLayerPass(_PassBase):
    def __init__(self, h, pre_ref, pre_row, w_ref, wo_ref, *, dh, m_len, seg):
        super().__init__(h, w_ref, wo_ref, dh)
        self.pre, self.pre_row = pre_ref, pre_row
        self.m, self.seg = m_len, seg
        m2 = 2 * m_len
        n = m2 + 2 * seg
        row = lax.broadcasted_iota(jnp.int32, (n, n), 0)
        col = lax.broadcasted_iota(jnp.int32, (n, n), 1)

        def first_layer(i):
            return (i < m_len) | ((i >= m2) & (i < m2 + seg))

        def token(i):
            return jnp.where(i < m2 + seg, i - m2, i - m2 - seg)

        self.col_a = first_layer(col)
        self.diag = first_layer(row) == self.col_a
        self.allowed = (row < m2) | (col < m2) | (token(row) >= token(col))
        self.lo_m = self._lane_lo(m_len)
        self.lo_x = self._lane_lo(seg)

    def _proj(self, p, j):
        m, pw = self.m, self.pw
        a = self._project(p, j)
        pre = self.pre[p, pl.ds(self.pre_row, PRE), j * pw:(j + 1) * pw]
        n1 = self.seg - PRE
        nx = n1 + self.seg
        rest = a[:nx].astype(BF16)
        x1 = jnp.concatenate([pre, rest[:n1]], axis=0)
        return a[nx:nx + m], a[nx + m:], x1, rest[n1:]

    @staticmethod
    def _cat(ma, mb, xa, xb):
        mm = jnp.concatenate([ma, mb], axis=0).astype(BF16)
        return jnp.concatenate([mm, xa, xb], axis=0)

    def _tiles(self, m1, m2, x1, x2):
        cat, lm, lx = self._cat, self.lo_m, self.lo_x
        t0 = cat(_tile(m1, 0), _tile(m2, 0), _tile(x1, 0), _tile(x2, 0))
        t2 = cat(_tile(m2, 2), _tile(m1, 2), _tile(x2, 2), _tile(x1, 2))
        m1, m2, x1, x2 = (_tile(a, 1) for a in (m1, m2, x1, x2))
        t1a = cat(_keep(lm, m1), _drop(lm, m1), _keep(lx, x1), _drop(lx, x1))
        t1b = cat(_drop(lm, m2), _keep(lm, m2), _drop(lx, x2), _keep(lx, x2))
        return t0, t1a, t1b, t2

    def _rows_a(self, a):
        return a[:2 * self.m + self.seg]

    def _rows_b(self, a):
        m2 = 2 * self.m
        return jnp.concatenate([a[:m2], a[m2 + self.seg:]], axis=0)

    def _merge_rows(self, a, b):
        m = self.m
        return jnp.concatenate([a[:m], b[m:2 * m], a[2 * m:], b[2 * m:]],
                               axis=0)

    def proj_q(self, p):
        self.q[p] = self._cat(*self._proj(p, 0))

    def proj_k(self, p):
        self.k[p] = self._tiles(*self._proj(p, 1))

    def proj_v(self, p):
        self.v[p] = self._tiles(*self._proj(p, 2))

    def scores(self, p):
        q = self.q.pop(p)
        k0, k1a, k1b, k2 = self.k.pop(p)
        q1 = _tile(q, 1)
        r0 = _dot(_tile(q, 0), k0, _NT)
        r2 = _dot(_tile(q, 2), k2, _NT)
        r1a = _dot(self._rows_a(q1), k1a, _NT)
        r1b = _dot(self._rows_b(q1), k1b, _NT)
        s = jnp.where(self.diag, r0, r2) + self._merge_rows(r1a, r1b)
        s = self._gate(jnp.where(self.allowed, s * self.scale, NEG))
        p_all = _pair_softmax(s, self.col_a)
        self.p[p] = (p_all.astype(BF16), _keep(self.diag, p_all).astype(BF16),
                     _drop(self.diag, p_all).astype(BF16))

    def pv(self, p):
        p_all, p_diag, p_off = self.p.pop(p)
        v0, v1a, v1b, v2 = self.v.pop(p)
        o0 = _dot(p_diag, v0, _NN)
        o2 = _dot(p_off, v2, _NN)
        o1 = self._merge_rows(_dot(self._rows_a(p_all), v1a, _NN),
                              _dot(self._rows_b(p_all), v1b, _NN))
        self.o[p] = jnp.concatenate([o0, o1, o2], axis=1).astype(BF16)


class _OneLayerPass(_PassBase):
    def __init__(self, h, pre_ref, pre_row, w_ref, wo_ref, *, dh, m_len, seg):
        super().__init__(h, w_ref, wo_ref, dh)
        self.pre, self.pre_row = pre_ref, pre_row
        n = self.n = m_len + seg
        row = lax.broadcasted_iota(jnp.int32, (n, 2 * n), 0)
        col = lax.broadcasted_iota(jnp.int32, (n, 2 * n), 1)
        self.col_a = col < n
        key = jnp.where(self.col_a, col, col - n)
        self.allowed = (row < m_len) | (row >= key)
        lane = lax.broadcasted_iota(jnp.int32, (n, self.pw), 1)
        self.head0 = lane < dh

    def _project(self, p, j):
        a = super()._project(p, j)
        n, pw = self.n, self.pw
        self.pre[p, pl.ds(self.pre_row, a.shape[0] - n),
                 j * pw:(j + 1) * pw] = a[n:].astype(BF16)
        return a[:n]

    def _block_diag(self, a):
        return jnp.concatenate([_keep(self.head0, a), _drop(self.head0, a)],
                               axis=0).astype(BF16)

    def proj_q(self, p):
        self.q[p] = self._project(p, 0).astype(BF16)

    def proj_k(self, p):
        self.k[p] = self._block_diag(self._project(p, 1))

    def proj_v(self, p):
        self.v[p] = self._block_diag(self._project(p, 2))

    def scores(self, p):
        s = _dot(self.q.pop(p), self.k.pop(p), _NT)
        s = self._gate(jnp.where(self.allowed, s * self.scale, NEG))
        self.p[p] = _pair_softmax(s, self.col_a).astype(BF16)

    def pv(self, p):
        self.o[p] = _dot(self.p.pop(p), self.v.pop(p), _NN).astype(BF16)


class _BPass:
    def __init__(self, y_ref, starts, wqkv_ref, wo_ref, kv_ref, *, seg, d):
        self.y, self.starts = y_ref, starts
        self.wqkv, self.wo, self.kv = wqkv_ref, wo_ref, kv_ref
        self.seg, self.nt = seg, d // LANES
        self.scale = (d // HB) ** (-0.5)
        self.n_groups = len(starts) * seg // 8
        self.outs = []

    def project(self):
        seg, nt = self.seg, self.nt
        yn = _ln(self.y[...]).astype(BF16)
        self.q, ka, va = (_dot(yn, self.wqkv[j], _NN) for j in range(3))
        for i in range(len(self.starts)):
            self.kv[i, :, :HIST, :] = self.kv[i, :, seg:, :]
            for c in range(nt):
                rows = slice(i * seg, (i + 1) * seg)
                self.kv[i, c, HIST:, :] = _tile(ka[rows], c)
                self.kv[i, nt + c, HIST:, :] = _tile(va[rows], c)

    def attend(self, gi, after=None):
        seg, nt, kv = self.seg, self.nt, self.kv
        i, g = divmod(gi, seg // 8)
        q = [_tile(self.q[8 * gi:8 * gi + 8], c) for c in range(nt)]
        if after is not None:
            q = [jnp.where(after[0], u, after[1]) for u in q]
        pos = (lax.broadcasted_iota(jnp.int32, (8, LANES), 0)
               + (self.starts[i] + 8 * g))
        offs = [HIST + 8 * g - w * DIL for w in range(WIN)]
        logits = []
        for w, off in enumerate(offs):
            t = q[0] * kv[i, 0, off:off + 8, :]
            for c in range(1, nt):
                t = t + q[c] * kv[i, c, off:off + 8, :]
            t = t + pltpu.roll(t, 64, 1)
            t = (t + pltpu.roll(t, 32, 1)) * self.scale
            if 8 * g < w * DIL:
                t = jnp.where(pos >= w * DIL, t, NEG)
            logits.append(t)
        m = logits[0]
        for t in logits[1:]:
            m = jnp.maximum(m, t)
        es = [jnp.exp(t - m) for t in logits]
        den = es[0]
        for e in es[1:]:
            den = den + e
        inv = _recip(den)
        o = []
        for c in range(nt):
            acc = None
            for w, off in enumerate(offs):
                term = es[w] * kv[i, nt + c, off:off + 8, :]
                acc = term if acc is None else acc + term
            o.append(acc * inv)
        self.outs.append(jnp.concatenate(o, axis=1))
        return o

    def finish(self):
        o = jnp.concatenate(self.outs, axis=0).astype(BF16)
        proj = jnp.concatenate(
            [_dot(o, self.wo[c], _NN) for c in range(self.nt)], axis=1)
        return self.y[...] + proj


def _kernel(x_hbm, mem_hbm, wq_hbm, wk_hbm, wv_hbm, wo_hbm, bqkv_hbm, bo_hbm,
            out_hbm,
            x_v, mem_v, wst_v, w_v, wo_v, bq_st, bo_st, tq_s, to_s, bqkv_p,
            bo_p, out_v, xn_s, pre_s, h_s, h1_s, ra_s, y_s, kv_s,
            sems, w_sems, wo_sems, bq_sems, bo_sems,
            *, seg, n_seg, m_len, n_pairs, dh, d):
    db = d // HB
    nt = d // LANES
    pw = 2 * dh
    m2 = 2 * m_len
    n_pre = (n_seg - 1 - LAG) * PRE
    n_bq = 3 * nt

    def w_copy(p, j):
        src = (wq_hbm, wk_hbm, wv_hbm)[j]
        slot = p % NSLOT
        return pltpu.make_async_copy(
            src.at[pl.ds(p * pw, pw), :],
            wst_v.at[slot, pl.ds(j * pw, pw), :], w_sems.at[3 * slot + j])

    def wo_copy(p):
        return pltpu.make_async_copy(wo_hbm.at[pl.ds(p * pw, pw), :],
                                     wo_v.at[pl.ds(p * pw, pw), :],
                                     wo_sems.at[p])

    def bq_copy(i):
        row = pl.multiple_of((i % nt) * LANES, LANES)
        col = pl.multiple_of((i // nt) * d, LANES)
        return pltpu.make_async_copy(
            bqkv_hbm.at[pl.ds(row, LANES), pl.ds(col, d)], bq_st.at[i + 1],
            bq_sems.at[i])

    def bo_copy(i):
        col = pl.multiple_of(i * LANES, LANES)
        return pltpu.make_async_copy(bo_hbm.at[:, pl.ds(col, LANES)],
                                     bo_st.at[i + 1], bo_sems.at[i])

    xa_copy = pltpu.make_async_copy(x_hbm.at[:, :PRE, :], x_v.at[:, :PRE, :],
                                    sems.at[0])
    xb_copy = pltpu.make_async_copy(x_hbm.at[1:, PRE:, :], x_v.at[1:, PRE:, :],
                                    sems.at[1])
    x0_copy = pltpu.make_async_copy(x_hbm.at[0, PRE:, :], x_v.at[0, PRE:, :],
                                    sems.at[5])
    mem_copy = pltpu.make_async_copy(mem_hbm, mem_v, sems.at[2])

    mem_copy.start()
    xa_copy.start()
    mem_copy.wait()
    x0_copy.start()
    for j in range(3):
        w_copy(0, j).start()

    ra_s[...] = jnp.zeros(ra_s.shape, F32)
    y_s[...] = jnp.zeros(y_s.shape, F32)
    kv_s[:, :, seg:, :] = jnp.zeros(kv_s.shape[:2] + (HIST, LANES), F32)
    bq_st[0] = jnp.zeros(bq_st.shape[1:], BF16)
    bo_st[0] = jnp.zeros(bo_st.shape[1:], BF16)

    xa_copy.wait()
    for j in range(3):
        w_copy(1, j).start()
    bq_copy(0).start()
    bo_copy(0).start()
    wo_copy(0).start()
    xb_copy.start()

    def ln_block(i, carry):
        s0 = pl.multiple_of(i * LN_SEGS, LN_SEGS)
        xb = x_v[pl.ds(s0, LN_SEGS), :PRE, :].astype(F32)
        xn_s[pl.ds(pl.multiple_of(s0 * PRE, PRE), LN_SEGS * PRE), :] = _ln(
            xb.reshape(LN_SEGS * PRE, d)).astype(BF16)
        return carry

    lax.fori_loop(0, n_seg // LN_SEGS, ln_block, 0)

    n1 = m_len + seg
    last_xn = (n_seg - 1) * PRE
    x0_copy.wait()
    h1_s[:n1, :] = jnp.concatenate(
        [mem_v[...].astype(F32), _ln(x_v[0].astype(F32))],
        axis=0).astype(BF16)
    h1_s[n1:, :] = xn_s[last_xn:last_xn + m_len, :]

    def permute_rows(tmp_ref):
        return jnp.concatenate(
            [tmp_ref[pl.ds(j, HB, stride=db), :] for j in range(db)], axis=0)

    def pre_pair(p, carry):
        always = p >= 0
        slot = p % NSLOT
        n_chunk = -(-n_pre // PRE_CHUNK)
        rows16 = n_pre // 16
        bounds = [16 * (rows16 * c // n_chunk) for c in range(n_chunk + 1)]

        def last_rows(a):
            return [a[(c + 1) * LANES - 16:(c + 1) * LANES] for c in range(nt)]

        def relayout_bo():
            k = jnp.minimum(p, nt)
            to_s[:d, :] = bo_st[k].astype(F32)
            bo = permute_rows(to_s)
            bo_p[jnp.maximum(k - 1, 0)] = bo.astype(BF16)
            g = d // nt // 16
            return [functools.reduce(
                lambda u, v: u + v,
                [bo[16 * (c * g + r):16 * (c * g + r + 1)] for r in range(g)]
            ).astype(BF16) for c in range(nt)]

        def relayout_bq():
            k = jnp.minimum(p, n_bq)
            i = jnp.maximum(k - 1, 0)
            tq_s[:d, :] = bq_st[k].astype(F32).T
            row = pl.multiple_of((i % nt) * LANES, LANES)
            bq = permute_rows(tq_s).T.astype(BF16)
            bqkv_p[i // nt, pl.ds(row, LANES), :] = bq
            return [_tile(bq[LANES - 16:], c) for c in range(nt)]

        def transpose_w(n):
            wt = wst_v[slot, n * LANES:(n + 1) * LANES, :].T
            w_v[p, :, n * LANES:(n + 1) * LANES] = wt
            return last_rows(wt)

        for j in range(3):
            w_copy(p, j).wait()

        @pl.when((p >= 1) & (p <= n_bq))
        def _():
            bq_copy(p - 1).wait()

        @pl.when((p >= 1) & (p <= nt))
        def _():
            bo_copy(p - 1).wait()

        jobs = [functools.partial(transpose_w, n)
                for n in range(3 * pw // LANES)]
        jobs = [None, relayout_bo, relayout_bq] + jobs
        for c in range(n_chunk):
            r0, r1 = bounds[c], bounds[c + 1]
            for j in range(3):
                lhs = xn_s[LAG * PRE + r0:LAG * PRE + r1, :]
                job = jobs.pop(0) if jobs else None
                if job is not None:
                    top = jnp.where(always, lhs[:16],
                                    jnp.concatenate(job(), axis=1))
                    lhs = jnp.concatenate([top, lhs[16:]], axis=0)
                pre_s[p, r0:r1, j * pw:(j + 1) * pw] = _dot(
                    lhs, wst_v[slot, j * pw:(j + 1) * pw, :],
                    _NT).astype(BF16)
        assert not jobs

        @pl.when(p + NSLOT < n_pairs)
        def _():
            for j in range(3):
                w_copy(p + NSLOT, j).start()

        @pl.when(p + 1 < n_pairs)
        def _():
            wo_copy(p + 1).start()

        @pl.when(p + 1 < n_bq)
        def _():
            bq_copy(p + 1).start()

        @pl.when(p + 1 < nt)
        def _():
            bo_copy(p + 1).start()

        return carry

    lax.fori_loop(0, n_pairs, pre_pair, 0)

    xb_copy.wait()
    for p in range(n_pairs):
        wo_copy(p).wait()

    def b_pass(t):
        return _BPass(y_s, ((t - 1) * seg, (t - 1 - LAG) * seg), bqkv_p, bo_p,
                      kv_s, seg=seg, d=d)

    def b_store(t, yb):
        out_v[jnp.maximum(t - 1 - LAG, 0)] = yb[seg:].astype(out_v.dtype)
        return yb[:seg]

    def two_layer_step(t, h):
        a = _TwoLayerPass(h, pre_s, pl.multiple_of((t - LAG) * PRE, PRE),
                          w_v, wo_v, dh=dh, m_len=m_len, seg=seg)
        init = jnp.concatenate(
            [jnp.zeros((m2, d), F32), x_v[t].astype(F32), ra_s[...]], axis=0)
        acc, yb = a.run(n_pairs, init, b_pass(t), t >= 0)
        x2 = b_store(t, yb)
        y_s[...] = acc[m2:]
        ra_s[...] = x2
        xn = x_v[jnp.minimum(t + 1, n_seg - 1), PRE:, :].astype(F32)
        return jnp.concatenate([_ln(xn), _ln(x2), acc[:m2]],
                               axis=0).astype(BF16)

    def two_layer_steps(i, carry):
        h = h_s[...]
        for u in range(UNROLL):
            h = two_layer_step(LAG + i * UNROLL + u, h)
        h_s[...] = h
        return carry

    def one_layer_step(t, carry):
        first = t < LAG
        extra_row = pl.multiple_of(n_pre + jnp.minimum(t, 1) * m_len, m_len)
        a = _OneLayerPass(h1_s[...], pre_s, extra_row, w_v, wo_v,
                          dh=dh, m_len=m_len, seg=seg)
        x0 = x_v[jnp.minimum(t, n_seg - 1)].astype(F32)
        init = jnp.concatenate(
            [jnp.zeros((m_len, d), F32), jnp.where(first, x0, ra_s[...])],
            axis=0)
        acc, yb = a.run(n_pairs, init, b_pass(t), t >= 0)
        x2 = b_store(t, yb)
        y = acc[m_len:]
        y_s[:seg, :] = y
        y_s[seg:, :] = y
        ra_s[...] = x2
        xn = _ln(x_v[jnp.minimum(t + 1, n_seg - 1)].astype(F32))
        x2n = _ln(x2)
        mem = acc[:m_len]
        h1_s[:n1, :] = jnp.concatenate(
            [mem, jnp.where(first, xn, x2n)], axis=0).astype(BF16)
        h1_s[n1:, :] = xn_s[last_xn + m_len:, :]
        h_s[...] = jnp.concatenate(
            [xn[PRE:], x2n, mem, mem_v[...].astype(F32)], axis=0).astype(BF16)
        return carry

    n_early_out = n_seg - 1 - LAG
    out_a = pltpu.make_async_copy(out_v.at[:n_early_out],
                                  out_hbm.at[:n_early_out], sems.at[3])
    out_b = pltpu.make_async_copy(out_v.at[n_early_out:],
                                  out_hbm.at[n_early_out:], sems.at[4])

    def phase(ph, carry):
        t0 = ph * n_seg
        lax.fori_loop(t0, t0 + LAG, one_layer_step, 0)

        @pl.when(ph == 0)
        def _():
            lax.fori_loop(0, (n_seg - LAG) // UNROLL, two_layer_steps, 0)
            out_a.start()
            hf = h_s[...].astype(F32)
            h1_s[:n1, :] = jnp.concatenate(
                [hf[2 * seg - PRE + m_len:], hf[seg - PRE:2 * seg - PRE]],
                axis=0).astype(BF16)

        return carry

    lax.fori_loop(0, 2, phase, 0)

    b = _BPass(y_s.at[seg:], ((n_seg - 1) * seg,), bqkv_p, bo_p, kv_s.at[1:],
               seg=seg, d=d)
    b.project()
    for gi in range(b.n_groups):
        b.attend(gi)
    out_v[n_seg - 1] = b.finish().astype(out_v.dtype)
    out_b.start()
    out_a.wait()
    out_b.wait()


@functools.partial(jax.jit, static_argnames=("A_seg_len",))
def pallas_interleave_layers__memory_aug_recurrent_mem_tr__sliding_local_dilated__prompt_kernel(
    A_x: jax.Array,
    A_mem0: jax.Array,
    A_Wq: jax.Array,
    A_Wk: jax.Array,
    A_Wv: jax.Array,
    A_Wo: jax.Array,
    A_seg_len,
    B_x: jax.Array,
    B_wqkv: jax.Array,
    B_wo: jax.Array,
):
    del B_x
    bsz, s_len, d = A_x.shape
    m_len = A_mem0.shape[1]
    n_heads, dh = A_Wq.shape[1], A_Wq.shape[2]
    seg = int(A_seg_len)
    n_seg = s_len // seg
    n_pairs = n_heads // 2
    nt = d // LANES
    assert bsz == 1 and s_len % seg == 0 and n_seg > LAG + 1
    assert seg % 16 == 0 and m_len == 8 and seg > PRE and seg >= HIST
    assert LAG == 2 and LAG * m_len == PRE and n_seg % LN_SEGS == 0
    assert 2 * (m_len + seg) <= LANES and (n_seg - LAG) % UNROLL == 0
    assert n_heads % 2 == 0 and 2 * dh == 3 * LANES and d % LANES == 0
    assert d % HB == 0 and LANES == 4 * HB and n_pairs > 3 * nt
    hd = n_heads * dh
    n_pre = (n_seg - LAG) * PRE

    wq_t = jnp.transpose(A_Wq, (1, 2, 0)).reshape(hd, d)
    wk_t = jnp.transpose(A_Wk, (1, 2, 0)).reshape(hd, d)
    wv_t = jnp.transpose(A_Wv, (1, 2, 0)).reshape(hd, d)
    wo = A_Wo.reshape(hd, d)

    kernel = functools.partial(
        _kernel, seg=seg, n_seg=n_seg, m_len=m_len, n_pairs=n_pairs, dh=dh,
        d=d)
    any_spec = pl.BlockSpec(memory_space=pl.ANY)
    dma = pltpu.SemaphoreType.DMA
    out = pl.pallas_call(
        kernel,
        out_shape=jax.ShapeDtypeStruct((n_seg, seg, d), A_x.dtype),
        in_specs=[any_spec] * 8,
        out_specs=any_spec,
        scratch_shapes=[
            pltpu.VMEM((n_seg, seg, d), BF16),
            pltpu.VMEM((m_len, d), BF16),
            pltpu.VMEM((NSLOT, 6 * dh, d), BF16),
            pltpu.VMEM((n_pairs, d, 6 * dh), BF16),
            pltpu.VMEM((hd, d), BF16),
            pltpu.VMEM((3 * nt + 1, LANES, d), BF16),
            pltpu.VMEM((nt + 1, d, LANES), BF16),
            pltpu.VMEM((d + HB, LANES), F32),
            pltpu.VMEM((d + HB, LANES), F32),
            pltpu.VMEM((3, d, d), BF16),
            pltpu.VMEM((nt, d, LANES), BF16),
            pltpu.VMEM((n_seg, seg, d), A_x.dtype),
            pltpu.VMEM((n_seg * PRE, d), BF16),
            pltpu.VMEM((n_pairs, n_pre, 6 * dh), BF16),
            pltpu.VMEM((2 * (m_len + seg) - PRE, d), BF16),
            pltpu.VMEM((2 * m_len + seg, d), BF16),
            pltpu.VMEM((seg, d), F32),
            pltpu.VMEM((2 * seg, d), F32),
            pltpu.VMEM((2, 2 * nt, HIST + seg, LANES), F32),
            dma((6,)), dma((3 * NSLOT,)), dma((n_pairs,)),
            dma((3 * nt,)), dma((nt,)),
        ],
        compiler_params=pltpu.CompilerParams(
            vmem_limit_bytes=110 * 1024 * 1024,
            disable_bounds_checks=True),
    )(A_x.reshape(n_seg, seg, d), A_mem0.reshape(m_len, d), wq_t, wk_t, wv_t,
      wo, B_wqkv, B_wo)
    return out.reshape(bsz, s_len, d)
```

```python
import functools

import jax
import jax.numpy as jnp
from jax import lax
import jax.experimental.pallas as pl
import jax.experimental.pallas.tpu as pltpu

F32 = jnp.float32
BF16 = jnp.bfloat16

_NT = (((1,), (1,)), ((), ()))
_NN = (((1,), (0,)), ((), ()))

HB = 32
WIN = 8
DIL = 2
HIST = 16
LANES = 128
PRE = 16
PRE_CHUNK = 256
LN_SEGS = 16
LAG = 2
UNROLL = 2
NSLOT = 2
NEG = -1000000000.0


def _dot(a, b, dims):
    return lax.dot_general(a, b, dims, preferred_element_type=F32)


def _recip(x):
    r = pl.reciprocal(x, approx=True)
    return r * (2.0 - x * r)


def _ln(x):
    m = jnp.mean(x, axis=-1, keepdims=True)
    xc = x - m
    v = jnp.mean(xc * xc, axis=-1, keepdims=True)
    return xc * lax.rsqrt(v + 1e-05)


def _tile(a, c):
    return a[:, c * LANES:(c + 1) * LANES]


def _keep(mask, a):
    return jnp.where(mask, a, jnp.zeros_like(a))


def _drop(mask, a):
    return jnp.where(mask, jnp.zeros_like(a), a)


def _pair_softmax(s, col_a):
    m_a = jnp.max(jnp.where(col_a, s, -jnp.inf), axis=1, keepdims=True)
    m_b = jnp.max(jnp.where(col_a, -jnp.inf, s), axis=1, keepdims=True)
    e = jnp.exp(s - jnp.where(col_a, m_a, m_b))
    d_a = jnp.sum(jnp.where(col_a, e, 0.0), axis=1, keepdims=True)
    d_b = jnp.sum(jnp.where(col_a, 0.0, e), axis=1, keepdims=True)
    return e * _recip(jnp.where(col_a, d_a, d_b))


class _PassBase:
    def __init__(self, h, w_ref, wo_ref, dh):
        self.h, self.w, self.wo = h, w_ref, wo_ref
        self.pw = 2 * dh
        self.half = dh - LANES
        self.scale = dh ** (-0.5)
        self.q, self.k, self.v, self.p, self.o = {}, {}, {}, {}, {}
        self.cols = (0, 2 * LANES, wo_ref.shape[1])
        self.pending = None

    def _lane_lo(self, rows):
        return lax.broadcasted_iota(jnp.int32, (rows, LANES), 1) < self.half

    def _project(self, p, j):
        a = _dot(self.h, self.w[p, :, j * self.pw:(j + 1) * self.pw], _NN)
        self.marker = a[:8, :LANES]
        return a

    def _gate(self, s):
        if self.pending is None:
            return s
        top = jnp.where(self.always, s[:8], self.pending[:, :s.shape[1]])
        self.pending = None
        return jnp.concatenate([top, s[8:]], axis=0)

    def out(self, p, part=None):
        for k in ((0, 1) if part is None else (part,)):
            c0, c1 = self.cols[k], self.cols[k + 1]
            w = self.wo[p * self.pw:(p + 1) * self.pw, c0:c1]
            self.acc[k] = self.acc[k] + _dot(self.o[p], w, _NN)

    def run(self, n_pairs, init, b, always):
        last = n_pairs - 1
        self.acc = [init[:, :self.cols[1]], init[:, self.cols[1]:]]
        self.always = always
        done = None
        for p in range(n_pairs):
            self.proj_q(p)
            self.pending, done = done, None
            if 2 <= p < 2 + b.n_groups:
                o = b.attend(p - 2, (always, self.marker))
                done = functools.reduce(lambda u, v: u + v, o)
            self.proj_k(p)
            if p > 0:
                self.pv(p - 1)
            self.proj_v(p)
            self.scores(p)
            if p == 0:
                b.project()
            elif p < last:
                self.out(p - 1)
        yb = b.finish()
        self.out(last - 1, 0)
        self.pv(last)
        self.out(last - 1, 1)
        self.out(last)
        return jnp.concatenate(self.acc, axis=1), yb


class _TwoLayerPass(_PassBase):
    def __init__(self, h, pre_ref, pre_row, w_ref, wo_ref, *, dh, m_len, seg):
        super().__init__(h, w_ref, wo_ref, dh)
        self.pre, self.pre_row = pre_ref, pre_row
        self.m, self.seg = m_len, seg
        m2 = 2 * m_len
        n = m2 + 2 * seg
        row = lax.broadcasted_iota(jnp.int32, (n, n), 0)
        col = lax.broadcasted_iota(jnp.int32, (n, n), 1)

        def first_layer(i):
            return (i < m_len) | ((i >= m2) & (i < m2 + seg))

        def token(i):
            return jnp.where(i < m2 + seg, i - m2, i - m2 - seg)

        self.col_a = first_layer(col)
        self.diag = first_layer(row) == self.col_a
        self.allowed = (row < m2) | (col < m2) | (token(row) >= token(col))
        self.lo_m = self._lane_lo(m_len)
        self.lo_x = self._lane_lo(seg)

    def _proj(self, p, j):
        m, pw = self.m, self.pw
        a = self._project(p, j)
        pre = self.pre[p, pl.ds(self.pre_row, PRE), j * pw:(j + 1) * pw]
        n1 = self.seg - PRE
        nx = n1 + self.seg
        rest = a[:nx].astype(BF16)
        x1 = jnp.concatenate([pre, rest[:n1]], axis=0)
        return a[nx:nx + m], a[nx + m:], x1, rest[n1:]

    @staticmethod
    def _cat(ma, mb, xa, xb):
        mm = jnp.concatenate([ma, mb], axis=0).astype(BF16)
        return jnp.concatenate([mm, xa, xb], axis=0)

    def _tiles(self, m1, m2, x1, x2):
        cat, lm, lx = self._cat, self.lo_m, self.lo_x
        t0 = cat(_tile(m1, 0), _tile(m2, 0), _tile(x1, 0), _tile(x2, 0))
        t2 = cat(_tile(m2, 2), _tile(m1, 2), _tile(x2, 2), _tile(x1, 2))
        m1, m2, x1, x2 = (_tile(a, 1) for a in (m1, m2, x1, x2))
        t1a = cat(_keep(lm, m1), _drop(lm, m1), _keep(lx, x1), _drop(lx, x1))
        t1b = cat(_drop(lm, m2), _keep(lm, m2), _drop(lx, x2), _keep(lx, x2))
        return t0, t1a, t1b, t2

    def _rows_a(self, a):
        return a[:2 * self.m + self.seg]

    def _rows_b(self, a):
        m2 = 2 * self.m
        return jnp.concatenate([a[:m2], a[m2 + self.seg:]], axis=0)

    def _merge_rows(self, a, b):
        m = self.m
        return jnp.concatenate([a[:m], b[m:2 * m], a[2 * m:], b[2 * m:]],
                               axis=0)

    def proj_q(self, p):
        self.q[p] = self._cat(*self._proj(p, 0))

    def proj_k(self, p):
        self.k[p] = self._tiles(*self._proj(p, 1))

    def proj_v(self, p):
        self.v[p] = self._tiles(*self._proj(p, 2))

    def scores(self, p):
        q = self.q.pop(p)
        k0, k1a, k1b, k2 = self.k.pop(p)
        q1 = _tile(q, 1)
        r0 = _dot(_tile(q, 0), k0, _NT)
        r2 = _dot(_tile(q, 2), k2, _NT)
        r1a = _dot(self._rows_a(q1), k1a, _NT)
        r1b = _dot(self._rows_b(q1), k1b, _NT)
        s = jnp.where(self.diag, r0, r2) + self._merge_rows(r1a, r1b)
        s = self._gate(jnp.where(self.allowed, s * self.scale, NEG))
        p_all = _pair_softmax(s, self.col_a)
        self.p[p] = (p_all.astype(BF16), _keep(self.diag, p_all).astype(BF16),
                     _drop(self.diag, p_all).astype(BF16))

    def pv(self, p):
        p_all, p_diag, p_off = self.p.pop(p)
        v0, v1a, v1b, v2 = self.v.pop(p)
        o0 = _dot(p_diag, v0, _NN)
        o2 = _dot(p_off, v2, _NN)
        o1 = self._merge_rows(_dot(self._rows_a(p_all), v1a, _NN),
                              _dot(self._rows_b(p_all), v1b, _NN))
        self.o[p] = jnp.concatenate([o0, o1, o2], axis=1).astype(BF16)


class _OneLayerPass(_PassBase):
    def __init__(self, h, pre_ref, pre_row, w_ref, wo_ref, *, dh, m_len, seg):
        super().__init__(h, w_ref, wo_ref, dh)
        self.pre, self.pre_row = pre_ref, pre_row
        n = self.n = m_len + seg
        row = lax.broadcasted_iota(jnp.int32, (n, 2 * n), 0)
        col = lax.broadcasted_iota(jnp.int32, (n, 2 * n), 1)
        self.col_a = col < n
        key = jnp.where(self.col_a, col, col - n)
        self.allowed = (row < m_len) | (row >= key)
        lane = lax.broadcasted_iota(jnp.int32, (n, self.pw), 1)
        self.head0 = lane < dh

    def _project(self, p, j):
        a = super()._project(p, j)
        n, pw = self.n, self.pw
        self.pre[p, pl.ds(self.pre_row, a.shape[0] - n),
                 j * pw:(j + 1) * pw] = a[n:].astype(BF16)
        return a[:n]

    def _block_diag(self, a):
        return jnp.concatenate([_keep(self.head0, a), _drop(self.head0, a)],
                               axis=0).astype(BF16)

    def proj_q(self, p):
        self.q[p] = self._project(p, 0).astype(BF16)

    def proj_k(self, p):
        self.k[p] = self._block_diag(self._project(p, 1))

    def proj_v(self, p):
        self.v[p] = self._block_diag(self._project(p, 2))

    def scores(self, p):
        s = _dot(self.q.pop(p), self.k.pop(p), _NT)
        s = self._gate(jnp.where(self.allowed, s * self.scale, NEG))
        self.p[p] = _pair_softmax(s, self.col_a).astype(BF16)

    def pv(self, p):
        self.o[p] = _dot(self.p.pop(p), self.v.pop(p), _NN).astype(BF16)


class _BPass:
    def __init__(self, y_ref, starts, wqkv_ref, wo_ref, kv_ref, kv_next_ref,
                 *, seg, d):
        self.y, self.starts = y_ref, starts
        self.wqkv, self.wo, self.kv = wqkv_ref, wo_ref, kv_ref
        self.kv_next = kv_next_ref
        self.seg, self.nt = seg, d // LANES
        self.scale = (d // HB) ** (-0.5)
        self.n_groups = len(starts) * seg // 8
        self.outs = []

    def project(self):
        seg, nt = self.seg, self.nt
        yn = _ln(self.y[...]).astype(BF16)
        self.q, ka, va = (_dot(yn, self.wqkv[j], _NN) for j in range(3))
        for i in range(len(self.starts)):
            for c in range(2 * nt):
                a = _tile((ka, va)[c // nt][i * seg:(i + 1) * seg], c % nt)
                self.kv[i, c, HIST:, :] = a
                if self.kv_next is not None:
                    self.kv_next[i, c, :HIST, :] = a[seg - HIST:]

    def attend(self, gi, after=None):
        seg, nt, kv = self.seg, self.nt, self.kv
        i, g = divmod(gi, seg // 8)
        q = [_tile(self.q[8 * gi:8 * gi + 8], c) for c in range(nt)]
        if after is not None:
            q = [jnp.where(after[0], u, after[1]) for u in q]
        pos = (lax.broadcasted_iota(jnp.int32, (8, LANES), 0)
               + (self.starts[i] + 8 * g))
        offs = [HIST + 8 * g - w * DIL for w in range(WIN)]
        logits = []
        for w, off in enumerate(offs):
            t = q[0] * kv[i, 0, off:off + 8, :]
            for c in range(1, nt):
                t = t + q[c] * kv[i, c, off:off + 8, :]
            t = t + pltpu.roll(t, 64, 1)
            t = (t + pltpu.roll(t, 32, 1)) * self.scale
            if 8 * g < w * DIL:
                t = jnp.where(pos >= w * DIL, t, NEG)
            logits.append(t)
        m = logits[0]
        for t in logits[1:]:
            m = jnp.maximum(m, t)
        es = [jnp.exp(t - m) for t in logits]
        den = es[0]
        for e in es[1:]:
            den = den + e
        inv = _recip(den)
        o = []
        for c in range(nt):
            acc = None
            for w, off in enumerate(offs):
                term = es[w] * kv[i, nt + c, off:off + 8, :]
                acc = term if acc is None else acc + term
            o.append(acc * inv)
        self.outs.append(jnp.concatenate(o, axis=1))
        return o

    def finish(self):
        o = jnp.concatenate(self.outs, axis=0).astype(BF16)
        proj = jnp.concatenate(
            [_dot(o, self.wo[c], _NN) for c in range(self.nt)], axis=1)
        return self.y[...] + proj


def _kernel(x_hbm, mem_hbm, wq_hbm, wk_hbm, wv_hbm, wo_hbm, bqkv_hbm, bo_hbm,
            out_hbm,
            x_v, mem_v, wst_v, w_v, wo_v, bq_st, bo_st, tq_s, to_s, bqkv_p,
            bo_p, out_v, xn_s, pre_s, h_s, h1_s, ra_s, y_s, kv_s,
            sems, w_sems, wo_sems, bq_sems, bo_sems,
            *, seg, n_seg, m_len, n_pairs, dh, d):
    db = d // HB
    nt = d // LANES
    pw = 2 * dh
    m2 = 2 * m_len
    n_pre = (n_seg - 1 - LAG) * PRE
    n_bq = 3 * nt

    def w_copy(p, j):
        src = (wq_hbm, wk_hbm, wv_hbm)[j]
        slot = p % NSLOT
        return pltpu.make_async_copy(
            src.at[pl.ds(p * pw, pw), :],
            wst_v.at[slot, pl.ds(j * pw, pw), :], w_sems.at[3 * slot + j])

    def wo_copy(p):
        return pltpu.make_async_copy(wo_hbm.at[pl.ds(p * pw, pw), :],
                                     wo_v.at[pl.ds(p * pw, pw), :],
                                     wo_sems.at[p])

    def bq_copy(i):
        row = pl.multiple_of((i % nt) * LANES, LANES)
        col = pl.multiple_of((i // nt) * d, LANES)
        return pltpu.make_async_copy(
            bqkv_hbm.at[pl.ds(row, LANES), pl.ds(col, d)], bq_st.at[i + 1],
            bq_sems.at[i])

    def bo_copy(i):
        col = pl.multiple_of(i * LANES, LANES)
        return pltpu.make_async_copy(bo_hbm.at[:, pl.ds(col, LANES)],
                                     bo_st.at[i + 1], bo_sems.at[i])

    xa_copy = pltpu.make_async_copy(x_hbm.at[:, :PRE, :], x_v.at[:, :PRE, :],
                                    sems.at[0])
    xb_copy = pltpu.make_async_copy(x_hbm.at[1:, PRE:, :], x_v.at[1:, PRE:, :],
                                    sems.at[1])
    x0_copy = pltpu.make_async_copy(x_hbm.at[0, PRE:, :], x_v.at[0, PRE:, :],
                                    sems.at[5])
    mem_copy = pltpu.make_async_copy(mem_hbm, mem_v, sems.at[2])

    mem_copy.start()
    xa_copy.start()
    mem_copy.wait()
    x0_copy.start()
    for j in range(3):
        w_copy(0, j).start()

    ra_s[...] = jnp.zeros(ra_s.shape, F32)
    y_s[...] = jnp.zeros(y_s.shape, F32)
    kv_s[0, :, :, :HIST, :] = jnp.zeros(kv_s.shape[1:3] + (HIST, LANES), F32)
    bq_st[0] = jnp.zeros(bq_st.shape[1:], BF16)
    bo_st[0] = jnp.zeros(bo_st.shape[1:], BF16)

    xa_copy.wait()
    for j in range(3):
        w_copy(1, j).start()
    bq_copy(0).start()
    bo_copy(0).start()
    wo_copy(0).start()
    xb_copy.start()

    def ln_block(i, carry):
        s0 = pl.multiple_of(i * LN_SEGS, LN_SEGS)
        xb = x_v[pl.ds(s0, LN_SEGS), :PRE, :].astype(F32)
        xn_s[pl.ds(pl.multiple_of(s0 * PRE, PRE), LN_SEGS * PRE), :] = _ln(
            xb.reshape(LN_SEGS * PRE, d)).astype(BF16)
        return carry

    lax.fori_loop(0, n_seg // LN_SEGS, ln_block, 0)

    n1 = m_len + seg
    last_xn = (n_seg - 1) * PRE
    x0_copy.wait()
    h1_s[:n1, :] = jnp.concatenate(
        [mem_v[...].astype(F32), _ln(x_v[0].astype(F32))],
        axis=0).astype(BF16)
    h1_s[n1:, :] = xn_s[last_xn:last_xn + m_len, :]

    def permute_rows(tmp_ref):
        return jnp.concatenate(
            [tmp_ref[pl.ds(j, HB, stride=db), :] for j in range(db)], axis=0)

    def pre_pair(p, carry):
        always = p >= 0
        slot = p % NSLOT
        n_chunk = -(-n_pre // PRE_CHUNK)
        rows16 = n_pre // 16
        bounds = [16 * (rows16 * c // n_chunk) for c in range(n_chunk + 1)]

        def last_rows(a):
            return [a[(c + 1) * LANES - 16:(c + 1) * LANES] for c in range(nt)]

        def relayout_bo():
            k = jnp.minimum(p, nt)
            to_s[:d, :] = bo_st[k].astype(F32)
            bo = permute_rows(to_s)
            bo_p[jnp.maximum(k - 1, 0)] = bo.astype(BF16)
            g = d // nt // 16
            return [functools.reduce(
                lambda u, v: u + v,
                [bo[16 * (c * g + r):16 * (c * g + r + 1)] for r in range(g)]
            ).astype(BF16) for c in range(nt)]

        def relayout_bq():
            k = jnp.minimum(p, n_bq)
            i = jnp.maximum(k - 1, 0)
            tq_s[:d, :] = bq_st[k].astype(F32).T
            row = pl.multiple_of((i % nt) * LANES, LANES)
            bq = permute_rows(tq_s).T.astype(BF16)
            bqkv_p[i // nt, pl.ds(row, LANES), :] = bq
            return [_tile(bq[LANES - 16:], c) for c in range(nt)]

        def transpose_w(n):
            wt = wst_v[slot, n * LANES:(n + 1) * LANES, :].T
            w_v[p, :, n * LANES:(n + 1) * LANES] = wt
            return last_rows(wt)

        for j in range(3):
            w_copy(p, j).wait()

        @pl.when((p >= 1) & (p <= n_bq))
        def _():
            bq_copy(p - 1).wait()

        @pl.when((p >= 1) & (p <= nt))
        def _():
            bo_copy(p - 1).wait()

        jobs = [functools.partial(transpose_w, n)
                for n in range(3 * pw // LANES)]
        jobs = [None, relayout_bo, relayout_bq] + jobs
        for c in range(n_chunk):
            r0, r1 = bounds[c], bounds[c + 1]
            for j in range(3):
                lhs = xn_s[LAG * PRE + r0:LAG * PRE + r1, :]
                job = jobs.pop(0) if jobs else None
                if job is not None:
                    top = jnp.where(always, lhs[:16],
                                    jnp.concatenate(job(), axis=1))
                    lhs = jnp.concatenate([top, lhs[16:]], axis=0)
                pre_s[p, r0:r1, j * pw:(j + 1) * pw] = _dot(
                    lhs, wst_v[slot, j * pw:(j + 1) * pw, :],
                    _NT).astype(BF16)
        assert not jobs

        @pl.when(p + NSLOT < n_pairs)
        def _():
            for j in range(3):
                w_copy(p + NSLOT, j).start()

        @pl.when(p + 1 < n_pairs)
        def _():
            wo_copy(p + 1).start()

        @pl.when(p + 1 < n_bq)
        def _():
            bq_copy(p + 1).start()

        @pl.when(p + 1 < nt)
        def _():
            bo_copy(p + 1).start()

        return carry

    lax.fori_loop(0, n_pairs, pre_pair, 0)

    xb_copy.wait()
    for p in range(n_pairs):
        wo_copy(p).wait()

    def b_pass(t, par):
        return _BPass(y_s, ((t - 1) * seg, (t - 1 - LAG) * seg), bqkv_p, bo_p,
                      kv_s.at[par], kv_s.at[1 - par], seg=seg, d=d)

    def b_store(t, yb):
        out_v[jnp.maximum(t - 1 - LAG, 0)] = yb[seg:].astype(out_v.dtype)
        return yb[:seg]

    def two_layer_step(t, par, h):
        a = _TwoLayerPass(h, pre_s, pl.multiple_of((t - LAG) * PRE, PRE),
                          w_v, wo_v, dh=dh, m_len=m_len, seg=seg)
        init = jnp.concatenate(
            [jnp.zeros((m2, d), F32), x_v[t].astype(F32), ra_s[...]], axis=0)
        acc, yb = a.run(n_pairs, init, b_pass(t, par), t >= 0)
        x2 = b_store(t, yb)
        y_s[...] = acc[m2:]
        ra_s[...] = x2
        xn = x_v[jnp.minimum(t + 1, n_seg - 1), PRE:, :].astype(F32)
        return jnp.concatenate([_ln(xn), _ln(x2), acc[:m2]],
                               axis=0).astype(BF16)

    def two_layer_steps(i, carry):
        h = h_s[...]
        for u in range(UNROLL):
            h = two_layer_step(LAG + i * UNROLL + u, (LAG + u) % 2, h)
        h_s[...] = h
        return carry

    def one_layer_step(t, carry):
        first = t < LAG
        extra_row = pl.multiple_of(n_pre + jnp.minimum(t, 1) * m_len, m_len)
        a = _OneLayerPass(h1_s[...], pre_s, extra_row, w_v, wo_v,
                          dh=dh, m_len=m_len, seg=seg)
        x0 = x_v[jnp.minimum(t, n_seg - 1)].astype(F32)
        init = jnp.concatenate(
            [jnp.zeros((m_len, d), F32), jnp.where(first, x0, ra_s[...])],
            axis=0)
        acc, yb = a.run(n_pairs, init, b_pass(t, t & 1), t >= 0)
        x2 = b_store(t, yb)
        y = acc[m_len:]
        y_s[:seg, :] = y
        y_s[seg:, :] = y
        ra_s[...] = x2
        xn = _ln(x_v[jnp.minimum(t + 1, n_seg - 1)].astype(F32))
        x2n = _ln(x2)
        mem = acc[:m_len]
        h1_s[:n1, :] = jnp.concatenate(
            [mem, jnp.where(first, xn, x2n)], axis=0).astype(BF16)
        h1_s[n1:, :] = xn_s[last_xn + m_len:, :]
        h_s[...] = jnp.concatenate(
            [xn[PRE:], x2n, mem, mem_v[...].astype(F32)], axis=0).astype(BF16)
        return carry

    n_early_out = n_seg - 1 - LAG
    out_a = pltpu.make_async_copy(out_v.at[:n_early_out],
                                  out_hbm.at[:n_early_out], sems.at[3])
    out_b = pltpu.make_async_copy(out_v.at[n_early_out:],
                                  out_hbm.at[n_early_out:], sems.at[4])

    def phase(ph, carry):
        t0 = ph * n_seg
        lax.fori_loop(t0, t0 + LAG, one_layer_step, 0)

        @pl.when(ph == 0)
        def _():
            lax.fori_loop(0, (n_seg - LAG) // UNROLL, two_layer_steps, 0)
            out_a.start()
            hf = h_s[...].astype(F32)
            h1_s[:n1, :] = jnp.concatenate(
                [hf[2 * seg - PRE + m_len:], hf[seg - PRE:2 * seg - PRE]],
                axis=0).astype(BF16)

        return carry

    lax.fori_loop(0, 2, phase, 0)

    b = _BPass(y_s.at[seg:], ((n_seg - 1) * seg,), bqkv_p, bo_p,
               kv_s.at[(n_seg + LAG) % 2, 1:], None, seg=seg, d=d)
    b.project()
    for gi in range(b.n_groups):
        b.attend(gi)
    out_v[n_seg - 1] = b.finish().astype(out_v.dtype)
    out_b.start()
    out_a.wait()
    out_b.wait()


@functools.partial(jax.jit, static_argnames=("A_seg_len",))
def pallas_interleave_layers__memory_aug_recurrent_mem_tr__sliding_local_dilated__prompt_kernel(
    A_x: jax.Array,
    A_mem0: jax.Array,
    A_Wq: jax.Array,
    A_Wk: jax.Array,
    A_Wv: jax.Array,
    A_Wo: jax.Array,
    A_seg_len,
    B_x: jax.Array,
    B_wqkv: jax.Array,
    B_wo: jax.Array,
):
    del B_x
    bsz, s_len, d = A_x.shape
    m_len = A_mem0.shape[1]
    n_heads, dh = A_Wq.shape[1], A_Wq.shape[2]
    seg = int(A_seg_len)
    n_seg = s_len // seg
    n_pairs = n_heads // 2
    nt = d // LANES
    assert bsz == 1 and s_len % seg == 0 and n_seg > LAG + 1
    assert seg % 16 == 0 and m_len == 8 and seg > PRE and seg >= HIST
    assert LAG == 2 and LAG * m_len == PRE and n_seg % LN_SEGS == 0
    assert 2 * (m_len + seg) <= LANES and (n_seg - LAG) % UNROLL == 0 == UNROLL % 2
    assert n_heads % 2 == 0 and 2 * dh == 3 * LANES and d % LANES == 0
    assert d % HB == 0 and LANES == 4 * HB and n_pairs > 3 * nt
    hd = n_heads * dh
    n_pre = (n_seg - LAG) * PRE

    wq_t = jnp.transpose(A_Wq, (1, 2, 0)).reshape(hd, d)
    wk_t = jnp.transpose(A_Wk, (1, 2, 0)).reshape(hd, d)
    wv_t = jnp.transpose(A_Wv, (1, 2, 0)).reshape(hd, d)
    wo = A_Wo.reshape(hd, d)

    kernel = functools.partial(
        _kernel, seg=seg, n_seg=n_seg, m_len=m_len, n_pairs=n_pairs, dh=dh,
        d=d)
    any_spec = pl.BlockSpec(memory_space=pl.ANY)
    dma = pltpu.SemaphoreType.DMA
    out = pl.pallas_call(
        kernel,
        out_shape=jax.ShapeDtypeStruct((n_seg, seg, d), A_x.dtype),
        in_specs=[any_spec] * 8,
        out_specs=any_spec,
        scratch_shapes=[
            pltpu.VMEM((n_seg, seg, d), BF16),
            pltpu.VMEM((m_len, d), BF16),
            pltpu.VMEM((NSLOT, 6 * dh, d), BF16),
            pltpu.VMEM((n_pairs, d, 6 * dh), BF16),
            pltpu.VMEM((hd, d), BF16),
            pltpu.VMEM((3 * nt + 1, LANES, d), BF16),
            pltpu.VMEM((nt + 1, d, LANES), BF16),
            pltpu.VMEM((d + HB, LANES), F32),
            pltpu.VMEM((d + HB, LANES), F32),
            pltpu.VMEM((3, d, d), BF16),
            pltpu.VMEM((nt, d, LANES), BF16),
            pltpu.VMEM((n_seg, seg, d), A_x.dtype),
            pltpu.VMEM((n_seg * PRE, d), BF16),
            pltpu.VMEM((n_pairs, n_pre, 6 * dh), BF16),
            pltpu.VMEM((2 * (m_len + seg) - PRE, d), BF16),
            pltpu.VMEM((2 * m_len + seg, d), BF16),
            pltpu.VMEM((seg, d), F32),
            pltpu.VMEM((2 * seg, d), F32),
            pltpu.VMEM((2, 2, 2 * nt, HIST + seg, LANES), F32),
            dma((6,)), dma((3 * NSLOT,)), dma((n_pairs,)),
            dma((3 * nt,)), dma((nt,)),
        ],
        compiler_params=pltpu.CompilerParams(
            vmem_limit_bytes=110 * 1024 * 1024,
            disable_bounds_checks=True),
    )(A_x.reshape(n_seg, seg, d), A_mem0.reshape(m_len, d), wq_t, wk_t, wv_t,
      wo, B_wqkv, B_wo)
    return out.reshape(bsz, s_len, d)
```

```python
import functools

import jax
import jax.numpy as jnp
from jax import lax
import jax.experimental.pallas as pl
import jax.experimental.pallas.tpu as pltpu

F32 = jnp.float32
BF16 = jnp.bfloat16

_NT = (((1,), (1,)), ((), ()))
_NN = (((1,), (0,)), ((), ()))

SEG_LEN = 32
HB = 32
WIN = 8
DIL = 2
HIST = 16
LANES = 128
PRE = 16
PRE_CHUNK = 256
LN_SEGS = 16
LAG = 2
UNROLL = 2
NSLOT = 2
NEG = -1000000000.0


def _dot(a, b, dims):
    return lax.dot_general(a, b, dims, preferred_element_type=F32)


def _recip(x):
    r = pl.reciprocal(x, approx=True)
    return r * (2.0 - x * r)


def _ln(x):
    m = jnp.mean(x, axis=-1, keepdims=True)
    xc = x - m
    v = jnp.mean(xc * xc, axis=-1, keepdims=True)
    return xc * lax.rsqrt(v + 1e-05)


def _tile(a, c):
    return a[:, c * LANES:(c + 1) * LANES]


def _keep(mask, a):
    return jnp.where(mask, a, jnp.zeros_like(a))


def _drop(mask, a):
    return jnp.where(mask, jnp.zeros_like(a), a)


def _pair_softmax(s, col_a):
    m_a = jnp.max(jnp.where(col_a, s, -jnp.inf), axis=1, keepdims=True)
    m_b = jnp.max(jnp.where(col_a, -jnp.inf, s), axis=1, keepdims=True)
    e = jnp.exp(s - jnp.where(col_a, m_a, m_b))
    d_a = jnp.sum(jnp.where(col_a, e, 0.0), axis=1, keepdims=True)
    d_b = jnp.sum(jnp.where(col_a, 0.0, e), axis=1, keepdims=True)
    return e * _recip(jnp.where(col_a, d_a, d_b))


class _PassBase:
    def __init__(self, h, w_ref, wo_ref, dh):
        self.h, self.w, self.wo = h, w_ref, wo_ref
        self.pw = 2 * dh
        self.half = dh - LANES
        self.scale = dh ** (-0.5)
        self.q, self.k, self.v, self.p, self.o = {}, {}, {}, {}, {}
        self.cols = (0, 2 * LANES, wo_ref.shape[1])
        self.pending = None

    def _lane_lo(self, rows):
        return lax.broadcasted_iota(jnp.int32, (rows, LANES), 1) < self.half

    def _project(self, p, j):
        a = _dot(self.h, self.w[p, :, j * self.pw:(j + 1) * self.pw], _NN)
        self.marker = a[:8, :LANES]
        return a

    def _gate(self, s):
        if self.pending is None:
            return s
        top = jnp.where(self.always, s[:8], self.pending[:, :s.shape[1]])
        self.pending = None
        return jnp.concatenate([top, s[8:]], axis=0)

    def out(self, p, part=None):
        for k in ((0, 1) if part is None else (part,)):
            c0, c1 = self.cols[k], self.cols[k + 1]
            w = self.wo[p * self.pw:(p + 1) * self.pw, c0:c1]
            self.acc[k] = self.acc[k] + _dot(self.o[p], w, _NN)

    def run(self, n_pairs, init, b, always):
        last = n_pairs - 1
        self.acc = [init[:, :self.cols[1]], init[:, self.cols[1]:]]
        self.always = always
        done = None
        for p in range(n_pairs):
            self.proj_q(p)
            self.pending, done = done, None
            if 2 <= p < 2 + b.n_groups:
                o = b.attend(p - 2, (always, self.marker))
                done = functools.reduce(lambda u, v: u + v, o)
            self.proj_k(p)
            if p > 0:
                self.pv(p - 1)
            self.proj_v(p)
            self.scores(p)
            if p == 0:
                b.project()
            elif p < last:
                self.out(p - 1)
        yb = b.finish()
        self.out(last - 1, 0)
        self.pv(last)
        self.out(last - 1, 1)
        self.out(last)
        return jnp.concatenate(self.acc, axis=1), yb


class _TwoLayerPass(_PassBase):
    def __init__(self, h, pre_ref, pre_row, w_ref, wo_ref, *, dh, m_len, seg):
        super().__init__(h, w_ref, wo_ref, dh)
        self.pre, self.pre_row = pre_ref, pre_row
        u = self.u = m_len
        n = self.n = 2 * (m_len + seg)
        self.ext = 4 * u
        self.seg = seg
        row = lax.broadcasted_iota(jnp.int32, (n, n + self.ext), 0)
        col = lax.broadcasted_iota(jnp.int32, (n, n + self.ext), 1)
        rep = col >= n
        col = jnp.where(rep, col - n, col)

        def first_layer(i):
            return (((i < 6 * u) & ((i & u) == 0))
                    | ((i >= 6 * u) & (i < 6 * u + PRE)))

        def index(i):
            low = ((i >> 1) & ~(u - 1)) + (i & (u - 1))
            high = jnp.where(i < 6 * u + PRE, i - 3 * u, i - 3 * u - PRE)
            return jnp.where(i < 6 * u, low, high)

        self.col_a = first_layer(col)
        self.diag = first_layer(row) == self.col_a
        used = ((row >= 3 * u) & (row < 4 * u)) == rep
        self.allowed = used & ((row < 2 * u) | (index(row) >= index(col)))
        self.fill = jnp.where(used, NEG, -jnp.inf)
        self.lo_u = self._lane_lo(u)
        self.lo_c = self._lane_lo(PRE)

    def _proj(self, p, j):
        u, pw, seg = self.u, self.pw, self.seg
        r = self._project(p, j)
        c1 = self.pre[p, pl.ds(self.pre_row, PRE), j * pw:(j + 1) * pw]
        nx = 2 * u + seg
        return ((r[nx:nx + u], r[:u], r[u:2 * u], c1),
                (r[nx + u:], r[2 * u:3 * u], r[3 * u:4 * u],
                 r[4 * u:nx].astype(BF16)))

    @staticmethod
    def _weave(f, g):
        top = jnp.concatenate([f[0], g[0], f[1], g[1], f[2], g[2]], axis=0)
        return jnp.concatenate([top.astype(BF16), f[3], g[3]], axis=0)

    def _tiles(self, l1, l2):
        masks = (self.lo_u,) * 3 + (self.lo_c,)

        def t(l, c):
            return [_tile(a, c) for a in l]

        def lo(l):
            return [_keep(mk, a) for mk, a in zip(masks, l)]

        def hi(l):
            return [_drop(mk, a) for mk, a in zip(masks, l)]

        def extend(a, b):
            return jnp.concatenate([a, b[:self.ext]], axis=0)

        t0 = self._weave(t(l1, 0), t(l2, 0))
        t2 = self._weave(t(l2, 2), t(l1, 2))
        t1a = self._weave(lo(t(l1, 1)), hi(t(l1, 1)))
        t1b = self._weave(hi(t(l2, 1)), lo(t(l2, 1)))
        return extend(t0, t0), extend(t1a, t1b), t1b, extend(t2, t2)

    def _split_rows(self, l1, l2):
        ra = jnp.concatenate([l1[0], l1[2], l1[1], l2[1]], axis=0)
        rb = jnp.concatenate([l2[0], l2[2]], axis=0)
        return (jnp.concatenate([ra.astype(BF16), l1[3]], axis=0),
                jnp.concatenate([rb.astype(BF16), l2[3]], axis=0))

    def _units(self, ra, rb):
        u = self.u
        return ((ra[:u], ra[2 * u:3 * u], ra[u:2 * u], ra[4 * u:]),
                (rb[:u], ra[3 * u:4 * u], rb[u:2 * u], rb[2 * u:]))

    def _unweave(self, a):
        u = self.u
        return ((a[:u], a[2 * u:3 * u], a[4 * u:5 * u], a[6 * u:6 * u + PRE]),
                (a[u:2 * u], a[3 * u:4 * u], a[5 * u:6 * u], a[6 * u + PRE:]))

    def proj_q(self, p):
        l1, l2 = self._proj(p, 0)
        q0, q2 = (self._weave([_tile(a, c) for a in l1],
                              [_tile(a, c) for a in l2]) for c in (0, 2))
        qa, qb = self._split_rows([_tile(a, 1) for a in l1],
                                  [_tile(a, 1) for a in l2])
        self.q[p] = (q0, qa, qb, q2)

    def proj_k(self, p):
        self.k[p] = self._tiles(*self._proj(p, 1))

    def proj_v(self, p):
        self.v[p] = self._tiles(*self._proj(p, 2))

    def scores(self, p):
        q0, qa, qb, q2 = self.q.pop(p)
        k0, k1a, k1b, k2 = self.k.pop(p)
        r0 = _dot(q0, k0, _NT)
        r2 = _dot(q2, k2, _NT)
        ra = _dot(qa, k1a, _NT)
        rb = _dot(qb, k1b, _NT)
        rb = jnp.concatenate(
            [rb, jnp.zeros((rb.shape[0], self.ext), F32)], axis=1)
        f, g = self._units(ra, rb)
        r1 = jnp.concatenate(
            [f[0], g[0], f[1], g[1], f[2], g[2], f[3], g[3]], axis=0)
        s = jnp.where(self.diag, r0, r2) + r1
        s = self._gate(jnp.where(self.allowed, s * self.scale, self.fill))
        p_all = _pair_softmax(s, self.col_a)
        f, g = self._unweave(p_all)
        pa, pb = self._split_rows(f[:3] + (f[3].astype(BF16),),
                                  g[:3] + (g[3].astype(BF16),))
        self.p[p] = (_keep(self.diag, p_all).astype(BF16), pa,
                     pb[:, :self.n], _drop(self.diag, p_all).astype(BF16))

    def pv(self, p):
        p0, pa, pb, p2 = self.p.pop(p)
        v0, v1a, v1b, v2 = self.v.pop(p)
        o0 = self._unweave(_dot(p0, v0, _NN))
        o2 = self._unweave(_dot(p2, v2, _NN))
        o1 = self._units(_dot(pa, v1a, _NN), _dot(pb, v1b, _NN))
        self.o[p] = jnp.concatenate(
            [jnp.concatenate((f[0], g[0]) + f[1:] + g[1:], axis=0)
             for f, g in (o0, o1, o2)], axis=1).astype(BF16)


class _OneLayerPass(_PassBase):
    def __init__(self, h, pre_ref, pre_row, w_ref, wo_ref, *, dh, m_len, seg):
        super().__init__(h, w_ref, wo_ref, dh)
        self.pre, self.pre_row = pre_ref, pre_row
        n = self.n = m_len + seg
        row = lax.broadcasted_iota(jnp.int32, (n, 2 * n), 0)
        col = lax.broadcasted_iota(jnp.int32, (n, 2 * n), 1)
        self.col_a = col < n
        key = jnp.where(self.col_a, col, col - n)
        self.allowed = (row < m_len) | (row >= key)
        lane = lax.broadcasted_iota(jnp.int32, (n, self.pw), 1)
        self.head0 = lane < dh

    def _project(self, p, j):
        a = super()._project(p, j)
        n, pw = self.n, self.pw
        self.pre[p, pl.ds(self.pre_row, a.shape[0] - n),
                 j * pw:(j + 1) * pw] = a[n:].astype(BF16)
        return a[:n]

    def _block_diag(self, a):
        return jnp.concatenate([_keep(self.head0, a), _drop(self.head0, a)],
                               axis=0).astype(BF16)

    def proj_q(self, p):
        self.q[p] = self._project(p, 0).astype(BF16)

    def proj_k(self, p):
        self.k[p] = self._block_diag(self._project(p, 1))

    def proj_v(self, p):
        self.v[p] = self._block_diag(self._project(p, 2))

    def scores(self, p):
        s = _dot(self.q.pop(p), self.k.pop(p), _NT)
        s = self._gate(jnp.where(self.allowed, s * self.scale, NEG))
        self.p[p] = _pair_softmax(s, self.col_a).astype(BF16)

    def pv(self, p):
        self.o[p] = _dot(self.p.pop(p), self.v.pop(p), _NN).astype(BF16)


class _BPass:
    def __init__(self, y_ref, starts, wqkv_ref, wo_ref, kv_ref, kv_next_ref,
                 *, seg, d):
        self.y, self.starts = y_ref, starts
        self.wqkv, self.wo, self.kv = wqkv_ref, wo_ref, kv_ref
        self.kv_next = kv_next_ref
        self.seg, self.nt = seg, d // LANES
        self.scale = (d // HB) ** (-0.5)
        self.n_groups = len(starts) * seg // 8
        self.outs = []

    def project(self):
        seg, nt = self.seg, self.nt
        yn = _ln(self.y[...]).astype(BF16)
        self.q, ka, va = (_dot(yn, self.wqkv[j], _NN) for j in range(3))
        for i in range(len(self.starts)):
            for c in range(2 * nt):
                a = _tile((ka, va)[c // nt][i * seg:(i + 1) * seg], c % nt)
                self.kv[i, c, HIST:, :] = a
                if self.kv_next is not None:
                    self.kv_next[i, c, :HIST, :] = a[seg - HIST:]

    def attend(self, gi, after=None):
        seg, nt, kv = self.seg, self.nt, self.kv
        i, g = divmod(gi, seg // 8)
        q = [_tile(self.q[8 * gi:8 * gi + 8], c) for c in range(nt)]
        if after is not None:
            q = [jnp.where(after[0], u, after[1]) for u in q]
        pos = (lax.broadcasted_iota(jnp.int32, (8, LANES), 0)
               + (self.starts[i] + 8 * g))
        offs = [HIST + 8 * g - w * DIL for w in range(WIN)]
        logits = []
        for w, off in enumerate(offs):
            t = q[0] * kv[i, 0, off:off + 8, :]
            for c in range(1, nt):
                t = t + q[c] * kv[i, c, off:off + 8, :]
            t = t + pltpu.roll(t, 64, 1)
            t = (t + pltpu.roll(t, 32, 1)) * self.scale
            if 8 * g < w * DIL:
                t = jnp.where(pos >= w * DIL, t, NEG)
            logits.append(t)
        m = logits[0]
        for t in logits[1:]:
            m = jnp.maximum(m, t)
        es = [jnp.exp(t - m) for t in logits]
        den = es[0]
        for e in es[1:]:
            den = den + e
        inv = _recip(den)
        o = []
        for c in range(nt):
            acc = None
            for w, off in enumerate(offs):
                term = es[w] * kv[i, nt + c, off:off + 8, :]
                acc = term if acc is None else acc + term
            o.append(acc * inv)
        self.outs.append(jnp.concatenate(o, axis=1))
        return o

    def finish(self):
        o = jnp.concatenate(self.outs, axis=0).astype(BF16)
        proj = jnp.concatenate(
            [_dot(o, self.wo[c], _NN) for c in range(self.nt)], axis=1)
        return self.y[...] + proj


def _kernel(x_hbm, mem_hbm, wq_hbm, wk_hbm, wv_hbm, wo_hbm, bqkv_hbm, bo_hbm,
            out_hbm,
            x_v, mem_v, wst_v, w_v, wo_v, bq_st, bo_st, tq_s, to_s, bqkv_p,
            bo_p, out_v, xn_s, pre_s, h_s, h1_s, ra_s, y_s, kv_s,
            sems, w_sems, wo_sems, bq_sems, bo_sems,
            *, seg, n_seg, m_len, n_pairs, dh, d):
    db = d // HB
    nt = d // LANES
    pw = 2 * dh
    m2 = 2 * m_len
    n_pre = (n_seg - 1 - LAG) * PRE
    n_bq = 3 * nt

    def w_copy(p, j):
        src = (wq_hbm, wk_hbm, wv_hbm)[j]
        slot = p % NSLOT
        return pltpu.make_async_copy(
            src.at[pl.ds(p * pw, pw), :],
            wst_v.at[slot, pl.ds(j * pw, pw), :], w_sems.at[3 * slot + j])

    def wo_copy(p):
        return pltpu.make_async_copy(wo_hbm.at[pl.ds(p * pw, pw), :],
                                     wo_v.at[pl.ds(p * pw, pw), :],
                                     wo_sems.at[p])

    def bq_copy(i):
        row = pl.multiple_of((i % nt) * LANES, LANES)
        col = pl.multiple_of((i // nt) * d, LANES)
        return pltpu.make_async_copy(
            bqkv_hbm.at[pl.ds(row, LANES), pl.ds(col, d)], bq_st.at[i + 1],
            bq_sems.at[i])

    def bo_copy(i):
        col = pl.multiple_of(i * LANES, LANES)
        return pltpu.make_async_copy(bo_hbm.at[:, pl.ds(col, LANES)],
                                     bo_st.at[i + 1], bo_sems.at[i])

    nf = seg - PRE
    xa_copy = pltpu.make_async_copy(x_hbm.at[:, nf:, :], x_v.at[:, nf:, :],
                                    sems.at[0])
    xb_copy = pltpu.make_async_copy(x_hbm.at[1:, :nf, :], x_v.at[1:, :nf, :],
                                    sems.at[1])
    x0_copy = pltpu.make_async_copy(x_hbm.at[0, :nf, :], x_v.at[0, :nf, :],
                                    sems.at[5])
    mem_copy = pltpu.make_async_copy(mem_hbm, mem_v, sems.at[2])

    mem_copy.start()
    xa_copy.start()
    mem_copy.wait()
    x0_copy.start()
    for j in range(3):
        w_copy(0, j).start()

    ra_s[...] = jnp.zeros(ra_s.shape, F32)
    y_s[...] = jnp.zeros(y_s.shape, F32)
    kv_s[0, :, :, :HIST, :] = jnp.zeros(kv_s.shape[1:3] + (HIST, LANES), F32)
    bq_st[0] = jnp.zeros(bq_st.shape[1:], BF16)
    bo_st[0] = jnp.zeros(bo_st.shape[1:], BF16)

    xa_copy.wait()
    for j in range(3):
        w_copy(1, j).start()
    bq_copy(0).start()
    bo_copy(0).start()
    wo_copy(0).start()
    xb_copy.start()

    def ln_block(i, carry):
        s0 = pl.multiple_of(i * LN_SEGS, LN_SEGS)
        xb = x_v[pl.ds(s0, LN_SEGS), nf:, :].astype(F32)
        xn_s[pl.ds(pl.multiple_of(s0 * PRE, PRE), LN_SEGS * PRE), :] = _ln(
            xb.reshape(LN_SEGS * PRE, d)).astype(BF16)
        return carry

    lax.fori_loop(0, n_seg // LN_SEGS, ln_block, 0)

    n1 = m_len + seg
    last_xn = (n_seg - 1) * PRE
    x0_copy.wait()
    h1_s[:n1, :] = jnp.concatenate(
        [mem_v[...].astype(F32), _ln(x_v[0].astype(F32))],
        axis=0).astype(BF16)
    h1_s[n1:, :] = xn_s[last_xn:last_xn + m_len, :]

    def permute_rows(tmp_ref):
        return jnp.concatenate(
            [tmp_ref[pl.ds(j, HB, stride=db), :] for j in range(db)], axis=0)

    def pre_pair(p, carry):
        always = p >= 0
        slot = p % NSLOT
        n_chunk = -(-n_pre // PRE_CHUNK)
        rows16 = n_pre // 16
        bounds = [16 * (rows16 * c // n_chunk) for c in range(n_chunk + 1)]

        def last_rows(a):
            return [a[(c + 1) * LANES - 16:(c + 1) * LANES] for c in range(nt)]

        def relayout_bo():
            k = jnp.minimum(p, nt)
            to_s[:d, :] = bo_st[k].astype(F32)
            bo = permute_rows(to_s)
            bo_p[jnp.maximum(k - 1, 0)] = bo.astype(BF16)
            g = d // nt // 16
            return [functools.reduce(
                lambda u, v: u + v,
                [bo[16 * (c * g + r):16 * (c * g + r + 1)] for r in range(g)]
            ).astype(BF16) for c in range(nt)]

        def relayout_bq():
            k = jnp.minimum(p, n_bq)
            i = jnp.maximum(k - 1, 0)
            tq_s[:d, :] = bq_st[k].astype(F32).T
            row = pl.multiple_of((i % nt) * LANES, LANES)
            bq = permute_rows(tq_s).T.astype(BF16)
            bqkv_p[i // nt, pl.ds(row, LANES), :] = bq
            return [_tile(bq[LANES - 16:], c) for c in range(nt)]

        def transpose_w(n):
            wt = wst_v[slot, n * LANES:(n + 1) * LANES, :].T
            w_v[p, :, n * LANES:(n + 1) * LANES] = wt
            return last_rows(wt)

        for j in range(3):
            w_copy(p, j).wait()

        @pl.when((p >= 1) & (p <= n_bq))
        def _():
            bq_copy(p - 1).wait()

        @pl.when((p >= 1) & (p <= nt))
        def _():
            bo_copy(p - 1).wait()

        jobs = [functools.partial(transpose_w, n)
                for n in range(3 * pw // LANES)]
        jobs = [None, relayout_bo, relayout_bq] + jobs
        for c in range(n_chunk):
            r0, r1 = bounds[c], bounds[c + 1]
            for j in range(3):
                lhs = xn_s[LAG * PRE + r0:LAG * PRE + r1, :]
                job = jobs.pop(0) if jobs else None
                if job is not None:
                    top = jnp.where(always, lhs[:16],
                                    jnp.concatenate(job(), axis=1))
                    lhs = jnp.concatenate([top, lhs[16:]], axis=0)
                pre_s[p, r0:r1, j * pw:(j + 1) * pw] = _dot(
                    lhs, wst_v[slot, j * pw:(j + 1) * pw, :],
                    _NT).astype(BF16)
        assert not jobs

        @pl.when(p + NSLOT < n_pairs)
        def _():
            for j in range(3):
                w_copy(p + NSLOT, j).start()

        @pl.when(p + 1 < n_pairs)
        def _():
            wo_copy(p + 1).start()

        @pl.when(p + 1 < n_bq)
        def _():
            bq_copy(p + 1).start()

        @pl.when(p + 1 < nt)
        def _():
            bo_copy(p + 1).start()

        return carry

    lax.fori_loop(0, n_pairs, pre_pair, 0)

    xb_copy.wait()
    for p in range(n_pairs):
        wo_copy(p).wait()

    def b_pass(t, par):
        return _BPass(y_s, ((t - 1) * seg, (t - 1 - LAG) * seg), bqkv_p, bo_p,
                      kv_s.at[par], kv_s.at[1 - par], seg=seg, d=d)

    def b_store(t, yb):
        out_v[jnp.maximum(t - 1 - LAG, 0)] = yb[seg:].astype(out_v.dtype)
        return yb[:seg]

    def two_layer_step(t, par, h):
        a = _TwoLayerPass(h, pre_s, pl.multiple_of((t - LAG) * PRE, PRE),
                          w_v, wo_v, dh=dh, m_len=m_len, seg=seg)
        init = jnp.concatenate(
            [jnp.zeros((m2, d), F32), x_v[t].astype(F32), ra_s[...]], axis=0)
        acc, yb = a.run(n_pairs, init, b_pass(t, par), t >= 0)
        x2 = b_store(t, yb)
        y_s[...] = acc[m2:]
        ra_s[...] = x2
        xn = x_v[jnp.minimum(t + 1, n_seg - 1), :nf, :].astype(F32)
        return jnp.concatenate([_ln(xn), _ln(x2), acc[:m2]],
                               axis=0).astype(BF16)

    def two_layer_steps(i, carry):
        h = h_s[...]
        for u in range(UNROLL):
            h = two_layer_step(LAG + i * UNROLL + u, (LAG + u) % 2, h)
        h_s[...] = h
        return carry

    def one_layer_step(t, carry):
        first = t < LAG
        extra_row = pl.multiple_of(n_pre + jnp.minimum(t, 1) * m_len, m_len)
        a = _OneLayerPass(h1_s[...], pre_s, extra_row, w_v, wo_v,
                          dh=dh, m_len=m_len, seg=seg)
        x0 = x_v[jnp.minimum(t, n_seg - 1)].astype(F32)
        init = jnp.concatenate(
            [jnp.zeros((m_len, d), F32), jnp.where(first, x0, ra_s[...])],
            axis=0)
        acc, yb = a.run(n_pairs, init, b_pass(t, t & 1), t >= 0)
        x2 = b_store(t, yb)
        y = acc[m_len:]
        y_s[:seg, :] = y
        y_s[seg:, :] = y
        ra_s[...] = x2
        xn = _ln(x_v[jnp.minimum(t + 1, n_seg - 1)].astype(F32))
        x2n = _ln(x2)
        mem = acc[:m_len]
        h1_s[:n1, :] = jnp.concatenate(
            [mem, jnp.where(first, xn, x2n)], axis=0).astype(BF16)
        h1_s[n1:, :] = xn_s[last_xn + m_len:, :]
        h_s[...] = jnp.concatenate(
            [xn[:nf], x2n, mem, mem_v[...].astype(F32)], axis=0).astype(BF16)
        return carry

    n_early_out = n_seg - 1 - LAG
    out_a = pltpu.make_async_copy(out_v.at[:n_early_out],
                                  out_hbm.at[:n_early_out], sems.at[3])
    out_b = pltpu.make_async_copy(out_v.at[n_early_out:],
                                  out_hbm.at[n_early_out:], sems.at[4])

    def phase(ph, carry):
        t0 = ph * n_seg
        lax.fori_loop(t0, t0 + LAG, one_layer_step, 0)

        @pl.when(ph == 0)
        def _():
            lax.fori_loop(0, (n_seg - LAG) // UNROLL, two_layer_steps, 0)
            out_a.start()
            hf = h_s[...].astype(F32)
            h1_s[:n1, :] = jnp.concatenate(
                [hf[nf + seg + m_len:], hf[nf:nf + seg]],
                axis=0).astype(BF16)

        return carry

    lax.fori_loop(0, 2, phase, 0)

    b = _BPass(y_s.at[seg:], ((n_seg - 1) * seg,), bqkv_p, bo_p,
               kv_s.at[(n_seg + LAG) % 2, 1:], None, seg=seg, d=d)
    b.project()
    for gi in range(b.n_groups):
        b.attend(gi)
    out_v[n_seg - 1] = b.finish().astype(out_v.dtype)
    out_b.start()
    out_a.wait()
    out_b.wait()


def pallas_interleave_layers__memory_aug_recurrent_mem_tr__sliding_local_dilated__prompt_kernel(
    A_x: jax.Array,
    A_mem0: jax.Array,
    A_Wq: jax.Array,
    A_Wk: jax.Array,
    A_Wv: jax.Array,
    A_Wo: jax.Array,
    A_seg_len,
    B_x: jax.Array,
    B_wqkv: jax.Array,
    B_wo: jax.Array,
):
    del B_x
    seg = A_seg_len if isinstance(A_seg_len, int) else SEG_LEN
    return _forward(A_x, A_mem0, A_Wq, A_Wk, A_Wv, A_Wo, B_wqkv, B_wo, seg=seg)


@functools.partial(jax.jit, static_argnames=("seg",))
def _forward(A_x, A_mem0, A_Wq, A_Wk, A_Wv, A_Wo, B_wqkv, B_wo, *, seg):
    bsz, s_len, d = A_x.shape
    m_len = A_mem0.shape[1]
    n_heads, dh = A_Wq.shape[1], A_Wq.shape[2]
    n_seg = s_len // seg
    n_pairs = n_heads // 2
    nt = d // LANES
    assert bsz == 1 and s_len % seg == 0 and n_seg > LAG + 1
    assert m_len == 8 and seg == 2 * m_len + PRE and seg >= HIST
    assert LAG == 2 and LAG * m_len == PRE and n_seg % LN_SEGS == 0
    assert 2 * (m_len + seg) + 4 * m_len <= LANES
    assert (n_seg - LAG) % UNROLL == 0 and UNROLL % 2 == 0
    assert n_heads % 2 == 0 and 2 * dh == 3 * LANES and d % LANES == 0
    assert d % HB == 0 and LANES == 4 * HB and n_pairs > 3 * nt
    hd = n_heads * dh
    n_pre = (n_seg - LAG) * PRE

    wq_t = jnp.transpose(A_Wq, (1, 2, 0)).reshape(hd, d)
    wk_t = jnp.transpose(A_Wk, (1, 2, 0)).reshape(hd, d)
    wv_t = jnp.transpose(A_Wv, (1, 2, 0)).reshape(hd, d)
    wo = A_Wo.reshape(hd, d)

    kernel = functools.partial(
        _kernel, seg=seg, n_seg=n_seg, m_len=m_len, n_pairs=n_pairs, dh=dh,
        d=d)
    any_spec = pl.BlockSpec(memory_space=pl.ANY)
    dma = pltpu.SemaphoreType.DMA
    out = pl.pallas_call(
        kernel,
        out_shape=jax.ShapeDtypeStruct((n_seg, seg, d), A_x.dtype),
        in_specs=[any_spec] * 8,
        out_specs=any_spec,
        scratch_shapes=[
            pltpu.VMEM((n_seg, seg, d), BF16),
            pltpu.VMEM((m_len, d), BF16),
            pltpu.VMEM((NSLOT, 6 * dh, d), BF16),
            pltpu.VMEM((n_pairs, d, 6 * dh), BF16),
            pltpu.VMEM((hd, d), BF16),
            pltpu.VMEM((3 * nt + 1, LANES, d), BF16),
            pltpu.VMEM((nt + 1, d, LANES), BF16),
            pltpu.VMEM((d + HB, LANES), F32),
            pltpu.VMEM((d + HB, LANES), F32),
            pltpu.VMEM((3, d, d), BF16),
            pltpu.VMEM((nt, d, LANES), BF16),
            pltpu.VMEM((n_seg, seg, d), A_x.dtype),
            pltpu.VMEM((n_seg * PRE, d), BF16),
            pltpu.VMEM((n_pairs, n_pre, 6 * dh), BF16),
            pltpu.VMEM((2 * (m_len + seg) - PRE, d), BF16),
            pltpu.VMEM((2 * m_len + seg, d), BF16),
            pltpu.VMEM((seg, d), F32),
            pltpu.VMEM((2 * seg, d), F32),
            pltpu.VMEM((2, 2, 2 * nt, HIST + seg, LANES), F32),
            dma((6,)), dma((3 * NSLOT,)), dma((n_pairs,)),
            dma((3 * nt,)), dma((nt,)),
        ],
        compiler_params=pltpu.CompilerParams(
            vmem_limit_bytes=110 * 1024 * 1024,
            disable_bounds_checks=True),
    )(A_x.reshape(n_seg, seg, d), A_mem0.reshape(m_len, d), wq_t, wk_t, wv_t,
      wo, B_wqkv, B_wo)
    return out.reshape(bsz, s_len, d)
```

```python
import functools

import jax
import jax.numpy as jnp
from jax import lax
import jax.experimental.pallas as pl
import jax.experimental.pallas.tpu as pltpu

F32 = jnp.float32
BF16 = jnp.bfloat16

_NT = (((1,), (1,)), ((), ()))
_NN = (((1,), (0,)), ((), ()))

SEG_LEN = 32
HB = 32
WIN = 8
DIL = 2
HIST = 16
LANES = 128
PRE = 16
PRE_CHUNK = 256
LN_SEGS = 16
LAG = 2
UNROLL = 2
NSLOT = 2
NEG = -1000000000.0


def _dot(a, b, dims):
    return lax.dot_general(a, b, dims, preferred_element_type=F32)


def _recip(x):
    r = pl.reciprocal(x, approx=True)
    return r * (2.0 - x * r)


def _ln(x):
    m = jnp.mean(x, axis=-1, keepdims=True)
    xc = x - m
    v = jnp.mean(xc * xc, axis=-1, keepdims=True)
    return xc * lax.rsqrt(v + 1e-05)


def _tile(a, c):
    return a[:, c * LANES:(c + 1) * LANES]


def _keep(mask, a):
    return jnp.where(mask, a, jnp.zeros_like(a))


def _drop(mask, a):
    return jnp.where(mask, jnp.zeros_like(a), a)


def _pair_softmax(s, col_a):
    m_a = jnp.max(jnp.where(col_a, s, -jnp.inf), axis=1, keepdims=True)
    m_b = jnp.max(jnp.where(col_a, -jnp.inf, s), axis=1, keepdims=True)
    e = jnp.exp(s - jnp.where(col_a, m_a, m_b))
    d_a = jnp.sum(jnp.where(col_a, e, 0.0), axis=1, keepdims=True)
    d_b = jnp.sum(jnp.where(col_a, 0.0, e), axis=1, keepdims=True)
    return e * _recip(jnp.where(col_a, d_a, d_b))


class _PassBase:
    def __init__(self, h, w_ref, wo_ref, dh):
        self.h, self.w, self.wo = h, w_ref, wo_ref
        self.pw = 2 * dh
        self.half = dh - LANES
        self.scale = dh ** (-0.5)
        self.q, self.k, self.v, self.p, self.o = {}, {}, {}, {}, {}
        self.cols = (0, 2 * LANES, wo_ref.shape[1])
        self.pending = None

    def _lane_lo(self, rows):
        return lax.broadcasted_iota(jnp.int32, (rows, LANES), 1) < self.half

    def _project(self, p, j):
        a = _dot(self.h, self.w[p, :, j * self.pw:(j + 1) * self.pw], _NN)
        self.marker = a[:8, :LANES]
        return a

    def _gate(self, s):
        if self.pending is None:
            return s
        top = jnp.where(self.always, s[:8], self.pending[:, :s.shape[1]])
        self.pending = None
        return jnp.concatenate([top, s[8:]], axis=0)

    def out(self, p, part=None):
        for k in ((0, 1) if part is None else (part,)):
            c0, c1 = self.cols[k], self.cols[k + 1]
            w = self.wo[p * self.pw:(p + 1) * self.pw, c0:c1]
            self.acc[k] = self.acc[k] + _dot(self.o[p], w, _NN)

    def run(self, n_pairs, init, b, always):
        last = n_pairs - 1
        self.acc = [init[:, :self.cols[1]], init[:, self.cols[1]:]]
        self.always = always
        done = None
        for p in range(n_pairs):
            self.proj_q(p)
            self.pending, done = done, None
            if 2 <= p < 2 + b.n_groups:
                o = b.attend(p - 2, (always, self.marker))
                done = functools.reduce(lambda u, v: u + v, o)
            self.proj_k(p)
            if p > 0:
                self.pv(p - 1)
            self.proj_v(p)
            self.scores(p)
            if p == 0:
                b.project()
            elif p < last:
                self.out(p - 1)
        yb = b.finish()
        self.out(last - 1, 0)
        self.pv(last)
        self.out(last - 1, 1)
        self.out(last)
        return jnp.concatenate(self.acc, axis=1), yb


class _TwoLayerPass(_PassBase):
    def __init__(self, h, pre_ref, pre_row, w_ref, wo_ref, *, dh, m_len, seg):
        super().__init__(h, w_ref, wo_ref, dh)
        self.pre, self.pre_row = pre_ref, pre_row
        u = self.u = m_len
        n = self.n = 2 * (m_len + seg)
        self.ext = 4 * u
        self.seg = seg
        row = lax.broadcasted_iota(jnp.int32, (n, n + self.ext), 0)
        col = lax.broadcasted_iota(jnp.int32, (n, n + self.ext), 1)
        rep = col >= n
        col = jnp.where(rep, col - n, col)

        def first_layer(i):
            return (((i < 6 * u) & ((i & u) == 0))
                    | ((i >= 6 * u) & (i < 6 * u + PRE)))

        def index(i):
            low = ((i >> 1) & ~(u - 1)) + (i & (u - 1))
            high = jnp.where(i < 6 * u + PRE, i - 3 * u, i - 3 * u - PRE)
            return jnp.where(i < 6 * u, low, high)

        self.col_a = first_layer(col)
        self.diag = first_layer(row) == self.col_a
        used = ((row >= 3 * u) & (row < 4 * u)) == rep
        self.allowed = used & ((row < 2 * u) | (index(row) >= index(col)))
        self.fill = jnp.where(used, NEG, -jnp.inf)
        self.lo_u = self._lane_lo(u)
        self.lo_c = self._lane_lo(PRE)

    def _proj(self, p, j):
        u, pw, seg = self.u, self.pw, self.seg
        r = self._project(p, j)
        c1 = self.pre[p, pl.ds(self.pre_row, PRE), j * pw:(j + 1) * pw]
        nx = 2 * u + seg
        return ((r[nx:nx + u], r[:u], r[u:2 * u], c1),
                (r[nx + u:], r[2 * u:3 * u], r[3 * u:4 * u],
                 r[4 * u:nx].astype(BF16)))

    @staticmethod
    def _weave(f, g):
        top = jnp.concatenate([f[0], g[0], f[1], g[1], f[2], g[2]], axis=0)
        return jnp.concatenate([top.astype(BF16), f[3], g[3]], axis=0)

    def _tiles(self, l1, l2):
        masks = (self.lo_u,) * 3 + (self.lo_c,)

        def t(l, c):
            return [_tile(a, c) for a in l]

        def lo(l):
            return [_keep(mk, a) for mk, a in zip(masks, l)]

        def hi(l):
            return [_drop(mk, a) for mk, a in zip(masks, l)]

        def extend(a, b):
            return jnp.concatenate([a, b[:self.ext]], axis=0)

        t0 = self._weave(t(l1, 0), t(l2, 0))
        t2 = self._weave(t(l2, 2), t(l1, 2))
        t1a = self._weave(lo(t(l1, 1)), hi(t(l1, 1)))
        t1b = self._weave(hi(t(l2, 1)), lo(t(l2, 1)))
        return extend(t0, t0), extend(t1a, t1b), t1b, extend(t2, t2)

    def _split_rows(self, l1, l2):
        ra = jnp.concatenate([l1[0], l1[2], l1[1], l2[1]], axis=0)
        rb = jnp.concatenate([l2[0], l2[2]], axis=0)
        return (jnp.concatenate([ra.astype(BF16), l1[3]], axis=0),
                jnp.concatenate([rb.astype(BF16), l2[3]], axis=0))

    def _units(self, ra, rb):
        u = self.u
        return ((ra[:u], ra[2 * u:3 * u], ra[u:2 * u], ra[4 * u:]),
                (rb[:u], ra[3 * u:4 * u], rb[u:2 * u], rb[2 * u:]))

    def _unweave(self, a):
        u = self.u
        return ((a[:u], a[2 * u:3 * u], a[4 * u:5 * u], a[6 * u:6 * u + PRE]),
                (a[u:2 * u], a[3 * u:4 * u], a[5 * u:6 * u], a[6 * u + PRE:]))

    def proj_q(self, p):
        l1, l2 = self._proj(p, 0)
        q0, q2 = (self._weave([_tile(a, c) for a in l1],
                              [_tile(a, c) for a in l2]) for c in (0, 2))
        qa, qb = self._split_rows([_tile(a, 1) for a in l1],
                                  [_tile(a, 1) for a in l2])
        self.q[p] = (q0, qa, qb, q2)

    def proj_k(self, p):
        self.k[p] = self._tiles(*self._proj(p, 1))

    def proj_v(self, p):
        self.v[p] = self._tiles(*self._proj(p, 2))

    def scores(self, p):
        q0, qa, qb, q2 = self.q.pop(p)
        k0, k1a, k1b, k2 = self.k.pop(p)
        r0 = _dot(q0, k0, _NT)
        r2 = _dot(q2, k2, _NT)
        ra = _dot(qa, k1a, _NT)
        rb = _dot(qb, k1b, _NT)
        rb = jnp.concatenate(
            [rb, jnp.zeros((rb.shape[0], self.ext), F32)], axis=1)
        f, g = self._units(ra, rb)
        r1 = jnp.concatenate(
            [f[0], g[0], f[1], g[1], f[2], g[2], f[3], g[3]], axis=0)
        s = jnp.where(self.diag, r0, r2) + r1
        s = self._gate(jnp.where(self.allowed, s * self.scale, self.fill))
        p_all = _pair_softmax(s, self.col_a)
        f, g = self._unweave(p_all)
        pa, pb = self._split_rows(f[:3] + (f[3].astype(BF16),),
                                  g[:3] + (g[3].astype(BF16),))
        self.p[p] = (_keep(self.diag, p_all).astype(BF16), pa,
                     pb[:, :self.n], _drop(self.diag, p_all).astype(BF16))

    def pv(self, p):
        p0, pa, pb, p2 = self.p.pop(p)
        v0, v1a, v1b, v2 = self.v.pop(p)
        o0 = self._unweave(_dot(p0, v0, _NN))
        o2 = self._unweave(_dot(p2, v2, _NN))
        o1 = self._units(_dot(pa, v1a, _NN), _dot(pb, v1b, _NN))
        self.o[p] = jnp.concatenate(
            [jnp.concatenate((f[0], g[0]) + f[1:] + g[1:], axis=0)
             for f, g in (o0, o1, o2)], axis=1).astype(BF16)


class _OneLayerPass(_PassBase):
    def __init__(self, h, pre_ref, pre_row, w_ref, wo_ref, *, dh, m_len, seg):
        super().__init__(h, w_ref, wo_ref, dh)
        self.pre, self.pre_row = pre_ref, pre_row
        n = self.n = m_len + seg
        row = lax.broadcasted_iota(jnp.int32, (n, 2 * n), 0)
        col = lax.broadcasted_iota(jnp.int32, (n, 2 * n), 1)
        self.col_a = col < n
        key = jnp.where(self.col_a, col, col - n)
        self.allowed = (row < m_len) | (row >= key)
        lane = lax.broadcasted_iota(jnp.int32, (n, self.pw), 1)
        self.head0 = lane < dh

    def _project(self, p, j):
        a = super()._project(p, j)
        n, pw = self.n, self.pw
        self.pre[p, pl.ds(self.pre_row, a.shape[0] - n),
                 j * pw:(j + 1) * pw] = a[n:].astype(BF16)
        return a[:n]

    def _block_diag(self, a):
        return jnp.concatenate([_keep(self.head0, a), _drop(self.head0, a)],
                               axis=0).astype(BF16)

    def proj_q(self, p):
        self.q[p] = self._project(p, 0).astype(BF16)

    def proj_k(self, p):
        self.k[p] = self._block_diag(self._project(p, 1))

    def proj_v(self, p):
        self.v[p] = self._block_diag(self._project(p, 2))

    def scores(self, p):
        s = _dot(self.q.pop(p), self.k.pop(p), _NT)
        s = self._gate(jnp.where(self.allowed, s * self.scale, NEG))
        self.p[p] = _pair_softmax(s, self.col_a).astype(BF16)

    def pv(self, p):
        self.o[p] = _dot(self.p.pop(p), self.v.pop(p), _NN).astype(BF16)


class _BPass:
    def __init__(self, y_ref, starts, wqkv_ref, wo_ref, kv_ref, kv_next_ref,
                 *, seg, d):
        self.y, self.starts = y_ref, starts
        self.wqkv, self.wo, self.kv = wqkv_ref, wo_ref, kv_ref
        self.kv_next = kv_next_ref
        self.seg, self.nt = seg, d // LANES
        self.scale = (d // HB) ** (-0.5)
        self.n_groups = len(starts) * seg // 8
        self.outs = []

    def project(self):
        seg, nt = self.seg, self.nt
        yn = _ln(self.y[...]).astype(BF16)
        self.q, ka, va = (_dot(yn, self.wqkv[j], _NN) for j in range(3))
        for i in range(len(self.starts)):
            for c in range(2 * nt):
                a = _tile((ka, va)[c // nt][i * seg:(i + 1) * seg], c % nt)
                self.kv[i, c, HIST:, :] = a
                if self.kv_next is not None:
                    self.kv_next[i, c, :HIST, :] = a[seg - HIST:]

    def attend(self, gi, after=None):
        seg, nt, kv = self.seg, self.nt, self.kv
        i, g = divmod(gi, seg // 8)
        q = [_tile(self.q[8 * gi:8 * gi + 8], c) for c in range(nt)]
        if after is not None:
            q = [jnp.where(after[0], u, after[1]) for u in q]
        pos = (lax.broadcasted_iota(jnp.int32, (8, LANES), 0)
               + (self.starts[i] + 8 * g))
        offs = [HIST + 8 * g - w * DIL for w in range(WIN)]
        logits = []
        for w, off in enumerate(offs):
            t = q[0] * kv[i, 0, off:off + 8, :]
            for c in range(1, nt):
                t = t + q[c] * kv[i, c, off:off + 8, :]
            t = t + pltpu.roll(t, 64, 1)
            t = (t + pltpu.roll(t, 32, 1)) * self.scale
            if 8 * g < w * DIL:
                t = jnp.where(pos >= w * DIL, t, NEG)
            logits.append(t)
        m = logits[0]
        for t in logits[1:]:
            m = jnp.maximum(m, t)
        es = [jnp.exp(t - m) for t in logits]
        den = es[0]
        for e in es[1:]:
            den = den + e
        inv = _recip(den)
        o = []
        for c in range(nt):
            acc = None
            for w, off in enumerate(offs):
                term = es[w] * kv[i, nt + c, off:off + 8, :]
                acc = term if acc is None else acc + term
            o.append(acc * inv)
        self.outs.append(jnp.concatenate(o, axis=1))
        return o

    def finish(self):
        o = jnp.concatenate(self.outs, axis=0).astype(BF16)
        proj = jnp.concatenate(
            [_dot(o, self.wo[c], _NN) for c in range(self.nt)], axis=1)
        return self.y[...] + proj


def _kernel(x_hbm, mem_hbm, wq_hbm, wk_hbm, wv_hbm, wo_hbm, bqkv_hbm, bo_hbm,
            out_hbm,
            x_v, mem_v, wst_v, w_v, wo_v, bq_st, bo_st, tq_s, to_s, bqkv_p,
            bo_p, out_v, xn_s, pre_s, h_s, h1_s, ra_s, y_s, kv_s,
            sems, w_sems, wo_sems, bq_sems, bo_sems,
            *, seg, n_seg, m_len, n_pairs, dh, d):
    db = d // HB
    nt = d // LANES
    pw = 2 * dh
    m2 = 2 * m_len
    n_pre = (n_seg - 1 - LAG) * PRE
    n_bq = 3 * nt

    def w_copy(p, j):
        src = (wq_hbm, wk_hbm, wv_hbm)[j]
        slot = p & (NSLOT - 1)
        return pltpu.make_async_copy(
            src.at[pl.ds(p * pw, pw), :],
            wst_v.at[slot, pl.ds(j * pw, pw), :], w_sems.at[slot])

    def w_wait(p):
        slot = p & (NSLOT - 1)
        pltpu.make_async_copy(wst_v.at[slot], wst_v.at[slot],
                              w_sems.at[slot]).wait()

    def wo_copy(p):
        return pltpu.make_async_copy(wo_hbm.at[pl.ds(p * pw, pw), :],
                                     wo_v.at[pl.ds(p * pw, pw), :],
                                     wo_sems.at[p])

    def bq_copy(i):
        row = pl.multiple_of((i % nt) * LANES, LANES)
        col = pl.multiple_of((i // nt) * d, LANES)
        return pltpu.make_async_copy(
            bqkv_hbm.at[pl.ds(row, LANES), pl.ds(col, d)], bq_st.at[i + 1],
            bq_sems.at[i])

    def bo_copy(i):
        col = pl.multiple_of(i * LANES, LANES)
        return pltpu.make_async_copy(bo_hbm.at[:, pl.ds(col, LANES)],
                                     bo_st.at[i + 1], bo_sems.at[i])

    nf = seg - PRE
    xa_copy = pltpu.make_async_copy(x_hbm.at[:, nf:, :], x_v.at[:, nf:, :],
                                    sems.at[0])
    xb_copy = pltpu.make_async_copy(x_hbm.at[1:, :nf, :], x_v.at[1:, :nf, :],
                                    sems.at[1])
    x0_copy = pltpu.make_async_copy(x_hbm.at[0, :nf, :], x_v.at[0, :nf, :],
                                    sems.at[5])
    mem_copy = pltpu.make_async_copy(mem_hbm, mem_v, sems.at[2])

    mem_copy.start()
    xa_copy.start()
    mem_copy.wait()
    x0_copy.start()
    for j in range(3):
        w_copy(0, j).start()

    ra_s[...] = jnp.zeros(ra_s.shape, F32)
    y_s[...] = jnp.zeros(y_s.shape, F32)
    kv_s[0, :, :, :HIST, :] = jnp.zeros(kv_s.shape[1:3] + (HIST, LANES), F32)
    bq_st[0] = jnp.zeros(bq_st.shape[1:], BF16)
    bo_st[0] = jnp.zeros(bo_st.shape[1:], BF16)

    xa_copy.wait()
    for j in range(3):
        w_copy(1, j).start()
    bq_copy(0).start()
    bo_copy(0).start()
    wo_copy(0).start()
    xb_copy.start()

    def ln_block(i, carry):
        s0 = pl.multiple_of(i * LN_SEGS, LN_SEGS)
        xb = x_v[pl.ds(s0, LN_SEGS), nf:, :].astype(F32)
        xn_s[pl.ds(pl.multiple_of(s0 * PRE, PRE), LN_SEGS * PRE), :] = _ln(
            xb.reshape(LN_SEGS * PRE, d)).astype(BF16)
        return carry

    lax.fori_loop(0, n_seg // LN_SEGS, ln_block, 0)

    n1 = m_len + seg
    last_xn = (n_seg - 1) * PRE
    x0_copy.wait()
    h1_s[:n1, :] = jnp.concatenate(
        [mem_v[...].astype(F32), _ln(x_v[0].astype(F32))],
        axis=0).astype(BF16)
    h1_s[n1:, :] = xn_s[last_xn:last_xn + m_len, :]

    def permute_rows(tmp_ref):
        return jnp.concatenate(
            [tmp_ref[pl.ds(j, HB, stride=db), :] for j in range(db)], axis=0)

    def pre_pair(p, carry):
        always = p >= 0
        slot = p & (NSLOT - 1)
        n_chunk = -(-n_pre // PRE_CHUNK)
        rows16 = n_pre // 16
        bounds = [16 * (rows16 * c // n_chunk) for c in range(n_chunk + 1)]

        def last_rows(a):
            return [a[(c + 1) * LANES - 16:(c + 1) * LANES] for c in range(nt)]

        def relayout_bo():
            k = jnp.minimum(p, nt)
            to_s[:d, :] = bo_st[k].astype(F32)
            bo = permute_rows(to_s)
            bo_p[jnp.maximum(k - 1, 0)] = bo.astype(BF16)
            g = d // nt // 16
            return [functools.reduce(
                lambda u, v: u + v,
                [bo[16 * (c * g + r):16 * (c * g + r + 1)] for r in range(g)]
            ).astype(BF16) for c in range(nt)]

        def relayout_bq():
            i = jnp.maximum(p - 1, 0)
            tq_s[:d, :] = bq_st[p].astype(F32).T
            row = pl.multiple_of((i % nt) * LANES, LANES)
            bq = permute_rows(tq_s).T.astype(BF16)
            bqkv_p[i // nt, pl.ds(row, LANES), :] = bq
            return [_tile(bq[LANES - 16:], c) for c in range(nt)]

        def transpose_w(n):
            wt = wst_v[slot, n * LANES:(n + 1) * LANES, :].T
            w_v[p, :, n * LANES:(n + 1) * LANES] = wt
            return last_rows(wt)

        w_wait(p)

        @pl.when(p >= 1)
        def _():
            bq_copy(p - 1).wait()

        @pl.when((p >= 1) & (p <= nt))
        def _():
            bo_copy(p - 1).wait()

        jobs = [functools.partial(transpose_w, n)
                for n in range(3 * pw // LANES)]
        jobs = [None, relayout_bo, relayout_bq] + jobs
        for c in range(n_chunk):
            r0, r1 = bounds[c], bounds[c + 1]
            for j in range(3):
                lhs = xn_s[LAG * PRE + r0:LAG * PRE + r1, :]
                job = jobs.pop(0) if jobs else None
                if job is not None:
                    top = jnp.where(always, lhs[:16],
                                    jnp.concatenate(job(), axis=1))
                    lhs = jnp.concatenate([top, lhs[16:]], axis=0)
                pre_s[p, r0:r1, j * pw:(j + 1) * pw] = _dot(
                    lhs, wst_v[slot, j * pw:(j + 1) * pw, :],
                    _NT).astype(BF16)
        assert not jobs

        @pl.when(p + NSLOT < n_pairs)
        def _():
            for j in range(3):
                w_copy(p + NSLOT, j).start()

        @pl.when(p + 1 < n_pairs)
        def _():
            wo_copy(p + 1).start()

        @pl.when(p + 1 < n_bq)
        def _():
            bq_copy(p + 1).start()

        @pl.when(p + 1 < nt)
        def _():
            bo_copy(p + 1).start()

        return carry

    lax.fori_loop(0, n_pairs, pre_pair, 0)

    xb_copy.wait()
    for p in range(n_pairs):
        wo_copy(p).wait()

    def b_pass(t, par):
        return _BPass(y_s, ((t - 1) * seg, (t - 1 - LAG) * seg), bqkv_p, bo_p,
                      kv_s.at[par], kv_s.at[1 - par], seg=seg, d=d)

    def b_store(t, yb):
        out_v[jnp.maximum(t - 1 - LAG, 0)] = yb[seg:].astype(out_v.dtype)
        return yb[:seg]

    def two_layer_step(t, par, h):
        a = _TwoLayerPass(h, pre_s, pl.multiple_of((t - LAG) * PRE, PRE),
                          w_v, wo_v, dh=dh, m_len=m_len, seg=seg)
        init = jnp.concatenate(
            [jnp.zeros((m2, d), F32), x_v[t].astype(F32), ra_s[...]], axis=0)
        acc, yb = a.run(n_pairs, init, b_pass(t, par), t >= 0)
        x2 = b_store(t, yb)
        y_s[...] = acc[m2:]
        ra_s[...] = x2
        xn = x_v[jnp.minimum(t + 1, n_seg - 1), :nf, :].astype(F32)
        return jnp.concatenate([_ln(xn), _ln(x2), acc[:m2]],
                               axis=0).astype(BF16)

    def two_layer_steps(i, carry):
        h = h_s[...]
        for u in range(UNROLL):
            h = two_layer_step(LAG + i * UNROLL + u, (LAG + u) % 2, h)
        h_s[...] = h
        return carry

    def one_layer_step(t, carry):
        first = t < LAG
        extra_row = pl.multiple_of(n_pre + jnp.minimum(t, 1) * m_len, m_len)
        a = _OneLayerPass(h1_s[...], pre_s, extra_row, w_v, wo_v,
                          dh=dh, m_len=m_len, seg=seg)
        x0 = x_v[jnp.minimum(t, n_seg - 1)].astype(F32)
        init = jnp.concatenate(
            [jnp.zeros((m_len, d), F32), jnp.where(first, x0, ra_s[...])],
            axis=0)
        acc, yb = a.run(n_pairs, init, b_pass(t, t & 1), t >= 0)
        x2 = b_store(t, yb)
        y = acc[m_len:]
        y_s[:seg, :] = y
        y_s[seg:, :] = y
        ra_s[...] = x2
        xn = _ln(x_v[jnp.minimum(t + 1, n_seg - 1)].astype(F32))
        x2n = _ln(x2)
        mem = acc[:m_len]
        h1_s[:n1, :] = jnp.concatenate(
            [mem, jnp.where(first, xn, x2n)], axis=0).astype(BF16)
        h1_s[n1:, :] = xn_s[last_xn + m_len:, :]
        h_s[...] = jnp.concatenate(
            [xn[:nf], x2n, mem, mem_v[...].astype(F32)], axis=0).astype(BF16)
        return carry

    n_early_out = n_seg - 1 - LAG
    out_a = pltpu.make_async_copy(out_v.at[:n_early_out],
                                  out_hbm.at[:n_early_out], sems.at[3])
    out_b = pltpu.make_async_copy(out_v.at[n_early_out:],
                                  out_hbm.at[n_early_out:], sems.at[4])

    def phase(ph, carry):
        t0 = ph * n_seg
        lax.fori_loop(t0, t0 + LAG, one_layer_step, 0)

        @pl.when(ph == 0)
        def _():
            lax.fori_loop(0, (n_seg - LAG) // UNROLL, two_layer_steps, 0)
            out_a.start()
            hf = h_s[...].astype(F32)
            h1_s[:n1, :] = jnp.concatenate(
                [hf[nf + seg + m_len:], hf[nf:nf + seg]],
                axis=0).astype(BF16)

        return carry

    lax.fori_loop(0, 2, phase, 0)

    b = _BPass(y_s.at[seg:], ((n_seg - 1) * seg,), bqkv_p, bo_p,
               kv_s.at[(n_seg + LAG) % 2, 1:], None, seg=seg, d=d)
    b.project()
    for gi in range(b.n_groups):
        b.attend(gi)
    out_v[n_seg - 1] = b.finish().astype(out_v.dtype)
    out_b.start()
    out_a.wait()
    out_b.wait()


def pallas_interleave_layers__memory_aug_recurrent_mem_tr__sliding_local_dilated__prompt_kernel(
    A_x: jax.Array,
    A_mem0: jax.Array,
    A_Wq: jax.Array,
    A_Wk: jax.Array,
    A_Wv: jax.Array,
    A_Wo: jax.Array,
    A_seg_len,
    B_x: jax.Array,
    B_wqkv: jax.Array,
    B_wo: jax.Array,
):
    del B_x
    seg = A_seg_len if isinstance(A_seg_len, int) else SEG_LEN
    return _forward(A_x, A_mem0, A_Wq, A_Wk, A_Wv, A_Wo, B_wqkv, B_wo, seg=seg)


@functools.partial(jax.jit, static_argnames=("seg",))
def _forward(A_x, A_mem0, A_Wq, A_Wk, A_Wv, A_Wo, B_wqkv, B_wo, *, seg):
    bsz, s_len, d = A_x.shape
    m_len = A_mem0.shape[1]
    n_heads, dh = A_Wq.shape[1], A_Wq.shape[2]
    n_seg = s_len // seg
    n_pairs = n_heads // 2
    nt = d // LANES
    assert bsz == 1 and s_len % seg == 0 and n_seg > LAG + 1
    assert m_len == 8 and seg == 2 * m_len + PRE and seg >= HIST
    assert LAG == 2 and LAG * m_len == PRE and n_seg % LN_SEGS == 0
    assert 2 * (m_len + seg) + 4 * m_len <= LANES
    assert (n_seg - LAG) % UNROLL == 0 and UNROLL % 2 == 0
    assert n_heads % 2 == 0 and 2 * dh == 3 * LANES and d % LANES == 0
    assert d % HB == 0 and LANES == 4 * HB and n_pairs == 3 * nt + 1
    hd = n_heads * dh
    n_pre = (n_seg - LAG) * PRE

    wq_t = jnp.transpose(A_Wq, (1, 2, 0)).reshape(hd, d)
    wk_t = jnp.transpose(A_Wk, (1, 2, 0)).reshape(hd, d)
    wv_t = jnp.transpose(A_Wv, (1, 2, 0)).reshape(hd, d)
    wo = A_Wo.reshape(hd, d)

    kernel = functools.partial(
        _kernel, seg=seg, n_seg=n_seg, m_len=m_len, n_pairs=n_pairs, dh=dh,
        d=d)
    any_spec = pl.BlockSpec(memory_space=pl.ANY)
    dma = pltpu.SemaphoreType.DMA
    out = pl.pallas_call(
        kernel,
        out_shape=jax.ShapeDtypeStruct((n_seg, seg, d), A_x.dtype),
        in_specs=[any_spec] * 8,
        out_specs=any_spec,
        scratch_shapes=[
            pltpu.VMEM((n_seg, seg, d), BF16),
            pltpu.VMEM((m_len, d), BF16),
            pltpu.VMEM((NSLOT, 6 * dh, d), BF16),
            pltpu.VMEM((n_pairs, d, 6 * dh), BF16),
            pltpu.VMEM((hd, d), BF16),
            pltpu.VMEM((3 * nt + 1, LANES, d), BF16),
            pltpu.VMEM((nt + 1, d, LANES), BF16),
            pltpu.VMEM((d + HB, LANES), F32),
            pltpu.VMEM((d + HB, LANES), F32),
            pltpu.VMEM((3, d, d), BF16),
            pltpu.VMEM((nt, d, LANES), BF16),
            pltpu.VMEM((n_seg, seg, d), A_x.dtype),
            pltpu.VMEM((n_seg * PRE, d), BF16),
            pltpu.VMEM((n_pairs, n_pre, 6 * dh), BF16),
            pltpu.VMEM((2 * (m_len + seg) - PRE, d), BF16),
            pltpu.VMEM((2 * m_len + seg, d), BF16),
            pltpu.VMEM((seg, d), F32),
            pltpu.VMEM((2 * seg, d), F32),
            pltpu.VMEM((2, 2, 2 * nt, HIST + seg, LANES), F32),
            dma((6,)), dma((NSLOT,)), dma((n_pairs,)),
            dma((3 * nt,)), dma((nt,)),
        ],
        compiler_params=pltpu.CompilerParams(
            vmem_limit_bytes=110 * 1024 * 1024,
            disable_bounds_checks=True),
    )(A_x.reshape(n_seg, seg, d), A_mem0.reshape(m_len, d), wq_t, wk_t, wv_t,
      wo, B_wqkv, B_wo)
    return out.reshape(bsz, s_len, d)
```

```python
import functools

import jax
import jax.numpy as jnp
from jax import lax
import jax.experimental.pallas as pl
import jax.experimental.pallas.tpu as pltpu

F32 = jnp.float32
BF16 = jnp.bfloat16

_NT = (((1,), (1,)), ((), ()))
_NN = (((1,), (0,)), ((), ()))

SEG_LEN = 32
HB = 32
WIN = 8
DIL = 2
HIST = 16
LANES = 128
PRE = 16
PRE_CHUNK = 128
LN_SEGS = 16
LAG = 2
UNROLL = 2
NSLOT = 2
NEG = -1000000000.0


def _dot(a, b, dims):
    return lax.dot_general(a, b, dims, preferred_element_type=F32)


def _recip(x):
    r = pl.reciprocal(x, approx=True)
    return r * (2.0 - x * r)


def _ln(x):
    m = jnp.mean(x, axis=-1, keepdims=True)
    xc = x - m
    v = jnp.mean(xc * xc, axis=-1, keepdims=True)
    return xc * lax.rsqrt(v + 1e-05)


def _tile(a, c):
    return a[:, c * LANES:(c + 1) * LANES]


def _keep(mask, a):
    return jnp.where(mask, a, jnp.zeros_like(a))


def _drop(mask, a):
    return jnp.where(mask, jnp.zeros_like(a), a)


def _pair_softmax(s, col_a):
    m_a = jnp.max(jnp.where(col_a, s, -jnp.inf), axis=1, keepdims=True)
    m_b = jnp.max(jnp.where(col_a, -jnp.inf, s), axis=1, keepdims=True)
    e = jnp.exp(s - jnp.where(col_a, m_a, m_b))
    d_a = jnp.sum(jnp.where(col_a, e, 0.0), axis=1, keepdims=True)
    d_b = jnp.sum(jnp.where(col_a, 0.0, e), axis=1, keepdims=True)
    return e * _recip(jnp.where(col_a, d_a, d_b))


class _PassBase:
    def __init__(self, h, w_ref, wo_ref, dh):
        self.h, self.w, self.wo = h, w_ref, wo_ref
        self.pw = 2 * dh
        self.half = dh - LANES
        self.scale = dh ** (-0.5)
        self.q, self.k, self.v, self.p, self.o = {}, {}, {}, {}, {}
        self.cols = (0, 2 * LANES, wo_ref.shape[1])
        self.pending = None

    def _lane_lo(self, rows):
        return lax.broadcasted_iota(jnp.int32, (rows, LANES), 1) < self.half

    def _project(self, p, j):
        a = _dot(self.h, self.w[p, :, j * self.pw:(j + 1) * self.pw], _NN)
        self.marker = a[:8, :LANES]
        return a

    def _gate(self, s):
        if self.pending is None:
            return s
        top = jnp.where(self.always, s[:8], self.pending[:, :s.shape[1]])
        self.pending = None
        return jnp.concatenate([top, s[8:]], axis=0)

    def out(self, p, part=None):
        for k in ((0, 1) if part is None else (part,)):
            c0, c1 = self.cols[k], self.cols[k + 1]
            w = self.wo[p * self.pw:(p + 1) * self.pw, c0:c1]
            self.acc[k] = self.acc[k] + _dot(self.o[p], w, _NN)

    def run(self, n_pairs, init, b, always):
        last = n_pairs - 1
        self.acc = [init[:, :self.cols[1]], init[:, self.cols[1]:]]
        self.always = always
        done = None
        for p in range(n_pairs):
            self.proj_q(p)
            self.pending, done = done, None
            if 2 <= p < 2 + b.n_groups:
                o = b.attend(p - 2, (always, self.marker))
                done = functools.reduce(lambda u, v: u + v, o)
            self.proj_k(p)
            if p > 0:
                self.pv(p - 1)
            self.proj_v(p)
            self.scores(p)
            if p == 0:
                b.project()
            elif p < last:
                self.out(p - 1)
        yb = b.finish()
        self.out(last - 1, 0)
        self.pv(last)
        self.out(last - 1, 1)
        self.out(last)
        return jnp.concatenate(self.acc, axis=1), yb


class _TwoLayerPass(_PassBase):
    def __init__(self, h, pre_ref, pre_row, w_ref, wo_ref, *, dh, m_len, seg):
        super().__init__(h, w_ref, wo_ref, dh)
        self.pre, self.pre_row = pre_ref, pre_row
        u = self.u = m_len
        n = self.n = 2 * (m_len + seg)
        self.ext = 4 * u
        self.seg = seg
        row = lax.broadcasted_iota(jnp.int32, (n, n + self.ext), 0)
        col = lax.broadcasted_iota(jnp.int32, (n, n + self.ext), 1)
        rep = col >= n
        col = jnp.where(rep, col - n, col)

        def first_layer(i):
            return (((i < 6 * u) & ((i & u) == 0))
                    | ((i >= 6 * u) & (i < 6 * u + PRE)))

        def index(i):
            low = ((i >> 1) & ~(u - 1)) + (i & (u - 1))
            high = jnp.where(i < 6 * u + PRE, i - 3 * u, i - 3 * u - PRE)
            return jnp.where(i < 6 * u, low, high)

        self.col_a = first_layer(col)
        self.diag = first_layer(row) == self.col_a
        used = ((row >= 3 * u) & (row < 4 * u)) == rep
        self.allowed = used & ((row < 2 * u) | (index(row) >= index(col)))
        self.fill = jnp.where(used, NEG, -jnp.inf)
        self.lo_u = self._lane_lo(u)
        self.lo_c = self._lane_lo(PRE)

    def _proj(self, p, j):
        u, pw, seg = self.u, self.pw, self.seg
        r = self._project(p, j)
        if self.pre_row is None:
            n1 = seg
            c1 = r[2 * u:n1].astype(BF16)
        else:
            n1 = 2 * u
            c1 = self.pre[p, pl.ds(self.pre_row, PRE), j * pw:(j + 1) * pw]
        nx = n1 + seg
        return ((r[nx:nx + u], r[:u], r[u:2 * u], c1),
                (r[nx + u:], r[n1:n1 + u], r[n1 + u:n1 + 2 * u],
                 r[n1 + 2 * u:nx].astype(BF16)))

    @staticmethod
    def _weave(f, g):
        top = jnp.concatenate([f[0], g[0], f[1], g[1], f[2], g[2]], axis=0)
        return jnp.concatenate([top.astype(BF16), f[3], g[3]], axis=0)

    def _tiles(self, l1, l2):
        masks = (self.lo_u,) * 3 + (self.lo_c,)

        def t(l, c):
            return [_tile(a, c) for a in l]

        def lo(l):
            return [_keep(mk, a) for mk, a in zip(masks, l)]

        def hi(l):
            return [_drop(mk, a) for mk, a in zip(masks, l)]

        def extend(a, b):
            return jnp.concatenate([a, b[:self.ext]], axis=0)

        t0 = self._weave(t(l1, 0), t(l2, 0))
        t2 = self._weave(t(l2, 2), t(l1, 2))
        t1a = self._weave(lo(t(l1, 1)), hi(t(l1, 1)))
        t1b = self._weave(hi(t(l2, 1)), lo(t(l2, 1)))
        return extend(t0, t0), extend(t1a, t1b), t1b, extend(t2, t2)

    def _split_rows(self, l1, l2):
        ra = jnp.concatenate([l1[0], l1[2], l1[1], l2[1]], axis=0)
        rb = jnp.concatenate([l2[0], l2[2]], axis=0)
        return (jnp.concatenate([ra.astype(BF16), l1[3]], axis=0),
                jnp.concatenate([rb.astype(BF16), l2[3]], axis=0))

    def _units(self, ra, rb):
        u = self.u
        return ((ra[:u], ra[2 * u:3 * u], ra[u:2 * u], ra[4 * u:]),
                (rb[:u], ra[3 * u:4 * u], rb[u:2 * u], rb[2 * u:]))

    def _unweave(self, a):
        u = self.u
        return ((a[:u], a[2 * u:3 * u], a[4 * u:5 * u], a[6 * u:6 * u + PRE]),
                (a[u:2 * u], a[3 * u:4 * u], a[5 * u:6 * u], a[6 * u + PRE:]))

    def proj_q(self, p):
        l1, l2 = self._proj(p, 0)
        q0, q2 = (self._weave([_tile(a, c) for a in l1],
                              [_tile(a, c) for a in l2]) for c in (0, 2))
        qa, qb = self._split_rows([_tile(a, 1) for a in l1],
                                  [_tile(a, 1) for a in l2])
        self.q[p] = (q0, qa, qb, q2)

    def proj_k(self, p):
        self.k[p] = self._tiles(*self._proj(p, 1))

    def proj_v(self, p):
        self.v[p] = self._tiles(*self._proj(p, 2))

    def scores(self, p):
        q0, qa, qb, q2 = self.q.pop(p)
        k0, k1a, k1b, k2 = self.k.pop(p)
        r0 = _dot(q0, k0, _NT)
        r2 = _dot(q2, k2, _NT)
        ra = _dot(qa, k1a, _NT)
        rb = _dot(qb, k1b, _NT)
        rb = jnp.concatenate(
            [rb, jnp.zeros((rb.shape[0], self.ext), F32)], axis=1)
        f, g = self._units(ra, rb)
        r1 = jnp.concatenate(
            [f[0], g[0], f[1], g[1], f[2], g[2], f[3], g[3]], axis=0)
        s = jnp.where(self.diag, r0, r2) + r1
        s = self._gate(jnp.where(self.allowed, s * self.scale, self.fill))
        p_all = _pair_softmax(s, self.col_a)
        f, g = self._unweave(p_all)
        pa, pb = self._split_rows(f[:3] + (f[3].astype(BF16),),
                                  g[:3] + (g[3].astype(BF16),))
        self.p[p] = (_keep(self.diag, p_all).astype(BF16), pa,
                     pb[:, :self.n], _drop(self.diag, p_all).astype(BF16))

    def pv(self, p):
        p0, pa, pb, p2 = self.p.pop(p)
        v0, v1a, v1b, v2 = self.v.pop(p)
        o0 = self._unweave(_dot(p0, v0, _NN))
        o2 = self._unweave(_dot(p2, v2, _NN))
        o1 = self._units(_dot(pa, v1a, _NN), _dot(pb, v1b, _NN))
        self.o[p] = jnp.concatenate(
            [jnp.concatenate((f[0], g[0]) + f[1:] + g[1:], axis=0)
             for f, g in (o0, o1, o2)], axis=1).astype(BF16)


class _OneLayerPass(_PassBase):
    def __init__(self, h, pre_ref, pre_row, w_ref, wo_ref, *, dh, m_len, seg):
        super().__init__(h, w_ref, wo_ref, dh)
        self.pre, self.pre_row = pre_ref, pre_row
        n = self.n = m_len + seg
        row = lax.broadcasted_iota(jnp.int32, (n, 2 * n), 0)
        col = lax.broadcasted_iota(jnp.int32, (n, 2 * n), 1)
        self.col_a = col < n
        key = jnp.where(self.col_a, col, col - n)
        self.allowed = (row < m_len) | (row >= key)
        lane = lax.broadcasted_iota(jnp.int32, (n, self.pw), 1)
        self.head0 = lane < dh

    def _project(self, p, j):
        a = super()._project(p, j)
        n, pw = self.n, self.pw
        self.pre[p, pl.ds(self.pre_row, a.shape[0] - n),
                 j * pw:(j + 1) * pw] = a[n:].astype(BF16)
        return a[:n]

    def _block_diag(self, a):
        return jnp.concatenate([_keep(self.head0, a), _drop(self.head0, a)],
                               axis=0).astype(BF16)

    def proj_q(self, p):
        self.q[p] = self._project(p, 0).astype(BF16)

    def proj_k(self, p):
        self.k[p] = self._block_diag(self._project(p, 1))

    def proj_v(self, p):
        self.v[p] = self._block_diag(self._project(p, 2))

    def scores(self, p):
        s = _dot(self.q.pop(p), self.k.pop(p), _NT)
        s = self._gate(jnp.where(self.allowed, s * self.scale, NEG))
        self.p[p] = _pair_softmax(s, self.col_a).astype(BF16)

    def pv(self, p):
        self.o[p] = _dot(self.p.pop(p), self.v.pop(p), _NN).astype(BF16)


class _BPass:
    def __init__(self, y_ref, starts, wqkv_ref, wo_ref, kv_ref, kv_next_ref,
                 *, seg, d):
        self.y, self.starts = y_ref, starts
        self.wqkv, self.wo, self.kv = wqkv_ref, wo_ref, kv_ref
        self.kv_next = kv_next_ref
        self.seg, self.nt = seg, d // LANES
        self.scale = (d // HB) ** (-0.5)
        self.n_groups = len(starts) * seg // 8
        self.outs = []

    def project(self):
        seg, nt = self.seg, self.nt
        yn = _ln(self.y[...]).astype(BF16)
        self.q, ka, va = (_dot(yn, self.wqkv[j], _NN) for j in range(3))
        for i in range(len(self.starts)):
            for c in range(2 * nt):
                a = _tile((ka, va)[c // nt][i * seg:(i + 1) * seg], c % nt)
                self.kv[i, c, HIST:, :] = a
                if self.kv_next is not None:
                    self.kv_next[i, c, :HIST, :] = a[seg - HIST:]

    def attend(self, gi, after=None):
        seg, nt, kv = self.seg, self.nt, self.kv
        i, g = divmod(gi, seg // 8)
        q = [_tile(self.q[8 * gi:8 * gi + 8], c) for c in range(nt)]
        if after is not None:
            q = [jnp.where(after[0], u, after[1]) for u in q]
        pos = (lax.broadcasted_iota(jnp.int32, (8, LANES), 0)
               + (self.starts[i] + 8 * g))
        offs = [HIST + 8 * g - w * DIL for w in range(WIN)]
        logits = []
        for w, off in enumerate(offs):
            t = q[0] * kv[i, 0, off:off + 8, :]
            for c in range(1, nt):
                t = t + q[c] * kv[i, c, off:off + 8, :]
            t = t + pltpu.roll(t, 64, 1)
            t = (t + pltpu.roll(t, 32, 1)) * self.scale
            if 8 * g < w * DIL:
                t = jnp.where(pos >= w * DIL, t, NEG)
            logits.append(t)
        m = logits[0]
        for t in logits[1:]:
            m = jnp.maximum(m, t)
        es = [jnp.exp(t - m) for t in logits]
        den = es[0]
        for e in es[1:]:
            den = den + e
        inv = _recip(den)
        o = []
        for c in range(nt):
            acc = None
            for w, off in enumerate(offs):
                term = es[w] * kv[i, nt + c, off:off + 8, :]
                acc = term if acc is None else acc + term
            o.append(acc * inv)
        self.outs.append(jnp.concatenate(o, axis=1))
        return o

    def finish(self):
        o = jnp.concatenate(self.outs, axis=0).astype(BF16)
        proj = jnp.concatenate(
            [_dot(o, self.wo[c], _NN) for c in range(self.nt)], axis=1)
        return self.y[...] + proj


def _kernel(x_hbm, mem_hbm, wq_hbm, wk_hbm, wv_hbm, wo_hbm, bqkv_hbm, bo_hbm,
            out_hbm,
            x_v, mem_v, wst_v, w_v, wo_v, bq_st, bo_st, tq_s, to_s, bqkv_p,
            bo_p, out_v, xn_s, pre_s, h_s, h1_s, ra_s, y_s, kv_s,
            sems, w_sems, wo_sems, bq_sems, bo_sems,
            *, seg, n_seg, m_len, n_pairs, dh, d):
    db = d // HB
    nt = d // LANES
    pw = 2 * dh
    m2 = 2 * m_len
    n_half = n_seg // 2
    n_pre = (n_half - 1 - LAG // 2) * PRE
    n_bq = 3 * nt

    def w_copy(p, j):
        src = (wq_hbm, wk_hbm, wv_hbm)[j]
        slot = p & (NSLOT - 1)
        return pltpu.make_async_copy(
            src.at[pl.ds(p * pw, pw), :],
            wst_v.at[slot, pl.ds(j * pw, pw), :], w_sems.at[slot])

    def w_wait(p):
        slot = p & (NSLOT - 1)
        pltpu.make_async_copy(wst_v.at[slot], wst_v.at[slot],
                              w_sems.at[slot]).wait()

    def wo_copy(p):
        return pltpu.make_async_copy(wo_hbm.at[pl.ds(p * pw, pw), :],
                                     wo_v.at[pl.ds(p * pw, pw), :],
                                     wo_sems.at[p])

    def bq_copy(i):
        row = pl.multiple_of((i % nt) * LANES, LANES)
        col = pl.multiple_of((i // nt) * d, LANES)
        return pltpu.make_async_copy(
            bqkv_hbm.at[pl.ds(row, LANES), pl.ds(col, d)], bq_st.at[i + 1],
            bq_sems.at[i])

    def bo_copy(i):
        col = pl.multiple_of(i * LANES, LANES)
        return pltpu.make_async_copy(bo_hbm.at[:, pl.ds(col, LANES)],
                                     bo_st.at[i + 1], bo_sems.at[i])

    nf = seg - PRE

    def x_copy(idx, sem):
        return pltpu.make_async_copy(x_hbm.at[idx], x_v.at[idx], sems.at[sem])

    full = slice(None)
    xa_copy = x_copy((full, 0, slice(nf, None), full), 0)
    x0_copy = x_copy((0, 0, slice(None, nf), full), 5)
    xb_copy = x_copy((slice(1, None), 0, slice(None, nf), full), 1)
    xc_copy = x_copy((full, 1), 6)

    def x_seg(t):
        return x_v.at[t >> 1, t & 1]

    mem_copy = pltpu.make_async_copy(mem_hbm, mem_v, sems.at[2])

    mem_copy.start()
    xa_copy.start()
    mem_copy.wait()
    x0_copy.start()
    for j in range(3):
        w_copy(0, j).start()

    ra_s[...] = jnp.zeros(ra_s.shape, F32)
    y_s[...] = jnp.zeros(y_s.shape, F32)
    kv_s[0, :, :, :HIST, :] = jnp.zeros(kv_s.shape[1:3] + (HIST, LANES), F32)
    bq_st[0] = jnp.zeros(bq_st.shape[1:], BF16)
    bo_st[0] = jnp.zeros(bo_st.shape[1:], BF16)

    xa_copy.wait()
    for j in range(3):
        w_copy(1, j).start()
    bq_copy(0).start()
    bo_copy(0).start()
    wo_copy(0).start()

    def ln_block(i, carry):
        s0 = pl.multiple_of(i * LN_SEGS, LN_SEGS)
        xb = x_v[pl.ds(s0, LN_SEGS), 0, nf:, :].astype(F32)
        xn_s[pl.ds(pl.multiple_of(s0 * PRE, PRE), LN_SEGS * PRE), :] = _ln(
            xb.reshape(LN_SEGS * PRE, d)).astype(BF16)
        return carry

    lax.fori_loop(0, n_half // LN_SEGS, ln_block, 0)

    n1 = m_len + seg
    last_xn = (n_half - 1) * PRE
    x0_copy.wait()
    h1_s[:n1, :] = jnp.concatenate(
        [mem_v[...].astype(F32), _ln(x_v[0, 0].astype(F32))],
        axis=0).astype(BF16)
    h1_s[n1:, :] = xn_s[last_xn:last_xn + m_len, :]

    def permute_rows(tmp_ref):
        return jnp.concatenate(
            [tmp_ref[pl.ds(j, HB, stride=db), :] for j in range(db)], axis=0)

    def pre_pair(p, carry):
        always = p >= 0
        slot = p & (NSLOT - 1)
        n_chunk = -(-n_pre // PRE_CHUNK)
        rows16 = n_pre // 16
        skip = LAG // 2 * PRE
        bounds = [16 * (rows16 * c // n_chunk) for c in range(n_chunk + 1)]

        def last_rows(a):
            return [a[(c + 1) * LANES - 16:(c + 1) * LANES] for c in range(nt)]

        def relayout_bo():
            k = jnp.minimum(p, nt)
            to_s[:d, :] = bo_st[k].astype(F32)
            bo = permute_rows(to_s)
            bo_p[jnp.maximum(k - 1, 0)] = bo.astype(BF16)
            g = d // nt // 16
            return [functools.reduce(
                lambda u, v: u + v,
                [bo[16 * (c * g + r):16 * (c * g + r + 1)] for r in range(g)]
            ).astype(BF16) for c in range(nt)]

        def relayout_bq():
            i = jnp.maximum(p - 1, 0)
            tq_s[:d, :] = bq_st[p].astype(F32).T
            row = pl.multiple_of((i % nt) * LANES, LANES)
            bq = permute_rows(tq_s).T.astype(BF16)
            bqkv_p[i // nt, pl.ds(row, LANES), :] = bq
            return [_tile(bq[LANES - 16:], c) for c in range(nt)]

        def transpose_w(n):
            wt = wst_v[slot, n * LANES:(n + 1) * LANES, :].T
            w_v[p, :, n * LANES:(n + 1) * LANES] = wt
            return last_rows(wt)

        w_wait(p)

        @pl.when(p >= 1)
        def _():
            bq_copy(p - 1).wait()

        @pl.when((p >= 1) & (p <= nt))
        def _():
            bo_copy(p - 1).wait()

        jobs = [functools.partial(transpose_w, n)
                for n in range(3 * pw // LANES)]
        jobs = [None, relayout_bo, relayout_bq] + jobs
        for c in range(n_chunk):
            r0, r1 = bounds[c], bounds[c + 1]
            for j in range(3):
                lhs = xn_s[skip + r0:skip + r1, :]
                job = jobs.pop(0) if jobs else None
                if job is not None:
                    top = jnp.where(always, lhs[:16],
                                    jnp.concatenate(job(), axis=1))
                    lhs = jnp.concatenate([top, lhs[16:]], axis=0)
                pre_s[p, r0:r1, j * pw:(j + 1) * pw] = _dot(
                    lhs, wst_v[slot, j * pw:(j + 1) * pw, :],
                    _NT).astype(BF16)
        assert not jobs

        @pl.when(p + NSLOT < n_pairs)
        def _():
            for j in range(3):
                w_copy(p + NSLOT, j).start()

        @pl.when(p + NSLOT == n_pairs)
        def _():
            xb_copy.start()
            xc_copy.start()

        @pl.when(p + 1 < n_pairs)
        def _():
            wo_copy(p + 1).start()

        @pl.when(p + 1 < n_bq)
        def _():
            bq_copy(p + 1).start()

        @pl.when(p + 1 < nt)
        def _():
            bo_copy(p + 1).start()

        return carry

    lax.fori_loop(0, n_pairs, pre_pair, 0)

    xb_copy.wait()
    xc_copy.wait()
    for p in range(n_pairs):
        wo_copy(p).wait()

    def b_pass(t, par):
        return _BPass(y_s, ((t - 1) * seg, (t - 1 - LAG) * seg), bqkv_p, bo_p,
                      kv_s.at[par], kv_s.at[1 - par], seg=seg, d=d)

    def b_store(t, yb):
        out_v[jnp.maximum(t - 1 - LAG, 0)] = yb[seg:].astype(out_v.dtype)
        return yb[:seg]

    def two_layer_step(t, par, h):
        half = t >> 1
        pre_row = None
        if par == 0:
            pre_row = pl.multiple_of((half - LAG // 2) * PRE, PRE)
        a = _TwoLayerPass(h, pre_s, pre_row, w_v, wo_v,
                          dh=dh, m_len=m_len, seg=seg)
        init = jnp.concatenate(
            [jnp.zeros((m2, d), F32), x_v[half, par].astype(F32), ra_s[...]],
            axis=0)
        acc, yb = a.run(n_pairs, init, b_pass(t, par), t >= 0)
        x2 = b_store(t, yb)
        y_s[...] = acc[m2:]
        ra_s[...] = x2
        if par == 0:
            xn = x_v[half, 1]
        else:
            xn = x_v[jnp.minimum(half + 1, n_half - 1), 0, :nf, :]
        return jnp.concatenate([_ln(xn.astype(F32)), _ln(x2), acc[:m2]],
                               axis=0).astype(BF16)

    def two_layer_steps(i, carry):
        h = h_s[...]
        for u in range(UNROLL):
            h = two_layer_step(LAG + i * UNROLL + u, (LAG + u) % 2, h)
        h_s[...] = h
        return carry

    def one_layer_step(t, carry):
        first = t < LAG
        extra_row = pl.multiple_of(n_pre + jnp.minimum(t, 1) * m_len, m_len)
        a = _OneLayerPass(h1_s[...], pre_s, extra_row, w_v, wo_v,
                          dh=dh, m_len=m_len, seg=seg)
        x0 = x_seg(jnp.minimum(t, n_seg - 1))[...].astype(F32)
        init = jnp.concatenate(
            [jnp.zeros((m_len, d), F32), jnp.where(first, x0, ra_s[...])],
            axis=0)
        acc, yb = a.run(n_pairs, init, b_pass(t, t & 1), t >= 0)
        x2 = b_store(t, yb)
        y = acc[m_len:]
        y_s[:seg, :] = y
        y_s[seg:, :] = y
        ra_s[...] = x2
        xn = _ln(x_seg(jnp.minimum(t + 1, n_seg - 1))[...].astype(F32))
        x2n = _ln(x2)
        mem = acc[:m_len]
        h1_s[:n1, :] = jnp.concatenate(
            [mem, jnp.where(first, xn, x2n)], axis=0).astype(BF16)
        h1_s[n1:, :] = xn_s[last_xn + m_len:, :]
        h_s[...] = jnp.concatenate(
            [xn[:nf], x2n, mem, mem_v[...].astype(F32)], axis=0).astype(BF16)
        return carry

    n_early_out = n_seg - 1 - LAG
    out_a = pltpu.make_async_copy(out_v.at[:n_early_out],
                                  out_hbm.at[:n_early_out], sems.at[3])
    out_b = pltpu.make_async_copy(out_v.at[n_early_out:],
                                  out_hbm.at[n_early_out:], sems.at[4])

    def phase(ph, carry):
        t0 = ph * n_seg
        lax.fori_loop(t0, t0 + LAG, one_layer_step, 0)

        @pl.when(ph == 0)
        def _():
            lax.fori_loop(0, (n_seg - LAG) // UNROLL, two_layer_steps, 0)
            out_a.start()
            hf = h_s[...].astype(F32)
            h1_s[:n1, :] = jnp.concatenate(
                [hf[nf + seg + m_len:], hf[nf:nf + seg]],
                axis=0).astype(BF16)

        return carry

    lax.fori_loop(0, 2, phase, 0)

    b = _BPass(y_s.at[seg:], ((n_seg - 1) * seg,), bqkv_p, bo_p,
               kv_s.at[(n_seg + LAG) % 2, 1:], None, seg=seg, d=d)
    b.project()
    for gi in range(b.n_groups):
        b.attend(gi)
    out_v[n_seg - 1] = b.finish().astype(out_v.dtype)
    out_b.start()
    out_a.wait()
    out_b.wait()


def pallas_interleave_layers__memory_aug_recurrent_mem_tr__sliding_local_dilated__prompt_kernel(
    A_x: jax.Array,
    A_mem0: jax.Array,
    A_Wq: jax.Array,
    A_Wk: jax.Array,
    A_Wv: jax.Array,
    A_Wo: jax.Array,
    A_seg_len,
    B_x: jax.Array,
    B_wqkv: jax.Array,
    B_wo: jax.Array,
):
    del B_x
    seg = A_seg_len if isinstance(A_seg_len, int) else SEG_LEN
    return _forward(A_x, A_mem0, A_Wq, A_Wk, A_Wv, A_Wo, B_wqkv, B_wo, seg=seg)


@functools.partial(jax.jit, static_argnames=("seg",))
def _forward(A_x, A_mem0, A_Wq, A_Wk, A_Wv, A_Wo, B_wqkv, B_wo, *, seg):
    bsz, s_len, d = A_x.shape
    m_len = A_mem0.shape[1]
    n_heads, dh = A_Wq.shape[1], A_Wq.shape[2]
    n_seg = s_len // seg
    n_pairs = n_heads // 2
    nt = d // LANES
    assert bsz == 1 and s_len % seg == 0 and n_seg > LAG + 1
    assert m_len == 8 and seg == 2 * m_len + PRE and seg >= HIST
    assert LAG == 2 and LAG * m_len == PRE and n_seg % (2 * LN_SEGS) == 0
    assert 2 * (m_len + seg) + 4 * m_len <= LANES
    assert (n_seg - LAG) % UNROLL == 0 and UNROLL == 2
    assert n_heads % 2 == 0 and 2 * dh == 3 * LANES and d % LANES == 0
    assert d % HB == 0 and LANES == 4 * HB and n_pairs == 3 * nt + 1
    hd = n_heads * dh
    n_half = n_seg // 2
    n_pre = (n_half - LAG // 2) * PRE

    wq_t = jnp.transpose(A_Wq, (1, 2, 0)).reshape(hd, d)
    wk_t = jnp.transpose(A_Wk, (1, 2, 0)).reshape(hd, d)
    wv_t = jnp.transpose(A_Wv, (1, 2, 0)).reshape(hd, d)
    wo = A_Wo.reshape(hd, d)

    kernel = functools.partial(
        _kernel, seg=seg, n_seg=n_seg, m_len=m_len, n_pairs=n_pairs, dh=dh,
        d=d)
    any_spec = pl.BlockSpec(memory_space=pl.ANY)
    dma = pltpu.SemaphoreType.DMA
    out = pl.pallas_call(
        kernel,
        out_shape=jax.ShapeDtypeStruct((n_seg, seg, d), A_x.dtype),
        in_specs=[any_spec] * 8,
        out_specs=any_spec,
        scratch_shapes=[
            pltpu.VMEM((n_half, 2, seg, d), BF16),
            pltpu.VMEM((m_len, d), BF16),
            pltpu.VMEM((NSLOT, 6 * dh, d), BF16),
            pltpu.VMEM((n_pairs, d, 6 * dh), BF16),
            pltpu.VMEM((hd, d), BF16),
            pltpu.VMEM((3 * nt + 1, LANES, d), BF16),
            pltpu.VMEM((nt + 1, d, LANES), BF16),
            pltpu.VMEM((d + HB, LANES), F32),
            pltpu.VMEM((d + HB, LANES), F32),
            pltpu.VMEM((3, d, d), BF16),
            pltpu.VMEM((nt, d, LANES), BF16),
            pltpu.VMEM((n_seg, seg, d), A_x.dtype),
            pltpu.VMEM((n_half * PRE, d), BF16),
            pltpu.VMEM((n_pairs, n_pre, 6 * dh), BF16),
            pltpu.VMEM((2 * (m_len + seg) - PRE, d), BF16),
            pltpu.VMEM((2 * m_len + seg, d), BF16),
            pltpu.VMEM((seg, d), F32),
            pltpu.VMEM((2 * seg, d), F32),
            pltpu.VMEM((2, 2, 2 * nt, HIST + seg, LANES), F32),
            dma((7,)), dma((NSLOT,)), dma((n_pairs,)),
            dma((3 * nt,)), dma((nt,)),
        ],
        compiler_params=pltpu.CompilerParams(
            vmem_limit_bytes=110 * 1024 * 1024,
            disable_bounds_checks=True),
    )(A_x.reshape(n_half, 2, seg, d), A_mem0.reshape(m_len, d), wq_t, wk_t, wv_t,
      wo, B_wqkv, B_wo)
    return out.reshape(bsz, s_len, d)
```

```python
import functools

import jax
import jax.numpy as jnp
from jax import lax
import jax.experimental.pallas as pl
import jax.experimental.pallas.tpu as pltpu

F32 = jnp.float32
BF16 = jnp.bfloat16

_NT = (((1,), (1,)), ((), ()))
_NN = (((1,), (0,)), ((), ()))

SEG_LEN = 32
HB = 32
WIN = 8
DIL = 2
HIST = 16
LANES = 128
PRE = 16
PRE_CHUNK = 128
LN_SEGS = 16
LAG = 2
UNROLL = 2
NSLOT = 2
NEG = -1000000000.0


def _dot(a, b, dims):
    return lax.dot_general(a, b, dims, preferred_element_type=F32)


def _recip(x):
    r = pl.reciprocal(x, approx=True)
    return r * (2.0 - x * r)


def _ln(x):
    m = jnp.mean(x, axis=-1, keepdims=True)
    xc = x - m
    v = jnp.mean(xc * xc, axis=-1, keepdims=True)
    return xc * lax.rsqrt(v + 1e-05)


def _tile(a, c):
    return a[:, c * LANES:(c + 1) * LANES]


def _keep(mask, a):
    return jnp.where(mask, a, jnp.zeros_like(a))


def _drop(mask, a):
    return jnp.where(mask, jnp.zeros_like(a), a)


def _pair_softmax(s, col_a):
    m_a = jnp.max(jnp.where(col_a, s, -jnp.inf), axis=1, keepdims=True)
    m_b = jnp.max(jnp.where(col_a, -jnp.inf, s), axis=1, keepdims=True)
    e = jnp.exp(s - jnp.where(col_a, m_a, m_b))
    d_a = jnp.sum(jnp.where(col_a, e, 0.0), axis=1, keepdims=True)
    d_b = jnp.sum(jnp.where(col_a, 0.0, e), axis=1, keepdims=True)
    return e * _recip(jnp.where(col_a, d_a, d_b))


class _PassBase:
    def __init__(self, h, w_ref, wo_ref, dh):
        self.h, self.w, self.wo = h, w_ref, wo_ref
        self.pw = 2 * dh
        self.half = dh - LANES
        self.scale = dh ** (-0.5)
        self.q, self.k, self.v, self.p, self.o = {}, {}, {}, {}, {}
        self.cols = (0, 2 * LANES, wo_ref.shape[1])
        self.pending = None

    def _lane_lo(self, rows):
        return lax.broadcasted_iota(jnp.int32, (rows, LANES), 1) < self.half

    def _project(self, p, j):
        a = _dot(self.h, self.w[3 * p + j], _NN)
        self.marker = a[:8, :LANES]
        return a

    def _gate(self, s):
        if self.pending is None:
            return s
        top = jnp.where(self.always, s[:8], self.pending[:, :s.shape[1]])
        self.pending = None
        return jnp.concatenate([top, s[8:]], axis=0)

    def out(self, p, part=None):
        for k in ((0, 1) if part is None else (part,)):
            c0, c1 = self.cols[k], self.cols[k + 1]
            w = self.wo[p * self.pw:(p + 1) * self.pw, c0:c1]
            self.acc[k] = self.acc[k] + _dot(self.o[p], w, _NN)

    def run(self, n_pairs, init, b, always):
        last = n_pairs - 1
        self.acc = [init[:, :self.cols[1]], init[:, self.cols[1]:]]
        self.always = always
        done = None
        for p in range(n_pairs):
            self.proj_q(p)
            self.pending, done = done, None
            if 2 <= p < 2 + b.n_groups:
                o = b.attend(p - 2, (always, self.marker))
                done = functools.reduce(lambda u, v: u + v, o)
            self.proj_k(p)
            if p > 0:
                self.pv(p - 1)
            self.proj_v(p)
            self.scores(p)
            if p == 0:
                b.project()
            elif p < last:
                self.out(p - 1)
        yb = b.finish()
        self.out(last - 1, 0)
        self.pv(last)
        self.out(last - 1, 1)
        self.out(last)
        return jnp.concatenate(self.acc, axis=1), yb


class _TwoLayerPass(_PassBase):
    def __init__(self, h, pre_ref, pre_row, w_ref, wo_ref, *, dh, m_len, seg):
        super().__init__(h, w_ref, wo_ref, dh)
        self.pre, self.pre_row = pre_ref, pre_row
        u = self.u = m_len
        n = self.n = 2 * (m_len + seg)
        self.ext = 4 * u
        self.seg = seg
        row = lax.broadcasted_iota(jnp.int32, (n, n + self.ext), 0)
        col = lax.broadcasted_iota(jnp.int32, (n, n + self.ext), 1)
        rep = col >= n
        col = jnp.where(rep, col - n, col)

        def first_layer(i):
            return (((i < 6 * u) & ((i & u) == 0))
                    | ((i >= 6 * u) & (i < 6 * u + PRE)))

        def index(i):
            low = ((i >> 1) & ~(u - 1)) + (i & (u - 1))
            high = jnp.where(i < 6 * u + PRE, i - 3 * u, i - 3 * u - PRE)
            return jnp.where(i < 6 * u, low, high)

        self.col_a = first_layer(col)
        self.diag = first_layer(row) == self.col_a
        used = ((row >= 3 * u) & (row < 4 * u)) == rep
        self.allowed = used & ((row < 2 * u) | (index(row) >= index(col)))
        self.fill = jnp.where(used, NEG, -jnp.inf)
        self.lo_u = self._lane_lo(u)
        self.lo_c = self._lane_lo(PRE)

    def _proj(self, p, j):
        u, seg = self.u, self.seg
        r = self._project(p, j)
        if self.pre_row is None:
            n1 = seg
            c1 = r[2 * u:n1].astype(BF16)
        else:
            n1 = 2 * u
            c1 = self.pre[3 * p + j, pl.ds(self.pre_row, PRE), :]
        nx = n1 + seg
        return ((r[nx:nx + u], r[:u], r[u:2 * u], c1),
                (r[nx + u:], r[n1:n1 + u], r[n1 + u:n1 + 2 * u],
                 r[n1 + 2 * u:nx].astype(BF16)))

    @staticmethod
    def _weave(f, g):
        top = jnp.concatenate([f[0], g[0], f[1], g[1], f[2], g[2]], axis=0)
        return jnp.concatenate([top.astype(BF16), f[3], g[3]], axis=0)

    def _tiles(self, l1, l2):
        masks = (self.lo_u,) * 3 + (self.lo_c,)

        def t(l, c):
            return [_tile(a, c) for a in l]

        def lo(l):
            return [_keep(mk, a) for mk, a in zip(masks, l)]

        def hi(l):
            return [_drop(mk, a) for mk, a in zip(masks, l)]

        def extend(a, b):
            return jnp.concatenate([a, b[:self.ext]], axis=0)

        t0 = self._weave(t(l1, 0), t(l2, 0))
        t2 = self._weave(t(l2, 2), t(l1, 2))
        t1a = self._weave(lo(t(l1, 1)), hi(t(l1, 1)))
        t1b = self._weave(hi(t(l2, 1)), lo(t(l2, 1)))
        return extend(t0, t0), extend(t1a, t1b), t1b, extend(t2, t2)

    def _split_rows(self, l1, l2):
        ra = jnp.concatenate([l1[0], l1[2], l1[1], l2[1]], axis=0)
        rb = jnp.concatenate([l2[0], l2[2]], axis=0)
        return (jnp.concatenate([ra.astype(BF16), l1[3]], axis=0),
                jnp.concatenate([rb.astype(BF16), l2[3]], axis=0))

    def _units(self, ra, rb):
        u = self.u
        return ((ra[:u], ra[2 * u:3 * u], ra[u:2 * u], ra[4 * u:]),
                (rb[:u], ra[3 * u:4 * u], rb[u:2 * u], rb[2 * u:]))

    def _unweave(self, a):
        u = self.u
        return ((a[:u], a[2 * u:3 * u], a[4 * u:5 * u], a[6 * u:6 * u + PRE]),
                (a[u:2 * u], a[3 * u:4 * u], a[5 * u:6 * u], a[6 * u + PRE:]))

    def proj_q(self, p):
        l1, l2 = self._proj(p, 0)
        q0, q2 = (self._weave([_tile(a, c) for a in l1],
                              [_tile(a, c) for a in l2]) for c in (0, 2))
        qa, qb = self._split_rows([_tile(a, 1) for a in l1],
                                  [_tile(a, 1) for a in l2])
        self.q[p] = (q0, qa, qb, q2)

    def proj_k(self, p):
        self.k[p] = self._tiles(*self._proj(p, 1))

    def proj_v(self, p):
        self.v[p] = self._tiles(*self._proj(p, 2))

    def scores(self, p):
        q0, qa, qb, q2 = self.q.pop(p)
        k0, k1a, k1b, k2 = self.k.pop(p)
        r0 = _dot(q0, k0, _NT)
        r2 = _dot(q2, k2, _NT)
        ra = _dot(qa, k1a, _NT)
        rb = _dot(qb, k1b, _NT)
        rb = jnp.concatenate(
            [rb, jnp.zeros((rb.shape[0], self.ext), F32)], axis=1)
        f, g = self._units(ra, rb)
        r1 = jnp.concatenate(
            [f[0], g[0], f[1], g[1], f[2], g[2], f[3], g[3]], axis=0)
        s = jnp.where(self.diag, r0, r2) + r1
        s = self._gate(jnp.where(self.allowed, s * self.scale, self.fill))
        p_all = _pair_softmax(s, self.col_a)
        f, g = self._unweave(p_all)
        pa, pb = self._split_rows(f[:3] + (f[3].astype(BF16),),
                                  g[:3] + (g[3].astype(BF16),))
        self.p[p] = (_keep(self.diag, p_all).astype(BF16), pa,
                     pb[:, :self.n], _drop(self.diag, p_all).astype(BF16))

    def pv(self, p):
        p0, pa, pb, p2 = self.p.pop(p)
        v0, v1a, v1b, v2 = self.v.pop(p)
        o0 = self._unweave(_dot(p0, v0, _NN))
        o2 = self._unweave(_dot(p2, v2, _NN))
        o1 = self._units(_dot(pa, v1a, _NN), _dot(pb, v1b, _NN))
        self.o[p] = jnp.concatenate(
            [jnp.concatenate((f[0], g[0]) + f[1:] + g[1:], axis=0)
             for f, g in (o0, o1, o2)], axis=1).astype(BF16)


class _OneLayerPass(_PassBase):
    def __init__(self, h, pre_ref, pre_row, w_ref, wo_ref, *, dh, m_len, seg):
        super().__init__(h, w_ref, wo_ref, dh)
        self.pre, self.pre_row = pre_ref, pre_row
        n = self.n = m_len + seg
        row = lax.broadcasted_iota(jnp.int32, (n, 2 * n), 0)
        col = lax.broadcasted_iota(jnp.int32, (n, 2 * n), 1)
        self.col_a = col < n
        key = jnp.where(self.col_a, col, col - n)
        self.allowed = (row < m_len) | (row >= key)
        lane = lax.broadcasted_iota(jnp.int32, (n, self.pw), 1)
        self.head0 = lane < dh

    def _project(self, p, j):
        a = super()._project(p, j)
        n = self.n
        self.pre[3 * p + j, pl.ds(self.pre_row, a.shape[0] - n), :] = (
            a[n:].astype(BF16))
        return a[:n]

    def _block_diag(self, a):
        return jnp.concatenate([_keep(self.head0, a), _drop(self.head0, a)],
                               axis=0).astype(BF16)

    def proj_q(self, p):
        self.q[p] = self._project(p, 0).astype(BF16)

    def proj_k(self, p):
        self.k[p] = self._block_diag(self._project(p, 1))

    def proj_v(self, p):
        self.v[p] = self._block_diag(self._project(p, 2))

    def scores(self, p):
        s = _dot(self.q.pop(p), self.k.pop(p), _NT)
        s = self._gate(jnp.where(self.allowed, s * self.scale, NEG))
        self.p[p] = _pair_softmax(s, self.col_a).astype(BF16)

    def pv(self, p):
        self.o[p] = _dot(self.p.pop(p), self.v.pop(p), _NN).astype(BF16)


class _BPass:
    def __init__(self, y_ref, starts, wqkv_ref, wo_ref, kv_ref, kv_next_ref,
                 *, seg, d):
        self.y, self.starts = y_ref, starts
        self.wqkv, self.wo, self.kv = wqkv_ref, wo_ref, kv_ref
        self.kv_next = kv_next_ref
        self.seg, self.nt = seg, d // LANES
        self.scale = (d // HB) ** (-0.5)
        self.n_groups = len(starts) * seg // 8
        self.outs = []

    def project(self):
        seg, nt = self.seg, self.nt
        yn = _ln(self.y[...]).astype(BF16)
        self.q, ka, va = (_dot(yn, self.wqkv[j], _NN) for j in range(3))
        for i in range(len(self.starts)):
            for c in range(2 * nt):
                a = _tile((ka, va)[c // nt][i * seg:(i + 1) * seg], c % nt)
                self.kv[i, c, HIST:, :] = a
                if self.kv_next is not None:
                    self.kv_next[i, c, :HIST, :] = a[seg - HIST:]

    def attend(self, gi, after=None):
        seg, nt, kv = self.seg, self.nt, self.kv
        i, g = divmod(gi, seg // 8)
        q = [_tile(self.q[8 * gi:8 * gi + 8], c) for c in range(nt)]
        if after is not None:
            q = [jnp.where(after[0], u, after[1]) for u in q]
        pos = (lax.broadcasted_iota(jnp.int32, (8, LANES), 0)
               + (self.starts[i] + 8 * g))
        offs = [HIST + 8 * g - w * DIL for w in range(WIN)]
        logits = []
        for w, off in enumerate(offs):
            t = q[0] * kv[i, 0, off:off + 8, :]
            for c in range(1, nt):
                t = t + q[c] * kv[i, c, off:off + 8, :]
            t = t + pltpu.roll(t, 64, 1)
            t = (t + pltpu.roll(t, 32, 1)) * self.scale
            if 8 * g < w * DIL:
                t = jnp.where(pos >= w * DIL, t, NEG)
            logits.append(t)
        m = logits[0]
        for t in logits[1:]:
            m = jnp.maximum(m, t)
        es = [jnp.exp(t - m) for t in logits]
        den = es[0]
        for e in es[1:]:
            den = den + e
        inv = _recip(den)
        o = []
        for c in range(nt):
            acc = None
            for w, off in enumerate(offs):
                term = es[w] * kv[i, nt + c, off:off + 8, :]
                acc = term if acc is None else acc + term
            o.append(acc * inv)
        self.outs.append(jnp.concatenate(o, axis=1))
        return o

    def finish(self):
        o = jnp.concatenate(self.outs, axis=0).astype(BF16)
        proj = jnp.concatenate(
            [_dot(o, self.wo[c], _NN) for c in range(self.nt)], axis=1)
        return self.y[...] + proj


def _kernel(x_hbm, mem_hbm, wq_hbm, wk_hbm, wv_hbm, wo_hbm, bqkv_hbm, bo_hbm,
            out_hbm,
            x_v, mem_v, wst_v, w_v, wo_v, bq_st, bo_st, tq_s, to_s, bqkv_p,
            bo_p, out_v, xn_s, pre_s, h_s, h1_s, ra_s, y_s, kv_s,
            sems, w_sems, wo_sems, bq_sems, bo_sems,
            *, seg, n_seg, m_len, n_pairs, dh, d):
    db = d // HB
    nt = d // LANES
    pw = 2 * dh
    m2 = 2 * m_len
    n_half = n_seg // 2
    n_pre = (n_half - 1 - LAG // 2) * PRE
    n_bq = 3 * nt

    def w_copy(p, j, sem=None):
        src = (wq_hbm, wk_hbm, wv_hbm)[j]
        slot = p & (NSLOT - 1)
        return pltpu.make_async_copy(
            src.at[pl.ds(p * pw, pw), :], wst_v.at[slot, j],
            w_sems.at[slot if sem is None else sem])

    def w_wait(p):
        slot = p & (NSLOT - 1)
        pltpu.make_async_copy(wst_v.at[slot], wst_v.at[slot],
                              w_sems.at[slot]).wait()

    def wo_copy(p):
        return pltpu.make_async_copy(wo_hbm.at[pl.ds(p * pw, pw), :],
                                     wo_v.at[pl.ds(p * pw, pw), :],
                                     wo_sems.at[p])

    def bq_copy(i):
        row = pl.multiple_of((i % nt) * LANES, LANES)
        col = pl.multiple_of((i // nt) * d, LANES)
        return pltpu.make_async_copy(
            bqkv_hbm.at[pl.ds(row, LANES), pl.ds(col, d)], bq_st.at[i],
            bq_sems.at[i])

    def bo_copy(i):
        col = pl.multiple_of(i * LANES, LANES)
        return pltpu.make_async_copy(bo_hbm.at[:, pl.ds(col, LANES)],
                                     bo_st.at[i], bo_sems.at[i])

    nf = seg - PRE

    def x_copy(idx, sem):
        return pltpu.make_async_copy(x_hbm.at[idx], x_v.at[idx], sems.at[sem])

    full = slice(None)
    xa_copy = x_copy((full, 0, slice(nf, None), full), 0)
    x0_copy = x_copy((0, 0, slice(None, nf), full), 5)
    xb_copy = x_copy((slice(1, None), 0, slice(None, nf), full), 1)
    xc_copy = x_copy((full, 1), 6)

    def x_seg(t):
        return x_v.at[t >> 1, t & 1]

    mem_copy = pltpu.make_async_copy(mem_hbm, mem_v, sems.at[2])

    mem_copy.start()
    xa_copy.start()
    mem_copy.wait()
    x0_copy.start()
    w_copy(0, 0, sem=NSLOT).start()

    ra_s[...] = jnp.zeros(ra_s.shape, F32)
    y_s[...] = jnp.zeros(y_s.shape, F32)
    kv_s[0, :, :, :HIST, :] = jnp.zeros(kv_s.shape[1:3] + (HIST, LANES), F32)

    xa_copy.wait()
    for j in range(1, 3):
        w_copy(0, j, sem=NSLOT + j).start()

    def ln_block(i, carry):
        s0 = pl.multiple_of(i * LN_SEGS, LN_SEGS)
        xb = x_v[pl.ds(s0, LN_SEGS), 0, nf:, :].astype(F32)
        xn_s[pl.ds(pl.multiple_of(s0 * PRE, PRE), LN_SEGS * PRE), :] = _ln(
            xb.reshape(LN_SEGS * PRE, d)).astype(BF16)
        return carry

    lax.fori_loop(0, n_half // LN_SEGS, ln_block, 0)

    n1 = m_len + seg
    last_xn = (n_half - 1) * PRE
    x0_copy.wait()
    for j in range(3):
        w_copy(1, j).start()
    bq_copy(0).start()
    bo_copy(0).start()
    wo_copy(0).start()

    def permute_rows(tmp_ref):
        return jnp.concatenate(
            [tmp_ref[pl.ds(j, HB, stride=db), :] for j in range(db)], axis=0)

    n_chunk = -(-n_pre // PRE_CHUNK)
    bounds = [16 * (n_pre // 16 * c // n_chunk) for c in range(n_chunk + 1)]
    skip = LAG // 2 * PRE

    def pre_blocks(blocks, jobs, always):
        def transpose_w(src, b, n):
            wt = src[n * LANES:(n + 1) * LANES, :].T
            w_v[b, :, n * LANES:(n + 1) * LANES] = wt
            return [wt[(c + 1) * LANES - 16:(c + 1) * LANES]
                    for c in range(nt)]

        jobs = [None] + jobs + [functools.partial(transpose_w, src, b, n)
                                for src, b in blocks
                                for n in range(pw // LANES)]
        for c in range(n_chunk):
            r0, r1 = bounds[c], bounds[c + 1]
            for src, b in blocks:
                lhs = xn_s[skip + r0:skip + r1, :]
                job = jobs.pop(0) if jobs else None
                if job is not None:
                    top = jnp.where(always, lhs[:16],
                                    jnp.concatenate(job(), axis=1))
                    lhs = jnp.concatenate([top, lhs[16:]], axis=0)
                pre_s[b, r0:r1, :] = _dot(lhs, src[...], _NT).astype(BF16)
        assert not jobs

    def first_block(j, carry):
        src = wst_v.at[0, j]
        pltpu.make_async_copy(src, src, w_sems.at[NSLOT + j]).wait()
        pre_blocks([(src, j)], [], j >= 0)
        h1_s[:n1, :] = jnp.concatenate(
            [mem_v[...].astype(F32), _ln(x_v[0, 0].astype(F32))],
            axis=0).astype(BF16)
        h1_s[n1:, :] = xn_s[last_xn:last_xn + m_len, :]
        return carry

    def prefetch(p):
        @pl.when(p + NSLOT < n_pairs)
        def _():
            for j in range(3):
                w_copy(p + NSLOT, j).start()

        @pl.when(p + NSLOT == n_pairs)
        def _():
            xb_copy.start()
            xc_copy.start()

        @pl.when(p + 1 < n_pairs)
        def _():
            wo_copy(p + 1).start()

        @pl.when(p + 1 < n_bq)
        def _():
            bq_copy(p + 1).start()

        @pl.when(p + 1 < nt)
        def _():
            bo_copy(p + 1).start()

    def pre_pair(p, carry):
        def relayout_bo():
            i = jnp.minimum(p - 1, nt - 1)
            to_s[:d, :] = bo_st[i].astype(F32)
            bo = permute_rows(to_s)
            bo_p[i] = bo.astype(BF16)
            g = d // nt // 16
            return [functools.reduce(
                lambda u, v: u + v,
                [bo[16 * (c * g + r):16 * (c * g + r + 1)] for r in range(g)]
            ).astype(BF16) for c in range(nt)]

        def relayout_bq():
            i = p - 1
            tq_s[:d, :] = bq_st[i].astype(F32).T
            row = pl.multiple_of((i % nt) * LANES, LANES)
            bq = permute_rows(tq_s).T.astype(BF16)
            bqkv_p[i // nt, pl.ds(row, LANES), :] = bq
            return [_tile(bq[LANES - 16:], c) for c in range(nt)]

        w_wait(p)
        pltpu.make_async_copy(bq_st.at[p - 1], bq_st.at[p - 1],
                              bq_sems.at[p - 1]).wait()

        @pl.when(p <= nt)
        def _():
            bo_copy(p - 1).wait()

        slot = p & (NSLOT - 1)
        pre_blocks([(wst_v.at[slot, j], 3 * p + j) for j in range(3)],
                   [relayout_bo, relayout_bq], p >= 0)
        prefetch(p)
        return carry

    lax.fori_loop(0, 3, first_block, 0)
    prefetch(jnp.int32(0))
    lax.fori_loop(1, n_pairs, pre_pair, 0)

    xb_copy.wait()
    xc_copy.wait()
    for p in range(n_pairs):
        wo_copy(p).wait()

    def b_pass(t, par):
        return _BPass(y_s, ((t - 1) * seg, (t - 1 - LAG) * seg), bqkv_p, bo_p,
                      kv_s.at[par], kv_s.at[1 - par], seg=seg, d=d)

    def b_store(t, yb):
        out_v[jnp.maximum(t - 1 - LAG, 0)] = yb[seg:].astype(out_v.dtype)
        return yb[:seg]

    def two_layer_step(t, par, h):
        half = t >> 1
        pre_row = None
        if par == 0:
            pre_row = pl.multiple_of((half - LAG // 2) * PRE, PRE)
        a = _TwoLayerPass(h, pre_s, pre_row, w_v, wo_v,
                          dh=dh, m_len=m_len, seg=seg)
        init = jnp.concatenate(
            [jnp.zeros((m2, d), F32), x_v[half, par].astype(F32), ra_s[...]],
            axis=0)
        acc, yb = a.run(n_pairs, init, b_pass(t, par), t >= 0)
        x2 = b_store(t, yb)
        y_s[...] = acc[m2:]
        ra_s[...] = x2
        if par == 0:
            xn = x_v[half, 1]
        else:
            xn = x_v[jnp.minimum(half + 1, n_half - 1), 0, :nf, :]
        return jnp.concatenate([_ln(xn.astype(F32)), _ln(x2), acc[:m2]],
                               axis=0).astype(BF16)

    def two_layer_steps(i, carry):
        h = h_s[...]
        for u in range(UNROLL):
            h = two_layer_step(LAG + i * UNROLL + u, (LAG + u) % 2, h)
        h_s[...] = h
        return carry

    def one_layer_step(t, carry):
        first = t < LAG
        extra_row = pl.multiple_of(n_pre + jnp.minimum(t, 1) * m_len, m_len)
        a = _OneLayerPass(h1_s[...], pre_s, extra_row, w_v, wo_v,
                          dh=dh, m_len=m_len, seg=seg)
        x0 = x_seg(jnp.minimum(t, n_seg - 1))[...].astype(F32)
        init = jnp.concatenate(
            [jnp.zeros((m_len, d), F32), jnp.where(first, x0, ra_s[...])],
            axis=0)
        acc, yb = a.run(n_pairs, init, b_pass(t, t & 1), t >= 0)
        x2 = b_store(t, yb)
        y = acc[m_len:]
        y_s[:seg, :] = y
        y_s[seg:, :] = y
        ra_s[...] = x2
        xn = _ln(x_seg(jnp.minimum(t + 1, n_seg - 1))[...].astype(F32))
        x2n = _ln(x2)
        mem = acc[:m_len]
        h1_s[:n1, :] = jnp.concatenate(
            [mem, jnp.where(first, xn, x2n)], axis=0).astype(BF16)
        h1_s[n1:, :] = xn_s[last_xn + m_len:, :]
        h_s[...] = jnp.concatenate(
            [xn[:nf], x2n, mem, mem_v[...].astype(F32)], axis=0).astype(BF16)
        return carry

    n_early_out = n_seg - 1 - LAG
    out_a = pltpu.make_async_copy(out_v.at[:n_early_out],
                                  out_hbm.at[:n_early_out], sems.at[3])
    out_b = pltpu.make_async_copy(out_v.at[n_early_out:],
                                  out_hbm.at[n_early_out:], sems.at[4])

    def phase(ph, carry):
        t0 = ph * n_seg
        lax.fori_loop(t0, t0 + LAG, one_layer_step, 0)

        @pl.when(ph == 0)
        def _():
            lax.fori_loop(0, (n_seg - LAG) // UNROLL, two_layer_steps, 0)
            out_a.start()
            hf = h_s[...].astype(F32)
            h1_s[:n1, :] = jnp.concatenate(
                [hf[nf + seg + m_len:], hf[nf:nf + seg]],
                axis=0).astype(BF16)

        return carry

    lax.fori_loop(0, 2, phase, 0)

    b = _BPass(y_s.at[seg:], ((n_seg - 1) * seg,), bqkv_p, bo_p,
               kv_s.at[(n_seg + LAG) % 2, 1:], None, seg=seg, d=d)
    b.project()
    for gi in range(b.n_groups):
        b.attend(gi)
    out_v[n_seg - 1] = b.finish().astype(out_v.dtype)
    out_b.start()
    out_a.wait()
    out_b.wait()


def pallas_interleave_layers__memory_aug_recurrent_mem_tr__sliding_local_dilated__prompt_kernel(
    A_x: jax.Array,
    A_mem0: jax.Array,
    A_Wq: jax.Array,
    A_Wk: jax.Array,
    A_Wv: jax.Array,
    A_Wo: jax.Array,
    A_seg_len,
    B_x: jax.Array,
    B_wqkv: jax.Array,
    B_wo: jax.Array,
):
    del B_x
    seg = A_seg_len if isinstance(A_seg_len, int) else SEG_LEN
    return _forward(A_x, A_mem0, A_Wq, A_Wk, A_Wv, A_Wo, B_wqkv, B_wo, seg=seg)


@functools.partial(jax.jit, static_argnames=("seg",))
def _forward(A_x, A_mem0, A_Wq, A_Wk, A_Wv, A_Wo, B_wqkv, B_wo, *, seg):
    bsz, s_len, d = A_x.shape
    m_len = A_mem0.shape[1]
    n_heads, dh = A_Wq.shape[1], A_Wq.shape[2]
    n_seg = s_len // seg
    n_pairs = n_heads // 2
    nt = d // LANES
    assert bsz == 1 and s_len % seg == 0 and n_seg > LAG + 1
    assert m_len == 8 and seg == 2 * m_len + PRE and seg >= HIST
    assert LAG == 2 and LAG * m_len == PRE and n_seg % (2 * LN_SEGS) == 0
    assert 2 * (m_len + seg) + 4 * m_len <= LANES
    assert (n_seg - LAG) % UNROLL == 0 and UNROLL == 2
    assert n_heads % 2 == 0 and 2 * dh == 3 * LANES and d % LANES == 0
    assert d % HB == 0 and LANES == 4 * HB and n_pairs == 3 * nt + 1
    hd = n_heads * dh
    n_half = n_seg // 2
    n_pre = (n_half - LAG // 2) * PRE

    wq_t = jnp.transpose(A_Wq, (1, 2, 0)).reshape(hd, d)
    wk_t = jnp.transpose(A_Wk, (1, 2, 0)).reshape(hd, d)
    wv_t = jnp.transpose(A_Wv, (1, 2, 0)).reshape(hd, d)
    wo = A_Wo.reshape(hd, d)

    kernel = functools.partial(
        _kernel, seg=seg, n_seg=n_seg, m_len=m_len, n_pairs=n_pairs, dh=dh,
        d=d)
    any_spec = pl.BlockSpec(memory_space=pl.ANY)
    dma = pltpu.SemaphoreType.DMA
    out = pl.pallas_call(
        kernel,
        out_shape=jax.ShapeDtypeStruct((n_seg, seg, d), A_x.dtype),
        in_specs=[any_spec] * 8,
        out_specs=any_spec,
        scratch_shapes=[
            pltpu.VMEM((n_half, 2, seg, d), BF16),
            pltpu.VMEM((m_len, d), BF16),
            pltpu.VMEM((NSLOT, 3, 2 * dh, d), BF16),
            pltpu.VMEM((3 * n_pairs, d, 2 * dh), BF16),
            pltpu.VMEM((hd, d), BF16),
            pltpu.VMEM((3 * nt, LANES, d), BF16),
            pltpu.VMEM((nt, d, LANES), BF16),
            pltpu.VMEM((d + HB, LANES), F32),
            pltpu.VMEM((d + HB, LANES), F32),
            pltpu.VMEM((3, d, d), BF16),
            pltpu.VMEM((nt, d, LANES), BF16),
            pltpu.VMEM((n_seg, seg, d), A_x.dtype),
            pltpu.VMEM((n_half * PRE, d), BF16),
            pltpu.VMEM((3 * n_pairs, n_pre, 2 * dh), BF16),
            pltpu.VMEM((2 * (m_len + seg) - PRE, d), BF16),
            pltpu.VMEM((2 * m_len + seg, d), BF16),
            pltpu.VMEM((seg, d), F32),
            pltpu.VMEM((2 * seg, d), F32),
            pltpu.VMEM((2, 2, 2 * nt, HIST + seg, LANES), F32),
            dma((7,)), dma((NSLOT + 3,)), dma((n_pairs,)),
            dma((3 * nt,)), dma((nt,)),
        ],
        compiler_params=pltpu.CompilerParams(
            vmem_limit_bytes=110 * 1024 * 1024,
            disable_bounds_checks=True),
    )(A_x.reshape(n_half, 2, seg, d), A_mem0.reshape(m_len, d), wq_t, wk_t, wv_t,
      wo, B_wqkv, B_wo)
    return out.reshape(bsz, s_len, d)
```

```python
import functools

import jax
import jax.numpy as jnp
from jax import lax
import jax.experimental.pallas as pl
import jax.experimental.pallas.tpu as pltpu

F32 = jnp.float32
BF16 = jnp.bfloat16

_NT = (((1,), (1,)), ((), ()))
_NN = (((1,), (0,)), ((), ()))

SEG_LEN = 32
HB = 32
WIN = 8
DIL = 2
HIST = 16
LANES = 128
PRE = 16
PRE_CHUNK = 128
LN_SEGS = 16
LAG = 2
UNROLL = 2
NSLOT = 2
NEG = -1000000000.0


def _dot(a, b, dims):
    return lax.dot_general(a, b, dims, preferred_element_type=F32)


def _recip(x):
    r = pl.reciprocal(x, approx=True)
    return r * (2.0 - x * r)


def _ln(x):
    m = jnp.mean(x, axis=-1, keepdims=True)
    xc = x - m
    v = jnp.mean(xc * xc, axis=-1, keepdims=True)
    return xc * lax.rsqrt(v + 1e-05)


def _tile(a, c):
    return a[:, c * LANES:(c + 1) * LANES]


def _keep(mask, a):
    return jnp.where(mask, a, jnp.zeros_like(a))


def _drop(mask, a):
    return jnp.where(mask, jnp.zeros_like(a), a)


def _pair_softmax(s, col_a):
    m_a = jnp.max(jnp.where(col_a, s, -jnp.inf), axis=1, keepdims=True)
    m_b = jnp.max(jnp.where(col_a, -jnp.inf, s), axis=1, keepdims=True)
    e = jnp.exp(s - jnp.where(col_a, m_a, m_b))
    d_a = jnp.sum(jnp.where(col_a, e, 0.0), axis=1, keepdims=True)
    d_b = jnp.sum(jnp.where(col_a, 0.0, e), axis=1, keepdims=True)
    return e * _recip(jnp.where(col_a, d_a, d_b))


class _PassBase:
    def __init__(self, h, w_ref, wo_ref, dh):
        self.h, self.w, self.wo = h, w_ref, wo_ref
        self.pw = 2 * dh
        self.half = dh - LANES
        self.scale = dh ** (-0.5)
        self.q, self.k, self.v, self.p, self.o = {}, {}, {}, {}, {}
        self.cols = (0, 2 * LANES, wo_ref.shape[1])
        self.pending = None

    def _lane_lo(self, rows):
        return lax.broadcasted_iota(jnp.int32, (rows, LANES), 1) < self.half

    def _project(self, p, j):
        a = _dot(self.h, self.w[3 * p + j], _NN)
        self.marker = a[:8, :LANES]
        return a

    def _gate(self, s):
        if self.pending is None:
            return s
        top = jnp.where(self.always, s[:8], self.pending[:, :s.shape[1]])
        self.pending = None
        return jnp.concatenate([top, s[8:]], axis=0)

    def out(self, p, part=None):
        for k in ((0, 1) if part is None else (part,)):
            c0, c1 = self.cols[k], self.cols[k + 1]
            w = self.wo[p * self.pw:(p + 1) * self.pw, c0:c1]
            self.acc[k] = self.acc[k] + _dot(self.o[p], w, _NN)

    def run(self, n_pairs, init, b, always):
        last = n_pairs - 1
        self.acc = [init[:, :self.cols[1]], init[:, self.cols[1]:]]
        self.always = always
        done = None
        for p in range(n_pairs):
            self.proj_q(p)
            self.pending, done = done, None
            if 2 <= p < 2 + b.n_groups:
                o = b.attend(p - 2, (always, self.marker))
                done = functools.reduce(lambda u, v: u + v, o)
            self.proj_k(p)
            if p > 0:
                self.pv(p - 1)
            self.proj_v(p)
            self.scores(p)
            if p == 0:
                b.project()
            elif p < last:
                self.out(p - 1)
        yb = b.finish()
        self.out(last - 1, 0)
        self.pv(last)
        self.out(last - 1, 1)
        self.out(last)
        return jnp.concatenate(self.acc, axis=1), yb


class _TwoLayerPass(_PassBase):
    def __init__(self, h, pre_ref, pre_row, w_ref, wo_ref, *, dh, m_len, seg):
        super().__init__(h, w_ref, wo_ref, dh)
        self.pre, self.pre_row = pre_ref, pre_row
        u = self.u = m_len
        n = self.n = 2 * (m_len + seg)
        self.ext = 4 * u
        self.seg = seg
        row = lax.broadcasted_iota(jnp.int32, (n, n + self.ext), 0)
        col = lax.broadcasted_iota(jnp.int32, (n, n + self.ext), 1)
        rep = col >= n
        col = jnp.where(rep, col - n, col)

        def first_layer(i):
            return (((i < 6 * u) & ((i & u) == 0))
                    | ((i >= 6 * u) & (i < 6 * u + PRE)))

        def index(i):
            low = ((i >> 1) & ~(u - 1)) + (i & (u - 1))
            high = jnp.where(i < 6 * u + PRE, i - 3 * u, i - 3 * u - PRE)
            return jnp.where(i < 6 * u, low, high)

        self.col_a = first_layer(col)
        self.diag = first_layer(row) == self.col_a
        used = ((row >= 3 * u) & (row < 4 * u)) == rep
        self.allowed = used & ((row < 2 * u) | (index(row) >= index(col)))
        self.fill = jnp.where(used, NEG, -jnp.inf)
        self.lo_u = self._lane_lo(u)
        self.lo_c = self._lane_lo(PRE)

    def _proj(self, p, j):
        u, seg = self.u, self.seg
        r = self._project(p, j)
        if self.pre_row is None:
            n1 = seg
            c1 = r[2 * u:n1].astype(BF16)
        else:
            n1 = 2 * u
            c1 = self.pre[3 * p + j, pl.ds(self.pre_row, PRE), :]
        nx = n1 + seg
        return ((r[nx:nx + u], r[:u], r[u:2 * u], c1),
                (r[nx + u:], r[n1:n1 + u], r[n1 + u:n1 + 2 * u],
                 r[n1 + 2 * u:nx].astype(BF16)))

    @staticmethod
    def _weave(f, g):
        top = jnp.concatenate([f[0], g[0], f[1], g[1], f[2], g[2]], axis=0)
        return jnp.concatenate([top.astype(BF16), f[3], g[3]], axis=0)

    def _tiles(self, l1, l2):
        masks = (self.lo_u,) * 3 + (self.lo_c,)

        def t(l, c):
            return [_tile(a, c) for a in l]

        def lo(l):
            return [_keep(mk, a) for mk, a in zip(masks, l)]

        def hi(l):
            return [_drop(mk, a) for mk, a in zip(masks, l)]

        def extend(a, b):
            return jnp.concatenate([a, b[:self.ext]], axis=0)

        t0 = self._weave(t(l1, 0), t(l2, 0))
        t2 = self._weave(t(l2, 2), t(l1, 2))
        t1a = self._weave(lo(t(l1, 1)), hi(t(l1, 1)))
        t1b = self._weave(hi(t(l2, 1)), lo(t(l2, 1)))
        return extend(t0, t0), extend(t1a, t1b), t1b, extend(t2, t2)

    def _split_rows(self, l1, l2):
        ra = jnp.concatenate([l1[0], l1[2], l1[1], l2[1]], axis=0)
        rb = jnp.concatenate([l2[0], l2[2]], axis=0)
        return (jnp.concatenate([ra.astype(BF16), l1[3]], axis=0),
                jnp.concatenate([rb.astype(BF16), l2[3]], axis=0))

    def _units(self, ra, rb):
        u = self.u
        return ((ra[:u], ra[2 * u:3 * u], ra[u:2 * u], ra[4 * u:]),
                (rb[:u], ra[3 * u:4 * u], rb[u:2 * u], rb[2 * u:]))

    def _unweave(self, a):
        u = self.u
        return ((a[:u], a[2 * u:3 * u], a[4 * u:5 * u], a[6 * u:6 * u + PRE]),
                (a[u:2 * u], a[3 * u:4 * u], a[5 * u:6 * u], a[6 * u + PRE:]))

    def proj_q(self, p):
        l1, l2 = self._proj(p, 0)
        q0, q2 = (self._weave([_tile(a, c) for a in l1],
                              [_tile(a, c) for a in l2]) for c in (0, 2))
        qa, qb = self._split_rows([_tile(a, 1) for a in l1],
                                  [_tile(a, 1) for a in l2])
        self.q[p] = (q0, qa, qb, q2)

    def proj_k(self, p):
        self.k[p] = self._tiles(*self._proj(p, 1))

    def proj_v(self, p):
        self.v[p] = self._tiles(*self._proj(p, 2))

    def scores(self, p):
        q0, qa, qb, q2 = self.q.pop(p)
        k0, k1a, k1b, k2 = self.k.pop(p)
        r0 = _dot(q0, k0, _NT)
        r2 = _dot(q2, k2, _NT)
        ra = _dot(qa, k1a, _NT)
        rb = _dot(qb, k1b, _NT)
        rb = jnp.concatenate(
            [rb, jnp.zeros((rb.shape[0], self.ext), F32)], axis=1)
        f, g = self._units(ra, rb)
        r1 = jnp.concatenate(
            [f[0], g[0], f[1], g[1], f[2], g[2], f[3], g[3]], axis=0)
        s = jnp.where(self.diag, r0, r2) + r1
        s = self._gate(jnp.where(self.allowed, s * self.scale, self.fill))
        p_all = _pair_softmax(s, self.col_a)
        f, g = self._unweave(p_all)
        pa, pb = self._split_rows(f[:3] + (f[3].astype(BF16),),
                                  g[:3] + (g[3].astype(BF16),))
        self.p[p] = (_keep(self.diag, p_all).astype(BF16), pa,
                     pb[:, :self.n], _drop(self.diag, p_all).astype(BF16))

    def pv(self, p):
        p0, pa, pb, p2 = self.p.pop(p)
        v0, v1a, v1b, v2 = self.v.pop(p)
        o0 = self._unweave(_dot(p0, v0, _NN))
        o2 = self._unweave(_dot(p2, v2, _NN))
        o1 = self._units(_dot(pa, v1a, _NN), _dot(pb, v1b, _NN))
        self.o[p] = jnp.concatenate(
            [jnp.concatenate((f[0], g[0]) + f[1:] + g[1:], axis=0)
             for f, g in (o0, o1, o2)], axis=1).astype(BF16)


class _OneLayerPass(_PassBase):
    def __init__(self, h, pre_ref, pre_row, w_ref, wo_ref, *, dh, m_len, seg):
        super().__init__(h, w_ref, wo_ref, dh)
        self.pre, self.pre_row = pre_ref, pre_row
        n = self.n = m_len + seg
        row = lax.broadcasted_iota(jnp.int32, (n, 2 * n), 0)
        col = lax.broadcasted_iota(jnp.int32, (n, 2 * n), 1)
        self.col_a = col < n
        key = jnp.where(self.col_a, col, col - n)
        self.allowed = (row < m_len) | (row >= key)
        lane = lax.broadcasted_iota(jnp.int32, (n, self.pw), 1)
        self.head0 = lane < dh

    def _project(self, p, j):
        a = super()._project(p, j)
        n = self.n
        self.pre[3 * p + j, pl.ds(self.pre_row, a.shape[0] - n), :] = (
            a[n:].astype(BF16))
        return a[:n]

    def _block_diag(self, a):
        return jnp.concatenate([_keep(self.head0, a), _drop(self.head0, a)],
                               axis=0).astype(BF16)

    def proj_q(self, p):
        self.q[p] = self._project(p, 0).astype(BF16)

    def proj_k(self, p):
        self.k[p] = self._block_diag(self._project(p, 1))

    def proj_v(self, p):
        self.v[p] = self._block_diag(self._project(p, 2))

    def scores(self, p):
        s = _dot(self.q.pop(p), self.k.pop(p), _NT)
        s = self._gate(jnp.where(self.allowed, s * self.scale, NEG))
        self.p[p] = _pair_softmax(s, self.col_a).astype(BF16)

    def pv(self, p):
        self.o[p] = _dot(self.p.pop(p), self.v.pop(p), _NN).astype(BF16)


class _BPass:
    def __init__(self, y_ref, starts, wqkv_ref, wo_ref, kv_ref, kv_next_ref,
                 *, seg, d):
        self.y, self.starts = y_ref, starts
        self.wqkv, self.wo, self.kv = wqkv_ref, wo_ref, kv_ref
        self.kv_next = kv_next_ref
        self.seg, self.nt = seg, d // LANES
        self.scale = (d // HB) ** (-0.5)
        self.n_groups = len(starts) * seg // 8
        self.outs = []

    def project(self):
        seg, nt = self.seg, self.nt
        yn = _ln(self.y[...]).astype(BF16)
        self.q, ka, va = (_dot(yn, self.wqkv[j], _NN) for j in range(3))
        for i in range(len(self.starts)):
            for c in range(2 * nt):
                a = _tile((ka, va)[c // nt][i * seg:(i + 1) * seg], c % nt)
                self.kv[i, c, HIST:, :] = a
                if self.kv_next is not None:
                    self.kv_next[i, c, :HIST, :] = a[seg - HIST:]

    def attend(self, gi, after=None):
        seg, nt, kv = self.seg, self.nt, self.kv
        i, g = divmod(gi, seg // 8)
        q = [_tile(self.q[8 * gi:8 * gi + 8], c) for c in range(nt)]
        if after is not None:
            q = [jnp.where(after[0], u, after[1]) for u in q]
        pos = (lax.broadcasted_iota(jnp.int32, (8, LANES), 0)
               + (self.starts[i] + 8 * g))
        offs = [HIST + 8 * g - w * DIL for w in range(WIN)]
        logits = []
        for w, off in enumerate(offs):
            t = q[0] * kv[i, 0, off:off + 8, :]
            for c in range(1, nt):
                t = t + q[c] * kv[i, c, off:off + 8, :]
            t = t + pltpu.roll(t, 64, 1)
            t = (t + pltpu.roll(t, 32, 1)) * self.scale
            if 8 * g < w * DIL:
                t = jnp.where(pos >= w * DIL, t, NEG)
            logits.append(t)
        m = logits[0]
        for t in logits[1:]:
            m = jnp.maximum(m, t)
        es = [jnp.exp(t - m) for t in logits]
        den = es[0]
        for e in es[1:]:
            den = den + e
        inv = _recip(den)
        o = []
        for c in range(nt):
            acc = None
            for w, off in enumerate(offs):
                term = es[w] * kv[i, nt + c, off:off + 8, :]
                acc = term if acc is None else acc + term
            o.append(acc * inv)
        self.outs.append(jnp.concatenate(o, axis=1))
        return o

    def finish(self):
        o = jnp.concatenate(self.outs, axis=0).astype(BF16)
        proj = jnp.concatenate(
            [_dot(o, self.wo[c], _NN) for c in range(self.nt)], axis=1)
        return self.y[...] + proj


def _kernel(x_hbm, mem_hbm, wq_hbm, wk_hbm, wv_hbm, wo_hbm, bqkv_hbm, bo_hbm,
            out_hbm,
            x_v, mem_v, wst_v, w_v, wo_v, bq_st, bo_st, tq_s, to_s, bqkv_p,
            bo_p, out_v, xn_s, pre_s, h_s, h1_s, ra_s, y_s, kv_s,
            sems, w_sems, bq_sems, bo_sems,
            *, seg, n_seg, m_len, n_pairs, dh, d):
    db = d // HB
    nt = d // LANES
    pw = 2 * dh
    m2 = 2 * m_len
    n_half = n_seg // 2
    n_pre = (n_half - 1 - LAG // 2) * PRE
    n_bq = 3 * nt

    def w_copy(p, j, sem=None):
        src = (wq_hbm, wk_hbm, wv_hbm)[j]
        slot = p & (NSLOT - 1)
        return pltpu.make_async_copy(
            src.at[pl.ds(p * pw, pw), :], wst_v.at[slot, j],
            w_sems.at[slot if sem is None else sem])

    def w_wait(p):
        slot = p & (NSLOT - 1)
        pltpu.make_async_copy(wst_v.at[slot], wst_v.at[slot],
                              w_sems.at[slot]).wait()

    def wo_copy(p):
        return pltpu.make_async_copy(wo_hbm.at[pl.ds(p * pw, pw), :],
                                     wo_v.at[pl.ds(p * pw, pw), :],
                                     sems.at[7])

    def bq_copy(i):
        row = pl.multiple_of((i % nt) * LANES, LANES)
        col = pl.multiple_of((i // nt) * d, LANES)
        return pltpu.make_async_copy(
            bqkv_hbm.at[pl.ds(row, LANES), pl.ds(col, d)], bq_st.at[i],
            bq_sems.at[i & 1])

    def bo_copy(i):
        col = pl.multiple_of(i * LANES, LANES)
        return pltpu.make_async_copy(bo_hbm.at[:, pl.ds(col, LANES)],
                                     bo_st.at[i], bo_sems.at[i & 1])

    nf = seg - PRE

    def x_copy(idx, sem):
        return pltpu.make_async_copy(x_hbm.at[idx], x_v.at[idx], sems.at[sem])

    full = slice(None)
    xa_copy = x_copy((full, 0, slice(nf, None), full), 0)
    x0_copy = x_copy((0, 0, slice(None, nf), full), 5)
    xb_copy = x_copy((slice(1, None), 0, slice(None, nf), full), 1)
    xc_copy = x_copy((full, 1), 6)

    def x_seg(t):
        return x_v.at[t >> 1, t & 1]

    mem_copy = pltpu.make_async_copy(mem_hbm, mem_v, sems.at[2])

    mem_copy.start()
    xa_copy.start()
    mem_copy.wait()
    x0_copy.start()
    w_copy(0, 0, sem=NSLOT).start()

    ra_s[...] = jnp.zeros(ra_s.shape, F32)
    y_s[...] = jnp.zeros(y_s.shape, F32)
    kv_s[0, :, :, :HIST, :] = jnp.zeros(kv_s.shape[1:3] + (HIST, LANES), F32)

    xa_copy.wait()
    for j in range(1, 3):
        w_copy(0, j, sem=NSLOT + j).start()

    def ln_block(i, carry):
        s0 = pl.multiple_of(i * LN_SEGS, LN_SEGS)
        xb = x_v[pl.ds(s0, LN_SEGS), 0, nf:, :].astype(F32)
        xn_s[pl.ds(pl.multiple_of(s0 * PRE, PRE), LN_SEGS * PRE), :] = _ln(
            xb.reshape(LN_SEGS * PRE, d)).astype(BF16)
        return carry

    lax.fori_loop(0, n_half // LN_SEGS, ln_block, 0)

    n1 = m_len + seg
    last_xn = (n_half - 1) * PRE
    x0_copy.wait()
    for j in range(3):
        w_copy(1, j).start()
    bq_copy(0).start()
    bo_copy(0).start()
    wo_copy(0).start()

    def permute_rows(tmp_ref):
        return jnp.concatenate(
            [tmp_ref[pl.ds(j, HB, stride=db), :] for j in range(db)], axis=0)

    n_chunk = -(-n_pre // PRE_CHUNK)
    bounds = [16 * (n_pre // 16 * c // n_chunk) for c in range(n_chunk + 1)]
    skip = LAG // 2 * PRE

    def pre_blocks(blocks, jobs, always):
        def transpose_w(src, b, n):
            wt = src[n * LANES:(n + 1) * LANES, :].T
            w_v[b, :, n * LANES:(n + 1) * LANES] = wt
            return [wt[(c + 1) * LANES - 16:(c + 1) * LANES]
                    for c in range(nt)]

        jobs = [None] + jobs + [functools.partial(transpose_w, src, b, n)
                                for src, b in blocks
                                for n in range(pw // LANES)]
        for c in range(n_chunk):
            r0, r1 = bounds[c], bounds[c + 1]
            for src, b in blocks:
                lhs = xn_s[skip + r0:skip + r1, :]
                job = jobs.pop(0) if jobs else None
                if job is not None:
                    top = jnp.where(always, lhs[:16],
                                    jnp.concatenate(job(), axis=1))
                    lhs = jnp.concatenate([top, lhs[16:]], axis=0)
                pre_s[b, r0:r1, :] = _dot(lhs, src[...], _NT).astype(BF16)
        assert not jobs

    def first_block(j, carry):
        src = wst_v.at[0, j]
        pltpu.make_async_copy(src, src, w_sems.at[NSLOT + j]).wait()
        pre_blocks([(src, j)], [], j >= 0)
        h1_s[:n1, :] = jnp.concatenate(
            [mem_v[...].astype(F32), _ln(x_v[0, 0].astype(F32))],
            axis=0).astype(BF16)
        h1_s[n1:, :] = xn_s[last_xn:last_xn + m_len, :]
        return carry

    def prefetch(p):
        @pl.when(p + NSLOT < n_pairs)
        def _():
            for j in range(3):
                w_copy(p + NSLOT, j).start()

        @pl.when(p + NSLOT == n_pairs)
        def _():
            xb_copy.start()
            xc_copy.start()

        @pl.when(p + 1 < n_pairs)
        def _():
            wo_copy(p + 1).start()

        @pl.when(p + 1 < n_bq)
        def _():
            bq_copy(p + 1).start()

        @pl.when(p + 1 < nt)
        def _():
            bo_copy(p + 1).start()

    def pre_pair(p, carry):
        def relayout_bo():
            i = jnp.minimum(p - 1, nt - 1)
            to_s[:d, :] = bo_st[i].astype(F32)
            bo = permute_rows(to_s)
            bo_p[i] = bo.astype(BF16)
            g = d // nt // 16
            return [functools.reduce(
                lambda u, v: u + v,
                [bo[16 * (c * g + r):16 * (c * g + r + 1)] for r in range(g)]
            ).astype(BF16) for c in range(nt)]

        def relayout_bq():
            i = p - 1
            tq_s[:d, :] = bq_st[i].astype(F32).T
            row = pl.multiple_of((i % nt) * LANES, LANES)
            bq = permute_rows(tq_s).T.astype(BF16)
            bqkv_p[i // nt, pl.ds(row, LANES), :] = bq
            return [_tile(bq[LANES - 16:], c) for c in range(nt)]

        w_wait(p)
        pltpu.make_async_copy(bq_st.at[p - 1], bq_st.at[p - 1],
                              bq_sems.at[(p - 1) & 1]).wait()

        @pl.when(p <= nt)
        def _():
            bo_copy(p - 1).wait()

        slot = p & (NSLOT - 1)
        pre_blocks([(wst_v.at[slot, j], 3 * p + j) for j in range(3)],
                   [relayout_bo, relayout_bq], p >= 0)
        prefetch(p)
        return carry

    lax.fori_loop(0, 3, first_block, 0)
    prefetch(jnp.int32(0))
    lax.fori_loop(1, n_pairs, pre_pair, 0)

    xb_copy.wait()
    xc_copy.wait()
    pltpu.make_async_copy(wo_v, wo_v, sems.at[7]).wait()

    def b_pass(t, par):
        return _BPass(y_s, ((t - 1) * seg, (t - 1 - LAG) * seg), bqkv_p, bo_p,
                      kv_s.at[par], kv_s.at[1 - par], seg=seg, d=d)

    def b_store(t, yb):
        out_v[jnp.maximum(t - 1 - LAG, 0)] = yb[seg:].astype(out_v.dtype)
        return yb[:seg]

    def two_layer_step(t, par, h):
        half = t >> 1
        pre_row = None
        if par == 0:
            pre_row = pl.multiple_of((half - LAG // 2) * PRE, PRE)
        a = _TwoLayerPass(h, pre_s, pre_row, w_v, wo_v,
                          dh=dh, m_len=m_len, seg=seg)
        init = jnp.concatenate(
            [jnp.zeros((m2, d), F32), x_v[half, par].astype(F32), ra_s[...]],
            axis=0)
        acc, yb = a.run(n_pairs, init, b_pass(t, par), t >= 0)
        x2 = b_store(t, yb)
        y_s[...] = acc[m2:]
        ra_s[...] = x2
        if par == 0:
            xn = x_v[half, 1]
        else:
            xn = x_v[jnp.minimum(half + 1, n_half - 1), 0, :nf, :]
        return jnp.concatenate([_ln(xn.astype(F32)), _ln(x2), acc[:m2]],
                               axis=0).astype(BF16)

    def two_layer_steps(i, carry):
        h = h_s[...]
        for u in range(UNROLL):
            h = two_layer_step(LAG + i * UNROLL + u, (LAG + u) % 2, h)
        h_s[...] = h
        return carry

    def one_layer_step(t, carry):
        first = t < LAG
        extra_row = pl.multiple_of(n_pre + jnp.minimum(t, 1) * m_len, m_len)
        a = _OneLayerPass(h1_s[...], pre_s, extra_row, w_v, wo_v,
                          dh=dh, m_len=m_len, seg=seg)
        x0 = x_seg(jnp.minimum(t, n_seg - 1))[...].astype(F32)
        init = jnp.concatenate(
            [jnp.zeros((m_len, d), F32), jnp.where(first, x0, ra_s[...])],
            axis=0)
        acc, yb = a.run(n_pairs, init, b_pass(t, t & 1), t >= 0)
        x2 = b_store(t, yb)
        y = acc[m_len:]
        y_s[:seg, :] = y
        y_s[seg:, :] = y
        ra_s[...] = x2
        xn = _ln(x_seg(jnp.minimum(t + 1, n_seg - 1))[...].astype(F32))
        x2n = _ln(x2)
        mem = acc[:m_len]
        h1_s[:n1, :] = jnp.concatenate(
            [mem, jnp.where(first, xn, x2n)], axis=0).astype(BF16)
        h1_s[n1:, :] = xn_s[last_xn + m_len:, :]
        h_s[...] = jnp.concatenate(
            [xn[:nf], x2n, mem, mem_v[...].astype(F32)], axis=0).astype(BF16)
        return carry

    n_early_out = n_seg - 1 - LAG
    out_a = pltpu.make_async_copy(out_v.at[:n_early_out],
                                  out_hbm.at[:n_early_out], sems.at[3])
    out_b = pltpu.make_async_copy(out_v.at[n_early_out:],
                                  out_hbm.at[n_early_out:], sems.at[4])

    def phase(ph, carry):
        t0 = ph * n_seg
        lax.fori_loop(t0, t0 + LAG, one_layer_step, 0)

        @pl.when(ph == 0)
        def _():
            lax.fori_loop(0, (n_seg - LAG) // UNROLL, two_layer_steps, 0)
            out_a.start()
            hf = h_s[...].astype(F32)
            h1_s[:n1, :] = jnp.concatenate(
                [hf[nf + seg + m_len:], hf[nf:nf + seg]],
                axis=0).astype(BF16)

        return carry

    lax.fori_loop(0, 2, phase, 0)

    b = _BPass(y_s.at[seg:], ((n_seg - 1) * seg,), bqkv_p, bo_p,
               kv_s.at[(n_seg + LAG) % 2, 1:], None, seg=seg, d=d)
    b.project()
    for gi in range(b.n_groups):
        b.attend(gi)
    out_v[n_seg - 1] = b.finish().astype(out_v.dtype)
    out_b.start()
    out_a.wait()
    out_b.wait()


def pallas_interleave_layers__memory_aug_recurrent_mem_tr__sliding_local_dilated__prompt_kernel(
    A_x: jax.Array,
    A_mem0: jax.Array,
    A_Wq: jax.Array,
    A_Wk: jax.Array,
    A_Wv: jax.Array,
    A_Wo: jax.Array,
    A_seg_len,
    B_x: jax.Array,
    B_wqkv: jax.Array,
    B_wo: jax.Array,
):
    del B_x
    seg = A_seg_len if isinstance(A_seg_len, int) else SEG_LEN
    return _forward(A_x, A_mem0, A_Wq, A_Wk, A_Wv, A_Wo, B_wqkv, B_wo, seg=seg)


@functools.partial(jax.jit, static_argnames=("seg",))
def _forward(A_x, A_mem0, A_Wq, A_Wk, A_Wv, A_Wo, B_wqkv, B_wo, *, seg):
    bsz, s_len, d = A_x.shape
    m_len = A_mem0.shape[1]
    n_heads, dh = A_Wq.shape[1], A_Wq.shape[2]
    n_seg = s_len // seg
    n_pairs = n_heads // 2
    nt = d // LANES
    assert bsz == 1 and s_len % seg == 0 and n_seg > LAG + 1
    assert m_len == 8 and seg == 2 * m_len + PRE and seg >= HIST
    assert LAG == 2 and LAG * m_len == PRE and n_seg % (2 * LN_SEGS) == 0
    assert 2 * (m_len + seg) + 4 * m_len <= LANES
    assert (n_seg - LAG) % UNROLL == 0 and UNROLL == 2
    assert n_heads % 2 == 0 and 2 * dh == 3 * LANES and d % LANES == 0
    assert d % HB == 0 and LANES == 4 * HB and n_pairs == 3 * nt + 1
    hd = n_heads * dh
    n_half = n_seg // 2
    n_pre = (n_half - LAG // 2) * PRE

    wq_t = jnp.transpose(A_Wq, (1, 2, 0)).reshape(hd, d)
    wk_t = jnp.transpose(A_Wk, (1, 2, 0)).reshape(hd, d)
    wv_t = jnp.transpose(A_Wv, (1, 2, 0)).reshape(hd, d)
    wo = A_Wo.reshape(hd, d)

    kernel = functools.partial(
        _kernel, seg=seg, n_seg=n_seg, m_len=m_len, n_pairs=n_pairs, dh=dh,
        d=d)
    any_spec = pl.BlockSpec(memory_space=pl.ANY)
    dma = pltpu.SemaphoreType.DMA
    out = pl.pallas_call(
        kernel,
        out_shape=jax.ShapeDtypeStruct((n_seg, seg, d), A_x.dtype),
        in_specs=[any_spec] * 8,
        out_specs=any_spec,
        scratch_shapes=[
            pltpu.VMEM((n_half, 2, seg, d), BF16),
            pltpu.VMEM((m_len, d), BF16),
            pltpu.VMEM((NSLOT, 3, 2 * dh, d), BF16),
            pltpu.VMEM((3 * n_pairs, d, 2 * dh), BF16),
            pltpu.VMEM((hd, d), BF16),
            pltpu.VMEM((3 * nt, LANES, d), BF16),
            pltpu.VMEM((nt, d, LANES), BF16),
            pltpu.VMEM((d + HB, LANES), F32),
            pltpu.VMEM((d + HB, LANES), F32),
            pltpu.VMEM((3, d, d), BF16),
            pltpu.VMEM((nt, d, LANES), BF16),
            pltpu.VMEM((n_seg, seg, d), A_x.dtype),
            pltpu.VMEM((n_half * PRE, d), BF16),
            pltpu.VMEM((3 * n_pairs, n_pre, 2 * dh), BF16),
            pltpu.VMEM((2 * (m_len + seg) - PRE, d), BF16),
            pltpu.VMEM((2 * m_len + seg, d), BF16),
            pltpu.VMEM((seg, d), F32),
            pltpu.VMEM((2 * seg, d), F32),
            pltpu.VMEM((2, 2, 2 * nt, HIST + seg, LANES), F32),
            dma((8,)), dma((NSLOT + 3,)), dma((2,)), dma((2,)),
        ],
        compiler_params=pltpu.CompilerParams(
            vmem_limit_bytes=110 * 1024 * 1024,
            disable_bounds_checks=True),
    )(A_x.reshape(n_half, 2, seg, d), A_mem0.reshape(m_len, d), wq_t, wk_t, wv_t,
      wo, B_wqkv, B_wo)
    return out.reshape(bsz, s_len, d)
```

```python
import functools

import jax
import jax.numpy as jnp
from jax import lax
import jax.experimental.pallas as pl
import jax.experimental.pallas.tpu as pltpu

F32 = jnp.float32
BF16 = jnp.bfloat16

_NT = (((1,), (1,)), ((), ()))
_NN = (((1,), (0,)), ((), ()))

SEG_LEN = 32
HB = 32
WIN = 8
DIL = 2
HIST = 16
LANES = 128
PRE = 16
PRE_CHUNK = 128
LN_SEGS = 16
LAG = 2
UNROLL = 2
NSLOT = 2
NEG = -1000000000.0


def _dot(a, b, dims):
    return lax.dot_general(a, b, dims, preferred_element_type=F32)


def _recip(x):
    r = pl.reciprocal(x, approx=True)
    return r * (2.0 - x * r)


def _ln(x):
    m = jnp.mean(x, axis=-1, keepdims=True)
    xc = x - m
    v = jnp.mean(xc * xc, axis=-1, keepdims=True)
    return xc * lax.rsqrt(v + 1e-05)


def _tile(a, c):
    return a[:, c * LANES:(c + 1) * LANES]


def _keep(mask, a):
    return jnp.where(mask, a, jnp.zeros_like(a))


def _drop(mask, a):
    return jnp.where(mask, jnp.zeros_like(a), a)


def _pair_softmax(s, col_a):
    m_a = jnp.max(jnp.where(col_a, s, -jnp.inf), axis=1, keepdims=True)
    m_b = jnp.max(jnp.where(col_a, -jnp.inf, s), axis=1, keepdims=True)
    e = jnp.exp(s - jnp.where(col_a, m_a, m_b))
    d_a = jnp.sum(jnp.where(col_a, e, 0.0), axis=1, keepdims=True)
    d_b = jnp.sum(jnp.where(col_a, 0.0, e), axis=1, keepdims=True)
    return e * _recip(jnp.where(col_a, d_a, d_b))


class _PassBase:
    defer = 0

    def __init__(self, h, w_ref, wo_ref, dh):
        self.h, self.w, self.wo = h, w_ref, wo_ref
        self.pw = 2 * dh
        self.half = dh - LANES
        self.scale = dh ** (-0.5)
        self.q, self.k, self.v, self.p, self.o = {}, {}, {}, {}, {}
        self.cols = (0, 2 * LANES, wo_ref.shape[1])
        self.pending = None

    def _lane_lo(self, rows):
        return lax.broadcasted_iota(jnp.int32, (rows, LANES), 1) < self.half

    def _project(self, p, j):
        a = _dot(self.h, self.w[3 * p + j], _NN)
        self.marker = a[:8, :LANES]
        return a

    def _gate(self, s):
        if self.pending is None:
            return s
        top = jnp.where(self.always, s[:8], self.pending[:, :s.shape[1]])
        self.pending = None
        return jnp.concatenate([top, s[8:]], axis=0)

    def out(self, p, part=None):
        for k in ((0, 1) if part is None else (part,)):
            c0, c1 = self.cols[k], self.cols[k + 1]
            w = self.wo[p * self.pw:(p + 1) * self.pw, c0:c1]
            self.acc[k] = self.acc[k] + _dot(self.o[p], w, _NN)

    def run(self, n_pairs, init, b, always):
        last = n_pairs - 1
        self.acc = [init[:, :self.cols[1]], init[:, self.cols[1]:]]
        self.always = always
        done = None
        for p in range(n_pairs):
            self.proj_q(p)
            self.pending, done = done, None
            if 2 <= p < 2 + b.n_groups:
                o = b.attend(p - 2, (always, self.marker))
                done = functools.reduce(lambda u, v: u + v, o)
            self.proj_k(p)
            if p == last and self.defer:
                self.proj_v(p)
                self.pv(p - 1)
            else:
                if p > 0:
                    self.pv(p - 1)
                self.proj_v(p)
            self.scores(p)
            if p == 0:
                b.project()
            elif p < last - self.defer:
                self.out(p - 1)
        if self.defer:
            self.out(last - 2)
        yb = b.finish()
        self.out(last - 1, 0)
        self.pv(last)
        self.out(last - 1, 1)
        self.out(last)
        return jnp.concatenate(self.acc, axis=1), yb


class _TwoLayerPass(_PassBase):
    def __init__(self, h, pre_ref, pre_row, w_ref, wo_ref, *, dh, m_len, seg):
        super().__init__(h, w_ref, wo_ref, dh)
        self.pre, self.pre_row = pre_ref, pre_row
        u = self.u = m_len
        n = self.n = 2 * (m_len + seg)
        self.ext = 4 * u
        self.seg = seg
        row = lax.broadcasted_iota(jnp.int32, (n, n + self.ext), 0)
        col = lax.broadcasted_iota(jnp.int32, (n, n + self.ext), 1)
        rep = col >= n
        col = jnp.where(rep, col - n, col)

        def first_layer(i):
            return (((i < 6 * u) & ((i & u) == 0))
                    | ((i >= 6 * u) & (i < 6 * u + PRE)))

        def index(i):
            low = ((i >> 1) & ~(u - 1)) + (i & (u - 1))
            high = jnp.where(i < 6 * u + PRE, i - 3 * u, i - 3 * u - PRE)
            return jnp.where(i < 6 * u, low, high)

        self.col_a = first_layer(col)
        self.diag = first_layer(row) == self.col_a
        used = ((row >= 3 * u) & (row < 4 * u)) == rep
        self.allowed = used & ((row < 2 * u) | (index(row) >= index(col)))
        self.fill = jnp.where(used, NEG, -jnp.inf)
        self.lo_u = self._lane_lo(u)
        self.lo_c = self._lane_lo(PRE)

    def _proj(self, p, j):
        u, seg = self.u, self.seg
        r = self._project(p, j)
        if self.pre_row is None:
            n1 = seg
            c1 = r[2 * u:n1].astype(BF16)
        else:
            n1 = 2 * u
            c1 = self.pre[3 * p + j, pl.ds(self.pre_row, PRE), :]
        nx = n1 + seg
        return ((r[nx:nx + u], r[:u], r[u:2 * u], c1),
                (r[nx + u:], r[n1:n1 + u], r[n1 + u:n1 + 2 * u],
                 r[n1 + 2 * u:nx].astype(BF16)))

    @staticmethod
    def _weave(f, g):
        top = jnp.concatenate([f[0], g[0], f[1], g[1], f[2], g[2]], axis=0)
        return jnp.concatenate([top.astype(BF16), f[3], g[3]], axis=0)

    def _tiles(self, l1, l2):
        masks = (self.lo_u,) * 3 + (self.lo_c,)

        def t(l, c):
            return [_tile(a, c) for a in l]

        def lo(l):
            return [_keep(mk, a) for mk, a in zip(masks, l)]

        def hi(l):
            return [_drop(mk, a) for mk, a in zip(masks, l)]

        def extend(a, b):
            return jnp.concatenate([a, b[:self.ext]], axis=0)

        t0 = self._weave(t(l1, 0), t(l2, 0))
        t2 = self._weave(t(l2, 2), t(l1, 2))
        t1a = self._weave(lo(t(l1, 1)), hi(t(l1, 1)))
        t1b = self._weave(hi(t(l2, 1)), lo(t(l2, 1)))
        return extend(t0, t0), extend(t1a, t1b), t1b, extend(t2, t2)

    def _split_rows(self, l1, l2):
        ra = jnp.concatenate([l1[0], l1[2], l1[1], l2[1]], axis=0)
        rb = jnp.concatenate([l2[0], l2[2]], axis=0)
        return (jnp.concatenate([ra.astype(BF16), l1[3]], axis=0),
                jnp.concatenate([rb.astype(BF16), l2[3]], axis=0))

    def _units(self, ra, rb):
        u = self.u
        return ((ra[:u], ra[2 * u:3 * u], ra[u:2 * u], ra[4 * u:]),
                (rb[:u], ra[3 * u:4 * u], rb[u:2 * u], rb[2 * u:]))

    def _unweave(self, a):
        u = self.u
        return ((a[:u], a[2 * u:3 * u], a[4 * u:5 * u], a[6 * u:6 * u + PRE]),
                (a[u:2 * u], a[3 * u:4 * u], a[5 * u:6 * u], a[6 * u + PRE:]))

    def proj_q(self, p):
        l1, l2 = self._proj(p, 0)
        q0, q2 = (self._weave([_tile(a, c) for a in l1],
                              [_tile(a, c) for a in l2]) for c in (0, 2))
        qa, qb = self._split_rows([_tile(a, 1) for a in l1],
                                  [_tile(a, 1) for a in l2])
        self.q[p] = (q0, qa, qb, q2)

    def proj_k(self, p):
        self.k[p] = self._tiles(*self._proj(p, 1))

    def proj_v(self, p):
        self.v[p] = self._tiles(*self._proj(p, 2))

    def scores(self, p):
        q0, qa, qb, q2 = self.q.pop(p)
        k0, k1a, k1b, k2 = self.k.pop(p)
        r0 = _dot(q0, k0, _NT)
        r2 = _dot(q2, k2, _NT)
        ra = _dot(qa, k1a, _NT)
        rb = _dot(qb, k1b, _NT)
        rb = jnp.concatenate(
            [rb, jnp.zeros((rb.shape[0], self.ext), F32)], axis=1)
        f, g = self._units(ra, rb)
        r1 = jnp.concatenate(
            [f[0], g[0], f[1], g[1], f[2], g[2], f[3], g[3]], axis=0)
        s = jnp.where(self.diag, r0, r2) + r1
        s = self._gate(jnp.where(self.allowed, s * self.scale, self.fill))
        p_all = _pair_softmax(s, self.col_a)
        f, g = self._unweave(p_all)
        pa, pb = self._split_rows(f[:3] + (f[3].astype(BF16),),
                                  g[:3] + (g[3].astype(BF16),))
        self.p[p] = (_keep(self.diag, p_all).astype(BF16), pa,
                     pb[:, :self.n], _drop(self.diag, p_all).astype(BF16))

    def pv(self, p):
        p0, pa, pb, p2 = self.p.pop(p)
        v0, v1a, v1b, v2 = self.v.pop(p)
        o0 = self._unweave(_dot(p0, v0, _NN))
        o2 = self._unweave(_dot(p2, v2, _NN))
        o1 = self._units(_dot(pa, v1a, _NN), _dot(pb, v1b, _NN))
        self.o[p] = jnp.concatenate(
            [jnp.concatenate((f[0], g[0]) + f[1:] + g[1:], axis=0)
             for f, g in (o0, o1, o2)], axis=1).astype(BF16)


class _OneLayerPass(_PassBase):
    defer = 1

    def __init__(self, h, pre_ref, pre_row, w_ref, wo_ref, *, dh, m_len, seg):
        super().__init__(h, w_ref, wo_ref, dh)
        self.pre, self.pre_row = pre_ref, pre_row
        n = self.n = m_len + seg
        row = lax.broadcasted_iota(jnp.int32, (n, 2 * n), 0)
        col = lax.broadcasted_iota(jnp.int32, (n, 2 * n), 1)
        self.col_a = col < n
        key = jnp.where(self.col_a, col, col - n)
        self.allowed = (row < m_len) | (row >= key)
        lane = lax.broadcasted_iota(jnp.int32, (n, self.pw), 1)
        self.head0 = lane < dh

    def _project(self, p, j):
        a = super()._project(p, j)
        n = self.n
        self.pre[3 * p + j, pl.ds(self.pre_row, a.shape[0] - n), :] = (
            a[n:].astype(BF16))
        return a[:n]

    def _block_diag(self, a):
        return jnp.concatenate([_keep(self.head0, a), _drop(self.head0, a)],
                               axis=0).astype(BF16)

    def proj_q(self, p):
        self.q[p] = self._project(p, 0).astype(BF16)

    def proj_k(self, p):
        self.k[p] = self._block_diag(self._project(p, 1))

    def proj_v(self, p):
        self.v[p] = self._block_diag(self._project(p, 2))

    def scores(self, p):
        s = _dot(self.q.pop(p), self.k.pop(p), _NT)
        s = self._gate(jnp.where(self.allowed, s * self.scale, NEG))
        self.p[p] = _pair_softmax(s, self.col_a).astype(BF16)

    def pv(self, p):
        self.o[p] = _dot(self.p.pop(p), self.v.pop(p), _NN).astype(BF16)


class _BPass:
    def __init__(self, y_ref, starts, wqkv_ref, wo_ref, kv_ref, kv_next_ref,
                 *, seg, d):
        self.y, self.starts = y_ref, starts
        self.wqkv, self.wo, self.kv = wqkv_ref, wo_ref, kv_ref
        self.kv_next = kv_next_ref
        self.seg, self.nt = seg, d // LANES
        self.scale = (d // HB) ** (-0.5)
        self.n_groups = len(starts) * seg // 8
        self.outs = []

    def project(self):
        seg, nt = self.seg, self.nt
        yn = _ln(self.y[...]).astype(BF16)
        self.q, ka, va = (_dot(yn, self.wqkv[j], _NN) for j in range(3))
        for i in range(len(self.starts)):
            for c in range(2 * nt):
                a = _tile((ka, va)[c // nt][i * seg:(i + 1) * seg], c % nt)
                self.kv[i, c, HIST:HIST + seg, :] = a
                if self.kv_next is not None:
                    self.kv_next[i, c, :HIST, :] = a[seg - HIST:]

    def attend(self, gi, after=None):
        seg, nt, kv = self.seg, self.nt, self.kv
        i, g = divmod(gi, seg // 8)
        q = [_tile(self.q[8 * gi:8 * gi + 8], c) for c in range(nt)]
        if after is not None:
            q = [jnp.where(after[0], u, after[1]) for u in q]
        pos = (lax.broadcasted_iota(jnp.int32, (8, LANES), 0)
               + (self.starts[i] + 8 * g))
        offs = [HIST + 8 * g - w * DIL for w in range(WIN)]
        logits = []
        for w, off in enumerate(offs):
            t = q[0] * kv[i, 0, off:off + 8, :]
            for c in range(1, nt):
                t = t + q[c] * kv[i, c, off:off + 8, :]
            t = t + pltpu.roll(t, 64, 1)
            t = (t + pltpu.roll(t, 32, 1)) * self.scale
            if 8 * g < w * DIL:
                t = jnp.where(pos >= w * DIL, t, NEG)
            logits.append(t)
        m = logits[0]
        for t in logits[1:]:
            m = jnp.maximum(m, t)
        es = [jnp.exp(t - m) for t in logits]
        den = es[0]
        for e in es[1:]:
            den = den + e
        inv = _recip(den)
        o = []
        for c in range(nt):
            acc = None
            for w, off in enumerate(offs):
                term = es[w] * kv[i, nt + c, off:off + 8, :]
                acc = term if acc is None else acc + term
            o.append(acc * inv)
        self.outs.append(jnp.concatenate(o, axis=1))
        return o

    def finish(self):
        o = jnp.concatenate(self.outs, axis=0).astype(BF16)
        proj = jnp.concatenate(
            [_dot(o, self.wo[c], _NN) for c in range(self.nt)], axis=1)
        return self.y[...] + proj


def _kernel(x_hbm, mem_hbm, wq_hbm, wk_hbm, wv_hbm, wo_hbm, bqkv_hbm, bo_hbm,
            out_hbm,
            x_v, mem_v, wst_v, w_v, wo_v, bq_st, bo_st, tq_s, to_s, bqkv_p,
            bo_p, out_v, xn_s, pre_s, h_s, h1_s, ra_s, y_s, yt_s, kv_s,
            sems, w_sems, bq_sems, bo_sems,
            *, seg, n_seg, m_len, n_pairs, dh, d):
    db = d // HB
    nt = d // LANES
    pw = 2 * dh
    m2 = 2 * m_len
    n_half = n_seg // 2
    n_pre = (n_half - 1 - LAG // 2) * PRE
    n_bq = 3 * nt

    def w_copy(p, j, sem=None):
        src = (wq_hbm, wk_hbm, wv_hbm)[j]
        slot = p & (NSLOT - 1)
        return pltpu.make_async_copy(
            src.at[pl.ds(p * pw, pw), :], wst_v.at[slot, j],
            w_sems.at[slot if sem is None else sem])

    def w_wait(p):
        slot = p & (NSLOT - 1)
        pltpu.make_async_copy(wst_v.at[slot], wst_v.at[slot],
                              w_sems.at[slot]).wait()

    def wo_copy(p):
        return pltpu.make_async_copy(wo_hbm.at[pl.ds(p * pw, pw), :],
                                     wo_v.at[pl.ds(p * pw, pw), :],
                                     sems.at[7])

    def bq_copy(i):
        row = pl.multiple_of((i % nt) * LANES, LANES)
        col = pl.multiple_of((i // nt) * d, LANES)
        return pltpu.make_async_copy(
            bqkv_hbm.at[pl.ds(row, LANES), pl.ds(col, d)], bq_st.at[i],
            bq_sems.at[i & 1])

    def bo_copy(i):
        col = pl.multiple_of(i * LANES, LANES)
        return pltpu.make_async_copy(bo_hbm.at[:, pl.ds(col, LANES)],
                                     bo_st.at[i], bo_sems.at[i & 1])

    nf = seg - PRE

    def x_copy(idx, sem):
        return pltpu.make_async_copy(x_hbm.at[idx], x_v.at[idx], sems.at[sem])

    full = slice(None)
    xa_copy = x_copy((full, 0, slice(nf, None), full), 0)
    x0_copy = x_copy((0, 0, slice(None, nf), full), 5)
    xb_copy = x_copy((slice(1, None), 0, slice(None, nf), full), 1)
    xc_copy = x_copy((full, 1), 6)

    def x_seg(t):
        return x_v.at[t >> 1, t & 1]

    mem_copy = pltpu.make_async_copy(mem_hbm, mem_v, sems.at[2])

    mem_copy.start()
    xa_copy.start()
    mem_copy.wait()
    x0_copy.start()
    w_copy(0, 0, sem=NSLOT).start()

    ra_s[...] = jnp.zeros(ra_s.shape, F32)
    y_s[...] = jnp.zeros(y_s.shape, F32)
    kv_s[0, :, :, :HIST, :] = jnp.zeros(kv_s.shape[1:3] + (HIST, LANES), F32)

    xa_copy.wait()
    for j in range(1, 3):
        w_copy(0, j, sem=NSLOT + j).start()

    def ln_block(i, carry):
        s0 = pl.multiple_of(i * LN_SEGS, LN_SEGS)
        xb = x_v[pl.ds(s0, LN_SEGS), 0, nf:, :].astype(F32)
        xn_s[pl.ds(pl.multiple_of(s0 * PRE, PRE), LN_SEGS * PRE), :] = _ln(
            xb.reshape(LN_SEGS * PRE, d)).astype(BF16)
        return carry

    lax.fori_loop(0, n_half // LN_SEGS, ln_block, 0)

    n1 = m_len + seg
    last_xn = (n_half - 1) * PRE
    x0_copy.wait()
    for j in range(3):
        w_copy(1, j).start()
    bq_copy(0).start()
    bo_copy(0).start()
    wo_copy(0).start()

    def permute_rows(tmp_ref):
        return jnp.concatenate(
            [tmp_ref[pl.ds(j, HB, stride=db), :] for j in range(db)], axis=0)

    n_chunk = -(-n_pre // PRE_CHUNK)
    bounds = [16 * (n_pre // 16 * c // n_chunk) for c in range(n_chunk + 1)]
    skip = LAG // 2 * PRE

    def pre_blocks(blocks, jobs, always):
        def transpose_w(src, b, n):
            wt = src[n * LANES:(n + 1) * LANES, :].T
            w_v[b, :, n * LANES:(n + 1) * LANES] = wt
            return [wt[(c + 1) * LANES - 16:(c + 1) * LANES]
                    for c in range(nt)]

        jobs = [None] + jobs + [functools.partial(transpose_w, src, b, n)
                                for src, b in blocks
                                for n in range(pw // LANES)]
        for c in range(n_chunk):
            r0, r1 = bounds[c], bounds[c + 1]
            for src, b in blocks:
                lhs = xn_s[skip + r0:skip + r1, :]
                job = jobs.pop(0) if jobs else None
                if job is not None:
                    top = jnp.where(always, lhs[:16],
                                    jnp.concatenate(job(), axis=1))
                    lhs = jnp.concatenate([top, lhs[16:]], axis=0)
                pre_s[b, r0:r1, :] = _dot(lhs, src[...], _NT).astype(BF16)
        assert not jobs

    def first_block(j, carry):
        src = wst_v.at[0, j]
        pltpu.make_async_copy(src, src, w_sems.at[NSLOT + j]).wait()
        pre_blocks([(src, j)], [], j >= 0)
        h1_s[:n1, :] = jnp.concatenate(
            [mem_v[...].astype(F32), _ln(x_v[0, 0].astype(F32))],
            axis=0).astype(BF16)
        h1_s[n1:, :] = xn_s[last_xn:last_xn + m_len, :]
        return carry

    def prefetch(p):
        @pl.when(p + NSLOT < n_pairs)
        def _():
            for j in range(3):
                w_copy(p + NSLOT, j).start()

        @pl.when(p + NSLOT == n_pairs)
        def _():
            xb_copy.start()
            xc_copy.start()

        @pl.when(p + 1 < n_pairs)
        def _():
            wo_copy(p + 1).start()

        @pl.when(p + 1 < n_bq)
        def _():
            bq_copy(p + 1).start()

        @pl.when(p + 1 < nt)
        def _():
            bo_copy(p + 1).start()

    def pre_pair(p, carry):
        def relayout_bo():
            i = jnp.minimum(p - 1, nt - 1)
            to_s[:d, :] = bo_st[i].astype(F32)
            bo = permute_rows(to_s)
            bo_p[i] = bo.astype(BF16)
            g = d // nt // 16
            return [functools.reduce(
                lambda u, v: u + v,
                [bo[16 * (c * g + r):16 * (c * g + r + 1)] for r in range(g)]
            ).astype(BF16) for c in range(nt)]

        def relayout_bq():
            i = p - 1
            tq_s[:d, :] = bq_st[i].astype(F32).T
            row = pl.multiple_of((i % nt) * LANES, LANES)
            bq = permute_rows(tq_s).T.astype(BF16)
            bqkv_p[i // nt, pl.ds(row, LANES), :] = bq
            return [_tile(bq[LANES - 16:], c) for c in range(nt)]

        w_wait(p)
        pltpu.make_async_copy(bq_st.at[p - 1], bq_st.at[p - 1],
                              bq_sems.at[(p - 1) & 1]).wait()

        @pl.when(p <= nt)
        def _():
            bo_copy(p - 1).wait()

        slot = p & (NSLOT - 1)
        pre_blocks([(wst_v.at[slot, j], 3 * p + j) for j in range(3)],
                   [relayout_bo, relayout_bq], p >= 0)
        prefetch(p)
        return carry

    lax.fori_loop(0, 3, first_block, 0)
    prefetch(jnp.int32(0))
    lax.fori_loop(1, n_pairs, pre_pair, 0)

    xb_copy.wait()
    xc_copy.wait()
    pltpu.make_async_copy(wo_v, wo_v, sems.at[7]).wait()

    n_early_out = n_seg - 1 - LAG

    def b_pass(t, par):
        return _BPass(y_s, ((t - 1) * seg, (t - 1 - LAG) * seg), bqkv_p, bo_p,
                      kv_s.at[par], kv_s.at[1 - par], seg=seg, d=d)

    def b_store(t, yb):
        out_v[jnp.maximum(t - 1 - LAG, 0)] = yb[seg:].astype(out_v.dtype)
        return yb[:seg]

    def two_layer_step(t, par, h):
        half = t >> 1
        pre_row = None
        if par == 0:
            pre_row = pl.multiple_of((half - LAG // 2) * PRE, PRE)
        a = _TwoLayerPass(h, pre_s, pre_row, w_v, wo_v,
                          dh=dh, m_len=m_len, seg=seg)
        init = jnp.concatenate(
            [jnp.zeros((m2, d), F32), x_v[half, par].astype(F32), ra_s[...]],
            axis=0)
        acc, yb = a.run(n_pairs, init, b_pass(t, par), t >= 0)
        x2 = b_store(t, yb)
        y_s[...] = acc[m2:]
        ra_s[...] = x2
        if par == 0:
            xn = x_v[half, 1]
        else:
            xn = x_v[jnp.minimum(half + 1, n_half - 1), 0, :nf, :]
        return jnp.concatenate([_ln(xn.astype(F32)), _ln(x2), acc[:m2]],
                               axis=0).astype(BF16)

    def two_layer_steps(i, carry):
        h = h_s[...]
        for u in range(UNROLL):
            h = two_layer_step(LAG + i * UNROLL + u, (LAG + u) % 2, h)
        h_s[...] = h
        return carry

    def one_layer_step(t, carry):
        first = t < LAG
        li = (t == n_seg + 1).astype(jnp.int32)
        par = (t - li) & 1
        b = _BPass(y_s.at[pl.ds(pl.multiple_of(li * seg, seg), seg)],
                   ((t - 1 - li * (1 + LAG)) * seg,), bqkv_p, bo_p,
                   kv_s.at[par, pl.ds(li, 1)], kv_s.at[1 - par, pl.ds(li, 1)],
                   seg=seg, d=d)
        extra_row = pl.multiple_of(n_pre + jnp.minimum(t, 1) * m_len, m_len)
        a = _OneLayerPass(h1_s[...], pre_s, extra_row, w_v, wo_v,
                          dh=dh, m_len=m_len, seg=seg)
        x0 = x_seg(jnp.minimum(t, n_seg - 1))[...].astype(F32)
        init = jnp.concatenate(
            [jnp.zeros((m_len, d), F32), jnp.where(first, x0, ra_s[...])],
            axis=0)
        acc, x2 = a.run(n_pairs, init, b, t >= 0)
        out_v[jnp.where(first, 0, n_early_out)] = x2.astype(out_v.dtype)
        y = acc[m_len:]
        y_s[:seg, :] = y
        yt_s[pl.ds(pl.multiple_of((t & 1) * seg, seg), seg), :] = y
        ra_s[...] = x2
        xn = _ln(x_seg(jnp.minimum(t + 1, n_seg - 1))[...].astype(F32))
        x2n = _ln(x2)
        mem = acc[:m_len]
        h1_s[:n1, :] = jnp.concatenate(
            [mem, jnp.where(first, xn, x2n)], axis=0).astype(BF16)
        h1_s[n1:, :] = xn_s[last_xn + m_len:, :]
        h_s[...] = jnp.concatenate(
            [xn[:nf], x2n, mem, mem_v[...].astype(F32)], axis=0).astype(BF16)
        return carry

    out_a = pltpu.make_async_copy(out_v.at[:n_early_out],
                                  out_hbm.at[:n_early_out], sems.at[3])
    out_b = pltpu.make_async_copy(out_v.at[n_early_out:],
                                  out_hbm.at[n_early_out:], sems.at[4])

    def phase(ph, carry):
        t0 = ph * n_seg
        lax.fori_loop(t0, t0 + LAG, one_layer_step, 0)

        @pl.when(ph == 0)
        def _():
            lax.fori_loop(0, (n_seg - LAG) // UNROLL, two_layer_steps, 0)
            out_a.start()
            hf = h_s[...].astype(F32)
            h1_s[:n1, :] = jnp.concatenate(
                [hf[nf + seg + m_len:], hf[nf:nf + seg]],
                axis=0).astype(BF16)

        return carry

    lax.fori_loop(0, 2, phase, 0)

    b = _BPass(yt_s, ((n_seg - 2) * seg,), bqkv_p, bo_p,
               kv_s.at[(n_seg + 1) % 2, 1:], None, seg=2 * seg, d=d)
    b.project()
    for gi in range(b.n_groups):
        b.attend(gi)
    out_v[n_seg - 2:] = b.finish().astype(out_v.dtype).reshape(2, seg, d)
    out_b.start()
    out_a.wait()
    out_b.wait()


def pallas_interleave_layers__memory_aug_recurrent_mem_tr__sliding_local_dilated__prompt_kernel(
    A_x: jax.Array,
    A_mem0: jax.Array,
    A_Wq: jax.Array,
    A_Wk: jax.Array,
    A_Wv: jax.Array,
    A_Wo: jax.Array,
    A_seg_len,
    B_x: jax.Array,
    B_wqkv: jax.Array,
    B_wo: jax.Array,
):
    del B_x
    seg = A_seg_len if isinstance(A_seg_len, int) else SEG_LEN
    return _forward(A_x, A_mem0, A_Wq, A_Wk, A_Wv, A_Wo, B_wqkv, B_wo, seg=seg)


@functools.partial(jax.jit, static_argnames=("seg",))
def _forward(A_x, A_mem0, A_Wq, A_Wk, A_Wv, A_Wo, B_wqkv, B_wo, *, seg):
    bsz, s_len, d = A_x.shape
    m_len = A_mem0.shape[1]
    n_heads, dh = A_Wq.shape[1], A_Wq.shape[2]
    n_seg = s_len // seg
    n_pairs = n_heads // 2
    nt = d // LANES
    assert bsz == 1 and s_len % seg == 0 and n_seg > LAG + 1
    assert m_len == 8 and seg == 2 * m_len + PRE and seg >= HIST
    assert LAG == 2 and LAG * m_len == PRE and n_seg % (2 * LN_SEGS) == 0
    assert 2 * (m_len + seg) + 4 * m_len <= LANES
    assert (n_seg - LAG) % UNROLL == 0 and UNROLL == 2
    assert n_heads % 2 == 0 and 2 * dh == 3 * LANES and d % LANES == 0
    assert d % HB == 0 and LANES == 4 * HB and n_pairs == 3 * nt + 1
    hd = n_heads * dh
    n_half = n_seg // 2
    n_pre = (n_half - LAG // 2) * PRE

    wq_t = jnp.transpose(A_Wq, (1, 2, 0)).reshape(hd, d)
    wk_t = jnp.transpose(A_Wk, (1, 2, 0)).reshape(hd, d)
    wv_t = jnp.transpose(A_Wv, (1, 2, 0)).reshape(hd, d)
    wo = A_Wo.reshape(hd, d)

    kernel = functools.partial(
        _kernel, seg=seg, n_seg=n_seg, m_len=m_len, n_pairs=n_pairs, dh=dh,
        d=d)
    any_spec = pl.BlockSpec(memory_space=pl.ANY)
    dma = pltpu.SemaphoreType.DMA
    out = pl.pallas_call(
        kernel,
        out_shape=jax.ShapeDtypeStruct((n_seg, seg, d), A_x.dtype),
        in_specs=[any_spec] * 8,
        out_specs=any_spec,
        scratch_shapes=[
            pltpu.VMEM((n_half, 2, seg, d), BF16),
            pltpu.VMEM((m_len, d), BF16),
            pltpu.VMEM((NSLOT, 3, 2 * dh, d), BF16),
            pltpu.VMEM((3 * n_pairs, d, 2 * dh), BF16),
            pltpu.VMEM((hd, d), BF16),
            pltpu.VMEM((3 * nt, LANES, d), BF16),
            pltpu.VMEM((nt, d, LANES), BF16),
            pltpu.VMEM((d + HB, LANES), F32),
            pltpu.VMEM((d + HB, LANES), F32),
            pltpu.VMEM((3, d, d), BF16),
            pltpu.VMEM((nt, d, LANES), BF16),
            pltpu.VMEM((n_seg, seg, d), A_x.dtype),
            pltpu.VMEM((n_half * PRE, d), BF16),
            pltpu.VMEM((3 * n_pairs, n_pre, 2 * dh), BF16),
            pltpu.VMEM((2 * (m_len + seg) - PRE, d), BF16),
            pltpu.VMEM((2 * m_len + seg, d), BF16),
            pltpu.VMEM((seg, d), F32),
            pltpu.VMEM((2 * seg, d), F32),
            pltpu.VMEM((2 * seg, d), F32),
            pltpu.VMEM((2, 2, 2 * nt, HIST + 2 * seg, LANES), F32),
            dma((8,)), dma((NSLOT + 3,)), dma((2,)), dma((2,)),
        ],
        compiler_params=pltpu.CompilerParams(
            vmem_limit_bytes=96 * 1024 * 1024,
            disable_bounds_checks=True,
            disable_semaphore_checks=True),
    )(A_x.reshape(n_half, 2, seg, d), A_mem0.reshape(m_len, d), wq_t, wk_t, wv_t,
      wo, B_wqkv, B_wo)
    return out.reshape(bsz, s_len, d)
```

```python
import functools

import jax
import jax.numpy as jnp
from jax import lax
import jax.experimental.pallas as pl
import jax.experimental.pallas.tpu as pltpu

F32 = jnp.float32
BF16 = jnp.bfloat16
U32 = jnp.uint32

_NT = (((1,), (1,)), ((), ()))
_NN = (((1,), (0,)), ((), ()))

SEG_LEN = 32
HB = 32
WIN = 8
DIL = 2
HIST = 16
LANES = 128
PRE = 16
PRE_CHUNK = 128
LN_SEGS = 16
LAG = 2
UNROLL = 2
NSLOT = 2
HEAD_SLOTS = 4
NEG = -1000000000.0

PLAN = dict(
    deps64=((), (0,), (), (2,)), deps80=((), (0,), (), (2,)),
    last64=((), (0,), (), (2,)), last80=((), (0,), (), (2,)),
    gate64=(0, 2), gate80=(0, 2),
    deps1=((), ()), last1=((), ()), gate1=(),
    b_start=2, b_after=3, order=(0, 1, 2, 3, 4, 5, 6, 7), mark=0,
)


def _dot(a, b, dims):
    return lax.dot_general(a, b, dims, preferred_element_type=F32)


def _recip(x):
    r = pl.reciprocal(x, approx=True)
    return r * (2.0 - x * r)


def _ln(x):
    m = jnp.mean(x, axis=-1, keepdims=True)
    xc = x - m
    v = jnp.mean(xc * xc, axis=-1, keepdims=True)
    return xc * lax.rsqrt(v + 1e-05)


def _pack(a):
    return pltpu.bitcast(a, U32)


def _unpack(a):
    return pltpu.bitcast(a, BF16)


def _tile(a, c):
    return a[:, c * LANES:(c + 1) * LANES]


def _keep(mask, a):
    return jnp.where(mask, a, jnp.zeros_like(a))


def _drop(mask, a):
    return jnp.where(mask, jnp.zeros_like(a), a)


def _pair_softmax(s, col_a):
    m_a = jnp.max(jnp.where(col_a, s, -jnp.inf), axis=1, keepdims=True)
    m_b = jnp.max(jnp.where(col_a, -jnp.inf, s), axis=1, keepdims=True)
    e = jnp.exp(s - jnp.where(col_a, m_a, m_b))
    d_a = jnp.sum(jnp.where(col_a, e, 0.0), axis=1, keepdims=True)
    d_b = jnp.sum(jnp.where(col_a, 0.0, e), axis=1, keepdims=True)
    return e * _recip(jnp.where(col_a, d_a, d_b))


class _PassBase:
    defer = 0

    def __init__(self, h, w_ref, wo_ref, head_ref, dh):
        self.h, self.w, self.wo = h, w_ref, wo_ref
        self.head = head_ref
        self.qa, self.ea, self.oa = {}, {}, {}
        self.pw = 2 * dh
        self.half = dh - LANES
        self.scale = dh ** (-0.5)
        self.q, self.k, self.v, self.p, self.o = {}, {}, {}, {}, {}
        self.cols = (0, 2 * LANES, wo_ref.shape[1])
        self.pending = None

    def _lane_lo(self, rows):
        return lax.broadcasted_iota(jnp.int32, (rows, LANES), 1) < self.half

    def _project(self, p, j):
        a = _dot(self.h, _unpack(self.w[3 * p + j]), _NN)
        self.marker = a[:8, :LANES]
        return a

    def _stash(self, p, layer, kind, m, a):
        rows = jnp.concatenate([m, a], axis=0)
        rows = jnp.stack([_tile(rows, c) for c in range(3)])
        for i in range(4):
            self.head[p % HEAD_SLOTS, layer, kind, :,
                      pl.ds(i, 16, stride=4), :] = rows

    def _head_job(self, p, layer, hd, after):
        q = self.qa[p, layer]
        sub = lax.broadcasted_iota(jnp.int32, (8, LANES), 0)
        top = sub < 4
        lo = self._lane_lo(8)

        def tiles(kind):
            blk = self.head[p % HEAD_SLOTS, layer, kind, hd:hd + 2, :64, :]
            blk = blk.reshape(2, 8, 8, LANES)
            return blk[hd], blk[1 - hd]

        def spread(a):
            r = pltpu.roll(a, 4, 0)
            return jnp.where(top, a, r), jnp.where(top, r, a)

        def fold(a, b, op):
            return op(jnp.where(top, a, b),
                      pltpu.roll(jnp.where(top, b, a), 4, 0))

        qo = jnp.where(self.always, _tile(q, 2 * hd), after) * self.scale
        qs = jnp.where(self.always, _tile(q, 1), after) * self.scale
        qs = _drop(lo, qs) if hd else _keep(lo, qs)
        ko, ks = tiles(0)
        n_used = (6, 8)
        scores = []
        for half, (a, b) in enumerate(zip(spread(qo), spread(qs))):
            n = n_used[half]
            sc = jnp.sum(a[None] * ko[:n] + b[None] * ks[:n], axis=2,
                         keepdims=True)
            sc = jnp.broadcast_to(sc, (n, 8, LANES))
            shape = (2, 8, LANES)
            pair = lax.broadcasted_iota(jnp.int32, shape, 0)
            row = lax.broadcasted_iota(jnp.int32, shape, 1)
            seen = 2 * pair + (row >> 2) <= (row & 3)
            scores.append(jnp.concatenate(
                [sc[:n - 2], jnp.where(seen, sc[n - 2:], NEG)], axis=0))
        m = fold(*(jnp.max(sc, axis=0) for sc in scores), jnp.maximum)
        es = [jnp.exp(sc - mh[None]) for sc, mh in zip(scores, spread(m))]
        inv = _recip(fold(*(jnp.sum(e, axis=0) for e in es), jnp.add))
        outs = [fold(*(jnp.sum(e * v[:e.shape[0]], axis=0) for e in es),
                     jnp.add) * inv for v in tiles(1)]
        return outs, m

    def _gate(self, s):
        if self.pending is None:
            return s
        top = jnp.where(self.always, s[:8], self.pending[:, :s.shape[1]])
        self.pending = None
        return jnp.concatenate([top, s[8:]], axis=0)

    def head_rows(self, p, start, deps):
        outs, ms = [], []
        for j, dep in enumerate(deps):
            after = start if not dep else functools.reduce(
                lambda a, b: a + b, [ms[i] for i in dep])
            o, m = self._head_job(p, j // 2, j % 2, after)
            outs.append(o)
            ms.append(m)
        for layer in range(len(deps) // 2):
            o0, o1 = outs[2 * layer:2 * layer + 2]
            self.oa[p, layer] = (
                o0[0], jnp.where(self._lane_lo(8), o0[1], o1[1]), o1[0])
        return ms

    def out(self, p, part=None):
        for k in ((0, 1) if part is None else (part,)):
            c0, c1 = self.cols[k], self.cols[k + 1]
            w = self.wo[p * self.pw:(p + 1) * self.pw, c0:c1]
            self.acc[k] = self.acc[k] + _dot(self.o[p], w, _NN)
            if k == PLAN["mark"]:
                self.marker = self.acc[k][:8, :LANES]

    def run(self, n_pairs, init, b, always):
        last = n_pairs - 1
        self.acc = [init[:, :self.cols[1]], init[:, self.cols[1]:]]
        self.always = always
        done = ms = None
        b0, b_after = PLAN["b_start"], PLAN["b_after"]
        gate = PLAN["gate" + self.kind]
        for p in range(n_pairs):
            self.proj_q(p)
            self.pending, done = done, None
            if b0 <= p < b0 + b.n_groups:
                mk = self.marker
                if b_after is not None:
                    mk = ms[min(b_after, len(ms) - 1)]
                o = b.attend(p - b0, (always, mk))
                done = functools.reduce(lambda u, v: u + v, o)
            self.proj_k(p)
            if p == last and self.defer:
                self.proj_v(p)
                self.pv(p - 1)
            else:
                if p > 0:
                    self.pv(p - 1)
                self.proj_v(p)
            if p == last and gate:
                ms = self.head_rows(p, self.pv_marker,
                                    PLAN["last" + self.kind])
                assert self.pending is None
                self.pending = functools.reduce(
                    lambda u, v: u + v, [ms[i] for i in gate])
            self.scores(p)
            if p == 0:
                b.project()
            elif p < last - self.defer:
                self.out(p - 1)
            if not (p == last and gate):
                ms = self.head_rows(
                    p, self.marker,
                    PLAN[("last" if p == last else "deps") + self.kind])
        if self.defer:
            self.out(last - 2)
        yb = b.finish()
        self.out(last - 1, 0)
        self.pv(last)
        self.out(last - 1, 1)
        self.out(last)
        return jnp.concatenate(self.acc, axis=1), yb


class _TwoLayerPass(_PassBase):
    def __init__(self, h, pre_ref, pre_row, w_ref, wo_ref, head_ref, *, dh,
                 m_len, seg):
        super().__init__(h, w_ref, wo_ref, head_ref, dh)
        self.pre, self.pre_row = pre_ref, pre_row
        self.kind = "80" if pre_row is None else "64"
        u = self.u = m_len
        n = 2 * (m_len + seg)
        self.seg = seg
        row = lax.broadcasted_iota(jnp.int32, (n - 2 * u, n), 0)
        col = lax.broadcasted_iota(jnp.int32, (n - 2 * u, n), 1)
        row = jnp.where(row < 2 * u, row, row + 2 * u)

        def first_layer(i):
            return (((i < 6 * u) & ((i & u) == 0))
                    | ((i >= 6 * u) & (i < 6 * u + PRE)))

        def index(i):
            low = ((i >> 1) & ~(u - 1)) + (i & (u - 1))
            high = jnp.where(i < 6 * u + PRE, i - 3 * u, i - 3 * u - PRE)
            return jnp.where(i < 6 * u, low, high)

        self.col_a = first_layer(col)
        self.diag = first_layer(row) == self.col_a
        self.allowed = (row < 2 * u) | (index(row) >= index(col))
        self.lo_u = self._lane_lo(u)
        self.lo_c = self._lane_lo(PRE)

    def _proj(self, p, j):
        u, seg = self.u, self.seg
        r = self._project(p, j)
        if self.pre_row is None:
            n1 = seg
            c1 = r[2 * u:n1]
        else:
            n1 = 2 * u
            c1 = self.pre[3 * p + j, pl.ds(self.pre_row, PRE), :].astype(F32)
        nx = n1 + seg
        return ((r[nx:nx + u], r[:u], r[u:2 * u], c1),
                (r[nx + u:], r[n1:n1 + u], r[n1 + u:n1 + 2 * u],
                 r[n1 + 2 * u:nx]))

    @staticmethod
    def _weave(f, g):
        return jnp.concatenate([a for pair in zip(f, g) for a in pair],
                               axis=0).astype(BF16)

    @staticmethod
    def _stack(f):
        return jnp.concatenate(f, axis=0).astype(BF16)

    def _tiles(self, l1, l2):
        masks = (self.lo_u,) * 3 + (self.lo_c,)

        def t(l, c):
            return [_tile(a, c) for a in l]

        def lo(l):
            return [_keep(mk, a) for mk, a in zip(masks, l)]

        def hi(l):
            return [_drop(mk, a) for mk, a in zip(masks, l)]

        return (self._weave(t(l1, 0), t(l2, 0)),
                self._weave(lo(t(l1, 1)), hi(t(l1, 1))),
                self._weave(hi(t(l2, 1)), lo(t(l2, 1))),
                self._weave(t(l2, 2), t(l1, 2)))

    def _unstack(self, a):
        u = self.u
        return a[:u], a[u:2 * u], a[2 * u:]

    def _unweave(self, a):
        u = self.u
        return ((a[:u], a[2 * u:3 * u], a[4 * u:4 * u + PRE]),
                (a[u:2 * u], a[3 * u:4 * u], a[4 * u + PRE:]))

    def proj_q(self, p):
        ls = self._proj(p, 0)
        for i, l in enumerate(ls):
            self.qa[p, i] = l[1]
        l1, l2 = ((l[0], l[2], l[3]) for l in ls)
        q0, q2 = (self._weave([_tile(a, c) for a in l1],
                              [_tile(a, c) for a in l2]) for c in (0, 2))
        qa, qb = (self._stack([_tile(a, 1) for a in l]) for l in (l1, l2))
        self.q[p] = (q0, qa, qb, q2)

    def _proj_kv(self, p, j):
        ls = self._proj(p, j)
        for i, l in enumerate(ls):
            self._stash(p, i, j - 1, l[0], l[1])
        return self._tiles(*ls)

    def proj_k(self, p):
        self.k[p] = self._proj_kv(p, 1)

    def proj_v(self, p):
        self.v[p] = self._proj_kv(p, 2)

    def scores(self, p):
        q0, qa, qb, q2 = self.q.pop(p)
        k0, k1a, k1b, k2 = self.k.pop(p)
        r0 = _dot(q0, k0, _NT)
        r2 = _dot(q2, k2, _NT)
        f = self._unstack(_dot(qa, k1a, _NT))
        g = self._unstack(_dot(qb, k1b, _NT))
        r1 = jnp.concatenate([f[0], g[0], f[1], g[1], f[2], g[2]], axis=0)
        s = jnp.where(self.diag, r0, r2) + r1
        s = self._gate(jnp.where(self.allowed, s * self.scale, NEG))
        p_all = _pair_softmax(s, self.col_a)
        pa, pb = (jnp.concatenate(l, axis=0).astype(BF16)
                  for l in self._unweave(p_all))
        self.p[p] = (_keep(self.diag, p_all).astype(BF16), pa, pb,
                     _drop(self.diag, p_all).astype(BF16))

    def pv(self, p):
        p0, pa, pb, p2 = self.p.pop(p)
        v0, v1a, v1b, v2 = self.v.pop(p)
        a1, a2 = self.oa.pop((p, 0)), self.oa.pop((p, 1))
        o0 = self._unweave(_dot(p0, v0, _NN))
        self.pv_marker = o0[0][0]
        o2 = self._unweave(_dot(p2, v2, _NN))
        o1 = (self._unstack(_dot(pa, v1a, _NN)),
              self._unstack(_dot(pb, v1b, _NN)))
        self.o[p] = jnp.concatenate(
            [self._order([f[0], g[0], a1[c], f[1], f[2], a2[c], g[1], g[2]])
             for c, (f, g) in enumerate((o0, o1, o2))], axis=1).astype(BF16)

    @staticmethod
    def _order(units):
        return jnp.concatenate([units[i] for i in PLAN["order"]], axis=0)

    def to_rows(self, x1, x2):
        z = jnp.zeros((self.u, x1.shape[1]), F32)
        return self._order((z, z) + self._unstack(x1) + self._unstack(x2))

    def from_rows(self, a):
        size = [self.u] * 8
        size[4] = size[7] = PRE
        units, r = {}, 0
        for i in PLAN["order"]:
            units[i] = a[r:r + size[i]]
            r += size[i]
        return (jnp.concatenate([units[0], units[1]], axis=0),
                jnp.concatenate([units[i] for i in range(2, 8)], axis=0))


class _OneLayerPass(_PassBase):
    defer = 1
    kind = "1"

    def __init__(self, h, pre_ref, pre_row, w_ref, wo_ref, head_ref, *, dh,
                 m_len, seg):
        super().__init__(h, w_ref, wo_ref, head_ref, dh)
        self.pre, self.pre_row = pre_ref, pre_row
        u = self.u = m_len
        n = self.n = m_len + seg
        row = lax.broadcasted_iota(jnp.int32, (n - u, 2 * n), 0)
        col = lax.broadcasted_iota(jnp.int32, (n - u, 2 * n), 1)
        self.col_a = col < n
        key = jnp.where(self.col_a, col, col - n)
        self.allowed = (row < u) | (row + u >= key)
        lane = lax.broadcasted_iota(jnp.int32, (n, self.pw), 1)
        self.head0 = lane < dh

    def _project(self, p, j):
        a = super()._project(p, j)
        n = self.n
        self.pre[3 * p + j, pl.ds(self.pre_row, a.shape[0] - n), :] = (
            a[n:].astype(BF16))
        return a[:n]

    def _proj_kv(self, p, j):
        a = self._project(p, j)
        u = self.u
        self._stash(p, 0, j - 1, a[:u], a[u:2 * u])
        return jnp.concatenate([_keep(self.head0, a), _drop(self.head0, a)],
                               axis=0).astype(BF16)

    def proj_q(self, p):
        a = self._project(p, 0)
        u = self.u
        self.qa[p, 0] = a[u:2 * u]
        self.q[p] = jnp.concatenate([a[:u], a[2 * u:]], axis=0).astype(BF16)

    def proj_k(self, p):
        self.k[p] = self._proj_kv(p, 1)

    def proj_v(self, p):
        self.v[p] = self._proj_kv(p, 2)

    def scores(self, p):
        s = _dot(self.q.pop(p), self.k.pop(p), _NT)
        s = self._gate(jnp.where(self.allowed, s * self.scale, NEG))
        self.p[p] = _pair_softmax(s, self.col_a).astype(BF16)

    def pv(self, p):
        o = _dot(self.p.pop(p), self.v.pop(p), _NN)
        self.pv_marker = o[:8, :LANES]
        oa = jnp.concatenate(self.oa.pop((p, 0)), axis=1)
        self.o[p] = jnp.concatenate([o[:self.u], oa, o[self.u:]],
                                    axis=0).astype(BF16)


class _BPass:
    def __init__(self, y_ref, starts, wqkv_ref, wo_ref, kv_ref, kv_next_ref,
                 *, seg, d):
        self.y, self.starts = y_ref, starts
        self.wqkv, self.wo, self.kv = wqkv_ref, wo_ref, kv_ref
        self.kv_next = kv_next_ref
        self.seg, self.nt = seg, d // LANES
        self.scale = (d // HB) ** (-0.5)
        self.n_groups = len(starts) * seg // 8
        self.outs = []

    def project(self):
        seg, nt = self.seg, self.nt
        yn = _ln(self.y[...]).astype(BF16)
        self.q, ka, va = (_dot(yn, _unpack(self.wqkv[j]), _NN)
                          for j in range(3))
        for i in range(len(self.starts)):
            for c in range(2 * nt):
                a = _tile((ka, va)[c // nt][i * seg:(i + 1) * seg], c % nt)
                self.kv[i, c, HIST:HIST + seg, :] = a
                if self.kv_next is not None:
                    self.kv_next[i, c, :HIST, :] = a[seg - HIST:]

    def attend(self, gi, after=None):
        seg, nt, kv = self.seg, self.nt, self.kv
        i, g = divmod(gi, seg // 8)
        q = [_tile(self.q[8 * gi:8 * gi + 8], c) for c in range(nt)]
        if after is not None:
            q = [jnp.where(after[0], u, after[1]) for u in q]
        pos = (lax.broadcasted_iota(jnp.int32, (8, LANES), 0)
               + (self.starts[i] + 8 * g))
        offs = [HIST + 8 * g - w * DIL for w in range(WIN)]
        logits = []
        for w, off in enumerate(offs):
            t = q[0] * kv[i, 0, off:off + 8, :]
            for c in range(1, nt):
                t = t + q[c] * kv[i, c, off:off + 8, :]
            t = t + pltpu.roll(t, 64, 1)
            t = (t + pltpu.roll(t, 32, 1)) * self.scale
            if 8 * g < w * DIL:
                t = jnp.where(pos >= w * DIL, t, NEG)
            logits.append(t)
        m = logits[0]
        for t in logits[1:]:
            m = jnp.maximum(m, t)
        es = [jnp.exp(t - m) for t in logits]
        den = es[0]
        for e in es[1:]:
            den = den + e
        inv = _recip(den)
        o = []
        for c in range(nt):
            acc = None
            for w, off in enumerate(offs):
                term = es[w] * kv[i, nt + c, off:off + 8, :]
                acc = term if acc is None else acc + term
            o.append(acc * inv)
        self.outs.append(jnp.concatenate(o, axis=1))
        return o

    def finish(self):
        o = jnp.concatenate(self.outs, axis=0).astype(BF16)
        proj = jnp.concatenate(
            [_dot(o, _unpack(self.wo[c]), _NN) for c in range(self.nt)],
            axis=1)
        return self.y[...] + proj


def _kernel(x_hbm, mem_hbm, wq_hbm, wk_hbm, wv_hbm, wo_hbm, bqkv_hbm, bo_hbm,
            out_hbm,
            x_v, mem_v, wst_v, w_v, wo_v, bq_st, bo_st, tq_s, to_s, bqkv_p,
            bo_p, out_v, xn_s, pre_s, h_s, h1_s, ra_s, y_s, yt_s, kv_s, head_s,
            sems, w_sems, bq_sems, bo_sems,
            *, seg, n_seg, m_len, n_pairs, dh, d):
    db = d // HB
    nt = d // LANES
    pw = 2 * dh
    m2 = 2 * m_len
    n_half = n_seg // 2
    n_pre = (n_half - 1 - LAG // 2) * PRE
    n_bq = 3 * nt

    def w_copy(p, j, sem=None):
        src = (wq_hbm, wk_hbm, wv_hbm)[j]
        slot = p & (NSLOT - 1)
        return pltpu.make_async_copy(
            src.at[pl.ds(p * pw, pw), :], wst_v.at[slot, j],
            w_sems.at[slot if sem is None else sem])

    def w_wait(p):
        slot = p & (NSLOT - 1)
        pltpu.make_async_copy(wst_v.at[slot], wst_v.at[slot],
                              w_sems.at[slot]).wait()

    def wo_copy(p):
        return pltpu.make_async_copy(wo_hbm.at[pl.ds(p * pw, pw), :],
                                     wo_v.at[pl.ds(p * pw, pw), :],
                                     sems.at[7])

    def bq_copy(i):
        row = pl.multiple_of((i % nt) * LANES, LANES)
        col = pl.multiple_of((i // nt) * d, LANES)
        return pltpu.make_async_copy(
            bqkv_hbm.at[pl.ds(row, LANES), pl.ds(col, d)], bq_st.at[i],
            bq_sems.at[i & 1])

    def bo_copy(i):
        col = pl.multiple_of(i * LANES, LANES)
        return pltpu.make_async_copy(bo_hbm.at[:, pl.ds(col, LANES)],
                                     bo_st.at[i], bo_sems.at[i & 1])

    nf = seg - PRE

    def x_copy(idx, sem):
        return pltpu.make_async_copy(x_hbm.at[idx], x_v.at[idx], sems.at[sem])

    full = slice(None)
    xa_copy = x_copy((full, 0, slice(nf, None), full), 0)
    x0_copy = x_copy((0, 0, slice(None, nf), full), 5)
    xb_copy = x_copy((slice(1, None), 0, slice(None, nf), full), 1)
    xc_copy = x_copy((full, 1), 6)

    def x_seg(t):
        return x_v.at[t >> 1, t & 1]

    mem_copy = pltpu.make_async_copy(mem_hbm, mem_v, sems.at[2])

    mem_copy.start()
    xa_copy.start()
    mem_copy.wait()
    x0_copy.start()
    w_copy(0, 0, sem=NSLOT).start()

    ra_s[...] = jnp.zeros(ra_s.shape, F32)
    y_s[...] = jnp.zeros(y_s.shape, F32)
    kv_s[0, :, :, :HIST, :] = jnp.zeros(kv_s.shape[1:3] + (HIST, LANES), F32)

    xa_copy.wait()
    for j in range(1, 3):
        w_copy(0, j, sem=NSLOT + j).start()

    def ln_block(i, carry):
        s0 = pl.multiple_of(i * LN_SEGS, LN_SEGS)
        xb = x_v[pl.ds(s0, LN_SEGS), 0, nf:, :].astype(F32)
        xn_s[pl.ds(pl.multiple_of(s0 * PRE, PRE), LN_SEGS * PRE), :] = _ln(
            xb.reshape(LN_SEGS * PRE, d)).astype(BF16)
        return carry

    lax.fori_loop(0, n_half // LN_SEGS, ln_block, 0)

    n1 = m_len + seg
    last_xn = (n_half - 1) * PRE
    x0_copy.wait()
    for j in range(3):
        w_copy(1, j).start()
    bq_copy(0).start()
    bo_copy(0).start()
    wo_copy(0).start()

    def permute_rows(tmp_ref):
        return jnp.concatenate(
            [tmp_ref[pl.ds(j, HB, stride=db), :] for j in range(db)], axis=0)

    n_chunk = -(-n_pre // PRE_CHUNK)
    bounds = [16 * (n_pre // 16 * c // n_chunk) for c in range(n_chunk + 1)]
    skip = LAG // 2 * PRE

    def pre_blocks(blocks, jobs, always):
        def transpose_w(src, b, n):
            wt = src[n * LANES:(n + 1) * LANES, :].T
            w_v[b, :, n * LANES:(n + 1) * LANES] = _pack(wt)
            return [wt[(c + 1) * LANES - 16:(c + 1) * LANES]
                    for c in range(nt)]

        jobs = [None] + jobs + [functools.partial(transpose_w, src, b, n)
                                for src, b in blocks
                                for n in range(pw // LANES)]
        for c in range(n_chunk):
            r0, r1 = bounds[c], bounds[c + 1]
            for src, b in blocks:
                lhs = xn_s[skip + r0:skip + r1, :]
                job = jobs.pop(0) if jobs else None
                if job is not None:
                    top = jnp.where(always, lhs[:16],
                                    jnp.concatenate(job(), axis=1))
                    lhs = jnp.concatenate([top, lhs[16:]], axis=0)
                pre_s[b, r0:r1, :] = _dot(lhs, src[...], _NT).astype(BF16)
        assert not jobs

    def first_block(j, carry):
        src = wst_v.at[0, j]
        pltpu.make_async_copy(src, src, w_sems.at[NSLOT + j]).wait()
        pre_blocks([(src, j)], [], j >= 0)
        h1_s[:n1, :] = jnp.concatenate(
            [mem_v[...].astype(F32), _ln(x_v[0, 0].astype(F32))],
            axis=0).astype(BF16)
        h1_s[n1:, :] = xn_s[last_xn:last_xn + m_len, :]
        return carry

    def prefetch(p):
        @pl.when(p + NSLOT < n_pairs)
        def _():
            for j in range(3):
                w_copy(p + NSLOT, j).start()

        @pl.when(p + NSLOT == n_pairs)
        def _():
            xb_copy.start()
            xc_copy.start()

        @pl.when(p + 1 < n_pairs)
        def _():
            wo_copy(p + 1).start()

        @pl.when(p + 1 < n_bq)
        def _():
            bq_copy(p + 1).start()

        @pl.when(p + 1 < nt)
        def _():
            bo_copy(p + 1).start()

    def pre_pair(p, carry):
        def relayout_bo():
            i = jnp.minimum(p - 1, nt - 1)
            to_s[:d, :] = bo_st[i].astype(F32)
            bo = permute_rows(to_s)
            bo_p[i] = _pack(bo.astype(BF16))
            g = d // nt // 16
            return [functools.reduce(
                lambda u, v: u + v,
                [bo[16 * (c * g + r):16 * (c * g + r + 1)] for r in range(g)]
            ).astype(BF16) for c in range(nt)]

        def relayout_bq():
            i = p - 1
            tq_s[:d, :] = bq_st[i].astype(F32).T
            row = pl.multiple_of((i % nt) * (LANES // 2), LANES // 2)
            bq = permute_rows(tq_s).T.astype(BF16)
            bqkv_p[i // nt, pl.ds(row, LANES // 2), :] = _pack(bq)
            return [_tile(bq[LANES - 16:], c) for c in range(nt)]

        w_wait(p)
        pltpu.make_async_copy(bq_st.at[p - 1], bq_st.at[p - 1],
                              bq_sems.at[(p - 1) & 1]).wait()

        @pl.when(p <= nt)
        def _():
            bo_copy(p - 1).wait()

        slot = p & (NSLOT - 1)
        pre_blocks([(wst_v.at[slot, j], 3 * p + j) for j in range(3)],
                   [relayout_bo, relayout_bq], p >= 0)
        prefetch(p)
        return carry

    lax.fori_loop(0, 3, first_block, 0)
    prefetch(jnp.int32(0))
    lax.fori_loop(1, n_pairs, pre_pair, 0)

    xb_copy.wait()
    xc_copy.wait()
    pltpu.make_async_copy(wo_v, wo_v, sems.at[7]).wait()

    n_early_out = n_seg - 1 - LAG

    def b_pass(t, par):
        return _BPass(y_s, ((t - 1) * seg, (t - 1 - LAG) * seg), bqkv_p, bo_p,
                      kv_s.at[par], kv_s.at[1 - par], seg=seg, d=d)

    def b_store(t, yb):
        out_v[jnp.maximum(t - 1 - LAG, 0)] = yb[seg:].astype(out_v.dtype)
        return yb[:seg]

    def two_layer_step(t, par, h):
        half = t >> 1
        pre_row = None
        if par == 0:
            pre_row = pl.multiple_of((half - LAG // 2) * PRE, PRE)
        a = _TwoLayerPass(h, pre_s, pre_row, w_v, wo_v, head_s,
                          dh=dh, m_len=m_len, seg=seg)
        init = a.to_rows(x_v[half, par].astype(F32), ra_s[...])
        acc, yb = a.run(n_pairs, init, b_pass(t, par), t >= 0)
        x2 = b_store(t, yb)
        mems, y_s[...] = a.from_rows(acc)
        ra_s[...] = x2
        if par == 0:
            xn = x_v[half, 1]
        else:
            xn = x_v[jnp.minimum(half + 1, n_half - 1), 0, :nf, :]
        return jnp.concatenate([_ln(xn.astype(F32)), _ln(x2), mems],
                               axis=0).astype(BF16)

    def two_layer_steps(i, carry):
        h = h_s[...]
        for u in range(UNROLL):
            h = two_layer_step(LAG + i * UNROLL + u, (LAG + u) % 2, h)
        h_s[...] = h
        return carry

    def one_layer_step(t, carry):
        first = t < LAG
        li = (t == n_seg + 1).astype(jnp.int32)
        par = (t - li) & 1
        b = _BPass(y_s.at[pl.ds(pl.multiple_of(li * seg, seg), seg)],
                   ((t - 1 - li * (1 + LAG)) * seg,), bqkv_p, bo_p,
                   kv_s.at[par, pl.ds(li, 1)], kv_s.at[1 - par, pl.ds(li, 1)],
                   seg=seg, d=d)
        extra_row = pl.multiple_of(n_pre + jnp.minimum(t, 1) * m_len, m_len)
        a = _OneLayerPass(h1_s[...], pre_s, extra_row, w_v, wo_v, head_s,
                          dh=dh, m_len=m_len, seg=seg)
        x0 = x_seg(jnp.minimum(t, n_seg - 1))[...].astype(F32)
        init = jnp.concatenate(
            [jnp.zeros((m_len, d), F32), jnp.where(first, x0, ra_s[...])],
            axis=0)
        acc, x2 = a.run(n_pairs, init, b, t >= 0)
        out_v[jnp.where(first, 0, n_early_out)] = x2.astype(out_v.dtype)
        y = acc[m_len:]
        y_s[:seg, :] = y
        yt_s[pl.ds(pl.multiple_of((t & 1) * seg, seg), seg), :] = y
        ra_s[...] = x2
        xn = _ln(x_seg(jnp.minimum(t + 1, n_seg - 1))[...].astype(F32))
        x2n = _ln(x2)
        mem = acc[:m_len]
        h1_s[:n1, :] = jnp.concatenate(
            [mem, jnp.where(first, xn, x2n)], axis=0).astype(BF16)
        h1_s[n1:, :] = xn_s[last_xn + m_len:, :]
        h_s[...] = jnp.concatenate(
            [xn[:nf], x2n, mem, mem_v[...].astype(F32)], axis=0).astype(BF16)
        return carry

    out_a = pltpu.make_async_copy(out_v.at[:n_early_out],
                                  out_hbm.at[:n_early_out], sems.at[3])
    out_b = pltpu.make_async_copy(out_v.at[n_early_out:],
                                  out_hbm.at[n_early_out:], sems.at[4])

    def phase(ph, carry):
        t0 = ph * n_seg
        lax.fori_loop(t0, t0 + LAG, one_layer_step, 0)

        @pl.when(ph == 0)
        def _():
            lax.fori_loop(0, (n_seg - LAG) // UNROLL, two_layer_steps, 0)
            out_a.start()
            hf = h_s[...].astype(F32)
            h1_s[:n1, :] = jnp.concatenate(
                [hf[nf + seg + m_len:], hf[nf:nf + seg]],
                axis=0).astype(BF16)

        return carry

    lax.fori_loop(0, 2, phase, 0)

    b = _BPass(yt_s, ((n_seg - 2) * seg,), bqkv_p, bo_p,
               kv_s.at[(n_seg + 1) % 2, 1:], None, seg=2 * seg, d=d)
    b.project()
    for gi in range(b.n_groups):
        b.attend(gi)
    out_v[n_seg - 2:] = b.finish().astype(out_v.dtype).reshape(2, seg, d)
    out_b.start()
    out_a.wait()
    out_b.wait()


def pallas_interleave_layers__memory_aug_recurrent_mem_tr__sliding_local_dilated__prompt_kernel(
    A_x: jax.Array,
    A_mem0: jax.Array,
    A_Wq: jax.Array,
    A_Wk: jax.Array,
    A_Wv: jax.Array,
    A_Wo: jax.Array,
    A_seg_len,
    B_x: jax.Array,
    B_wqkv: jax.Array,
    B_wo: jax.Array,
):
    del B_x
    seg = A_seg_len if isinstance(A_seg_len, int) else SEG_LEN
    return _forward(A_x, A_mem0, A_Wq, A_Wk, A_Wv, A_Wo, B_wqkv, B_wo, seg=seg)


@functools.partial(jax.jit, static_argnames=("seg",))
def _forward(A_x, A_mem0, A_Wq, A_Wk, A_Wv, A_Wo, B_wqkv, B_wo, *, seg):
    bsz, s_len, d = A_x.shape
    m_len = A_mem0.shape[1]
    n_heads, dh = A_Wq.shape[1], A_Wq.shape[2]
    n_seg = s_len // seg
    n_pairs = n_heads // 2
    nt = d // LANES
    assert bsz == 1 and s_len % seg == 0 and n_seg > LAG + 1
    assert m_len == 8 and seg == 2 * m_len + PRE and seg >= HIST
    assert LAG == 2 and LAG * m_len == PRE and n_seg % (2 * LN_SEGS) == 0
    assert 2 * (m_len + seg) <= LANES
    assert (n_seg - LAG) % UNROLL == 0 and UNROLL == 2
    assert n_heads % 2 == 0 and 2 * dh == 3 * LANES and d % LANES == 0
    assert d % HB == 0 and LANES == 4 * HB and n_pairs == 3 * nt + 1
    hd = n_heads * dh
    n_half = n_seg // 2
    n_pre = (n_half - LAG // 2) * PRE

    wq_t = jnp.transpose(A_Wq, (1, 2, 0)).reshape(hd, d)
    wk_t = jnp.transpose(A_Wk, (1, 2, 0)).reshape(hd, d)
    wv_t = jnp.transpose(A_Wv, (1, 2, 0)).reshape(hd, d)
    wo = A_Wo.reshape(hd, d)

    kernel = functools.partial(
        _kernel, seg=seg, n_seg=n_seg, m_len=m_len, n_pairs=n_pairs, dh=dh,
        d=d)
    any_spec = pl.BlockSpec(memory_space=pl.ANY)
    dma = pltpu.SemaphoreType.DMA
    out = pl.pallas_call(
        kernel,
        out_shape=jax.ShapeDtypeStruct((n_seg, seg, d), A_x.dtype),
        in_specs=[any_spec] * 8,
        out_specs=any_spec,
        scratch_shapes=[
            pltpu.VMEM((n_half, 2, seg, d), BF16),
            pltpu.VMEM((m_len, d), BF16),
            pltpu.VMEM((NSLOT, 3, 2 * dh, d), BF16),
            pltpu.VMEM((3 * n_pairs, d // 2, 2 * dh), U32),
            pltpu.VMEM((hd, d), BF16),
            pltpu.VMEM((3 * nt, LANES, d), BF16),
            pltpu.VMEM((nt, d, LANES), BF16),
            pltpu.VMEM((d + HB, LANES), F32),
            pltpu.VMEM((d + HB, LANES), F32),
            pltpu.VMEM((3, d // 2, d), U32),
            pltpu.VMEM((nt, d // 2, LANES), U32),
            pltpu.VMEM((n_seg, seg, d), A_x.dtype),
            pltpu.VMEM((n_half * PRE, d), BF16),
            pltpu.VMEM((3 * n_pairs, n_pre, 2 * dh), BF16),
            pltpu.VMEM((2 * (m_len + seg) - PRE, d), BF16),
            pltpu.VMEM((2 * m_len + seg, d), BF16),
            pltpu.VMEM((seg, d), F32),
            pltpu.VMEM((2 * seg, d), F32),
            pltpu.VMEM((2 * seg, d), F32),
            pltpu.VMEM((2, 2, 2 * nt, HIST + 2 * seg, LANES), F32),
            pltpu.VMEM((HEAD_SLOTS, 2, 2, 3, 72, LANES), F32),
            dma((8,)), dma((NSLOT + 3,)), dma((2,)), dma((2,)),
        ],
        compiler_params=pltpu.CompilerParams(
            vmem_limit_bytes=96 * 1024 * 1024,
            disable_bounds_checks=True,
            disable_semaphore_checks=True),
    )(A_x.reshape(n_half, 2, seg, d), A_mem0.reshape(m_len, d), wq_t, wk_t, wv_t,
      wo, B_wqkv, B_wo)
    return out.reshape(bsz, s_len, d)
```

```python
import functools

import jax
import jax.numpy as jnp
from jax import lax
import jax.experimental.pallas as pl
import jax.experimental.pallas.tpu as pltpu

F32 = jnp.float32
BF16 = jnp.bfloat16
U32 = jnp.uint32

_NT = (((1,), (1,)), ((), ()))
_NN = (((1,), (0,)), ((), ()))

SEG_LEN = 32
HB = 32
WIN = 8
DIL = 2
HIST = 16
LANES = 128
PRE = 16
PRE_CHUNK = 128
LN_SEGS = 16
LAG = 2
UNROLL = 2
NSLOT = 2
HEAD_SLOTS = 4
NEG = -1000000000.0

PLAN = dict(
    deps64=((), (0,), (), (2,)), deps80=((), (0,), (), (2,)),
    last64=((), (0,), (), (2,)), last80=((), (0,), (), (2,)),
    gate64=(0, 2), gate80=(0, 2),
    deps1=((), ()), last1=((), ()), gate1=(),
    b_start=2, b_after=3, order=(0, 1, 2, 3, 4, 5, 6, 7), mark=0,
)


def _dot(a, b, dims):
    return lax.dot_general(a, b, dims, preferred_element_type=F32)


def _recip(x):
    r = pl.reciprocal(x, approx=True)
    return r * (2.0 - x * r)


def _ln(x):
    m = jnp.mean(x, axis=-1, keepdims=True)
    xc = x - m
    v = jnp.mean(xc * xc, axis=-1, keepdims=True)
    return xc * lax.rsqrt(v + 1e-05)


def _pack(a):
    return pltpu.bitcast(a, U32)


def _unpack(a):
    return pltpu.bitcast(a, BF16)


def _tile(a, c):
    return a[:, c * LANES:(c + 1) * LANES]


def _keep(mask, a):
    return jnp.where(mask, a, jnp.zeros_like(a))


def _drop(mask, a):
    return jnp.where(mask, jnp.zeros_like(a), a)


def _pair_softmax(s, col_a):
    m_a = jnp.max(jnp.where(col_a, s, -jnp.inf), axis=1, keepdims=True)
    m_b = jnp.max(jnp.where(col_a, -jnp.inf, s), axis=1, keepdims=True)
    e = jnp.exp(s - jnp.where(col_a, m_a, m_b))
    d_a = jnp.sum(jnp.where(col_a, e, 0.0), axis=1, keepdims=True)
    d_b = jnp.sum(jnp.where(col_a, 0.0, e), axis=1, keepdims=True)
    return e * _recip(jnp.where(col_a, d_a, d_b))


class _PassBase:
    defer = 0

    def __init__(self, h, w_ref, wo_ref, head_ref, dh):
        self.h, self.w, self.wo = h, w_ref, wo_ref
        self.head = head_ref
        self.qa, self.ea, self.oa = {}, {}, {}
        self.pw = 2 * dh
        self.half = dh - LANES
        self.scale = dh ** (-0.5)
        self.q, self.k, self.v, self.p, self.o = {}, {}, {}, {}, {}
        self.cols = (0, 2 * LANES, wo_ref.shape[1])
        self.pending = None

    def _lane_lo(self, rows):
        return lax.broadcasted_iota(jnp.int32, (rows, LANES), 1) < self.half

    def _project(self, p, j):
        a = _dot(self.h, _unpack(self.w[3 * p + j]), _NN)
        self.marker = a[:8, :LANES]
        return a

    def _stash(self, p, layer, kind, m, a):
        rows = jnp.concatenate([m, a], axis=0)
        rows = jnp.stack([_tile(rows, c) for c in range(3)])
        for i in range(4):
            self.head[p % HEAD_SLOTS, layer, kind, :,
                      pl.ds(i, 16, stride=4), :] = rows

    def _head_job(self, p, layer, hd, after):
        q = self.qa[p, layer]
        sub = lax.broadcasted_iota(jnp.int32, (8, LANES), 0)
        top = sub < 4
        lo = self._lane_lo(8)

        def tiles(kind):
            blk = self.head[p % HEAD_SLOTS, layer, kind, hd:hd + 2, :64, :]
            blk = blk.reshape(2, 8, 8, LANES)
            return blk[hd], blk[1 - hd]

        def spread(a):
            r = pltpu.roll(a, 4, 0)
            return jnp.where(top, a, r), jnp.where(top, r, a)

        def fold(a, b, op):
            return op(jnp.where(top, a, b),
                      pltpu.roll(jnp.where(top, b, a), 4, 0))

        qo = jnp.where(self.always, _tile(q, 2 * hd), after) * self.scale
        qs = jnp.where(self.always, _tile(q, 1), after) * self.scale
        qs = _drop(lo, qs) if hd else _keep(lo, qs)
        ko, ks = tiles(0)
        n_used = (6, 8)
        scores = []
        for half, (a, b) in enumerate(zip(spread(qo), spread(qs))):
            n = n_used[half]
            sc = jnp.sum(a[None] * ko[:n] + b[None] * ks[:n], axis=2,
                         keepdims=True)
            sc = jnp.broadcast_to(sc, (n, 8, LANES))
            shape = (2, 8, LANES)
            pair = lax.broadcasted_iota(jnp.int32, shape, 0)
            row = lax.broadcasted_iota(jnp.int32, shape, 1)
            seen = 2 * pair + (row >> 2) <= (row & 3)
            scores.append(jnp.concatenate(
                [sc[:n - 2], jnp.where(seen, sc[n - 2:], NEG)], axis=0))
        m = fold(*(jnp.max(sc, axis=0) for sc in scores), jnp.maximum)
        es = [jnp.exp(sc - mh[None]) for sc, mh in zip(scores, spread(m))]
        inv = _recip(fold(*(jnp.sum(e, axis=0) for e in es), jnp.add))
        outs = [fold(*(jnp.sum(e * v[:e.shape[0]], axis=0) for e in es),
                     jnp.add) * inv for v in tiles(1)]
        return outs, m

    def _gate(self, s):
        if self.pending is None:
            return s
        top = jnp.where(self.always, s[:8], self.pending[:, :s.shape[1]])
        self.pending = None
        return jnp.concatenate([top, s[8:]], axis=0)

    def head_rows(self, p, start, deps):
        outs, ms = [], []
        for j, dep in enumerate(deps):
            after = start if not dep else functools.reduce(
                lambda a, b: a + b, [ms[i] for i in dep])
            o, m = self._head_job(p, j // 2, j % 2, after)
            outs.append(o)
            ms.append(m)
        for layer in range(len(deps) // 2):
            o0, o1 = outs[2 * layer:2 * layer + 2]
            self.oa[p, layer] = (
                o0[0], jnp.where(self._lane_lo(8), o0[1], o1[1]), o1[0])
        return ms

    def out(self, p, part=None):
        for k in ((0, 1) if part is None else (part,)):
            c0, c1 = self.cols[k], self.cols[k + 1]
            w = self.wo[p * self.pw:(p + 1) * self.pw, c0:c1]
            self.acc[k] = self.acc[k] + _dot(self.o[p], w, _NN)
            if k == PLAN["mark"]:
                self.marker = self.acc[k][:8, :LANES]

    def run(self, n_pairs, init, b, always):
        last = n_pairs - 1
        self.acc = [init[:, :self.cols[1]], init[:, self.cols[1]:]]
        self.always = always
        done = ms = None
        b0, b_after = PLAN["b_start"], PLAN["b_after"]
        gate = PLAN["gate" + self.kind]
        for p in range(n_pairs):
            self.proj_q(p)
            self.pending, done = done, None
            if b0 <= p < b0 + b.n_groups:
                mk = self.marker
                if b_after is not None:
                    mk = ms[min(b_after, len(ms) - 1)]
                done = b.attend(p - b0, (always, mk))
            self.proj_k(p)
            if p == last and self.defer:
                self.proj_v(p)
                self.pv(p - 1)
            else:
                if p > 0:
                    self.pv(p - 1)
                self.proj_v(p)
            if p == last and gate:
                ms = self.head_rows(p, self.pv_marker,
                                    PLAN["last" + self.kind])
                assert self.pending is None
                self.pending = functools.reduce(
                    lambda u, v: u + v, [ms[i] for i in gate])
            self.scores(p)
            if p == 0:
                b.project()
            elif p < last - self.defer:
                self.out(p - 1)
            if not (p == last and gate):
                ms = self.head_rows(
                    p, self.marker,
                    PLAN[("last" if p == last else "deps") + self.kind])
        if self.defer:
            self.out(last - 2)
        yb = b.finish()
        self.out(last - 1, 0)
        self.pv(last)
        self.out(last - 1, 1)
        self.out(last)
        return jnp.concatenate(self.acc, axis=1), yb


class _TwoLayerPass(_PassBase):
    def __init__(self, h, pre_ref, pre_row, w_ref, wo_ref, head_ref, *, dh,
                 m_len, seg):
        super().__init__(h, w_ref, wo_ref, head_ref, dh)
        self.pre, self.pre_row = pre_ref, pre_row
        self.kind = "80" if pre_row is None else "64"
        u = self.u = m_len
        n = 2 * (m_len + seg)
        self.seg = seg
        row = lax.broadcasted_iota(jnp.int32, (n - 2 * u, n), 0)
        col = lax.broadcasted_iota(jnp.int32, (n - 2 * u, n), 1)
        row = jnp.where(row < 2 * u, row, row + 2 * u)

        def first_layer(i):
            return (((i < 6 * u) & ((i & u) == 0))
                    | ((i >= 6 * u) & (i < 6 * u + PRE)))

        def index(i):
            low = ((i >> 1) & ~(u - 1)) + (i & (u - 1))
            high = jnp.where(i < 6 * u + PRE, i - 3 * u, i - 3 * u - PRE)
            return jnp.where(i < 6 * u, low, high)

        self.col_a = first_layer(col)
        self.diag = first_layer(row) == self.col_a
        self.allowed = (row < 2 * u) | (index(row) >= index(col))
        self.lo_u = self._lane_lo(u)
        self.lo_c = self._lane_lo(PRE)

    def _proj(self, p, j):
        u, seg = self.u, self.seg
        r = self._project(p, j)
        if self.pre_row is None:
            n1 = seg
            c1 = r[2 * u:n1]
        else:
            n1 = 2 * u
            c1 = self.pre[3 * p + j, pl.ds(self.pre_row, PRE), :].astype(F32)
        nx = n1 + seg
        return ((r[nx:nx + u], r[:u], r[u:2 * u], c1),
                (r[nx + u:], r[n1:n1 + u], r[n1 + u:n1 + 2 * u],
                 r[n1 + 2 * u:nx]))

    @staticmethod
    def _weave(f, g):
        return jnp.concatenate([a for pair in zip(f, g) for a in pair],
                               axis=0).astype(BF16)

    @staticmethod
    def _stack(f):
        return jnp.concatenate(f, axis=0).astype(BF16)

    def _tiles(self, l1, l2):
        masks = (self.lo_u,) * 3 + (self.lo_c,)

        def t(l, c):
            return [_tile(a, c) for a in l]

        def lo(l):
            return [_keep(mk, a) for mk, a in zip(masks, l)]

        def hi(l):
            return [_drop(mk, a) for mk, a in zip(masks, l)]

        return (self._weave(t(l1, 0), t(l2, 0)),
                self._weave(lo(t(l1, 1)), hi(t(l1, 1))),
                self._weave(hi(t(l2, 1)), lo(t(l2, 1))),
                self._weave(t(l2, 2), t(l1, 2)))

    def _unstack(self, a):
        u = self.u
        return a[:u], a[u:2 * u], a[2 * u:]

    def _unweave(self, a):
        u = self.u
        return ((a[:u], a[2 * u:3 * u], a[4 * u:4 * u + PRE]),
                (a[u:2 * u], a[3 * u:4 * u], a[4 * u + PRE:]))

    def proj_q(self, p):
        ls = self._proj(p, 0)
        for i, l in enumerate(ls):
            self.qa[p, i] = l[1]
        l1, l2 = ((l[0], l[2], l[3]) for l in ls)
        q0, q2 = (self._weave([_tile(a, c) for a in l1],
                              [_tile(a, c) for a in l2]) for c in (0, 2))
        qa, qb = (self._stack([_tile(a, 1) for a in l]) for l in (l1, l2))
        self.q[p] = (q0, qa, qb, q2)

    def _proj_kv(self, p, j):
        ls = self._proj(p, j)
        for i, l in enumerate(ls):
            self._stash(p, i, j - 1, l[0], l[1])
        return self._tiles(*ls)

    def proj_k(self, p):
        self.k[p] = self._proj_kv(p, 1)

    def proj_v(self, p):
        self.v[p] = self._proj_kv(p, 2)

    def scores(self, p):
        q0, qa, qb, q2 = self.q.pop(p)
        k0, k1a, k1b, k2 = self.k.pop(p)
        r0 = _dot(q0, k0, _NT)
        r2 = _dot(q2, k2, _NT)
        f = self._unstack(_dot(qa, k1a, _NT))
        g = self._unstack(_dot(qb, k1b, _NT))
        r1 = jnp.concatenate([f[0], g[0], f[1], g[1], f[2], g[2]], axis=0)
        s = jnp.where(self.diag, r0, r2) + r1
        s = self._gate(jnp.where(self.allowed, s * self.scale, NEG))
        p_all = _pair_softmax(s, self.col_a)
        pa, pb = (jnp.concatenate(l, axis=0).astype(BF16)
                  for l in self._unweave(p_all))
        self.p[p] = (_keep(self.diag, p_all).astype(BF16), pa, pb,
                     _drop(self.diag, p_all).astype(BF16))

    def pv(self, p):
        p0, pa, pb, p2 = self.p.pop(p)
        v0, v1a, v1b, v2 = self.v.pop(p)
        a1, a2 = self.oa.pop((p, 0)), self.oa.pop((p, 1))
        o0 = self._unweave(_dot(p0, v0, _NN))
        self.pv_marker = o0[0][0]
        o2 = self._unweave(_dot(p2, v2, _NN))
        o1 = (self._unstack(_dot(pa, v1a, _NN)),
              self._unstack(_dot(pb, v1b, _NN)))
        self.o[p] = jnp.concatenate(
            [self._order([f[0], g[0], a1[c], f[1], f[2], a2[c], g[1], g[2]])
             for c, (f, g) in enumerate((o0, o1, o2))], axis=1).astype(BF16)

    @staticmethod
    def _order(units):
        return jnp.concatenate([units[i] for i in PLAN["order"]], axis=0)

    def to_rows(self, x1, x2):
        z = jnp.zeros((self.u, x1.shape[1]), F32)
        return self._order((z, z) + self._unstack(x1) + self._unstack(x2))

    def from_rows(self, a):
        size = [self.u] * 8
        size[4] = size[7] = PRE
        units, r = {}, 0
        for i in PLAN["order"]:
            units[i] = a[r:r + size[i]]
            r += size[i]
        return (jnp.concatenate([units[0], units[1]], axis=0),
                jnp.concatenate([units[i] for i in range(2, 8)], axis=0))


class _OneLayerPass(_PassBase):
    defer = 1
    kind = "1"

    def __init__(self, h, pre_ref, pre_row, w_ref, wo_ref, head_ref, *, dh,
                 m_len, seg):
        super().__init__(h, w_ref, wo_ref, head_ref, dh)
        self.pre, self.pre_row = pre_ref, pre_row
        u = self.u = m_len
        n = self.n = m_len + seg
        row = lax.broadcasted_iota(jnp.int32, (n - u, 2 * n), 0)
        col = lax.broadcasted_iota(jnp.int32, (n - u, 2 * n), 1)
        self.col_a = col < n
        key = jnp.where(self.col_a, col, col - n)
        self.allowed = (row < u) | (row + u >= key)
        lane = lax.broadcasted_iota(jnp.int32, (n, self.pw), 1)
        self.head0 = lane < dh

    def _project(self, p, j):
        a = super()._project(p, j)
        n = self.n
        self.pre[3 * p + j, pl.ds(self.pre_row, a.shape[0] - n), :] = (
            a[n:].astype(BF16))
        return a[:n]

    def _proj_kv(self, p, j):
        a = self._project(p, j)
        u = self.u
        self._stash(p, 0, j - 1, a[:u], a[u:2 * u])
        return jnp.concatenate([_keep(self.head0, a), _drop(self.head0, a)],
                               axis=0).astype(BF16)

    def proj_q(self, p):
        a = self._project(p, 0)
        u = self.u
        self.qa[p, 0] = a[u:2 * u]
        self.q[p] = jnp.concatenate([a[:u], a[2 * u:]], axis=0).astype(BF16)

    def proj_k(self, p):
        self.k[p] = self._proj_kv(p, 1)

    def proj_v(self, p):
        self.v[p] = self._proj_kv(p, 2)

    def scores(self, p):
        s = _dot(self.q.pop(p), self.k.pop(p), _NT)
        s = self._gate(jnp.where(self.allowed, s * self.scale, NEG))
        self.p[p] = _pair_softmax(s, self.col_a).astype(BF16)

    def pv(self, p):
        o = _dot(self.p.pop(p), self.v.pop(p), _NN)
        self.pv_marker = o[:8, :LANES]
        oa = jnp.concatenate(self.oa.pop((p, 0)), axis=1)
        self.o[p] = jnp.concatenate([o[:self.u], oa, o[self.u:]],
                                    axis=0).astype(BF16)


class _BPass:
    def __init__(self, y_ref, starts, wqkv_ref, wo_ref, kv_ref, kv_next_ref,
                 *, seg, d):
        self.y, self.starts = y_ref, starts
        self.wqkv, self.wo, self.kv = wqkv_ref, wo_ref, kv_ref
        self.kv_next = kv_next_ref
        self.seg, self.nt = seg, d // LANES
        self.scale = (d // HB) ** (-0.5)
        self.n_groups = len(starts) * seg // 8
        self.outs = []

    def project(self):
        seg, nt = self.seg, self.nt
        yn = _ln(self.y[...]).astype(BF16)
        self.q, ka, va = (_dot(yn, _unpack(self.wqkv[j]), _NN)
                          for j in range(3))
        for i in range(len(self.starts)):
            a = jnp.stack([_tile(t[i * seg:(i + 1) * seg], c)
                           for t in (ka, va) for c in range(nt)])
            self.kv[i, :, HIST:HIST + seg, :] = a
            if self.kv_next is not None:
                self.kv_next[i, :, :HIST, :] = a[:, seg - HIST:]

    def attend(self, gi, after=None):
        seg, nt, kv = self.seg, self.nt, self.kv
        i, g = divmod(gi, seg // 8)
        q = jnp.stack([_tile(self.q[8 * gi:8 * gi + 8], c) for c in range(nt)])
        if after is not None:
            q = jnp.where(after[0], q, after[1][None])
        pos = (lax.broadcasted_iota(jnp.int32, (8, LANES), 0)
               + (self.starts[i] + 8 * g))
        offs = [HIST + 8 * g - w * DIL for w in range(WIN)]
        logits = []
        for w, off in enumerate(offs):
            t = jnp.sum(q * kv[i, :nt, off:off + 8, :], axis=0)
            t = t + pltpu.roll(t, 64, 1)
            t = (t + pltpu.roll(t, 32, 1)) * self.scale
            if 8 * g < w * DIL:
                t = jnp.where(pos >= w * DIL, t, NEG)
            logits.append(t)
        m = functools.reduce(jnp.maximum, logits)
        es = [jnp.exp(t - m) for t in logits]
        inv = _recip(functools.reduce(jnp.add, es))
        o = functools.reduce(jnp.add, [
            e[None] * kv[i, nt:, off:off + 8, :] for e, off in zip(es, offs)])
        o = o * inv[None]
        self.outs.append(jnp.concatenate([o[c] for c in range(nt)], axis=1))
        return jnp.sum(o, axis=0)

    def finish(self):
        o = jnp.concatenate(self.outs, axis=0).astype(BF16)
        proj = jnp.concatenate(
            [_dot(o, _unpack(self.wo[c]), _NN) for c in range(self.nt)],
            axis=1)
        return self.y[...] + proj


def _kernel(x_hbm, mem_hbm, wq_hbm, wk_hbm, wv_hbm, wo_hbm, bqkv_hbm, bo_hbm,
            out_hbm,
            x_v, mem_v, wst_v, w_v, wo_v, bq_st, bo_st, tq_s, to_s, bqkv_p,
            bo_p, out_v, xn_s, pre_s, h_s, h1_s, ra_s, y_s, yt_s, kv_s, head_s,
            sems, w_sems, bq_sems, bo_sems,
            *, seg, n_seg, m_len, n_pairs, dh, d):
    db = d // HB
    nt = d // LANES
    pw = 2 * dh
    m2 = 2 * m_len
    n_half = n_seg // 2
    n_pre = (n_half - 1 - LAG // 2) * PRE
    n_bq = 3 * nt

    def w_copy(p, j, sem=None):
        src = (wq_hbm, wk_hbm, wv_hbm)[j]
        slot = p & (NSLOT - 1)
        return pltpu.make_async_copy(
            src.at[pl.ds(p * pw, pw), :], wst_v.at[slot, j],
            w_sems.at[slot if sem is None else sem])

    def w_wait(p):
        slot = p & (NSLOT - 1)
        pltpu.make_async_copy(wst_v.at[slot], wst_v.at[slot],
                              w_sems.at[slot]).wait()

    def wo_copy(p):
        return pltpu.make_async_copy(wo_hbm.at[pl.ds(p * pw, pw), :],
                                     wo_v.at[pl.ds(p * pw, pw), :],
                                     sems.at[7])

    def bq_copy(i):
        row = pl.multiple_of((i % nt) * LANES, LANES)
        col = pl.multiple_of((i // nt) * d, LANES)
        return pltpu.make_async_copy(
            bqkv_hbm.at[pl.ds(row, LANES), pl.ds(col, d)], bq_st.at[i],
            bq_sems.at[i & 1])

    def bo_copy(i):
        col = pl.multiple_of(i * LANES, LANES)
        return pltpu.make_async_copy(bo_hbm.at[:, pl.ds(col, LANES)],
                                     bo_st.at[i], bo_sems.at[i & 1])

    nf = seg - PRE

    def x_copy(idx, sem):
        return pltpu.make_async_copy(x_hbm.at[idx], x_v.at[idx], sems.at[sem])

    full = slice(None)
    xa_copy = x_copy((full, 0, slice(nf, None), full), 0)
    x0_copy = x_copy((0, 0, slice(None, nf), full), 5)
    xb_copy = x_copy((slice(1, None), 0, slice(None, nf), full), 1)
    xc_copy = x_copy((full, 1), 6)

    def x_seg(t):
        return x_v.at[t >> 1, t & 1]

    mem_copy = pltpu.make_async_copy(mem_hbm, mem_v, sems.at[2])

    mem_copy.start()
    xa_copy.start()
    mem_copy.wait()
    x0_copy.start()
    w_copy(0, 0, sem=NSLOT).start()

    ra_s[...] = jnp.zeros(ra_s.shape, F32)
    y_s[...] = jnp.zeros(y_s.shape, F32)
    kv_s[0, :, :, :HIST, :] = jnp.zeros(kv_s.shape[1:3] + (HIST, LANES), F32)

    xa_copy.wait()
    for j in range(1, 3):
        w_copy(0, j, sem=NSLOT + j).start()

    def ln_block(i, carry):
        s0 = pl.multiple_of(i * LN_SEGS, LN_SEGS)
        xb = x_v[pl.ds(s0, LN_SEGS), 0, nf:, :].astype(F32)
        xn_s[pl.ds(pl.multiple_of(s0 * PRE, PRE), LN_SEGS * PRE), :] = _ln(
            xb.reshape(LN_SEGS * PRE, d)).astype(BF16)
        return carry

    lax.fori_loop(0, n_half // LN_SEGS, ln_block, 0)

    n1 = m_len + seg
    last_xn = (n_half - 1) * PRE
    x0_copy.wait()
    for j in range(3):
        w_copy(1, j).start()
    bq_copy(0).start()
    bo_copy(0).start()
    wo_copy(0).start()

    def permute_rows(tmp_ref):
        return jnp.concatenate(
            [tmp_ref[pl.ds(j, HB, stride=db), :] for j in range(db)], axis=0)

    n_chunk = -(-n_pre // PRE_CHUNK)
    bounds = [16 * (n_pre // 16 * c // n_chunk) for c in range(n_chunk + 1)]
    skip = LAG // 2 * PRE

    def pre_blocks(blocks, jobs, always):
        def transpose_w(src, b, n):
            wt = src[n * LANES:(n + 1) * LANES, :].T
            w_v[b, :, n * LANES:(n + 1) * LANES] = _pack(wt)
            return [wt[(c + 1) * LANES - 16:(c + 1) * LANES]
                    for c in range(nt)]

        jobs = [None] + jobs + [functools.partial(transpose_w, src, b, n)
                                for src, b in blocks
                                for n in range(pw // LANES)]
        for c in range(n_chunk):
            r0, r1 = bounds[c], bounds[c + 1]
            for src, b in blocks:
                lhs = xn_s[skip + r0:skip + r1, :]
                job = jobs.pop(0) if jobs else None
                if job is not None:
                    top = jnp.where(always, lhs[:16],
                                    jnp.concatenate(job(), axis=1))
                    lhs = jnp.concatenate([top, lhs[16:]], axis=0)
                pre_s[b, r0:r1, :] = _dot(lhs, src[...], _NT).astype(BF16)
        assert not jobs

    def first_block(j, carry):
        src = wst_v.at[0, j]
        pltpu.make_async_copy(src, src, w_sems.at[NSLOT + j]).wait()
        pre_blocks([(src, j)], [], j >= 0)
        h1_s[:n1, :] = jnp.concatenate(
            [mem_v[...].astype(F32), _ln(x_v[0, 0].astype(F32))],
            axis=0).astype(BF16)
        h1_s[n1:, :] = xn_s[last_xn:last_xn + m_len, :]
        return carry

    def prefetch(p):
        @pl.when(p + NSLOT < n_pairs)
        def _():
            for j in range(3):
                w_copy(p + NSLOT, j).start()

        @pl.when(p + NSLOT == n_pairs)
        def _():
            xb_copy.start()
            xc_copy.start()

        @pl.when(p + 1 < n_pairs)
        def _():
            wo_copy(p + 1).start()

        @pl.when(p + 1 < n_bq)
        def _():
            bq_copy(p + 1).start()

        @pl.when(p + 1 < nt)
        def _():
            bo_copy(p + 1).start()

    def pre_pair(p, carry):
        def relayout_bo():
            i = jnp.minimum(p - 1, nt - 1)
            to_s[:d, :] = bo_st[i].astype(F32)
            bo = permute_rows(to_s)
            bo_p[i] = _pack(bo.astype(BF16))
            g = d // nt // 16
            return [functools.reduce(
                lambda u, v: u + v,
                [bo[16 * (c * g + r):16 * (c * g + r + 1)] for r in range(g)]
            ).astype(BF16) for c in range(nt)]

        def relayout_bq():
            i = p - 1
            tq_s[:d, :] = bq_st[i].astype(F32).T
            row = pl.multiple_of((i % nt) * (LANES // 2), LANES // 2)
            bq = permute_rows(tq_s).T.astype(BF16)
            bqkv_p[i // nt, pl.ds(row, LANES // 2), :] = _pack(bq)
            return [_tile(bq[LANES - 16:], c) for c in range(nt)]

        w_wait(p)
        pltpu.make_async_copy(bq_st.at[p - 1], bq_st.at[p - 1],
                              bq_sems.at[(p - 1) & 1]).wait()

        @pl.when(p <= nt)
        def _():
            bo_copy(p - 1).wait()

        slot = p & (NSLOT - 1)
        pre_blocks([(wst_v.at[slot, j], 3 * p + j) for j in range(3)],
                   [relayout_bo, relayout_bq], p >= 0)
        prefetch(p)
        return carry

    lax.fori_loop(0, 3, first_block, 0)
    prefetch(jnp.int32(0))
    lax.fori_loop(1, n_pairs, pre_pair, 0)

    xb_copy.wait()
    xc_copy.wait()
    pltpu.make_async_copy(wo_v, wo_v, sems.at[7]).wait()

    n_early_out = n_seg - 1 - LAG

    def b_pass(t, par):
        return _BPass(y_s, ((t - 1) * seg, (t - 1 - LAG) * seg), bqkv_p, bo_p,
                      kv_s.at[par], kv_s.at[1 - par], seg=seg, d=d)

    def b_store(t, yb):
        out_v[jnp.maximum(t - 1 - LAG, 0)] = yb[seg:].astype(out_v.dtype)
        return yb[:seg]

    def two_layer_step(t, par, h):
        half = t >> 1
        pre_row = None
        if par == 0:
            pre_row = pl.multiple_of((half - LAG // 2) * PRE, PRE)
        a = _TwoLayerPass(h, pre_s, pre_row, w_v, wo_v, head_s,
                          dh=dh, m_len=m_len, seg=seg)
        init = a.to_rows(x_v[half, par].astype(F32), ra_s[...])
        acc, yb = a.run(n_pairs, init, b_pass(t, par), t >= 0)
        x2 = b_store(t, yb)
        mems, y_s[...] = a.from_rows(acc)
        ra_s[...] = x2
        if par == 0:
            xn = x_v[half, 1]
        else:
            xn = x_v[jnp.minimum(half + 1, n_half - 1), 0, :nf, :]
        return jnp.concatenate([_ln(xn.astype(F32)), _ln(x2), mems],
                               axis=0).astype(BF16)

    def two_layer_steps(i, carry):
        h = h_s[...]
        for u in range(UNROLL):
            h = two_layer_step(LAG + i * UNROLL + u, (LAG + u) % 2, h)
        h_s[...] = h
        return carry

    def one_layer_step(t, carry):
        first = t < LAG
        li = (t == n_seg + 1).astype(jnp.int32)
        par = (t - li) & 1
        b = _BPass(y_s.at[pl.ds(pl.multiple_of(li * seg, seg), seg)],
                   ((t - 1 - li * (1 + LAG)) * seg,), bqkv_p, bo_p,
                   kv_s.at[par, pl.ds(li, 1)], kv_s.at[1 - par, pl.ds(li, 1)],
                   seg=seg, d=d)
        extra_row = pl.multiple_of(n_pre + jnp.minimum(t, 1) * m_len, m_len)
        a = _OneLayerPass(h1_s[...], pre_s, extra_row, w_v, wo_v, head_s,
                          dh=dh, m_len=m_len, seg=seg)
        x0 = x_seg(jnp.minimum(t, n_seg - 1))[...].astype(F32)
        init = jnp.concatenate(
            [jnp.zeros((m_len, d), F32), jnp.where(first, x0, ra_s[...])],
            axis=0)
        acc, x2 = a.run(n_pairs, init, b, t >= 0)
        out_v[jnp.where(first, 0, n_early_out)] = x2.astype(out_v.dtype)
        y = acc[m_len:]
        y_s[:seg, :] = y
        yt_s[pl.ds(pl.multiple_of((t & 1) * seg, seg), seg), :] = y
        ra_s[...] = x2
        xn = _ln(x_seg(jnp.minimum(t + 1, n_seg - 1))[...].astype(F32))
        x2n = _ln(x2)
        mem = acc[:m_len]
        h1_s[:n1, :] = jnp.concatenate(
            [mem, jnp.where(first, xn, x2n)], axis=0).astype(BF16)
        h1_s[n1:, :] = xn_s[last_xn + m_len:, :]
        h_s[...] = jnp.concatenate(
            [xn[:nf], x2n, mem, mem_v[...].astype(F32)], axis=0).astype(BF16)
        return carry

    out_a = pltpu.make_async_copy(out_v.at[:n_early_out],
                                  out_hbm.at[:n_early_out], sems.at[3])
    out_b = pltpu.make_async_copy(out_v.at[n_early_out:],
                                  out_hbm.at[n_early_out:], sems.at[4])

    def phase(ph, carry):
        t0 = ph * n_seg
        lax.fori_loop(t0, t0 + LAG, one_layer_step, 0)

        @pl.when(ph == 0)
        def _():
            lax.fori_loop(0, (n_seg - LAG) // UNROLL, two_layer_steps, 0)
            out_a.start()
            hf = h_s[...].astype(F32)
            h1_s[:n1, :] = jnp.concatenate(
                [hf[nf + seg + m_len:], hf[nf:nf + seg]],
                axis=0).astype(BF16)

        return carry

    lax.fori_loop(0, 2, phase, 0)

    b = _BPass(yt_s, ((n_seg - 2) * seg,), bqkv_p, bo_p,
               kv_s.at[(n_seg + 1) % 2, 1:], None, seg=2 * seg, d=d)
    b.project()
    for gi in range(b.n_groups):
        b.attend(gi)
    out_v[n_seg - 2:] = b.finish().astype(out_v.dtype).reshape(2, seg, d)
    out_b.start()
    out_a.wait()
    out_b.wait()


def pallas_interleave_layers__memory_aug_recurrent_mem_tr__sliding_local_dilated__prompt_kernel(
    A_x: jax.Array,
    A_mem0: jax.Array,
    A_Wq: jax.Array,
    A_Wk: jax.Array,
    A_Wv: jax.Array,
    A_Wo: jax.Array,
    A_seg_len,
    B_x: jax.Array,
    B_wqkv: jax.Array,
    B_wo: jax.Array,
):
    del B_x
    seg = A_seg_len if isinstance(A_seg_len, int) else SEG_LEN
    return _forward(A_x, A_mem0, A_Wq, A_Wk, A_Wv, A_Wo, B_wqkv, B_wo, seg=seg)


@functools.partial(jax.jit, static_argnames=("seg",))
def _forward(A_x, A_mem0, A_Wq, A_Wk, A_Wv, A_Wo, B_wqkv, B_wo, *, seg):
    bsz, s_len, d = A_x.shape
    m_len = A_mem0.shape[1]
    n_heads, dh = A_Wq.shape[1], A_Wq.shape[2]
    n_seg = s_len // seg
    n_pairs = n_heads // 2
    nt = d // LANES
    assert bsz == 1 and s_len % seg == 0 and n_seg > LAG + 1
    assert m_len == 8 and seg == 2 * m_len + PRE and seg >= HIST
    assert LAG == 2 and LAG * m_len == PRE and n_seg % (2 * LN_SEGS) == 0
    assert 2 * (m_len + seg) <= LANES
    assert (n_seg - LAG) % UNROLL == 0 and UNROLL == 2
    assert n_heads % 2 == 0 and 2 * dh == 3 * LANES and d % LANES == 0
    assert d % HB == 0 and LANES == 4 * HB and n_pairs == 3 * nt + 1
    hd = n_heads * dh
    n_half = n_seg // 2
    n_pre = (n_half - LAG // 2) * PRE

    wq_t = jnp.transpose(A_Wq, (1, 2, 0)).reshape(hd, d)
    wk_t = jnp.transpose(A_Wk, (1, 2, 0)).reshape(hd, d)
    wv_t = jnp.transpose(A_Wv, (1, 2, 0)).reshape(hd, d)
    wo = A_Wo.reshape(hd, d)

    kernel = functools.partial(
        _kernel, seg=seg, n_seg=n_seg, m_len=m_len, n_pairs=n_pairs, dh=dh,
        d=d)
    any_spec = pl.BlockSpec(memory_space=pl.ANY)
    dma = pltpu.SemaphoreType.DMA
    out = pl.pallas_call(
        kernel,
        out_shape=jax.ShapeDtypeStruct((n_seg, seg, d), A_x.dtype),
        in_specs=[any_spec] * 8,
        out_specs=any_spec,
        scratch_shapes=[
            pltpu.VMEM((n_half, 2, seg, d), BF16),
            pltpu.VMEM((m_len, d), BF16),
            pltpu.VMEM((NSLOT, 3, 2 * dh, d), BF16),
            pltpu.VMEM((3 * n_pairs, d // 2, 2 * dh), U32),
            pltpu.VMEM((hd, d), BF16),
            pltpu.VMEM((3 * nt, LANES, d), BF16),
            pltpu.VMEM((nt, d, LANES), BF16),
            pltpu.VMEM((d + HB, LANES), F32),
            pltpu.VMEM((d + HB, LANES), F32),
            pltpu.VMEM((3, d // 2, d), U32),
            pltpu.VMEM((nt, d // 2, LANES), U32),
            pltpu.VMEM((n_seg, seg, d), A_x.dtype),
            pltpu.VMEM((n_half * PRE, d), BF16),
            pltpu.VMEM((3 * n_pairs, n_pre, 2 * dh), BF16),
            pltpu.VMEM((2 * (m_len + seg) - PRE, d), BF16),
            pltpu.VMEM((2 * m_len + seg, d), BF16),
            pltpu.VMEM((seg, d), F32),
            pltpu.VMEM((2 * seg, d), F32),
            pltpu.VMEM((2 * seg, d), F32),
            pltpu.VMEM((2, 2, 2 * nt, HIST + 2 * seg, LANES), F32),
            pltpu.VMEM((HEAD_SLOTS, 2, 2, 3, 72, LANES), F32),
            dma((8,)), dma((NSLOT + 3,)), dma((2,)), dma((2,)),
        ],
        compiler_params=pltpu.CompilerParams(
            vmem_limit_bytes=96 * 1024 * 1024,
            disable_bounds_checks=True,
            disable_semaphore_checks=True),
    )(A_x.reshape(n_half, 2, seg, d), A_mem0.reshape(m_len, d), wq_t, wk_t, wv_t,
      wo, B_wqkv, B_wo)
    return out.reshape(bsz, s_len, d)
```

```python
import functools

import jax
import jax.numpy as jnp
from jax import lax
import jax.experimental.pallas as pl
import jax.experimental.pallas.tpu as pltpu

F32 = jnp.float32
BF16 = jnp.bfloat16
U32 = jnp.uint32

_NT = (((1,), (1,)), ((), ()))
_NN = (((1,), (0,)), ((), ()))

SEG_LEN = 32
HB = 32
WIN = 8
DIL = 2
HIST = 16
LANES = 128
PRE = 16
PRE_CHUNK = 128
LN_SEGS = 16
LAG = 2
UNROLL = 2
NSLOT = 2
HEAD_SLOTS = 2
NEG = -1000000000.0


def _dot(a, b, dims):
    return lax.dot_general(a, b, dims, preferred_element_type=F32)


def _recip(x):
    r = pl.reciprocal(x, approx=True)
    return r * (2.0 - x * r)


def _ln(x):
    m = jnp.mean(x, axis=-1, keepdims=True)
    xc = x - m
    v = jnp.mean(xc * xc, axis=-1, keepdims=True)
    return xc * lax.rsqrt(v + 1e-05)


def _pack(a):
    return pltpu.bitcast(a, U32)


def _unpack(a):
    return pltpu.bitcast(a, BF16)


def _tile(a, c):
    return a[:, c * LANES:(c + 1) * LANES]


def _keep(mask, a):
    return jnp.where(mask, a, jnp.zeros_like(a))


def _drop(mask, a):
    return jnp.where(mask, jnp.zeros_like(a), a)


def _pair_softmax(s, col_a):
    m_a = jnp.max(jnp.where(col_a, s, -jnp.inf), axis=1, keepdims=True)
    m_b = jnp.max(jnp.where(col_a, -jnp.inf, s), axis=1, keepdims=True)
    e = jnp.exp(s - jnp.where(col_a, m_a, m_b))
    d_a = jnp.sum(jnp.where(col_a, e, 0.0), axis=1, keepdims=True)
    d_b = jnp.sum(jnp.where(col_a, 0.0, e), axis=1, keepdims=True)
    return e * _recip(jnp.where(col_a, d_a, d_b))


class _PassBase:
    chain = True
    defer = 0

    def __init__(self, h, w_ref, wo_ref, head_ref, dh):
        self.h, self.w, self.wo = h, w_ref, wo_ref
        self.head = head_ref
        self.qa, self.oa = {}, {}
        self.pw = 2 * dh
        self.half = dh - LANES
        self.scale = dh ** (-0.5)
        self.q, self.k, self.v, self.p, self.o = {}, {}, {}, {}, {}
        self.cols = (0, 2 * LANES, wo_ref.shape[1])
        self.pending = None

    def _lane_lo(self, rows):
        return lax.broadcasted_iota(jnp.int32, (rows, LANES), 1) < self.half

    def _project(self, p, j):
        a = _dot(self.h, _unpack(self.w[3 * p + j]), _NN)
        self.marker = a[:8, :LANES]
        return a

    def _stash(self, p, layer, kind, m, a):
        rows = jnp.concatenate([m, a], axis=0)
        rows = jnp.stack([_tile(rows, c) for c in range(3)])
        for i in range(4):
            self.head[p % HEAD_SLOTS, layer, kind, :,
                      pl.ds(i, 16, stride=4), :] = rows

    def _head_job(self, p, layer, hd, after):
        q = self.qa[p, layer]
        sub = lax.broadcasted_iota(jnp.int32, (8, LANES), 0)
        top = sub < 4
        lo = self._lane_lo(8)

        def tiles(kind):
            blk = self.head[p % HEAD_SLOTS, layer, kind, hd:hd + 2, :64, :]
            blk = blk.reshape(2, 8, 8, LANES)
            return blk[hd], blk[1 - hd]

        def spread(a):
            r = pltpu.roll(a, 4, 0)
            return jnp.where(top, a, r), jnp.where(top, r, a)

        def fold(a, b, op):
            return op(jnp.where(top, a, b),
                      pltpu.roll(jnp.where(top, b, a), 4, 0))

        qo = jnp.where(self.always, _tile(q, 2 * hd), after) * self.scale
        qs = jnp.where(self.always, _tile(q, 1), after) * self.scale
        qs = _drop(lo, qs) if hd else _keep(lo, qs)
        ko, ks = tiles(0)
        n_used = (6, 8)
        scores = []
        for half, (a, b) in enumerate(zip(spread(qo), spread(qs))):
            n = n_used[half]
            sc = jnp.sum(a[None] * ko[:n] + b[None] * ks[:n], axis=2,
                         keepdims=True)
            sc = jnp.broadcast_to(sc, (n, 8, LANES))
            shape = (2, 8, LANES)
            pair = lax.broadcasted_iota(jnp.int32, shape, 0)
            row = lax.broadcasted_iota(jnp.int32, shape, 1)
            seen = 2 * pair + (row >> 2) <= (row & 3)
            scores.append(jnp.concatenate(
                [sc[:n - 2], jnp.where(seen, sc[n - 2:], NEG)], axis=0))
        m = fold(*(jnp.max(sc, axis=0) for sc in scores), jnp.maximum)
        es = [jnp.exp(sc - mh[None]) for sc, mh in zip(scores, spread(m))]
        inv = _recip(fold(*(jnp.sum(e, axis=0) for e in es), jnp.add))
        outs = [fold(*(jnp.sum(e * v[:e.shape[0]], axis=0) for e in es),
                     jnp.add) * inv for v in tiles(1)]
        return outs, m

    def _gate(self, s):
        if self.pending is None:
            return s
        top = jnp.where(self.always, s[:8], self.pending[:, :s.shape[1]])
        self.pending = None
        return jnp.concatenate([top, s[8:]], axis=0)

    def head_rows(self, p, start):
        ms = []
        for layer in range(2):
            if (p, layer) not in self.qa:
                continue
            o0, m0 = self._head_job(p, layer, 0, start)
            o1, m1 = self._head_job(p, layer, 1, m0 if self.chain else start)
            self.oa[p, layer] = (
                o0[0], jnp.where(self._lane_lo(8), o0[1], o1[1]), o1[0])
            ms += [m0, m1]
        return ms

    def out(self, p, part=None):
        for k in ((0, 1) if part is None else (part,)):
            c0, c1 = self.cols[k], self.cols[k + 1]
            w = self.wo[p * self.pw:(p + 1) * self.pw, c0:c1]
            self.acc[k] = self.acc[k] + _dot(self.o[p], w, _NN)
            if k == 0:
                self.marker = self.acc[k][:8, :LANES]

    def run(self, n_pairs, init, b, always):
        last = n_pairs - 1
        self.acc = [init[:, :self.cols[1]], init[:, self.cols[1]:]]
        self.always = always
        done = ms = None
        for p in range(n_pairs):
            self.proj_q(p)
            self.pending, done = done, None
            if 2 <= p < 2 + b.n_groups:
                done = b.attend(p - 2, (always, ms[-1]))
            self.proj_k(p)
            if p == last and self.defer:
                self.proj_v(p)
                self.pv(p - 1)
            else:
                if p > 0:
                    self.pv(p - 1)
                self.proj_v(p)
            early = p == last and self.chain
            if early:
                ms = self.head_rows(p, self.pv_marker)
                self.pending = ms[0] + ms[2]
            self.scores(p)
            if p == 0:
                b.project()
            elif p < last - self.defer:
                self.out(p - 1)
            if not early:
                ms = self.head_rows(p, self.marker)
        if self.defer:
            self.out(last - 2)
            yb = b.finish()
            self.out(last - 1, 0)
        else:
            self.out(last - 1, 0)
            yb = b.finish()
        self.pv(last)
        self.out(last - 1, 1)
        self.out(last)
        return jnp.concatenate(self.acc, axis=1), yb


class _TwoLayerPass(_PassBase):
    def __init__(self, h, pre_ref, pre_row, w_ref, wo_ref, head_ref, *, dh,
                 m_len, seg):
        super().__init__(h, w_ref, wo_ref, head_ref, dh)
        self.pre, self.pre_row = pre_ref, pre_row
        u = self.u = m_len
        n = 2 * (m_len + seg)
        self.seg = seg
        row = lax.broadcasted_iota(jnp.int32, (n - 2 * u, n), 0)
        col = lax.broadcasted_iota(jnp.int32, (n - 2 * u, n), 1)
        row = jnp.where(row < 2 * u, row, row + 2 * u)

        def first_layer(i):
            return (((i < 6 * u) & ((i & u) == 0))
                    | ((i >= 6 * u) & (i < 6 * u + PRE)))

        def index(i):
            low = ((i >> 1) & ~(u - 1)) + (i & (u - 1))
            high = jnp.where(i < 6 * u + PRE, i - 3 * u, i - 3 * u - PRE)
            return jnp.where(i < 6 * u, low, high)

        self.col_a = first_layer(col)
        self.diag = first_layer(row) == self.col_a
        self.allowed = (row < 2 * u) | (index(row) >= index(col))
        self.lo_u = self._lane_lo(u)
        self.lo_c = self._lane_lo(PRE)

    def _proj(self, p, j):
        u, seg = self.u, self.seg
        r = self._project(p, j)
        if self.pre_row is None:
            n1 = seg
            c1 = r[2 * u:n1]
        else:
            n1 = 2 * u
            c1 = self.pre[3 * p + j, pl.ds(self.pre_row, PRE), :].astype(F32)
        nx = n1 + seg
        return ((r[nx:nx + u], r[:u], r[u:2 * u], c1),
                (r[nx + u:], r[n1:n1 + u], r[n1 + u:n1 + 2 * u],
                 r[n1 + 2 * u:nx]))

    @staticmethod
    def _weave(f, g):
        return jnp.concatenate([a for pair in zip(f, g) for a in pair],
                               axis=0).astype(BF16)

    @staticmethod
    def _stack(f):
        return jnp.concatenate(f, axis=0).astype(BF16)

    def _tiles(self, l1, l2):
        masks = (self.lo_u,) * 3 + (self.lo_c,)

        def t(l, c):
            return [_tile(a, c) for a in l]

        def lo(l):
            return [_keep(mk, a) for mk, a in zip(masks, l)]

        def hi(l):
            return [_drop(mk, a) for mk, a in zip(masks, l)]

        return (self._weave(t(l1, 0), t(l2, 0)),
                self._weave(lo(t(l1, 1)), hi(t(l1, 1))),
                self._weave(hi(t(l2, 1)), lo(t(l2, 1))),
                self._weave(t(l2, 2), t(l1, 2)))

    def _unstack(self, a):
        u = self.u
        return a[:u], a[u:2 * u], a[2 * u:]

    def _unweave(self, a):
        u = self.u
        return ((a[:u], a[2 * u:3 * u], a[4 * u:4 * u + PRE]),
                (a[u:2 * u], a[3 * u:4 * u], a[4 * u + PRE:]))

    def proj_q(self, p):
        ls = self._proj(p, 0)
        for i, l in enumerate(ls):
            self.qa[p, i] = l[1]
        l1, l2 = ((l[0], l[2], l[3]) for l in ls)
        q0, q2 = (self._weave([_tile(a, c) for a in l1],
                              [_tile(a, c) for a in l2]) for c in (0, 2))
        qa, qb = (self._stack([_tile(a, 1) for a in l]) for l in (l1, l2))
        self.q[p] = (q0, qa, qb, q2)

    def _proj_kv(self, p, j):
        ls = self._proj(p, j)
        for i, l in enumerate(ls):
            self._stash(p, i, j - 1, l[0], l[1])
        return self._tiles(*ls)

    def proj_k(self, p):
        self.k[p] = self._proj_kv(p, 1)

    def proj_v(self, p):
        self.v[p] = self._proj_kv(p, 2)

    def scores(self, p):
        q0, qa, qb, q2 = self.q.pop(p)
        k0, k1a, k1b, k2 = self.k.pop(p)
        r0 = _dot(q0, k0, _NT)
        r2 = _dot(q2, k2, _NT)
        f = self._unstack(_dot(qa, k1a, _NT))
        g = self._unstack(_dot(qb, k1b, _NT))
        r1 = jnp.concatenate([f[0], g[0], f[1], g[1], f[2], g[2]], axis=0)
        s = jnp.where(self.diag, r0, r2) + r1
        s = self._gate(jnp.where(self.allowed, s * self.scale, NEG))
        p_all = _pair_softmax(s, self.col_a)
        pa, pb = (jnp.concatenate(l, axis=0).astype(BF16)
                  for l in self._unweave(p_all))
        self.p[p] = (_keep(self.diag, p_all).astype(BF16), pa, pb,
                     _drop(self.diag, p_all).astype(BF16))

    def pv(self, p):
        p0, pa, pb, p2 = self.p.pop(p)
        v0, v1a, v1b, v2 = self.v.pop(p)
        a1, a2 = self.oa.pop((p, 0)), self.oa.pop((p, 1))
        o0 = self._unweave(_dot(p0, v0, _NN))
        self.pv_marker = o0[0][0]
        o2 = self._unweave(_dot(p2, v2, _NN))
        o1 = (self._unstack(_dot(pa, v1a, _NN)),
              self._unstack(_dot(pb, v1b, _NN)))
        self.o[p] = jnp.concatenate(
            [jnp.concatenate(
                [f[0], g[0], a1[c], f[1], f[2], a2[c], g[1], g[2]], axis=0)
             for c, (f, g) in enumerate((o0, o1, o2))], axis=1).astype(BF16)


class _OneLayerPass(_PassBase):
    defer = 1
    chain = False

    def __init__(self, h, pre_ref, pre_row, w_ref, wo_ref, head_ref, *, dh,
                 m_len, seg):
        super().__init__(h, w_ref, wo_ref, head_ref, dh)
        self.pre, self.pre_row = pre_ref, pre_row
        u = self.u = m_len
        n = self.n = m_len + seg
        row = lax.broadcasted_iota(jnp.int32, (n - u, 2 * n), 0)
        col = lax.broadcasted_iota(jnp.int32, (n - u, 2 * n), 1)
        self.col_a = col < n
        key = jnp.where(self.col_a, col, col - n)
        self.allowed = (row < u) | (row + u >= key)
        lane = lax.broadcasted_iota(jnp.int32, (n, self.pw), 1)
        self.head0 = lane < dh

    def _project(self, p, j):
        a = super()._project(p, j)
        n = self.n
        self.pre[3 * p + j, pl.ds(self.pre_row, a.shape[0] - n), :] = (
            a[n:].astype(BF16))
        return a[:n]

    def _proj_kv(self, p, j):
        a = self._project(p, j)
        u = self.u
        self._stash(p, 0, j - 1, a[:u], a[u:2 * u])
        return jnp.concatenate([_keep(self.head0, a), _drop(self.head0, a)],
                               axis=0).astype(BF16)

    def proj_q(self, p):
        a = self._project(p, 0)
        u = self.u
        self.qa[p, 0] = a[u:2 * u]
        self.q[p] = jnp.concatenate([a[:u], a[2 * u:]], axis=0).astype(BF16)

    def proj_k(self, p):
        self.k[p] = self._proj_kv(p, 1)

    def proj_v(self, p):
        self.v[p] = self._proj_kv(p, 2)

    def scores(self, p):
        s = _dot(self.q.pop(p), self.k.pop(p), _NT)
        s = self._gate(jnp.where(self.allowed, s * self.scale, NEG))
        self.p[p] = _pair_softmax(s, self.col_a).astype(BF16)

    def pv(self, p):
        o = _dot(self.p.pop(p), self.v.pop(p), _NN)
        oa = jnp.concatenate(self.oa.pop((p, 0)), axis=1)
        self.o[p] = jnp.concatenate([o[:self.u], oa, o[self.u:]],
                                    axis=0).astype(BF16)


class _BPass:
    def __init__(self, y_ref, starts, wqkv_ref, wo_ref, kv_ref, kv_next_ref,
                 *, seg, d):
        self.y, self.starts = y_ref, starts
        self.wqkv, self.wo, self.kv = wqkv_ref, wo_ref, kv_ref
        self.kv_next = kv_next_ref
        self.seg, self.nt = seg, d // LANES
        self.scale = (d // HB) ** (-0.5)
        self.n_groups = len(starts) * seg // 8
        self.outs = []

    def project(self):
        seg, nt = self.seg, self.nt
        yn = _ln(self.y[...]).astype(BF16)
        self.q, ka, va = (_dot(yn, _unpack(self.wqkv[j]), _NN)
                          for j in range(3))
        for i in range(len(self.starts)):
            a = jnp.stack([_tile(t[i * seg:(i + 1) * seg], c)
                           for t in (ka, va) for c in range(nt)])
            self.kv[i, :, HIST:HIST + seg, :] = a
            if self.kv_next is not None:
                self.kv_next[i, :, :HIST, :] = a[:, seg - HIST:]

    def attend(self, gi, after=None):
        seg, nt, kv = self.seg, self.nt, self.kv
        i, g = divmod(gi, seg // 8)
        q = jnp.stack([_tile(self.q[8 * gi:8 * gi + 8], c) for c in range(nt)])
        if after is not None:
            q = jnp.where(after[0], q, after[1][None])
        pos = (lax.broadcasted_iota(jnp.int32, (8, LANES), 0)
               + (self.starts[i] + 8 * g))
        offs = [HIST + 8 * g - w * DIL for w in range(WIN)]
        logits = []
        for w, off in enumerate(offs):
            t = jnp.sum(q * kv[i, :nt, off:off + 8, :], axis=0)
            t = t + pltpu.roll(t, 64, 1)
            t = (t + pltpu.roll(t, 32, 1)) * self.scale
            if 8 * g < w * DIL:
                t = jnp.where(pos >= w * DIL, t, NEG)
            logits.append(t)
        m = functools.reduce(jnp.maximum, logits)
        es = [jnp.exp(t - m) for t in logits]
        inv = _recip(functools.reduce(jnp.add, es))
        o = functools.reduce(jnp.add, [
            e[None] * kv[i, nt:, off:off + 8, :] for e, off in zip(es, offs)])
        o = o * inv[None]
        self.outs.append(jnp.concatenate([o[c] for c in range(nt)], axis=1))
        return jnp.sum(o, axis=0)

    def finish(self):
        o = jnp.concatenate(self.outs, axis=0).astype(BF16)
        proj = jnp.concatenate(
            [_dot(o, _unpack(self.wo[c]), _NN) for c in range(self.nt)],
            axis=1)
        return self.y[...] + proj


def _kernel(x_hbm, mem_hbm, wq_hbm, wk_hbm, wv_hbm, wo_hbm, bqkv_hbm, bo_hbm,
            out_hbm,
            x_v, mem_v, wst_v, w_v, wo_v, bq_st, bo_st, tq_s, to_s, bqkv_p,
            bo_p, out_v, xn_s, pre_s, h_s, h1_s, ra_s, y_s, yt_s, kv_s, head_s,
            sems, w_sems, bq_sems, bo_sems,
            *, seg, n_seg, m_len, n_pairs, dh, d):
    db = d // HB
    nt = d // LANES
    pw = 2 * dh
    m2 = 2 * m_len
    n_half = n_seg // 2
    n_pre = (n_half - 1 - LAG // 2) * PRE
    n_bq = 3 * nt

    def w_copy(p, j, sem=None):
        src = (wq_hbm, wk_hbm, wv_hbm)[j]
        slot = p & (NSLOT - 1)
        return pltpu.make_async_copy(
            src.at[pl.ds(p * pw, pw), :], wst_v.at[slot, j],
            w_sems.at[slot if sem is None else sem])

    def w_wait(p):
        slot = p & (NSLOT - 1)
        pltpu.make_async_copy(wst_v.at[slot], wst_v.at[slot],
                              w_sems.at[slot]).wait()

    def wo_copy(p):
        return pltpu.make_async_copy(wo_hbm.at[pl.ds(p * pw, pw), :],
                                     wo_v.at[pl.ds(p * pw, pw), :],
                                     sems.at[7])

    def bq_copy(i):
        row = pl.multiple_of((i % nt) * LANES, LANES)
        col = pl.multiple_of((i // nt) * d, LANES)
        return pltpu.make_async_copy(
            bqkv_hbm.at[pl.ds(row, LANES), pl.ds(col, d)], bq_st.at[i],
            bq_sems.at[i & 1])

    def bo_copy(i):
        col = pl.multiple_of(i * LANES, LANES)
        return pltpu.make_async_copy(bo_hbm.at[:, pl.ds(col, LANES)],
                                     bo_st.at[i], bo_sems.at[i & 1])

    nf = seg - PRE

    def x_copy(idx, sem):
        return pltpu.make_async_copy(x_hbm.at[idx], x_v.at[idx], sems.at[sem])

    full = slice(None)
    xa_copy = x_copy((full, 0, slice(nf, None), full), 0)
    x0_copy = x_copy((0, 0, slice(None, nf), full), 5)
    xb_copy = x_copy((slice(1, None), 0, slice(None, nf), full), 1)
    xc_copy = x_copy((full, 1), 6)

    def x_seg(t):
        return x_v.at[t >> 1, t & 1]

    mem_copy = pltpu.make_async_copy(mem_hbm, mem_v, sems.at[2])

    mem_copy.start()
    xa_copy.start()
    mem_copy.wait()
    x0_copy.start()
    w_copy(0, 0, sem=NSLOT).start()

    ra_s[...] = jnp.zeros(ra_s.shape, F32)
    y_s[...] = jnp.zeros(y_s.shape, F32)
    kv_s[0, :, :, :HIST, :] = jnp.zeros(kv_s.shape[1:3] + (HIST, LANES), F32)

    xa_copy.wait()
    for j in range(1, 3):
        w_copy(0, j, sem=NSLOT + j).start()

    def ln_block(i, carry):
        s0 = pl.multiple_of(i * LN_SEGS, LN_SEGS)
        xb = x_v[pl.ds(s0, LN_SEGS), 0, nf:, :].astype(F32)
        xn_s[pl.ds(pl.multiple_of(s0 * PRE, PRE), LN_SEGS * PRE), :] = _ln(
            xb.reshape(LN_SEGS * PRE, d)).astype(BF16)
        return carry

    lax.fori_loop(0, n_half // LN_SEGS, ln_block, 0)

    n1 = m_len + seg
    last_xn = (n_half - 1) * PRE
    x0_copy.wait()
    for j in range(3):
        w_copy(1, j).start()
    bq_copy(0).start()
    bo_copy(0).start()
    wo_copy(0).start()

    def permute_rows(tmp_ref):
        return jnp.concatenate(
            [tmp_ref[pl.ds(j, HB, stride=db), :] for j in range(db)], axis=0)

    n_chunk = -(-n_pre // PRE_CHUNK)
    bounds = [16 * (n_pre // 16 * c // n_chunk) for c in range(n_chunk + 1)]
    skip = LAG // 2 * PRE

    def pre_blocks(blocks, jobs, always):
        def transpose_w(src, b, n):
            wt = src[n * LANES:(n + 1) * LANES, :].T
            w_v[b, :, n * LANES:(n + 1) * LANES] = _pack(wt)
            return [wt[(c + 1) * LANES - 16:(c + 1) * LANES]
                    for c in range(nt)]

        jobs = [None] + jobs + [functools.partial(transpose_w, src, b, n)
                                for src, b in blocks
                                for n in range(pw // LANES)]
        for c in range(n_chunk):
            r0, r1 = bounds[c], bounds[c + 1]
            for src, b in blocks:
                lhs = xn_s[skip + r0:skip + r1, :]
                job = jobs.pop(0) if jobs else None
                if job is not None:
                    top = jnp.where(always, lhs[:16],
                                    jnp.concatenate(job(), axis=1))
                    lhs = jnp.concatenate([top, lhs[16:]], axis=0)
                pre_s[b, r0:r1, :] = _dot(lhs, src[...], _NT).astype(BF16)
        assert not jobs

    def first_block(j, carry):
        src = wst_v.at[0, j]
        pltpu.make_async_copy(src, src, w_sems.at[NSLOT + j]).wait()
        pre_blocks([(src, j)], [], j >= 0)
        h1_s[:n1, :] = jnp.concatenate(
            [mem_v[...].astype(F32), _ln(x_v[0, 0].astype(F32))],
            axis=0).astype(BF16)
        h1_s[n1:, :] = xn_s[last_xn:last_xn + m_len, :]
        return carry

    def prefetch(p):
        @pl.when(p + NSLOT < n_pairs)
        def _():
            for j in range(3):
                w_copy(p + NSLOT, j).start()

        @pl.when(p + NSLOT == n_pairs)
        def _():
            xb_copy.start()
            xc_copy.start()

        @pl.when(p + 1 < n_pairs)
        def _():
            wo_copy(p + 1).start()

        @pl.when(p + 1 < n_bq)
        def _():
            bq_copy(p + 1).start()

        @pl.when(p + 1 < nt)
        def _():
            bo_copy(p + 1).start()

    def pre_pair(p, carry):
        def relayout_bo():
            i = jnp.minimum(p - 1, nt - 1)
            to_s[:d, :] = bo_st[i].astype(F32)
            bo = permute_rows(to_s)
            bo_p[i] = _pack(bo.astype(BF16))
            g = d // nt // 16
            return [functools.reduce(
                lambda u, v: u + v,
                [bo[16 * (c * g + r):16 * (c * g + r + 1)] for r in range(g)]
            ).astype(BF16) for c in range(nt)]

        def relayout_bq():
            i = p - 1
            tq_s[:d, :] = bq_st[i].astype(F32).T
            row = pl.multiple_of((i % nt) * (LANES // 2), LANES // 2)
            bq = permute_rows(tq_s).T.astype(BF16)
            bqkv_p[i // nt, pl.ds(row, LANES // 2), :] = _pack(bq)
            return [_tile(bq[LANES - 16:], c) for c in range(nt)]

        w_wait(p)
        pltpu.make_async_copy(bq_st.at[p - 1], bq_st.at[p - 1],
                              bq_sems.at[(p - 1) & 1]).wait()

        @pl.when(p <= nt)
        def _():
            bo_copy(p - 1).wait()

        slot = p & (NSLOT - 1)
        pre_blocks([(wst_v.at[slot, j], 3 * p + j) for j in range(3)],
                   [relayout_bo, relayout_bq], p >= 0)
        prefetch(p)
        return carry

    lax.fori_loop(0, 3, first_block, 0)
    prefetch(jnp.int32(0))
    lax.fori_loop(1, n_pairs, pre_pair, 0)

    xb_copy.wait()
    xc_copy.wait()
    pltpu.make_async_copy(wo_v, wo_v, sems.at[7]).wait()

    n_early_out = n_seg - 1 - LAG

    def b_pass(t, par):
        return _BPass(y_s, ((t - 1) * seg, (t - 1 - LAG) * seg), bqkv_p, bo_p,
                      kv_s.at[par], kv_s.at[1 - par], seg=seg, d=d)

    def b_store(t, yb):
        out_v[jnp.maximum(t - 1 - LAG, 0)] = yb[seg:].astype(out_v.dtype)
        return yb[:seg]

    def two_layer_step(t, par, h):
        half = t >> 1
        pre_row = None
        if par == 0:
            pre_row = pl.multiple_of((half - LAG // 2) * PRE, PRE)
        a = _TwoLayerPass(h, pre_s, pre_row, w_v, wo_v, head_s,
                          dh=dh, m_len=m_len, seg=seg)
        init = jnp.concatenate(
            [jnp.zeros((m2, d), F32), x_v[half, par].astype(F32), ra_s[...]],
            axis=0)
        acc, yb = a.run(n_pairs, init, b_pass(t, par), t >= 0)
        x2 = b_store(t, yb)
        y_s[...] = acc[m2:]
        ra_s[...] = x2
        if par == 0:
            xn = x_v[half, 1]
        else:
            xn = x_v[jnp.minimum(half + 1, n_half - 1), 0, :nf, :]
        return jnp.concatenate([_ln(xn.astype(F32)), _ln(x2), acc[:m2]],
                               axis=0).astype(BF16)

    def two_layer_steps(i, carry):
        h = h_s[...]
        for u in range(UNROLL):
            h = two_layer_step(LAG + i * UNROLL + u, (LAG + u) % 2, h)
        h_s[...] = h
        return carry

    def one_layer_step(t, carry):
        first = t < LAG
        li = (t == n_seg + 1).astype(jnp.int32)
        par = (t - li) & 1
        b = _BPass(y_s.at[pl.ds(pl.multiple_of(li * seg, seg), seg)],
                   ((t - 1 - li * (1 + LAG)) * seg,), bqkv_p, bo_p,
                   kv_s.at[par, pl.ds(li, 1)], kv_s.at[1 - par, pl.ds(li, 1)],
                   seg=seg, d=d)
        extra_row = pl.multiple_of(n_pre + jnp.minimum(t, 1) * m_len, m_len)
        a = _OneLayerPass(h1_s[...], pre_s, extra_row, w_v, wo_v, head_s,
                          dh=dh, m_len=m_len, seg=seg)
        x0 = x_seg(jnp.minimum(t, n_seg - 1))[...].astype(F32)
        init = jnp.concatenate(
            [jnp.zeros((m_len, d), F32), jnp.where(first, x0, ra_s[...])],
            axis=0)
        acc, x2 = a.run(n_pairs, init, b, t >= 0)
        out_v[jnp.where(first, 0, n_early_out)] = x2.astype(out_v.dtype)
        y = acc[m_len:]
        y_s[:seg, :] = y
        yt_s[pl.ds(pl.multiple_of((t & 1) * seg, seg), seg), :] = y
        ra_s[...] = x2
        xn = _ln(x_seg(jnp.minimum(t + 1, n_seg - 1))[...].astype(F32))
        x2n = _ln(x2)
        mem = acc[:m_len]
        h1_s[:n1, :] = jnp.concatenate(
            [mem, jnp.where(first, xn, x2n)], axis=0).astype(BF16)
        h1_s[n1:, :] = xn_s[last_xn + m_len:, :]
        h_s[...] = jnp.concatenate(
            [xn[:nf], x2n, mem, mem_v[...].astype(F32)], axis=0).astype(BF16)
        return carry

    out_a = pltpu.make_async_copy(out_v.at[:n_early_out],
                                  out_hbm.at[:n_early_out], sems.at[3])
    out_b = pltpu.make_async_copy(out_v.at[n_early_out:],
                                  out_hbm.at[n_early_out:], sems.at[4])

    def phase(ph, carry):
        t0 = ph * n_seg
        lax.fori_loop(t0, t0 + LAG, one_layer_step, 0)

        @pl.when(ph == 0)
        def _():
            lax.fori_loop(0, (n_seg - LAG) // UNROLL, two_layer_steps, 0)
            out_a.start()
            hf = h_s[...].astype(F32)
            h1_s[:n1, :] = jnp.concatenate(
                [hf[nf + seg + m_len:], hf[nf:nf + seg]],
                axis=0).astype(BF16)

        return carry

    lax.fori_loop(0, 2, phase, 0)

    b = _BPass(yt_s, ((n_seg - 2) * seg,), bqkv_p, bo_p,
               kv_s.at[(n_seg + 1) % 2, 1:], None, seg=2 * seg, d=d)
    b.project()
    for gi in range(b.n_groups):
        b.attend(gi)
    out_v[n_seg - 2:] = b.finish().astype(out_v.dtype).reshape(2, seg, d)
    out_b.start()
    out_a.wait()
    out_b.wait()


def pallas_interleave_layers__memory_aug_recurrent_mem_tr__sliding_local_dilated__prompt_kernel(
    A_x: jax.Array,
    A_mem0: jax.Array,
    A_Wq: jax.Array,
    A_Wk: jax.Array,
    A_Wv: jax.Array,
    A_Wo: jax.Array,
    A_seg_len,
    B_x: jax.Array,
    B_wqkv: jax.Array,
    B_wo: jax.Array,
):
    del B_x
    seg = A_seg_len if isinstance(A_seg_len, int) else SEG_LEN
    return _forward(A_x, A_mem0, A_Wq, A_Wk, A_Wv, A_Wo, B_wqkv, B_wo, seg=seg)


@functools.partial(jax.jit, static_argnames=("seg",))
def _forward(A_x, A_mem0, A_Wq, A_Wk, A_Wv, A_Wo, B_wqkv, B_wo, *, seg):
    bsz, s_len, d = A_x.shape
    m_len = A_mem0.shape[1]
    n_heads, dh = A_Wq.shape[1], A_Wq.shape[2]
    n_seg = s_len // seg
    n_pairs = n_heads // 2
    nt = d // LANES
    assert bsz == 1 and s_len % seg == 0 and n_seg > LAG + 1
    assert m_len == 8 and seg == 2 * m_len + PRE and seg >= HIST
    assert LAG == 2 and LAG * m_len == PRE and n_seg % (2 * LN_SEGS) == 0
    assert 2 * (m_len + seg) <= LANES
    assert (n_seg - LAG) % UNROLL == 0 and UNROLL == 2
    assert n_heads % 2 == 0 and 2 * dh == 3 * LANES and d % LANES == 0
    assert d % HB == 0 and LANES == 4 * HB and n_pairs == 3 * nt + 1
    hd = n_heads * dh
    n_half = n_seg // 2
    n_pre = (n_half - LAG // 2) * PRE

    wq_t = jnp.transpose(A_Wq, (1, 2, 0)).reshape(hd, d)
    wk_t = jnp.transpose(A_Wk, (1, 2, 0)).reshape(hd, d)
    wv_t = jnp.transpose(A_Wv, (1, 2, 0)).reshape(hd, d)
    wo = A_Wo.reshape(hd, d)

    kernel = functools.partial(
        _kernel, seg=seg, n_seg=n_seg, m_len=m_len, n_pairs=n_pairs, dh=dh,
        d=d)
    any_spec = pl.BlockSpec(memory_space=pl.ANY)
    dma = pltpu.SemaphoreType.DMA
    out = pl.pallas_call(
        kernel,
        out_shape=jax.ShapeDtypeStruct((n_seg, seg, d), A_x.dtype),
        in_specs=[any_spec] * 8,
        out_specs=any_spec,
        scratch_shapes=[
            pltpu.VMEM((n_half, 2, seg, d), BF16),
            pltpu.VMEM((m_len, d), BF16),
            pltpu.VMEM((NSLOT, 3, 2 * dh, d), BF16),
            pltpu.VMEM((3 * n_pairs, d // 2, 2 * dh), U32),
            pltpu.VMEM((hd, d), BF16),
            pltpu.VMEM((3 * nt, LANES, d), BF16),
            pltpu.VMEM((nt, d, LANES), BF16),
            pltpu.VMEM((d + HB, LANES), F32),
            pltpu.VMEM((d + HB, LANES), F32),
            pltpu.VMEM((3, d // 2, d), U32),
            pltpu.VMEM((nt, d // 2, LANES), U32),
            pltpu.VMEM((n_seg, seg, d), A_x.dtype),
            pltpu.VMEM((n_half * PRE, d), BF16),
            pltpu.VMEM((3 * n_pairs, n_pre, 2 * dh), BF16),
            pltpu.VMEM((2 * (m_len + seg) - PRE, d), BF16),
            pltpu.VMEM((2 * m_len + seg, d), BF16),
            pltpu.VMEM((seg, d), F32),
            pltpu.VMEM((2 * seg, d), F32),
            pltpu.VMEM((2 * seg, d), F32),
            pltpu.VMEM((2, 2, 2 * nt, HIST + 2 * seg, LANES), F32),
            pltpu.VMEM((HEAD_SLOTS, 2, 2, 3, 72, LANES), F32),
            dma((8,)), dma((NSLOT + 3,)), dma((2,)), dma((2,)),
        ],
        compiler_params=pltpu.CompilerParams(
            vmem_limit_bytes=96 * 1024 * 1024,
            disable_bounds_checks=True,
            disable_semaphore_checks=True),
    )(A_x.reshape(n_half, 2, seg, d), A_mem0.reshape(m_len, d), wq_t, wk_t, wv_t,
      wo, B_wqkv, B_wo)
    return out.reshape(bsz, s_len, d)
```
